```python
import jax
import jax.numpy as jnp

def _softmax(x, axis=-1):
    return jax.nn.softmax(x, axis=axis)

def _gelu(x):
    return jax.nn.gelu(x, approximate=True)

def _silu(x):
    return jax.nn.silu(x)

def _sigmoid(x):
    return jax.nn.sigmoid(x)

def _layernorm(x, axis=-1, eps=1e-05):
    m = jnp.mean(x, axis=axis, keepdims=True)
    v = jnp.var(x, axis=axis, keepdims=True)
    return (x - m) / jnp.sqrt(v + eps)

def _scatter_add(tgt, idx, src, axis=0):
    return tgt.at[idx].add(src)

def _segment_sum(src, seg, n):
    return jax.ops.segment_sum(src, seg, n)

class _Rng:

    def __init__(self, key):
        self._k = key

    def _next(self):
        self._k, sub = jax.random.split(self._k)
        return sub

    def normal(self, shape):
        return jax.random.normal(self._next(), shape, dtype=jnp.bfloat16)

    def randint(self, lo, hi, shape):
        return jax.random.randint(self._next(), shape, lo, hi, dtype=jnp.int32)

    def uniform(self, shape, lo=0.0, hi=1.0):
        return jax.random.uniform(self._next(), shape, jnp.bfloat16, lo, hi)

    def permutation(self, n):
        return jax.random.permutation(self._next(), n)
kernel_name = 'adaLN_cond__mha_block_cached__moe_arch_mod__prompt'

def setup_inputs():
    _rng = _Rng(jax.random.key(int.from_bytes(__import__("os").urandom(4), "little")))
    _w = lambda a: (lambda t: t.astype(jnp.bfloat16) if jnp.issubdtype(t.dtype, jnp.floating) else t)(jnp.asarray(a))

    def _A_setup():
        B, Sq, D = (1, 2048, 1024)
        H, Sk, Dh = (32, 2048, 128)
        return {'x': _w((lambda *s: _rng.normal(s) * 0.05)(B, Sq, D)), 'k_cache': _w((lambda *s: _rng.normal(s) * 0.05)(B, H, Sk, Dh)), 'v_cache': _w((lambda *s: _rng.normal(s) * 0.05)(B, H, Sk, Dh)), 'wq': _w((lambda *s: _rng.normal(s) * 0.05)(D, H * Dh) * D ** (-0.5)), 'wo': _w((lambda *s: _rng.normal(s) * 0.05)(H * Dh, D) * (H * Dh) ** (-0.5))}
    _A_in = _A_setup()

    def _B_setup():
        B, S, D, F, C = (1, 2048, 1024, 3584, 2)
        return {'x': _w((lambda *s: _rng.normal(s) * 0.05)(B, S, D)), 'w_r': _w((lambda *s: _rng.normal(s) * 0.05)(D)), 'w_gate': _w((lambda *s: _rng.normal(s) * 0.05)(D, F)), 'w_up': _w((lambda *s: _rng.normal(s) * 0.05)(D, F)), 'w_down': _w((lambda *s: _rng.normal(s) * 0.05)(F, D))}
    _B_in = _B_setup()
    return {'A_x': _A_in['x'], 'A_k_cache': _A_in['k_cache'], 'A_v_cache': _A_in['v_cache'], 'A_wq': _A_in['wq'], 'A_wo': _A_in['wo'], 'B_x': _B_in['x'], 'B_w_r': _B_in['w_r'], 'B_w_gate': _B_in['w_gate'], 'B_w_up': _B_in['w_up'], 'B_w_down': _B_in['w_down'], 'c': _w((lambda *s: _rng.normal(s) * 0.05)(1, 1024)), 'w_mod': _w((lambda *s: _rng.normal(s) * 0.05)(1024, 6 * 1024) * 1024 ** (-0.5))}

def reference(A_x, A_k_cache, A_v_cache, A_wq, A_wo, B_x, B_w_r, B_w_gate, B_w_up, B_w_down, c, w_mod):

    def _A_ref(x, k_cache, v_cache, wq, wo):
        B, Sq, D = x.shape
        H, Dh = (32, 128)
        q = (lambda x, *d: x.transpose(*d))((x @ wq).reshape(B, Sq, H, Dh), 0, 2, 1, 3)
        scores = jnp.einsum('bhqd,bhkd->bhqk', q, k_cache) * Dh ** (-0.5)
        p = _softmax(scores, axis=-1)
        o = jnp.einsum('bhqk,bhkd->bhqd', p, v_cache)
        return (lambda x, *d: x.transpose(*d))(o, 0, 2, 1, 3).reshape(B, Sq, H * Dh) @ wo

    def _B_ref(x, w_r, w_gate, w_up, w_down):
        B, S, D = x.shape
        C = 2
        r = x @ w_r
        idx = jnp.argsort(-r, axis=-1)[:, :C]
        idx_e = jnp.repeat(idx.reshape(B, C, 1), D, axis=2)
        x_sel = jnp.take_along_axis(x, idx_e, axis=1)
        g = _silu(x_sel @ w_gate)
        u = x_sel @ w_up
        y = g * u @ w_down
        r_sel = _sigmoid(jnp.take_along_axis(r, idx, axis=1))
        y = y * r_sel.reshape(B, C, 1)
        b_off = (jnp.arange(B) * S).reshape(B, 1)
        flat_idx = (idx + b_off).reshape(B * C)
        zero = (x * 0.0).reshape(B * S, D)
        upd = _scatter_add(zero, flat_idx, y.reshape(B * C, D), axis=0)
        return x + upd.reshape(B, S, D)
    x = A_x
    mod = (_silu(c) @ w_mod).reshape(c.shape[0], 6, 1, -1)
    sa, ca, ga, sb, cb, gb = (mod[:, 0].copy(), mod[:, 1].copy(), mod[:, 2].copy(), mod[:, 3].copy(), mod[:, 4].copy(), mod[:, 5].copy())
    h = _layernorm(x, axis=-1) * (1 + ca) + sa
    x = x + ga * _A_ref(h, A_k_cache, A_v_cache, A_wq, A_wo)
    h = _layernorm(x, axis=-1) * (1 + cb) + sb
    x = x + gb * _B_ref(h, B_w_r, B_w_gate, B_w_up, B_w_down)
    return x
```

```python
import jax
import jax.numpy as jnp
from jax import lax
import jax.experimental.pallas as pl
import jax.experimental.pallas.tpu as pltpu

S = 2048
D = 1024
H = 32
DH = 128
F = 3584
TQ = 512
SUB = 256
HG = 4
NQ = S // TQ
NG = H // HG
NSUB = TQ // SUB
RC = TQ // NG
NCH = S // RC
GW = HG * DH
PAD = 128
EPS = 1e-5
QSCALE = float(DH ** -0.5) * 1.4426950408889634

F32 = jnp.float32
BF16 = jnp.bfloat16


def _r(v):
    return v.astype(BF16).astype(F32)


def _ln_mod(xf, scale1, shift):
    m = jnp.mean(xf, axis=-1, keepdims=True)
    xc = xf - m
    v = jnp.mean(xc * xc, axis=-1, keepdims=True)
    den = _r(jnp.sqrt(_r(_r(v) + EPS)))
    n = _r(_r(xf - _r(m)) / den)
    return _r(_r(n * scale1) + shift)


def _kernel(x_hbm, k_hbm, v_hbm, wq_hbm, wo_hbm, wr_ref, wg_hbm, wu_hbm, wd_hbm,
            c_ref, wmod_hbm, out_hbm,
            x_buf, k_buf, v_buf, wq_buf, wo_buf, wa_buf, wb_buf, wd_buf,
            h_buf, acc, x2_buf, out_buf, r_buf, mod_buf, q_car, o_car,
            sem_x, sem_k, sem_v, sem_wq, sem_wo, sem_w, sem_out):
    i = pl.program_id(0)
    g = pl.program_id(1)
    step = i * NG + g

    def cp_x(b):
        return pltpu.make_async_copy(x_hbm.at[pl.ds(b * TQ, TQ), :],
                                     x_buf.at[pl.ds(b * TQ, TQ), :], sem_x.at[b])

    def cp_k(gg):
        return pltpu.make_async_copy(k_hbm.at[pl.ds(gg * HG, HG)],
                                     k_buf.at[pl.ds(gg * HG, HG)], sem_k.at[gg])

    def cp_v(gg):
        return pltpu.make_async_copy(v_hbm.at[pl.ds(gg * HG, HG)],
                                     v_buf.at[pl.ds(gg * HG, HG)], sem_v.at[gg])

    def cp_wq(gg):
        return pltpu.make_async_copy(wq_hbm.at[:, pl.ds(gg * GW, GW)],
                                     wq_buf.at[gg], sem_wq.at[gg])

    def cp_wo(gg):
        return pltpu.make_async_copy(wo_hbm.at[pl.ds(gg * GW, GW), :],
                                     wo_buf.at[gg], sem_wo.at[gg])

    cp_m0 = pltpu.make_async_copy(wmod_hbm.at[:, 0:2 * D], wa_buf.at[:, 0:2 * D], sem_w.at[0])
    cp_m1 = pltpu.make_async_copy(wmod_hbm.at[:, 2 * D:3 * D], wa_buf.at[:, 2 * D:3 * D], sem_w.at[1])
    cp_m2 = pltpu.make_async_copy(wmod_hbm.at[:, 3 * D:6 * D], wb_buf.at[:, 0:3 * D], sem_w.at[2])
    cp_wg = pltpu.make_async_copy(wg_hbm, wa_buf.at[:, 0:F], sem_w.at[3])
    cp_wu = pltpu.make_async_copy(wu_hbm, wb_buf.at[:, 0:F], sem_w.at[4])
    cp_wd = pltpu.make_async_copy(wd_hbm, wd_buf.at[:, 0:D], sem_w.at[5])

    def cp_out(b):
        return pltpu.make_async_copy(out_buf.at[pl.ds(b * TQ, TQ), :],
                                     out_hbm.at[pl.ds(b * TQ, TQ), :], sem_out.at[b])

    def silu_c():
        cf = c_ref[...].astype(F32)
        sc = (cf * _r(jax.nn.sigmoid(cf))).astype(BF16)
        return jnp.broadcast_to(sc, (16, D))

    def qproj(hs, w):
        q = jnp.dot(hs, w, preferred_element_type=F32)
        return (q * QSCALE).astype(BF16)

    def finalize(xrows, arows, dst_row, chunk):
        ga = mod_buf[2:3, :]
        sb = mod_buf[3:4, :]
        cb1 = mod_buf[4:5, :]
        gb = mod_buf[5:6, :]
        x2 = _r(xrows.astype(F32) + _r(ga * _r(arows)))
        h2 = _ln_mod(x2, cb1, sb)
        r = _r(jnp.sum(h2 * wr_ref[...].astype(F32), axis=-1, keepdims=True))
        x2_buf[pl.ds(dst_row, RC), :] = x2.astype(BF16)
        out_buf[pl.ds(dst_row, RC), :] = (x2 + _r(gb * h2)).astype(BF16)
        lane = lax.broadcasted_iota(jnp.int32, (RC, 128), 1)
        r_buf[...] = jnp.where(lane == chunk, r, r_buf[...])

    @pl.when(step == 0)
    def _():
        cp_x(0).start()
        cp_m0.start()
        cp_wq(0).start()
        cp_k(0).start()
        cp_v(0).start()
        cp_wo(0).start()
        cp_wq(1).start()
        for b in range(1, NQ):
            cp_x(b).start()
        acc[...] = jnp.zeros(acc.shape, F32)
        o_car[...] = jnp.zeros(o_car.shape, BF16)
        r_buf[...] = jnp.full(r_buf.shape, -jnp.inf, F32)
        mod_buf[...] = jnp.zeros(mod_buf.shape, F32)
        cp_m0.wait()
        m = _r(jnp.dot(silu_c(), wa_buf[:, 0:2 * D], preferred_element_type=F32)[0:1, :])
        mod_buf[0:1, :] = m[:, 0:D]
        mod_buf[1:2, :] = _r(1.0 + m[:, D:2 * D])
        cp_x(0).wait()
        for cidx in range(NG):
            xr = x_buf[pl.ds(cidx * RC, RC), :].astype(F32)
            h_buf[0, pl.ds(cidx * RC, RC), :] = _ln_mod(
                xr, mod_buf[1:2, :], mod_buf[0:1, :]).astype(BF16)
        cp_wq(0).wait()
        q_car[...] = qproj(h_buf[0, 0:SUB, :], wq_buf[0, :, 0:DH])
        for b in range(1, NQ):
            cp_x(b).wait()

    @pl.when(i == 0)
    def _():
        @pl.when(g + 1 < NG)
        def _():
            cp_k(g + 1).start()
            cp_v(g + 1).start()
            cp_wo(g + 1).start()

        @pl.when(g + 2 < NG)
        def _():
            cp_wq(g + 2).start()

        @pl.when(g == 2)
        def _():
            cp_m1.start()
            cp_m2.start()

        @pl.when(g == NG - 1)
        def _():
            cp_m1.wait()
            cp_m2.wait()
            sc = silu_c()
            m1 = _r(jnp.dot(sc, wa_buf[:, 2 * D:3 * D], preferred_element_type=F32)[0:1, :])
            m2 = _r(jnp.dot(sc, wb_buf[:, 0:3 * D], preferred_element_type=F32)[0:1, :])
            mod_buf[2:3, :] = m1
            mod_buf[3:4, :] = m2[:, 0:D]
            mod_buf[4:5, :] = _r(1.0 + m2[:, D:2 * D])
            mod_buf[5:6, :] = m2[:, 2 * D:3 * D]
            cp_wg.start()
            cp_wu.start()
            cp_wd.start()

        cp_k(g).wait()
        cp_v(g).wait()
        cp_wo(g).wait()

        @pl.when(g + 1 < NG)
        def _():
            cp_wq(g + 1).wait()

    @pl.when(jnp.logical_and(i >= 2, g == 0))
    def _():
        cp_out(i - 2).start()

    slot = lax.rem(i, 2)
    oslot = 1 - slot
    head0 = g * HG
    prev_g = jnp.where(step == 0, 0, lax.rem(g + NG - 1, NG))
    prev_slot = jnp.where(g == 0, oslot, slot)
    next_g = lax.rem(g + 1, NG)
    next_slot = jnp.where(g == NG - 1, oslot, slot)

    units = [(s, j) for s in range(NSUB) for j in range(HG)]
    nu = len(units)

    def oproj(o, gg, j, sl, s):
        w = wo_buf[gg, j * DH:(j + 1) * DH, :]
        acc[sl, s * SUB:(s + 1) * SUB, :] += jnp.dot(o, w, preferred_element_type=F32)

    q = q_car[...]
    o_prev = o_car[...]
    for u, (s, j) in enumerate(units):
        kk = k_buf[head0 + j]
        sc = lax.dot_general(q, kk, (((1,), (1,)), ((), ())), preferred_element_type=F32)
        if u == 0:
            oproj(o_prev, prev_g, HG - 1, prev_slot, NSUB - 1)
        else:
            ps, pj = units[u - 1]
            oproj(o_prev, g, pj, slot, ps)
        if u + 1 < nu:
            ns, nj = units[u + 1]
            q = qproj(h_buf[slot, ns * SUB:(ns + 1) * SUB, :],
                      wq_buf[g, :, nj * DH:(nj + 1) * DH])
        m = jnp.max(sc, axis=-1, keepdims=True)
        p = jnp.exp2(sc - m)
        l = jnp.sum(p, axis=-1, keepdims=True)
        pv = jnp.dot(p.astype(BF16), v_buf[head0 + j], preferred_element_type=F32)
        o_prev = (pv / l).astype(BF16)
    o_car[...] = o_prev
    q_car[...] = qproj(h_buf[next_slot, 0:SUB, :], wq_buf[next_g, :, 0:DH])

    roff = pl.multiple_of(g * RC, RC)
    nrow = pl.multiple_of(jnp.minimum(i + 1, NQ - 1) * TQ + roff, RC)
    h_buf[oslot, pl.ds(roff, RC), :] = _ln_mod(
        x_buf[pl.ds(nrow, RC), :].astype(F32), mod_buf[1:2, :], mod_buf[0:1, :]).astype(BF16)

    src_row = pl.multiple_of(jnp.maximum(i - 1, 0) * TQ + roff, RC)
    dst_blk = lax.rem(i + NQ - 1, NQ)
    dst_row = pl.multiple_of(dst_blk * TQ + roff, RC)
    finalize(x_buf[pl.ds(src_row, RC), :], acc[oslot, pl.ds(roff, RC), :],
             dst_row, dst_blk * NG + g)
    acc[oslot, pl.ds(roff, RC), :] = jnp.zeros((RC, D), F32)

    @pl.when(step == NQ * NG - 1)
    def _():
        lslot = (NQ - 1) % 2
        cp_out(NQ - 2).start()
        oproj(o_car[...], NG - 1, HG - 1, lslot, NSUB - 1)
        for cidx in range(NG):
            row = (NQ - 1) * TQ + cidx * RC
            finalize(x_buf[row:row + RC, :], acc[lslot, cidx * RC:(cidx + 1) * RC, :],
                     row, (NQ - 1) * NG + cidx)
        cp_out(NQ - 1).start()

        rr = r_buf[...]
        ridx = (lax.broadcasted_iota(jnp.int32, (RC, 128), 1) * RC
                + lax.broadcasted_iota(jnp.int32, (RC, 128), 0))
        big = jnp.int32(S - 1)
        m1 = jnp.max(jnp.max(rr, axis=0, keepdims=True), axis=1, keepdims=True)
        i1 = jnp.minimum(jnp.min(jnp.where(rr == m1, ridx, big)), big)
        rr2 = jnp.where(ridx == i1, -jnp.inf, rr)
        m2 = jnp.max(jnp.max(rr2, axis=0, keepdims=True), axis=1, keepdims=True)
        i2 = jnp.minimum(jnp.min(jnp.where(
            jnp.logical_and(rr2 == m2, ridx != i1), ridx, big)), big)

        sb = mod_buf[3:4, :]
        cb1 = mod_buf[4:5, :]
        gb = mod_buf[5:6, :]
        rowid = lax.broadcasted_iota(jnp.int32, (16, D), 0)
        g1 = pl.multiple_of((i1 // 16) * 16, 16)
        g2 = pl.multiple_of((i2 // 16) * 16, 16)
        x2a = x2_buf[pl.ds(g1, 16), :].astype(F32)
        x2b = x2_buf[pl.ds(g2, 16), :].astype(F32)
        h2a = _ln_mod(x2a, cb1, sb)
        h2b = _ln_mod(x2b, cb1, sb)
        row1 = jnp.sum(jnp.where(rowid + g1 == i1, h2a, 0.0), axis=0, keepdims=True)
        row2 = jnp.sum(jnp.where(rowid + g2 == i2, h2b, 0.0), axis=0, keepdims=True)
        xs = jnp.where(rowid == 0, row1, row2).astype(BF16)

        cp_wg.wait()
        cp_wu.wait()
        cp_wd.wait()
        gt = _r(jnp.dot(xs, wa_buf[:, 0:F], preferred_element_type=F32))
        up = _r(jnp.dot(xs, wb_buf[:, 0:F], preferred_element_type=F32))
        act = (_r(gt * _r(jax.nn.sigmoid(gt))) * up).astype(BF16)
        y = _r(jnp.dot(act, wd_buf[:, 0:D], preferred_element_type=F32))
        y1 = _r(y[0:1, :] * _r(jax.nn.sigmoid(m1)))
        y2 = _r(y[1:2, :] * _r(jax.nn.sigmoid(m2)))

        def fix(x2g, h2g, gbase):
            rid = rowid + gbase
            upd = jnp.where(rid == i1, y1, jnp.where(rid == i2, y2, 0.0))
            return (x2g + _r(gb * _r(h2g + upd))).astype(BF16)

        for b in range(NQ):
            cp_out(b).wait()
        out_buf[pl.ds(g1, 16), :] = fix(x2a, h2a, g1)
        out_buf[pl.ds(g2, 16), :] = fix(x2b, h2b, g2)
        f1 = pltpu.make_async_copy(out_buf.at[pl.ds(g1, 16), :],
                                   out_hbm.at[pl.ds(g1, 16), :], sem_out.at[0])
        f2 = pltpu.make_async_copy(out_buf.at[pl.ds(g2, 16), :],
                                   out_hbm.at[pl.ds(g2, 16), :], sem_out.at[1])
        f1.start()

        @pl.when(g1 != g2)
        def _():
            f2.start()
            f2.wait()

        f1.wait()


@jax.jit
def pallas_adaLN_cond__mha_block_cached__moe_arch_mod__prompt_kernel(
    A_x: jax.Array,
    A_k_cache: jax.Array,
    A_v_cache: jax.Array,
    A_wq: jax.Array,
    A_wo: jax.Array,
    B_x: jax.Array,
    B_w_r: jax.Array,
    B_w_gate: jax.Array,
    B_w_up: jax.Array,
    B_w_down: jax.Array,
    c: jax.Array,
    w_mod: jax.Array,
):
    del B_x
    hbm = pl.BlockSpec(memory_space=pl.ANY)
    vec = pl.BlockSpec((1, D), lambda i, g: (0, 0))
    out = pl.pallas_call(
        _kernel,
        grid=(NQ, NG),
        in_specs=[hbm, hbm, hbm, hbm, hbm, vec, hbm, hbm, hbm, vec, hbm],
        out_specs=hbm,
        out_shape=jax.ShapeDtypeStruct((S, D), BF16),
        scratch_shapes=[
            pltpu.VMEM((S, D), BF16),
            pltpu.VMEM((H, S, DH), BF16),
            pltpu.VMEM((H, S, DH), BF16),
            pltpu.VMEM((NG, D, GW), BF16),
            pltpu.VMEM((NG, GW, D), BF16),
            pltpu.VMEM((D, F + PAD), BF16),
            pltpu.VMEM((D, F + PAD), BF16),
            pltpu.VMEM((F, D + PAD), BF16),
            pltpu.VMEM((2, TQ, D), BF16),
            pltpu.VMEM((2, TQ, D), F32),
            pltpu.VMEM((S, D), BF16),
            pltpu.VMEM((S, D), BF16),
            pltpu.VMEM((RC, 128), F32),
            pltpu.VMEM((8, D), F32),
            pltpu.VMEM((SUB, DH), BF16),
            pltpu.VMEM((SUB, DH), BF16),
            pltpu.SemaphoreType.DMA((NQ,)),
            pltpu.SemaphoreType.DMA((NG,)),
            pltpu.SemaphoreType.DMA((NG,)),
            pltpu.SemaphoreType.DMA((NG,)),
            pltpu.SemaphoreType.DMA((NG,)),
            pltpu.SemaphoreType.DMA((6,)),
            pltpu.SemaphoreType.DMA((NQ,)),
        ],
        compiler_params=pltpu.CompilerParams(
            dimension_semantics=("arbitrary", "arbitrary"),
            vmem_limit_bytes=120 * 1024 * 1024,
        ),
        name="adaln_mha_mod",
    )(
        A_x.reshape(S, D),
        A_k_cache.reshape(H, S, DH),
        A_v_cache.reshape(H, S, DH),
        A_wq,
        A_wo,
        B_w_r.reshape(1, D),
        B_w_gate,
        B_w_up,
        B_w_down,
        c,
        w_mod,
    )
    return out.reshape(1, S, D)
```

```python
import jax
import jax.numpy as jnp
from jax import lax
import jax.experimental.pallas as pl
import jax.experimental.pallas.tpu as pltpu

S = 2048
D = 1024
H = 32
DH = 128
F = 3584
SUB = 256
NRB = S // SUB
NU = H * NRB
PR = 16
UM = 16
RAMP = 16
NM = (NU - RAMP) // UM
LN_START = 32
FIN_START = 129
PAD = 128
MCH = 4
EPS = 1e-5
QSCALE = float(DH ** -0.5) * 1.4426950408889634

F32 = jnp.float32
BF16 = jnp.bfloat16
I32 = jnp.int32
NT = (((1,), (1,)), ((), ()))

C_GA, C_SCALE, C_SHIFT, C_KEEP, C_GB = range(5)


def _r(v):
    return v.astype(BF16).astype(F32)


def _rows8(v, fn, c):
    n = v.shape[0] // 8
    return fn(v.reshape(n, 8, D), c[None]).reshape(v.shape)


def _lane_fold(p, fn):
    t = p[:, 0:128]
    for j in range(1, p.shape[1] // 128):
        t = fn(t, p[:, j * 128:(j + 1) * 128])
    return t


def _normalize(pv, ls):
    l = jnp.sum(ls, axis=-1, keepdims=True)
    r = pl.reciprocal(l, approx=True)
    r = r * (2.0 - l * r)
    return (pv * r).astype(BF16)


def _head_of(n):
    if isinstance(n, int):
        return (n % 64) // 2 if n < 192 else (n - 192) % H
    return jnp.where(n < 192, lax.shift_right_logical(n & 63, 1), (n - 192) & (H - 1))


def _row_of(n):
    if isinstance(n, int):
        return SUB * ((n // 64) * 2 + n % 2 if n < 192 else min(n // 32, NRB - 1))
    rb = jnp.where(n < 192, lax.shift_right_logical(n, 6) * 2 + (n & 1),
                   jnp.minimum(lax.shift_right_logical(n, 5), NRB - 1))
    return pl.multiple_of(rb * SUB, SUB)


def _kernel(x_hbm, k_hbm, v_hbm, wq_hbm, wo_hbm, wr_hbm, wg_hbm, wu_hbm, wd_hbm,
            c_hbm, wmod_hbm, out_hbm,
            x_buf, k_buf, v_buf, wq_buf, wo_buf, wa_buf, wb_buf, wd_buf,
            act, acc, r_buf, coef, wr_buf, wr_b, c_buf, zero_buf, q_car, pv_car, ls_car,
            sem_x, sem_k, sem_v, sem_wq, sem_wo, sem_m, sem_w, sem_out):
    def cp_x(b, nb=1):
        return pltpu.make_async_copy(x_hbm.at[pl.ds(b * SUB, nb * SUB), :],
                                     x_buf.at[pl.ds(b * SUB, nb * SUB), :], sem_x.at[b])

    def cp_k(h0, nh):
        return pltpu.make_async_copy(k_hbm.at[pl.ds(h0, nh)], k_buf.at[pl.ds(h0, nh)], sem_k.at[h0])

    def cp_v(h0, nh):
        return pltpu.make_async_copy(v_hbm.at[pl.ds(h0, nh)], v_buf.at[pl.ds(h0, nh)], sem_v.at[h0])

    def cp_wo(h0, nh):
        return pltpu.make_async_copy(wo_hbm.at[pl.ds(h0, nh)], wo_buf.at[pl.ds(h0, nh)], sem_wo.at[h0])

    def cp_wq(h):
        col = h * DH if isinstance(h, int) else pl.multiple_of(h * DH, DH)
        return pltpu.make_async_copy(wq_hbm.at[:, pl.ds(col, DH)], wq_buf.at[h], sem_wq.at[h])

    def heads(h0, nh):
        nq = nh - 1 if isinstance(h0, int) and h0 + nh == H else nh
        return [cp_k(h0, nh), cp_v(h0, nh), cp_wo(h0, nh)] + [
            cp_wq(h0 + 1 + j) for j in range(nq)]

    mrows = D // MCH
    cp_m0 = [pltpu.make_async_copy(wmod_hbm.at[pl.ds(j * mrows, mrows), 0:2 * D],
                                   wa_buf.at[pl.ds(j * mrows, mrows), 0:2 * D], sem_m.at[j])
             for j in range(MCH)]
    cp_c = pltpu.make_async_copy(c_hbm, c_buf, sem_w.at[0])
    cp_wr = pltpu.make_async_copy(wr_hbm, wr_buf, sem_w.at[1])
    cp_m1 = pltpu.make_async_copy(wmod_hbm.at[:, 2 * D:3 * D], wa_buf.at[:, 2 * D:3 * D], sem_w.at[2])
    cp_m2 = pltpu.make_async_copy(wmod_hbm.at[:, 3 * D:6 * D], wb_buf.at[:, 0:3 * D], sem_w.at[3])
    cp_wg = pltpu.make_async_copy(wg_hbm, wa_buf.at[:, 0:F], sem_w.at[4])
    cp_wu = pltpu.make_async_copy(wu_hbm, wb_buf.at[:, 0:F], sem_w.at[5])
    cp_wd = pltpu.make_async_copy(wd_hbm, wd_buf.at[:, 0:D], sem_w.at[6])

    def cp_out(b):
        row = b * SUB if isinstance(b, int) else pl.multiple_of(b * SUB, SUB)
        return pltpu.make_async_copy(act.at[pl.ds(row, SUB), :],
                                     out_hbm.at[pl.ds(row, SUB), :], sem_out.at[b])

    def silu_c():
        cf = c_buf[...].astype(F32)
        sc = (cf * _r(jax.nn.sigmoid(cf))).astype(BF16)
        return jnp.broadcast_to(sc, (16, D))

    def bcast8(v):
        return jnp.broadcast_to(v, (8, D))

    def packed(ref, h):
        return pltpu.bitcast(ref.bitcast(jnp.uint32)[h], BF16)

    def ada_ln(y, kind):
        m = jnp.mean(y, axis=-1, keepdims=True)
        yc = y - m
        v = jnp.mean(yc * yc, axis=-1, keepdims=True)
        den = _r(jnp.sqrt(_r(_r(v) + EPS)))
        n = (y - _r(m)) * (1.0 / den)
        n = _rows8(n, jnp.multiply, coef[kind, C_SCALE])
        return _rows8(n, jnp.add, coef[kind, C_SHIFT])

    def resid(row, nrows, kind):
        a = _rows8(acc[pl.ds(row, nrows), :], jnp.multiply, coef[kind, C_GA])
        return _r(x_buf[pl.ds(row, nrows), :].astype(F32) + a)

    def piece(src, dst, kind, lane_id):
        y = resid(src, PR, kind)
        hh = ada_ln(y, kind)
        r = jnp.sum(_rows8(hh, jnp.multiply, wr_b[...]), axis=-1, keepdims=True)
        oo = (_rows8(y, jnp.multiply, coef[kind, C_KEEP])
              + _rows8(hh, jnp.multiply, coef[kind, C_GB]))
        act[pl.ds(dst, PR), :] = oo.astype(BF16)
        lane = lax.broadcasted_iota(I32, (PR, 128), 1)
        rn = jnp.where(lane == lane_id, r, r_buf[...])
        r_buf[...] = rn
        return oo, rn

    def unit_piece(n):
        is_ln = jnp.logical_and(n >= LN_START, n < LN_START + (S - 2 * SUB) // PR)
        is_fin = jnp.logical_and(n >= FIN_START, n < FIN_START + (S - SUB) // PR)
        f = n - FIN_START
        src = jnp.where(is_ln, 2 * SUB + (n - LN_START) * PR, jnp.where(is_fin, f * PR, 0))
        dst = jnp.where(jnp.logical_or(is_ln, is_fin), src, S)
        oo, rn = piece(pl.multiple_of(src, PR), pl.multiple_of(dst, PR),
                       is_fin.astype(I32), jnp.where(is_fin, f, -1))
        bits = _lane_fold(pltpu.bitcast(oo, I32), jnp.bitwise_or) | pltpu.bitcast(rn, I32)
        return (bits[0:8] | bits[8:16]) & zero_buf[...]

    def qproj(n):
        q = jnp.dot(act[pl.ds(_row_of(n), SUB), :], packed(wq_buf, _head_of(n)),
                    preferred_element_type=F32)
        return (q * QSCALE).astype(BF16)

    def oproj(o, n):
        acc[pl.ds(_row_of(n), SUB), :] += jnp.dot(o, wo_buf[_head_of(n)],
                                                  preferred_element_type=F32)

    def unit_block(n0, nunits, with_piece):
        q = q_car[...]
        o = _normalize(pv_car[...], ls_car[...])
        for u in range(nunits):
            n = n0 + u
            hd = _head_of(n)
            z = unit_piece(n) if with_piece else None
            sc = lax.dot_general(q, packed(k_buf, hd), NT, preferred_element_type=F32)
            mm = _lane_fold(sc, jnp.maximum)
            if with_piece:
                mb = pltpu.bitcast(mm, I32)
                mm = pltpu.bitcast(jnp.concatenate([mb[0:8] | z, mb[8:]], axis=0), F32)
            m = jnp.max(mm, axis=-1, keepdims=True)
            p = jnp.exp2(sc - m)
            ls = _lane_fold(p, jnp.add)
            pv = jnp.dot(p.astype(BF16), packed(v_buf, hd), preferred_element_type=F32)
            q = qproj(n + 1)
            prev = max(n - 1, 0) if isinstance(n, int) else jnp.maximum(n - 1, 0)
            oproj(o, prev)
            if u + 1 < nunits:
                o = _normalize(pv, ls)
            else:
                pv_car[...] = pv
                ls_car[...] = ls
        q_car[...] = q

    def start(cps):
        for cp in cps:
            cp.start()

    def wait(cps):
        for cp in cps:
            cp.wait()

    start([cp_c, cp_x(0)] + cp_m0 + [cp_wq(0), cp_x(1), cp_wr])
    start(heads(0, 1) + heads(1, 1) + heads(2, 2) + heads(4, 4))
    acc[...] = jnp.zeros(acc.shape, F32)
    pv_car[...] = jnp.zeros(pv_car.shape, F32)
    ls_car[...] = jnp.ones(ls_car.shape, F32)
    r_buf[...] = jnp.zeros(r_buf.shape, F32)
    zero_buf[...] = jnp.zeros(zero_buf.shape, I32)
    coef[0, C_GA] = jnp.zeros((8, D), F32)
    coef[0, C_KEEP] = jnp.zeros((8, D), F32)
    coef[0, C_GB] = jnp.ones((8, D), F32)
    coef[1, C_KEEP] = jnp.ones((8, D), F32)
    cp_c.wait()
    sc16 = silu_c()
    m0 = None
    for j in range(MCH):
        cp_m0[j].wait()
        part = jnp.dot(sc16[:, j * mrows:(j + 1) * mrows],
                       wa_buf[j * mrows:(j + 1) * mrows, 0:2 * D], preferred_element_type=F32)
        m0 = part if m0 is None else m0 + part
    m0 = _r(m0[0:8, :])
    coef[0, C_SHIFT] = m0[:, 0:D]
    coef[0, C_SCALE] = _r(1.0 + m0[:, D:2 * D])
    for b in range(2):
        cp_x(b).wait()
        for j in range(SUB // 64):
            row = b * SUB + j * 64
            act[row:row + 64, :] = ada_ln(x_buf[row:row + 64, :].astype(F32), 0).astype(BF16)
        if b == 0:
            cp_wq(0).wait()
            q_car[...] = qproj(0)
    cp_wr.wait()
    wr_b[...] = bcast8(wr_buf[...].astype(F32))

    def ramp2(j, carry):
        wait(heads(j, 1))
        unit_block(2 * j, 2, False)
        return carry

    lax.fori_loop(0, 2, ramp2, 0)
    start(heads(8, 8))
    wait(heads(2, 2))
    unit_block(4, 4, False)
    start([cp_x(2, 6)] + heads(16, 8))
    wait(heads(4, 4))
    unit_block(8, 8, False)

    def main(k, carry):
        @pl.when(k == 0)
        def _():
            start(heads(24, 8) + [cp_m1, cp_m2])
            wait(heads(8, 8))

        @pl.when(k == 1)
        def _():
            wait(heads(16, 8) + [cp_x(2, 6)])

        @pl.when(k == 2)
        def _():
            wait(heads(24, 8))

        @pl.when(k == 3)
        def _():
            wait([cp_m1, cp_m2])
            sc = silu_c()
            m1 = _r(jnp.dot(sc, wa_buf[:, 2 * D:3 * D], preferred_element_type=F32)[0:8, :])
            m2 = _r(jnp.dot(sc, wb_buf[:, 0:3 * D], preferred_element_type=F32)[0:8, :])
            coef[1, C_GA] = m1
            coef[1, C_SHIFT] = m2[:, 0:D]
            coef[1, C_SCALE] = _r(1.0 + m2[:, D:2 * D])
            coef[1, C_GB] = m2[:, 2 * D:3 * D]
            start([cp_wg, cp_wu, cp_wd])

        @pl.when(k >= NM - 6)
        def _():
            cp_out(k - (NM - 6)).start()

        unit_block(RAMP + k * UM, UM, True)
        return carry

    lax.fori_loop(0, NM, main, 0)

    cp_out(NRB - 2).start()
    oproj(_normalize(pv_car[...], ls_car[...]), NU - 1)
    for j in range(SUB // PR):
        row = (NRB - 1) * SUB + j * PR
        piece(row, row, 1, row // PR)
    cp_out(NRB - 1).start()

    rr = r_buf[...]
    ridx = (lax.broadcasted_iota(I32, (PR, 128), 1) * PR
            + lax.broadcasted_iota(I32, (PR, 128), 0))
    big = jnp.int32(S - 1)
    m1 = jnp.max(jnp.max(rr, axis=0, keepdims=True), axis=1, keepdims=True)
    i1 = jnp.min(jnp.where(rr == m1, ridx, big))
    rr2 = jnp.where(ridx == i1, -jnp.inf, rr)
    m2 = jnp.max(jnp.max(rr2, axis=0, keepdims=True), axis=1, keepdims=True)
    i2 = jnp.min(jnp.where(jnp.logical_and(rr2 == m2, ridx != i1), ridx, big))

    rowid = lax.broadcasted_iota(I32, (PR, D), 0)
    g1 = pl.multiple_of(lax.shift_right_logical(i1, 4) * PR, PR)
    g2 = pl.multiple_of(lax.shift_right_logical(i2, 4) * PR, PR)
    x2a = resid(g1, PR, 1)
    x2b = resid(g2, PR, 1)
    h2a = _r(ada_ln(x2a, 1))
    h2b = _r(ada_ln(x2b, 1))
    row1 = jnp.sum(jnp.where(rowid + g1 == i1, h2a, 0.0), axis=0, keepdims=True)
    row2 = jnp.sum(jnp.where(rowid + g2 == i2, h2b, 0.0), axis=0, keepdims=True)
    xs = jnp.where(rowid == 0, row1, row2).astype(BF16)

    wait([cp_wg, cp_wu, cp_wd])
    gt = _r(jnp.dot(xs, wa_buf[:, 0:F], preferred_element_type=F32))
    up = _r(jnp.dot(xs, wb_buf[:, 0:F], preferred_element_type=F32))
    hid = (_r(gt * _r(jax.nn.sigmoid(gt))) * up).astype(BF16)
    y = _r(jnp.dot(hid, wd_buf[:, 0:D], preferred_element_type=F32))
    y1 = _r(y[0:1, :] * _r(jax.nn.sigmoid(_r(m1))))
    y2 = _r(y[1:2, :] * _r(jax.nn.sigmoid(_r(m2))))

    def fix(x2g, h2g, gbase):
        rid = rowid + gbase
        upd = jnp.where(rid == i1, y1, jnp.where(rid == i2, y2, 0.0))
        return (x2g + _rows8(h2g + upd, jnp.multiply, coef[1, C_GB])).astype(BF16)

    for b in range(NRB):
        cp_out(b).wait()
    act[pl.ds(g1, PR), :] = fix(x2a, h2a, g1)
    act[pl.ds(g2, PR), :] = fix(x2b, h2b, g2)
    f1 = pltpu.make_async_copy(act.at[pl.ds(g1, PR), :],
                               out_hbm.at[pl.ds(g1, PR), :], sem_out.at[0])
    f2 = pltpu.make_async_copy(act.at[pl.ds(g2, PR), :],
                               out_hbm.at[pl.ds(g2, PR), :], sem_out.at[1])
    f1.start()

    @pl.when(g1 != g2)
    def _():
        f2.start()
        f2.wait()

    f1.wait()


@jax.jit
def pallas_adaLN_cond__mha_block_cached__moe_arch_mod__prompt_kernel(
    A_x: jax.Array,
    A_k_cache: jax.Array,
    A_v_cache: jax.Array,
    A_wq: jax.Array,
    A_wo: jax.Array,
    B_x: jax.Array,
    B_w_r: jax.Array,
    B_w_gate: jax.Array,
    B_w_up: jax.Array,
    B_w_down: jax.Array,
    c: jax.Array,
    w_mod: jax.Array,
):
    del B_x
    hbm = pl.BlockSpec(memory_space=pl.ANY)
    out = pl.pallas_call(
        _kernel,
        in_specs=[hbm] * 11,
        out_specs=hbm,
        out_shape=jax.ShapeDtypeStruct((S, D), BF16),
        scratch_shapes=[
            pltpu.VMEM((S, D), BF16),
            pltpu.VMEM((H, S, DH), BF16),
            pltpu.VMEM((H, S, DH), BF16),
            pltpu.VMEM((H, D, DH), BF16),
            pltpu.VMEM((H, DH, D), BF16),
            pltpu.VMEM((D, F + PAD), BF16),
            pltpu.VMEM((D, F + PAD), BF16),
            pltpu.VMEM((F, D + PAD), BF16),
            pltpu.VMEM((S + PR, D), BF16),
            pltpu.VMEM((S, D), F32),
            pltpu.VMEM((PR, 128), F32),
            pltpu.VMEM((2, 5, 8, D), F32),
            pltpu.VMEM((1, D), BF16),
            pltpu.VMEM((8, D), F32),
            pltpu.VMEM((1, D), BF16),
            pltpu.VMEM((8, 128), I32),
            pltpu.VMEM((SUB, DH), BF16),
            pltpu.VMEM((SUB, DH), F32),
            pltpu.VMEM((SUB, DH), F32),
            pltpu.SemaphoreType.DMA((NRB,)),
            pltpu.SemaphoreType.DMA((H,)),
            pltpu.SemaphoreType.DMA((H,)),
            pltpu.SemaphoreType.DMA((H,)),
            pltpu.SemaphoreType.DMA((H,)),
            pltpu.SemaphoreType.DMA((MCH,)),
            pltpu.SemaphoreType.DMA((7,)),
            pltpu.SemaphoreType.DMA((NRB,)),
        ],
        compiler_params=pltpu.CompilerParams(
            vmem_limit_bytes=120 * 1024 * 1024,
        ),
        name="adaln_mha_mod",
    )(
        A_x.reshape(S, D),
        A_k_cache.reshape(H, S, DH),
        A_v_cache.reshape(H, S, DH),
        A_wq,
        A_wo.reshape(H, DH, D),
        B_w_r.reshape(1, D),
        B_w_gate,
        B_w_up,
        B_w_down,
        c,
        w_mod,
    )
    return out.reshape(1, S, D)
```

```python
import jax
import jax.numpy as jnp
from jax import lax
import jax.experimental.pallas as pl
import jax.experimental.pallas.tpu as pltpu

S = 2048
D = 1024
H = 32
DH = 128
F = 3584
SUB = 256
NRB = S // SUB
NU = H * NRB
PR = 16
UM = 8
R2 = 2
R4 = 1
RAMP = 2 * R2 + 4 * R4
NM = (NU - RAMP) // UM
HPI = UM // 2
NLOAD = (2 * H - RAMP) // UM
K_MOD = NLOAD
LN_START = 32
FIN_START = 129
PAD = 128
MCH = 4
EPS = 1e-5
QSCALE = float(DH ** -0.5) * 1.4426950408889634

F32 = jnp.float32
BF16 = jnp.bfloat16
I32 = jnp.int32
NT = (((1,), (1,)), ((), ()))

C_GA, C_SCALE, C_SHIFT, C_KEEP, C_GB = range(5)


def _r(v):
    return v.astype(BF16).astype(F32)


def _rows8(v, fn, c):
    n = v.shape[0] // 8
    return fn(v.reshape(n, 8, D), c[None]).reshape(v.shape)


def _lane_fold(p, fn):
    t = p[:, 0:128]
    for j in range(1, p.shape[1] // 128):
        t = fn(t, p[:, j * 128:(j + 1) * 128])
    return t


def _normalize(pv, ls):
    l = jnp.sum(ls, axis=-1, keepdims=True)
    r = pl.reciprocal(l, approx=True)
    r = r * (2.0 - l * r)
    return (pv * r).astype(BF16)


def _head_of(n):
    if isinstance(n, int):
        return (n % 64) // 2 if n < 192 else (n - 192) % H
    return jnp.where(n < 192, lax.shift_right_logical(n & 63, 1), (n - 192) & (H - 1))


def _row_of(n):
    if isinstance(n, int):
        return SUB * ((n // 64) * 2 + n % 2 if n < 192 else min(n // 32, NRB - 1))
    rb = jnp.where(n < 192, lax.shift_right_logical(n, 6) * 2 + (n & 1),
                   jnp.minimum(lax.shift_right_logical(n, 5), NRB - 1))
    return pl.multiple_of(rb * SUB, SUB)


(SEM_C, SEM_WR, SEM_X0, SEM_X1, SEM_XR, SEM_M12, SEM_FFN, SEM_OUT, SEM_FIX,
 SEM_M0) = range(10)
SEM_RAMP = SEM_M0 + MCH
SEM_MAIN = SEM_RAMP + R2 + R4
NSEM = SEM_MAIN + NLOAD


def _kernel(x_hbm, k_hbm, v_hbm, wq_hbm, wo_hbm, wr_hbm, wg_hbm, wu_hbm, wd_hbm,
            c_hbm, wmod_hbm, out_hbm,
            x_buf, k_buf, v_buf, wq_buf, wo_buf, wa_buf, wb_buf, wd_buf,
            act, acc, r_buf, coef, wr_buf, wr_b, c_buf, zero_buf, o_car, pv_car, ls_car,
            sems):
    def cp(src, dst, slot):
        return pltpu.make_async_copy(src, dst, sems.at[slot])

    def cp_x(b, nb, slot):
        return cp(x_hbm.at[pl.ds(b * SUB, nb * SUB), :],
                  x_buf.at[pl.ds(b * SUB, nb * SUB), :], slot)

    def heads(h0, nh, slot):
        cps = []
        for j in range(nh):
            col = (h0 + j) * DH
            if not isinstance(col, int):
                col = pl.multiple_of(col, DH)
            cps.append(cp(wq_hbm.at[:, pl.ds(col, DH)], wq_buf.at[h0 + j], slot))
        for src, dst in ((k_hbm, k_buf), (v_hbm, v_buf), (wo_hbm, wo_buf)):
            cps.append(cp(src.at[pl.ds(h0, nh)], dst.at[pl.ds(h0, nh)], slot))
        return cps

    def ramp_heads(j):
        return heads(j, 1, SEM_RAMP + j)

    def main_heads(k):
        return heads(RAMP // 2 + k * HPI, HPI, SEM_MAIN + k)

    mrows = D // MCH
    cp_m0 = [cp(wmod_hbm.at[pl.ds(j * mrows, mrows), 0:2 * D],
                wa_buf.at[pl.ds(j * mrows, mrows), 0:2 * D], SEM_M0 + j) for j in range(MCH)]
    cp_c = cp(c_hbm, c_buf, SEM_C)
    cp_wr = cp(wr_hbm, wr_buf, SEM_WR)
    cp_m12 = [cp(wmod_hbm.at[:, 2 * D:3 * D], wa_buf.at[:, 2 * D:3 * D], SEM_M12),
              cp(wmod_hbm.at[:, 3 * D:6 * D], wb_buf.at[:, 0:3 * D], SEM_M12)]
    cp_ffn = [cp(wg_hbm, wa_buf.at[:, 0:F], SEM_FFN),
              cp(wu_hbm, wb_buf.at[:, 0:F], SEM_FFN),
              cp(wd_hbm, wd_buf.at[:, 0:D], SEM_FFN)]

    def cp_out(b):
        row = b * SUB if isinstance(b, int) else pl.multiple_of(b * SUB, SUB)
        return cp(act.at[pl.ds(row, SUB), :], out_hbm.at[pl.ds(row, SUB), :], SEM_OUT)

    def silu_c():
        cf = c_buf[...].astype(F32)
        sc = (cf * _r(jax.nn.sigmoid(cf))).astype(BF16)
        return jnp.broadcast_to(sc, (16, D))

    def packed(ref, h):
        return pltpu.bitcast(ref.bitcast(jnp.uint32)[h], BF16)

    def ada_ln(y, kind):
        m = jnp.mean(y, axis=-1, keepdims=True)
        yc = y - m
        v = jnp.mean(yc * yc, axis=-1, keepdims=True)
        den = _r(jnp.sqrt(_r(_r(v) + EPS)))
        n = (y - _r(m)) * (1.0 / den)
        n = _rows8(n, jnp.multiply, coef[kind, C_SCALE])
        return _rows8(n, jnp.add, coef[kind, C_SHIFT])

    def resid(row, nrows, kind):
        a = _rows8(acc[pl.ds(row, nrows), :], jnp.multiply, coef[kind, C_GA])
        return _r(x_buf[pl.ds(row, nrows), :].astype(F32) + a)

    def piece(src, dst, kind, lane_id):
        y = resid(src, PR, kind)
        hh = ada_ln(y, kind)
        r = jnp.sum(_rows8(hh, jnp.multiply, wr_b[...]), axis=-1, keepdims=True)
        oo = (_rows8(y, jnp.multiply, coef[kind, C_KEEP])
              + _rows8(hh, jnp.multiply, coef[kind, C_GB]))
        act[pl.ds(dst, PR), :] = oo.astype(BF16)
        lane = lax.broadcasted_iota(I32, (PR, 128), 1)
        rn = jnp.where(lane == lane_id, r, r_buf[...])
        r_buf[...] = rn
        return oo, rn

    def unit_piece(n):
        is_ln = jnp.logical_and(n >= LN_START, n < LN_START + (S - 2 * SUB) // PR)
        is_fin = jnp.logical_and(n >= FIN_START, n < FIN_START + (S - SUB) // PR)
        f = n - FIN_START
        src = jnp.where(is_ln, 2 * SUB + (n - LN_START) * PR, jnp.where(is_fin, f * PR, 0))
        dst = jnp.where(jnp.logical_or(is_ln, is_fin), src, S)
        oo, rn = piece(pl.multiple_of(src, PR), pl.multiple_of(dst, PR),
                       is_fin.astype(I32), jnp.where(is_fin, f, -1))
        bits = _lane_fold(pltpu.bitcast(oo, I32), jnp.bitwise_or) | pltpu.bitcast(rn, I32)
        return (bits[0:8] | bits[8:16]) & zero_buf[...]

    def qproj(n):
        q = jnp.dot(act[pl.ds(_row_of(n), SUB), :], packed(wq_buf, _head_of(n)),
                    preferred_element_type=F32)
        return (q * QSCALE).astype(BF16)

    def oproj(o, n):
        acc[pl.ds(_row_of(n), SUB), :] += jnp.dot(o, wo_buf[_head_of(n)],
                                                  preferred_element_type=F32)

    def unit_block(n0, nunits, with_piece):
        o = o_car[...]
        raw = (pv_car[...], ls_car[...])
        for u in range(nunits):
            n = n0 + u
            hd = _head_of(n)
            q = qproj(n)
            oproj(o, max(n - 2, 0) if isinstance(n, int) else jnp.maximum(n - 2, 0))
            z = unit_piece(n) if with_piece else None
            sc = lax.dot_general(q, packed(k_buf, hd), NT, preferred_element_type=F32)
            mm = _lane_fold(sc, jnp.maximum)
            if with_piece:
                mb = pltpu.bitcast(mm, I32)
                mm = pltpu.bitcast(jnp.concatenate([mb[0:8] | z, mb[8:]], axis=0), F32)
            m = jnp.max(mm, axis=-1, keepdims=True)
            p = jnp.exp2(sc - m)
            ls = _lane_fold(p, jnp.add)
            pv = jnp.dot(p.astype(BF16), packed(v_buf, hd), preferred_element_type=F32)
            o = _normalize(*raw)
            raw = (pv, ls)
        o_car[...] = o
        pv_car[...] = raw[0]
        ls_car[...] = raw[1]

    def start(cps):
        for c_ in cps:
            c_.start()

    def wait(cps):
        for c_ in cps:
            c_.wait()

    start([cp_c, cp_x(0, 1, SEM_X0)] + cp_m0 + [cp_x(1, 1, SEM_X1)])
    for j in range(R2):
        start(ramp_heads(j))
    start([cp_wr])
    if R4:
        start(heads(R2, 2, SEM_RAMP + R2))
    n_early = (LN_START - RAMP) // UM
    for k in range(n_early):
        start(main_heads(k))

    def zero_acc(j, carry):
        acc[pl.ds(pl.multiple_of(j * 64, 64), 64), :] = jnp.zeros((64, D), F32)
        return carry

    lax.fori_loop(0, S // 64, zero_acc, 0)
    o_car[...] = jnp.zeros(o_car.shape, BF16)
    pv_car[...] = jnp.zeros(pv_car.shape, F32)
    ls_car[...] = jnp.ones(ls_car.shape, F32)
    r_buf[...] = jnp.zeros(r_buf.shape, F32)
    zero_buf[...] = jnp.zeros(zero_buf.shape, I32)
    coef[0, C_GA] = jnp.zeros((8, D), F32)
    coef[0, C_KEEP] = jnp.zeros((8, D), F32)
    coef[0, C_GB] = jnp.ones((8, D), F32)
    coef[1, C_KEEP] = jnp.ones((8, D), F32)
    cp_c.wait()
    sc16 = silu_c()
    m0 = None
    for j in range(MCH):
        cp_m0[j].wait()
        part = jnp.dot(sc16[:, j * mrows:(j + 1) * mrows],
                       wa_buf[j * mrows:(j + 1) * mrows, 0:2 * D], preferred_element_type=F32)
        m0 = part if m0 is None else m0 + part
    m0 = _r(m0[0:8, :])
    coef[0, C_SHIFT] = m0[:, 0:D]
    coef[0, C_SCALE] = _r(1.0 + m0[:, D:2 * D])
    for b in range(2):
        cp_x(b, 1, SEM_X0 + b).wait()
        for j in range(SUB // 64):
            row = b * SUB + j * 64
            act[row:row + 64, :] = ada_ln(x_buf[row:row + 64, :].astype(F32), 0).astype(BF16)

    def ramp2(j, carry):
        wait(ramp_heads(j))
        unit_block(2 * j, 2, False)
        return carry

    lax.fori_loop(0, R2, ramp2, 0)
    start([cp_x(2, NRB - 2, SEM_XR)])
    for k in range(n_early, NLOAD):
        start(main_heads(k))
    start(cp_m12)
    cp_wr.wait()
    w8 = wr_buf[...].astype(F32)
    for j in range(D // 128):
        wr_b[:, j * 128:(j + 1) * 128] = jnp.broadcast_to(w8[j:j + 1, :], (8, 128))
    if R4:
        wait(heads(R2, 2, SEM_RAMP + R2))
        unit_block(2 * R2, 4, False)

    def blocks_done(n0):
        return (n0 - FIN_START) // (SUB // PR)

    def main(k, carry):
        n0 = RAMP + k * UM

        @pl.when(k <= K_MOD)
        def _():
            @pl.when(k < NLOAD)
            def _():
                wait(main_heads(k))

            @pl.when(k == n_early)
            def _():
                cp_x(2, NRB - 2, SEM_XR).wait()

            @pl.when(k == K_MOD)
            def _():
                wait(cp_m12)
                sc = silu_c()
                m1 = _r(jnp.dot(sc, wa_buf[:, 2 * D:3 * D], preferred_element_type=F32)[0:8, :])
                m2 = _r(jnp.dot(sc, wb_buf[:, 0:3 * D], preferred_element_type=F32)[0:8, :])
                coef[1, C_GA] = m1
                coef[1, C_SHIFT] = m2[:, 0:D]
                coef[1, C_SCALE] = _r(1.0 + m2[:, D:2 * D])
                coef[1, C_GB] = m2[:, 2 * D:3 * D]
                start(cp_ffn)

        done = lax.shift_right_arithmetic(n0 - FIN_START, 4)
        done_before = lax.shift_right_arithmetic(n0 - UM - FIN_START, 4)

        @pl.when(jnp.logical_and(done >= 1, done > done_before))
        def _():
            cp_out(jnp.maximum(done - 1, 0)).start()

        unit_block(n0, UM, True)
        return carry

    lax.fori_loop(0, NM, main, 0)

    for b in range(blocks_done(RAMP + (NM - 1) * UM), NRB - 1):
        cp_out(b).start()
    oproj(o_car[...], NU - 2)
    oproj(_normalize(pv_car[...], ls_car[...]), NU - 1)
    for j in range(SUB // PR):
        row = (NRB - 1) * SUB + j * PR
        piece(row, row, 1, row // PR)
    cp_out(NRB - 1).start()

    rr = r_buf[...]
    ridx = (lax.broadcasted_iota(I32, (PR, 128), 1) * PR
            + lax.broadcasted_iota(I32, (PR, 128), 0))
    big = jnp.int32(S - 1)
    m1 = jnp.max(jnp.max(rr, axis=0, keepdims=True), axis=1, keepdims=True)
    i1 = jnp.min(jnp.where(rr == m1, ridx, big))
    rr2 = jnp.where(ridx == i1, -jnp.inf, rr)
    m2 = jnp.max(jnp.max(rr2, axis=0, keepdims=True), axis=1, keepdims=True)
    i2 = jnp.min(jnp.where(jnp.logical_and(rr2 == m2, ridx != i1), ridx, big))

    rowid = lax.broadcasted_iota(I32, (PR, D), 0)
    g1 = pl.multiple_of(lax.shift_right_logical(i1, 4) * PR, PR)
    g2 = pl.multiple_of(lax.shift_right_logical(i2, 4) * PR, PR)
    x2a = resid(g1, PR, 1)
    x2b = resid(g2, PR, 1)
    h2a = _r(ada_ln(x2a, 1))
    h2b = _r(ada_ln(x2b, 1))
    row1 = jnp.sum(jnp.where(rowid + g1 == i1, h2a, 0.0), axis=0, keepdims=True)
    row2 = jnp.sum(jnp.where(rowid + g2 == i2, h2b, 0.0), axis=0, keepdims=True)
    xs = jnp.where(rowid == 0, row1, row2).astype(BF16)

    wait(cp_ffn)
    gt = _r(jnp.dot(xs, wa_buf[:, 0:F], preferred_element_type=F32))
    up = _r(jnp.dot(xs, wb_buf[:, 0:F], preferred_element_type=F32))
    hid = (_r(gt * _r(jax.nn.sigmoid(gt))) * up).astype(BF16)
    y = _r(jnp.dot(hid, wd_buf[:, 0:D], preferred_element_type=F32))
    y1 = _r(y[0:1, :] * _r(jax.nn.sigmoid(_r(m1))))
    y2 = _r(y[1:2, :] * _r(jax.nn.sigmoid(_r(m2))))

    def fix(x2g, h2g, gbase):
        rid = rowid + gbase
        upd = jnp.where(rid == i1, y1, jnp.where(rid == i2, y2, 0.0))
        return (x2g + _rows8(h2g + upd, jnp.multiply, coef[1, C_GB])).astype(BF16)

    for b in range(NRB):
        cp_out(b).wait()
    act[pl.ds(g1, PR), :] = fix(x2a, h2a, g1)
    act[pl.ds(g2, PR), :] = fix(x2b, h2b, g2)
    f1 = cp(act.at[pl.ds(g1, PR), :], out_hbm.at[pl.ds(g1, PR), :], SEM_OUT)
    f2 = cp(act.at[pl.ds(g2, PR), :], out_hbm.at[pl.ds(g2, PR), :], SEM_FIX)
    f1.start()

    @pl.when(g1 != g2)
    def _():
        f2.start()
        f2.wait()

    f1.wait()


@jax.jit
def pallas_adaLN_cond__mha_block_cached__moe_arch_mod__prompt_kernel(
    A_x: jax.Array,
    A_k_cache: jax.Array,
    A_v_cache: jax.Array,
    A_wq: jax.Array,
    A_wo: jax.Array,
    B_x: jax.Array,
    B_w_r: jax.Array,
    B_w_gate: jax.Array,
    B_w_up: jax.Array,
    B_w_down: jax.Array,
    c: jax.Array,
    w_mod: jax.Array,
):
    del B_x
    hbm = pl.BlockSpec(memory_space=pl.ANY)
    out = pl.pallas_call(
        _kernel,
        in_specs=[hbm] * 11,
        out_specs=hbm,
        out_shape=jax.ShapeDtypeStruct((S, D), BF16),
        scratch_shapes=[
            pltpu.VMEM((S, D), BF16),
            pltpu.VMEM((H, S, DH), BF16),
            pltpu.VMEM((H, S, DH), BF16),
            pltpu.VMEM((H, D, DH), BF16),
            pltpu.VMEM((H, DH, D), BF16),
            pltpu.VMEM((D, F + PAD), BF16),
            pltpu.VMEM((D, F + PAD), BF16),
            pltpu.VMEM((F, D + PAD), BF16),
            pltpu.VMEM((S + PR, D), BF16),
            pltpu.VMEM((S, D), F32),
            pltpu.VMEM((PR, 128), F32),
            pltpu.VMEM((2, 5, 8, D), F32),
            pltpu.VMEM((8, 128), BF16),
            pltpu.VMEM((8, D), F32),
            pltpu.VMEM((1, D), BF16),
            pltpu.VMEM((8, 128), I32),
            pltpu.VMEM((SUB, DH), BF16),
            pltpu.VMEM((SUB, DH), F32),
            pltpu.VMEM((SUB, DH), F32),
            pltpu.SemaphoreType.DMA((NSEM,)),
        ],
        compiler_params=pltpu.CompilerParams(
            vmem_limit_bytes=120 * 1024 * 1024,
        ),
        name="adaln_mha_mod",
    )(
        A_x.reshape(S, D),
        A_k_cache.reshape(H, S, DH),
        A_v_cache.reshape(H, S, DH),
        A_wq,
        A_wo.reshape(H, DH, D),
        B_w_r.reshape(8, 128),
        B_w_gate,
        B_w_up,
        B_w_down,
        c,
        w_mod,
    )
    return out.reshape(1, S, D)
```

```python
import jax
import jax.numpy as jnp
from jax import lax
import jax.experimental.pallas as pl
import jax.experimental.pallas.tpu as pltpu

S = 2048
D = 1024
H = 32
DH = 128
F = 3584
SUB = 256
NRB = S // SUB
NU = H * NRB
PR = 16
UM = 12
R2 = 8
R4 = 0
RAMP = 2 * R2 + 4 * R4
NM = (NU - RAMP) // UM
HPI = UM // 2
NLOAD = (2 * H - RAMP) // UM
K_MOD = NLOAD
LN_START = 32
FIN_START = 129
FILL = 48
PAD = 128
MCH = 4
EPS = 1e-5
QSCALE = float(DH ** -0.5) * 1.4426950408889634

F32 = jnp.float32
BF16 = jnp.bfloat16
I32 = jnp.int32
NT = (((1,), (1,)), ((), ()))

C_GA, C_SCALE, C_SHIFT, C_KEEP, C_GB = range(5)


def _r(v):
    return v.astype(BF16).astype(F32)


def _rows8(v, fn, c):
    n = v.shape[0] // 8
    return fn(v.reshape(n, 8, D), c[None]).reshape(v.shape)


def _lane_fold(p, fn):
    t = p[:, 0:128]
    for j in range(1, p.shape[1] // 128):
        t = fn(t, p[:, j * 128:(j + 1) * 128])
    return t


def _normalize(pv, ls):
    l = jnp.sum(ls, axis=-1, keepdims=True)
    r = pl.reciprocal(l, approx=True)
    r = r * (2.0 - l * r)
    return (pv * r).astype(BF16)


def _head_of(n):
    if isinstance(n, int):
        return (n % 64) // 2 if n < 192 else (n - 192) % H
    return jnp.where(n < 192, lax.shift_right_logical(n & 63, 1), (n - 192) & (H - 1))


def _row_of(n):
    if isinstance(n, int):
        return SUB * ((n // 64) * 2 + n % 2 if n < 192 else min(n // 32, NRB - 1))
    rb = jnp.where(n < 192, lax.shift_right_logical(n, 6) * 2 + (n & 1),
                   jnp.minimum(lax.shift_right_logical(n, 5), NRB - 1))
    return pl.multiple_of(rb * SUB, SUB)


(SEM_C, SEM_WR, SEM_X0, SEM_X1, SEM_XR, SEM_M12, SEM_FFN, SEM_OUT, SEM_FIX,
 SEM_WQ0, SEM_M0) = range(11)
SEM_RAMP = SEM_M0 + MCH
SEM_MAIN = SEM_RAMP + R2 + R4
NSEM = SEM_MAIN + NLOAD


def _kernel(x_hbm, k_hbm, v_hbm, wq_hbm, wo_hbm, wr_hbm, wg_hbm, wu_hbm, wd_hbm,
            c_hbm, wmod_hbm, out_hbm,
            x_buf, k_buf, v_buf, wq_buf, wo_buf, wa_buf, wb_buf, wd_buf,
            act, acc, r_buf, coef, wr_buf, wr_b, c_buf, zero_buf, qa_car, pv_car, ls_car,
            sems):
    def cp(src, dst, slot):
        return pltpu.make_async_copy(src, dst, sems.at[slot])

    def cp_x(b, nb, slot):
        return cp(x_hbm.at[pl.ds(b * SUB, nb * SUB), :],
                  x_buf.at[pl.ds(b * SUB, nb * SUB), :], slot)

    def cp_wq(h, slot):
        col = h * DH if isinstance(h, int) else pl.multiple_of(h * DH, DH)
        return cp(wq_hbm.at[:, pl.ds(col, DH)], wq_buf.at[h], slot)

    def heads(h0, nh, slot, nq=None):
        cps = [cp(src.at[pl.ds(h0, nh)], dst.at[pl.ds(h0, nh)], slot)
               for src, dst in ((k_hbm, k_buf), (v_hbm, v_buf), (wo_hbm, wo_buf))]
        return cps + [cp_wq(h0 + 1 + j, slot) for j in range(nh if nq is None else nq)]

    def ramp_heads(j):
        return heads(j, 1, SEM_RAMP + j)

    def main_heads(k, last=False):
        return heads(RAMP // 2 + k * HPI, HPI, SEM_MAIN + k, HPI - 1 if last else HPI)

    mrows = D // MCH
    cp_m0 = [cp(wmod_hbm.at[pl.ds(j * mrows, mrows), 0:2 * D],
                wa_buf.at[pl.ds(j * mrows, mrows), 0:2 * D], SEM_M0 + j) for j in range(MCH)]
    cp_c = cp(c_hbm, c_buf, SEM_C)
    cp_wr = cp(wr_hbm, wr_buf, SEM_WR)
    cp_m12 = [cp(wmod_hbm.at[:, 2 * D:3 * D], wa_buf.at[:, 2 * D:3 * D], SEM_M12),
              cp(wmod_hbm.at[:, 3 * D:6 * D], wb_buf.at[:, 0:3 * D], SEM_M12)]
    cp_ffn = [cp(wg_hbm, wa_buf.at[:, 0:F], SEM_FFN),
              cp(wu_hbm, wb_buf.at[:, 0:F], SEM_FFN),
              cp(wd_hbm, wd_buf.at[:, 0:D], SEM_FFN)]

    def cp_out(b):
        row = b * SUB if isinstance(b, int) else pl.multiple_of(b * SUB, SUB)
        return cp(act.at[pl.ds(row, SUB), :], out_hbm.at[pl.ds(row, SUB), :], SEM_OUT)

    def silu_c():
        cf = c_buf[...].astype(F32)
        sc = (cf * _r(jax.nn.sigmoid(cf))).astype(BF16)
        return jnp.broadcast_to(sc, (16, D))

    def packed(ref, h):
        return pltpu.bitcast(ref.bitcast(jnp.uint32)[h], BF16)

    def ada_ln(y, kind):
        m = jnp.mean(y, axis=-1, keepdims=True)
        yc = y - m
        v = jnp.mean(yc * yc, axis=-1, keepdims=True)
        den = _r(jnp.sqrt(_r(_r(v) + EPS)))
        n = (y - _r(m)) * (1.0 / den)
        n = _rows8(n, jnp.multiply, coef[kind, C_SCALE])
        return _rows8(n, jnp.add, coef[kind, C_SHIFT])

    def resid(row, nrows, kind):
        a = _rows8(acc[pl.ds(row, nrows), :], jnp.multiply, coef[kind, C_GA])
        return _r(x_buf[pl.ds(row, nrows), :].astype(F32) + a)

    def piece(src, dst, kind, lane_id):
        y = resid(src, PR, kind)
        hh = ada_ln(y, kind)
        r = jnp.sum(_rows8(hh, jnp.multiply, wr_b[...]), axis=-1, keepdims=True)
        oo = (_rows8(y, jnp.multiply, coef[kind, C_KEEP])
              + _rows8(hh, jnp.multiply, coef[kind, C_GB]))
        act[pl.ds(dst, PR), :] = oo.astype(BF16)
        lane = lax.broadcasted_iota(I32, (PR, 128), 1)
        rn = jnp.where(lane == lane_id, r, r_buf[...])
        r_buf[...] = rn
        return oo, rn

    def unit_piece(n):
        is_ln = jnp.logical_and(n >= LN_START, n < LN_START + (S - 2 * SUB) // PR)
        is_fin = jnp.logical_and(n >= FIN_START, n < FIN_START + (S - SUB) // PR)
        f = n - FIN_START
        src = jnp.where(is_ln, 2 * SUB + (n - LN_START) * PR, jnp.where(is_fin, f * PR, 0))
        dst = jnp.where(jnp.logical_or(is_ln, is_fin), src, S)
        oo, rn = piece(pl.multiple_of(src, PR), pl.multiple_of(dst, PR),
                       is_fin.astype(I32), jnp.where(is_fin, f, -1))
        bits = _lane_fold(pltpu.bitcast(oo, I32), jnp.bitwise_or) | pltpu.bitcast(rn, I32)
        return (bits[0:8] | bits[8:16]) & zero_buf[...]

    def qproj_head(n):
        return jnp.dot(act[pl.ds(_row_of(n), FILL), 0:D // 2],
                       packed(wq_buf, _head_of(n))[0:D // 2], preferred_element_type=F32)

    def qproj_rest(n, qa):
        row = _row_of(n)
        w = packed(wq_buf, _head_of(n))
        row2 = row + FILL if isinstance(row, int) else pl.multiple_of(row + FILL, 16)
        qb = jnp.dot(act[pl.ds(row, SUB), D // 2:D], w[D // 2:D], preferred_element_type=F32)
        qc = jnp.dot(act[pl.ds(row2, SUB - FILL), 0:D // 2], w[0:D // 2],
                     preferred_element_type=F32)
        return ((qb + jnp.concatenate([qa, qc], axis=0)) * QSCALE).astype(BF16)

    def oproj(o, n):
        acc[pl.ds(_row_of(n), SUB), :] += jnp.dot(o, wo_buf[_head_of(n)],
                                                  preferred_element_type=F32)

    def unit_block(n0, nunits, with_piece):
        o = _normalize(pv_car[0], ls_car[0])
        raw = (pv_car[1], ls_car[1])
        qa = qa_car[...]
        for u in range(nunits):
            n = n0 + u
            hd = _head_of(n)
            q = qproj_rest(n, qa)
            oproj(o, max(n - 2, 0) if isinstance(n, int) else jnp.maximum(n - 2, 0))
            z = unit_piece(n) if with_piece else None
            sc = lax.dot_general(q, packed(k_buf, hd), NT, preferred_element_type=F32)
            qa = qproj_head(n + 1)
            mm = _lane_fold(sc, jnp.maximum)
            if with_piece:
                mb = pltpu.bitcast(mm, I32)
                mm = pltpu.bitcast(jnp.concatenate([mb[0:8] | z, mb[8:]], axis=0), F32)
            m = jnp.max(mm, axis=-1, keepdims=True)
            p = jnp.exp2(sc - m)
            ls = _lane_fold(p, jnp.add)
            pv = jnp.dot(p.astype(BF16), packed(v_buf, hd), preferred_element_type=F32)
            if u + 1 < nunits:
                zb = (pltpu.bitcast(pv, I32).reshape(SUB // 8, 8, 128)
                      & zero_buf[...][None]).reshape(SUB, 128)
                o = _normalize(raw[0], pltpu.bitcast(pltpu.bitcast(raw[1], I32) | zb, F32))
            else:
                pv_car[0] = raw[0]
                ls_car[0] = raw[1]
            raw = (pv, ls)
        pv_car[1] = raw[0]
        ls_car[1] = raw[1]
        qa_car[...] = qa

    def start(cps):
        for c_ in cps:
            c_.start()

    def wait(cps):
        for c_ in cps:
            c_.wait()

    start([cp_c, cp_x(0, 1, SEM_X0)] + cp_m0 + [cp_wq(0, SEM_WQ0), cp_x(1, 1, SEM_X1)])
    for j in range(R2):
        start(ramp_heads(j))
    start([cp_wr])
    if R4:
        start(heads(R2, 2, SEM_RAMP + R2))
    n_early = (LN_START - RAMP) // UM
    for k in range(n_early):
        start(main_heads(k))

    def zero_acc(j, carry):
        acc[pl.ds(pl.multiple_of(j * 64, 64), 64), :] = jnp.zeros((64, D), F32)
        return carry

    lax.fori_loop(0, S // 64, zero_acc, 0)
    pv_car[...] = jnp.zeros(pv_car.shape, F32)
    ls_car[...] = jnp.ones(ls_car.shape, F32)
    r_buf[...] = jnp.zeros(r_buf.shape, F32)
    zero_buf[...] = jnp.zeros(zero_buf.shape, I32)
    coef[0, C_GA] = jnp.zeros((8, D), F32)
    coef[0, C_KEEP] = jnp.zeros((8, D), F32)
    coef[0, C_GB] = jnp.ones((8, D), F32)
    coef[1, C_KEEP] = jnp.ones((8, D), F32)
    cp_c.wait()
    sc16 = silu_c()
    m0 = None
    for j in range(MCH):
        cp_m0[j].wait()
        part = jnp.dot(sc16[:, j * mrows:(j + 1) * mrows],
                       wa_buf[j * mrows:(j + 1) * mrows, 0:2 * D], preferred_element_type=F32)
        m0 = part if m0 is None else m0 + part
    m0 = _r(m0[0:8, :])
    coef[0, C_SHIFT] = m0[:, 0:D]
    coef[0, C_SCALE] = _r(1.0 + m0[:, D:2 * D])
    for b in range(2):
        cp_x(b, 1, SEM_X0 + b).wait()
        for j in range(SUB // 64):
            row = b * SUB + j * 64
            act[row:row + 64, :] = ada_ln(x_buf[row:row + 64, :].astype(F32), 0).astype(BF16)
        if b == 0:
            cp_wq(0, SEM_WQ0).wait()
            qa_car[...] = qproj_head(0)

    def ramp2(j, carry):
        wait(ramp_heads(j))
        unit_block(2 * j, 2, False)
        return carry

    lax.fori_loop(0, R2, ramp2, 0)
    start([cp_x(2, NRB - 2, SEM_XR)])
    for k in range(n_early, NLOAD):
        start(main_heads(k, k == NLOAD - 1))
    start(cp_m12)
    cp_wr.wait()
    w8 = wr_buf[...].astype(F32)
    for j in range(D // 128):
        wr_b[:, j * 128:(j + 1) * 128] = jnp.broadcast_to(w8[j:j + 1, :], (8, 128))
    if R4:
        wait(heads(R2, 2, SEM_RAMP + R2))
        unit_block(2 * R2, 4, False)

    def blocks_done(n0):
        return (n0 - FIN_START) // (SUB // PR)

    def main(k, carry):
        n0 = RAMP + k * UM

        @pl.when(k <= K_MOD)
        def _():
            @pl.when(k < NLOAD - 1)
            def _():
                wait(main_heads(k))

            @pl.when(k == NLOAD - 1)
            def _():
                wait(main_heads(NLOAD - 1, True))

            @pl.when(k == n_early)
            def _():
                cp_x(2, NRB - 2, SEM_XR).wait()

            @pl.when(k == K_MOD)
            def _():
                wait(cp_m12)
                sc = silu_c()
                m1 = _r(jnp.dot(sc, wa_buf[:, 2 * D:3 * D], preferred_element_type=F32)[0:8, :])
                m2 = _r(jnp.dot(sc, wb_buf[:, 0:3 * D], preferred_element_type=F32)[0:8, :])
                coef[1, C_GA] = m1
                coef[1, C_SHIFT] = m2[:, 0:D]
                coef[1, C_SCALE] = _r(1.0 + m2[:, D:2 * D])
                coef[1, C_GB] = m2[:, 2 * D:3 * D]
                start(cp_ffn)

        done = lax.shift_right_arithmetic(n0 - FIN_START, 4)
        done_before = lax.shift_right_arithmetic(n0 - UM - FIN_START, 4)

        @pl.when(jnp.logical_and(done >= 1, done > done_before))
        def _():
            cp_out(jnp.maximum(done - 1, 0)).start()

        unit_block(n0, UM, True)
        return carry

    lax.fori_loop(0, NM, main, 0)

    for b in range(blocks_done(RAMP + (NM - 1) * UM), NRB - 1):
        cp_out(b).start()
    oproj(_normalize(pv_car[0], ls_car[0]), NU - 2)
    oproj(_normalize(pv_car[1], ls_car[1]), NU - 1)
    for j in range(SUB // PR):
        row = (NRB - 1) * SUB + j * PR
        piece(row, row, 1, row // PR)
    cp_out(NRB - 1).start()

    rr = r_buf[...]
    ridx = (lax.broadcasted_iota(I32, (PR, 128), 1) * PR
            + lax.broadcasted_iota(I32, (PR, 128), 0))
    big = jnp.int32(S - 1)
    m1 = jnp.max(jnp.max(rr, axis=0, keepdims=True), axis=1, keepdims=True)
    i1 = jnp.min(jnp.where(rr == m1, ridx, big))
    rr2 = jnp.where(ridx == i1, -jnp.inf, rr)
    m2 = jnp.max(jnp.max(rr2, axis=0, keepdims=True), axis=1, keepdims=True)
    i2 = jnp.min(jnp.where(jnp.logical_and(rr2 == m2, ridx != i1), ridx, big))

    rowid = lax.broadcasted_iota(I32, (PR, D), 0)
    g1 = pl.multiple_of(lax.shift_right_logical(i1, 4) * PR, PR)
    g2 = pl.multiple_of(lax.shift_right_logical(i2, 4) * PR, PR)
    x2a = resid(g1, PR, 1)
    x2b = resid(g2, PR, 1)
    h2a = _r(ada_ln(x2a, 1))
    h2b = _r(ada_ln(x2b, 1))
    row1 = jnp.sum(jnp.where(rowid + g1 == i1, h2a, 0.0), axis=0, keepdims=True)
    row2 = jnp.sum(jnp.where(rowid + g2 == i2, h2b, 0.0), axis=0, keepdims=True)
    xs = jnp.where(rowid == 0, row1, row2).astype(BF16)

    wait(cp_ffn)
    gt = _r(jnp.dot(xs, wa_buf[:, 0:F], preferred_element_type=F32))
    up = _r(jnp.dot(xs, wb_buf[:, 0:F], preferred_element_type=F32))
    hid = (_r(gt * _r(jax.nn.sigmoid(gt))) * up).astype(BF16)
    y = _r(jnp.dot(hid, wd_buf[:, 0:D], preferred_element_type=F32))
    y1 = _r(y[0:1, :] * _r(jax.nn.sigmoid(_r(m1))))
    y2 = _r(y[1:2, :] * _r(jax.nn.sigmoid(_r(m2))))

    def fix(x2g, h2g, gbase):
        rid = rowid + gbase
        upd = jnp.where(rid == i1, y1, jnp.where(rid == i2, y2, 0.0))
        return (x2g + _rows8(h2g + upd, jnp.multiply, coef[1, C_GB])).astype(BF16)

    for b in range(NRB):
        cp_out(b).wait()
    act[pl.ds(g1, PR), :] = fix(x2a, h2a, g1)
    act[pl.ds(g2, PR), :] = fix(x2b, h2b, g2)
    f1 = cp(act.at[pl.ds(g1, PR), :], out_hbm.at[pl.ds(g1, PR), :], SEM_OUT)
    f2 = cp(act.at[pl.ds(g2, PR), :], out_hbm.at[pl.ds(g2, PR), :], SEM_FIX)
    f1.start()

    @pl.when(g1 != g2)
    def _():
        f2.start()
        f2.wait()

    f1.wait()


@jax.jit
def pallas_adaLN_cond__mha_block_cached__moe_arch_mod__prompt_kernel(
    A_x: jax.Array,
    A_k_cache: jax.Array,
    A_v_cache: jax.Array,
    A_wq: jax.Array,
    A_wo: jax.Array,
    B_x: jax.Array,
    B_w_r: jax.Array,
    B_w_gate: jax.Array,
    B_w_up: jax.Array,
    B_w_down: jax.Array,
    c: jax.Array,
    w_mod: jax.Array,
):
    del B_x
    hbm = pl.BlockSpec(memory_space=pl.ANY)
    out = pl.pallas_call(
        _kernel,
        in_specs=[hbm] * 11,
        out_specs=hbm,
        out_shape=jax.ShapeDtypeStruct((S, D), BF16),
        scratch_shapes=[
            pltpu.VMEM((S, D), BF16),
            pltpu.VMEM((H, S, DH), BF16),
            pltpu.VMEM((H, S, DH), BF16),
            pltpu.VMEM((H, D, DH), BF16),
            pltpu.VMEM((H, DH, D), BF16),
            pltpu.VMEM((D, F + PAD), BF16),
            pltpu.VMEM((D, F + PAD), BF16),
            pltpu.VMEM((F, D + PAD), BF16),
            pltpu.VMEM((S + PR, D), BF16),
            pltpu.VMEM((S, D), F32),
            pltpu.VMEM((PR, 128), F32),
            pltpu.VMEM((2, 5, 8, D), F32),
            pltpu.VMEM((8, 128), BF16),
            pltpu.VMEM((8, D), F32),
            pltpu.VMEM((1, D), BF16),
            pltpu.VMEM((8, 128), I32),
            pltpu.VMEM((FILL, DH), F32),
            pltpu.VMEM((2, SUB, DH), F32),
            pltpu.VMEM((2, SUB, DH), F32),
            pltpu.SemaphoreType.DMA((NSEM,)),
        ],
        compiler_params=pltpu.CompilerParams(
            vmem_limit_bytes=120 * 1024 * 1024,
        ),
        name="adaln_mha_mod",
    )(
        A_x.reshape(S, D),
        A_k_cache.reshape(H, S, DH),
        A_v_cache.reshape(H, S, DH),
        A_wq,
        A_wo.reshape(H, DH, D),
        B_w_r.reshape(8, 128),
        B_w_gate,
        B_w_up,
        B_w_down,
        c,
        w_mod,
    )
    return out.reshape(1, S, D)
```

```python
import jax
import jax.numpy as jnp
from jax import lax
import jax.experimental.pallas as pl
import jax.experimental.pallas.tpu as pltpu

S = 2048
D = 1024
H = 32
DH = 128
F = 3584
SUB = 256
NRB = S // SUB
NU = H * NRB
PR = 16
UM = 12
R2 = 8
RAMP = 2 * R2
NM = (NU - RAMP) // UM
HPI = UM // 2
NLOAD = (2 * H - RAMP) // UM
K_MOD = NLOAD
LN_START = 32
FIN_START = 129
FILL = 48
PAD = 128
MCH = 4
EPS = 1e-5
QSCALE = float(DH ** -0.5) * 1.4426950408889634

F32 = jnp.float32
BF16 = jnp.bfloat16
I32 = jnp.int32
NT = (((1,), (1,)), ((), ()))

C_GA, C_SCALE, C_SHIFT, C_KEEP, C_GB = range(5)


def _r(v):
    return v.astype(BF16).astype(F32)


def _rows8(v, fn, c):
    n = v.shape[0] // 8
    return fn(v.reshape(n, 8, D), c[None]).reshape(v.shape)


def _layernorm(y):
    m = jnp.mean(y, axis=-1, keepdims=True)
    yc = y - m
    v = jnp.mean(yc * yc, axis=-1, keepdims=True)
    den = _r(jnp.sqrt(_r(_r(v) + EPS)))
    return (y - _r(m)) * (1.0 / den)


def _lane_fold(p, fn):
    t = p[:, 0:128]
    for j in range(1, p.shape[1] // 128):
        t = fn(t, p[:, j * 128:(j + 1) * 128])
    return t


def _normalize(pv, ls):
    l = jnp.sum(ls, axis=-1, keepdims=True)
    r = pl.reciprocal(l, approx=True)
    r = r * (2.0 - l * r)
    return (pv * r).astype(BF16)


def _head_of(n):
    if isinstance(n, int):
        return (n % 64) // 2 if n < 192 else (n - 192) % H
    return jnp.where(n < 192, lax.shift_right_logical(n & 63, 1), (n - 192) & (H - 1))


def _row_of(n):
    if isinstance(n, int):
        return SUB * ((n // 64) * 2 + n % 2 if n < 192 else min(n // 32, NRB - 1))
    rb = jnp.where(n < 192, lax.shift_right_logical(n, 6) * 2 + (n & 1),
                   jnp.minimum(lax.shift_right_logical(n, 5), NRB - 1))
    return pl.multiple_of(rb * SUB, SUB)


(SEM_C, SEM_WR, SEM_X0, SEM_XR, SEM_M12, SEM_FFN, SEM_OUT, SEM_FIX,
 SEM_WQ0, SEM_K0, SEM_M0) = range(11)
SEM_RAMP = SEM_M0 + MCH
SEM_MAIN = SEM_RAMP + R2
NSEM = SEM_MAIN + NLOAD


def _kernel(x_hbm, k_hbm, v_hbm, wq_hbm, wo_hbm, wr_hbm, wg_hbm, wu_hbm, wd_hbm,
            c_hbm, wmod_hbm, out_hbm,
            x_buf, k_buf, v_buf, wq_buf, wo_buf, wa_buf, wb_buf, wd_buf,
            act, acc, n_buf, r_buf, coef, wr_buf, wr_b, c_buf, zero_buf, qa_car, pv_car, ls_car,
            sems):
    def cp(src, dst, slot):
        return pltpu.make_async_copy(src, dst, sems.at[slot])

    def cp_x(b, nb, slot):
        return cp(x_hbm.at[pl.ds(b * SUB, nb * SUB), :],
                  x_buf.at[pl.ds(b * SUB, nb * SUB), :], slot)

    def cp_wq(h, slot):
        col = h * DH if isinstance(h, int) else pl.multiple_of(h * DH, DH)
        return cp(wq_hbm.at[:, pl.ds(col, DH)], wq_buf.at[h], slot)

    def cp_h(src, dst, h0, nh, slot):
        return cp(src.at[pl.ds(h0, nh)], dst.at[pl.ds(h0, nh)], slot)

    def heads(h0, nh, slot, last=False):
        return [cp_h(k_hbm, k_buf, h0, nh, slot), cp_h(v_hbm, v_buf, h0, nh, slot),
                cp_h(wo_hbm, wo_buf, h0 - 1, nh + 1 if last else nh, slot)] + [
            cp_wq(h0 + 1 + j, slot) for j in range(nh - 1 if last else nh)]

    def ramp_heads(j):
        return heads(j, 1, SEM_RAMP + j)

    def main_heads(k, last=False):
        return heads(RAMP // 2 + k * HPI, HPI, SEM_MAIN + k, last)

    cp_k0 = cp_h(k_hbm, k_buf, 0, 1, SEM_K0)
    cp_v0 = [cp_h(v_hbm, v_buf, 0, 1, SEM_RAMP), cp_wq(1, SEM_RAMP)]
    mrows = D // MCH
    cp_m0 = [cp(wmod_hbm.at[pl.ds(j * mrows, mrows), 0:2 * D],
                wa_buf.at[pl.ds(j * mrows, mrows), 0:2 * D], SEM_M0 + j) for j in range(MCH)]
    cp_c = cp(c_hbm, c_buf, SEM_C)
    cp_wr = cp(wr_hbm, wr_buf, SEM_WR)
    cp_m12 = [cp(wmod_hbm.at[:, 2 * D:3 * D], wa_buf.at[:, 2 * D:3 * D], SEM_M12),
              cp(wmod_hbm.at[:, 3 * D:6 * D], wb_buf.at[:, 0:3 * D], SEM_M12)]
    cp_ffn = [cp(wg_hbm, wa_buf.at[:, 0:F], SEM_FFN),
              cp(wu_hbm, wb_buf.at[:, 0:F], SEM_FFN),
              cp(wd_hbm, wd_buf.at[:, 0:D], SEM_FFN)]

    def cp_out(b):
        row = b * SUB if isinstance(b, int) else pl.multiple_of(b * SUB, SUB)
        return cp(act.at[pl.ds(row, SUB), :], out_hbm.at[pl.ds(row, SUB), :], SEM_OUT)

    def silu_c():
        cf = c_buf[...].astype(F32)
        sc = (cf * _r(jax.nn.sigmoid(cf))).astype(BF16)
        return jnp.broadcast_to(sc, (16, D))

    def packed(ref, h):
        return pltpu.bitcast(ref.bitcast(jnp.uint32)[h], BF16)

    def modulate(n, kind):
        n = _rows8(n, jnp.multiply, coef[kind, C_SCALE])
        return _rows8(n, jnp.add, coef[kind, C_SHIFT])

    def ada_ln(y, kind):
        return modulate(_layernorm(y), kind)

    def resid(row, nrows, kind):
        a = _rows8(acc[pl.ds(row, nrows), :], jnp.multiply, coef[kind, C_GA])
        return _r(x_buf[pl.ds(row, nrows), :].astype(F32) + a)

    def piece(src, dst, kind, lane_id):
        y = resid(src, PR, kind)
        hh = ada_ln(y, kind)
        r = jnp.sum(_rows8(hh, jnp.multiply, wr_b[...]), axis=-1, keepdims=True)
        oo = (_rows8(y, jnp.multiply, coef[kind, C_KEEP])
              + _rows8(hh, jnp.multiply, coef[kind, C_GB]))
        act[pl.ds(dst, PR), :] = oo.astype(BF16)
        lane = lax.broadcasted_iota(I32, (PR, 128), 1)
        rn = jnp.where(lane == lane_id, r, r_buf[...])
        r_buf[...] = rn
        return oo, rn

    def unit_piece(n):
        is_ln = jnp.logical_and(n >= LN_START, n < LN_START + (S - 2 * SUB) // PR)
        is_fin = jnp.logical_and(n >= FIN_START, n < FIN_START + (S - SUB) // PR)
        f = n - FIN_START
        src = jnp.where(is_ln, 2 * SUB + (n - LN_START) * PR, jnp.where(is_fin, f * PR, 0))
        dst = jnp.where(jnp.logical_or(is_ln, is_fin), src, S)
        oo, rn = piece(pl.multiple_of(src, PR), pl.multiple_of(dst, PR),
                       is_fin.astype(I32), jnp.where(is_fin, f, -1))
        bits = _lane_fold(pltpu.bitcast(oo, I32), jnp.bitwise_or) | pltpu.bitcast(rn, I32)
        return (bits[0:8] | bits[8:16]) & zero_buf[...]

    def qproj_head(n):
        return jnp.dot(act[pl.ds(_row_of(n), FILL), 0:D // 2],
                       packed(wq_buf, _head_of(n))[0:D // 2], preferred_element_type=F32)

    def qproj_rest(n, qa):
        row = _row_of(n)
        w = packed(wq_buf, _head_of(n))
        row2 = row + FILL if isinstance(row, int) else pl.multiple_of(row + FILL, 16)
        qb = jnp.dot(act[pl.ds(row, SUB), D // 2:D], w[D // 2:D], preferred_element_type=F32)
        qc = jnp.dot(act[pl.ds(row2, SUB - FILL), 0:D // 2], w[0:D // 2],
                     preferred_element_type=F32)
        return ((qb + jnp.concatenate([qa, qc], axis=0)) * QSCALE).astype(BF16)

    def oproj(o, n):
        acc[pl.ds(_row_of(n), SUB), :] += jnp.dot(o, wo_buf[_head_of(n)],
                                                  preferred_element_type=F32)

    def unit_block(n0, nunits, with_piece):
        o = _normalize(pv_car[0], ls_car[0])
        raw = (pv_car[1], ls_car[1])
        qa = qa_car[...]
        for u in range(nunits):
            n = n0 + u
            hd = _head_of(n)
            q = qproj_rest(n, qa)
            oproj(o, n - 2)
            z = unit_piece(n) if with_piece else None
            sc = lax.dot_general(q, packed(k_buf, hd), NT, preferred_element_type=F32)
            qa = qproj_head(n + 1)
            mm = _lane_fold(sc, jnp.maximum)
            if with_piece:
                mb = pltpu.bitcast(mm, I32)
                mm = pltpu.bitcast(jnp.concatenate([mb[0:8] | z, mb[8:]], axis=0), F32)
            m = jnp.max(mm, axis=-1, keepdims=True)
            p = jnp.exp2(sc - m)
            ls = _lane_fold(p, jnp.add)
            pv = jnp.dot(p.astype(BF16), packed(v_buf, hd), preferred_element_type=F32)
            if u + 1 < nunits:
                zb = (pltpu.bitcast(pv, I32).reshape(SUB // 8, 8, 128)
                      & zero_buf[...][None]).reshape(SUB, 128)
                o = _normalize(raw[0], pltpu.bitcast(pltpu.bitcast(raw[1], I32) | zb, F32))
            else:
                pv_car[0] = raw[0]
                ls_car[0] = raw[1]
            raw = (pv, ls)
        pv_car[1] = raw[0]
        ls_car[1] = raw[1]
        qa_car[...] = qa

    def start(cps):
        for c_ in cps:
            c_.start()

    def wait(cps):
        for c_ in cps:
            c_.wait()

    start([cp_c, cp_x(0, 2, SEM_X0)] + cp_m0 + [cp_wq(0, SEM_WQ0), cp_k0] + cp_v0)
    for j in range(1, R2):
        start(ramp_heads(j))
    start([cp_wr])
    n_early = (LN_START - RAMP) // UM
    for k in range(n_early):
        start(main_heads(k))

    def zero_acc(j, carry):
        acc[pl.ds(pl.multiple_of(j * 64, 64), 64), :] = jnp.zeros((64, D), F32)
        return carry

    lax.fori_loop(0, S // 64, zero_acc, 0)
    r_buf[...] = jnp.zeros(r_buf.shape, F32)
    zero_buf[...] = jnp.zeros(zero_buf.shape, I32)
    coef[0, C_GA] = jnp.zeros((8, D), F32)
    coef[0, C_KEEP] = jnp.zeros((8, D), F32)
    coef[0, C_GB] = jnp.ones((8, D), F32)
    coef[1, C_KEEP] = jnp.ones((8, D), F32)
    cp_c.wait()
    cp_x(0, 2, SEM_X0).wait()

    def norm_rows(j, carry):
        row = pl.multiple_of(j * 128, 128)
        n_buf[pl.ds(row, 128), :] = _layernorm(x_buf[pl.ds(row, 128), :].astype(F32))
        return carry

    lax.fori_loop(0, 2 * SUB // 128, norm_rows, 0)
    sc16 = silu_c()
    m0 = None
    for j in range(MCH):
        cp_m0[j].wait()
        part = jnp.dot(sc16[:, j * mrows:(j + 1) * mrows],
                       wa_buf[j * mrows:(j + 1) * mrows, 0:2 * D], preferred_element_type=F32)
        m0 = part if m0 is None else m0 + part
    m0 = _r(m0[0:8, :])
    coef[0, C_SHIFT] = m0[:, 0:D]
    coef[0, C_SCALE] = _r(1.0 + m0[:, D:2 * D])

    cp_wq(0, SEM_WQ0).wait()
    h01 = modulate(n_buf[...], 0).astype(BF16)
    act[0:2 * SUB, :] = h01
    q01 = (jnp.dot(h01, packed(wq_buf, 0), preferred_element_type=F32) * QSCALE).astype(BF16)
    cp_k0.wait()
    s01 = lax.dot_general(q01, packed(k_buf, 0), NT, preferred_element_type=F32)
    m01 = jnp.max(_lane_fold(s01, jnp.maximum), axis=-1, keepdims=True)
    wait(cp_v0)
    qa_car[...] = qproj_head(2)
    for u in range(2):
        p = jnp.exp2(s01[u * SUB:(u + 1) * SUB] - m01[u * SUB:(u + 1) * SUB])
        ls_car[u] = _lane_fold(p, jnp.add)
        pv_car[u] = jnp.dot(p.astype(BF16), packed(v_buf, 0), preferred_element_type=F32)

    def ramp2(j, carry):
        wait(ramp_heads(j))
        unit_block(2 * j, 2, False)
        return carry

    lax.fori_loop(1, R2, ramp2, 0)
    start([cp_x(2, NRB - 2, SEM_XR)])
    for k in range(n_early, NLOAD):
        start(main_heads(k, k == NLOAD - 1))
    start(cp_m12)
    cp_wr.wait()
    w8 = wr_buf[...].astype(F32)
    for j in range(D // 128):
        wr_b[:, j * 128:(j + 1) * 128] = jnp.broadcast_to(w8[j:j + 1, :], (8, 128))

    def blocks_done(n0):
        return (n0 - FIN_START) // (SUB // PR)

    def main(k, carry):
        n0 = RAMP + k * UM

        @pl.when(k <= K_MOD)
        def _():
            @pl.when(k < NLOAD - 1)
            def _():
                wait(main_heads(k))

            @pl.when(k == NLOAD - 1)
            def _():
                wait(main_heads(NLOAD - 1, True))

            @pl.when(k == n_early)
            def _():
                cp_x(2, NRB - 2, SEM_XR).wait()

            @pl.when(k == K_MOD)
            def _():
                wait(cp_m12)
                sc = silu_c()
                m1 = _r(jnp.dot(sc, wa_buf[:, 2 * D:3 * D], preferred_element_type=F32)[0:8, :])
                m2 = _r(jnp.dot(sc, wb_buf[:, 0:3 * D], preferred_element_type=F32)[0:8, :])
                coef[1, C_GA] = m1
                coef[1, C_SHIFT] = m2[:, 0:D]
                coef[1, C_SCALE] = _r(1.0 + m2[:, D:2 * D])
                coef[1, C_GB] = m2[:, 2 * D:3 * D]
                start(cp_ffn)

        done = lax.shift_right_arithmetic(n0 - FIN_START, 4)
        done_before = lax.shift_right_arithmetic(n0 - UM - FIN_START, 4)

        @pl.when(jnp.logical_and(done >= 1, done > done_before))
        def _():
            cp_out(jnp.maximum(done - 1, 0)).start()

        unit_block(n0, UM, True)
        return carry

    lax.fori_loop(0, NM, main, 0)

    for b in range(blocks_done(RAMP + (NM - 1) * UM), NRB - 1):
        cp_out(b).start()
    oproj(_normalize(pv_car[0], ls_car[0]), NU - 2)
    oproj(_normalize(pv_car[1], ls_car[1]), NU - 1)
    for j in range(SUB // PR):
        row = (NRB - 1) * SUB + j * PR
        piece(row, row, 1, row // PR)
    cp_out(NRB - 1).start()

    rr = r_buf[...]
    ridx = (lax.broadcasted_iota(I32, (PR, 128), 1) * PR
            + lax.broadcasted_iota(I32, (PR, 128), 0))
    big = jnp.int32(S - 1)
    m1 = jnp.max(jnp.max(rr, axis=0, keepdims=True), axis=1, keepdims=True)
    i1 = jnp.min(jnp.where(rr == m1, ridx, big))
    rr2 = jnp.where(ridx == i1, -jnp.inf, rr)
    m2 = jnp.max(jnp.max(rr2, axis=0, keepdims=True), axis=1, keepdims=True)
    i2 = jnp.min(jnp.where(jnp.logical_and(rr2 == m2, ridx != i1), ridx, big))

    rowid = lax.broadcasted_iota(I32, (PR, D), 0)
    g1 = pl.multiple_of(lax.shift_right_logical(i1, 4) * PR, PR)
    g2 = pl.multiple_of(lax.shift_right_logical(i2, 4) * PR, PR)
    x2a = resid(g1, PR, 1)
    x2b = resid(g2, PR, 1)
    h2a = _r(ada_ln(x2a, 1))
    h2b = _r(ada_ln(x2b, 1))
    row1 = jnp.sum(jnp.where(rowid + g1 == i1, h2a, 0.0), axis=0, keepdims=True)
    row2 = jnp.sum(jnp.where(rowid + g2 == i2, h2b, 0.0), axis=0, keepdims=True)
    xs = jnp.where(rowid == 0, row1, row2).astype(BF16)

    wait(cp_ffn)
    gt = _r(jnp.dot(xs, wa_buf[:, 0:F], preferred_element_type=F32))
    up = _r(jnp.dot(xs, wb_buf[:, 0:F], preferred_element_type=F32))
    hid = (_r(gt * _r(jax.nn.sigmoid(gt))) * up).astype(BF16)
    y = _r(jnp.dot(hid, wd_buf[:, 0:D], preferred_element_type=F32))
    y1 = _r(y[0:1, :] * _r(jax.nn.sigmoid(_r(m1))))
    y2 = _r(y[1:2, :] * _r(jax.nn.sigmoid(_r(m2))))

    def fix(x2g, h2g, gbase):
        rid = rowid + gbase
        upd = jnp.where(rid == i1, y1, jnp.where(rid == i2, y2, 0.0))
        return (x2g + _rows8(h2g + upd, jnp.multiply, coef[1, C_GB])).astype(BF16)

    for b in range(NRB):
        cp_out(b).wait()
    act[pl.ds(g1, PR), :] = fix(x2a, h2a, g1)
    act[pl.ds(g2, PR), :] = fix(x2b, h2b, g2)
    f1 = cp(act.at[pl.ds(g1, PR), :], out_hbm.at[pl.ds(g1, PR), :], SEM_OUT)
    f2 = cp(act.at[pl.ds(g2, PR), :], out_hbm.at[pl.ds(g2, PR), :], SEM_FIX)
    f1.start()

    @pl.when(g1 != g2)
    def _():
        f2.start()
        f2.wait()

    f1.wait()


@jax.jit
def pallas_adaLN_cond__mha_block_cached__moe_arch_mod__prompt_kernel(
    A_x: jax.Array,
    A_k_cache: jax.Array,
    A_v_cache: jax.Array,
    A_wq: jax.Array,
    A_wo: jax.Array,
    B_x: jax.Array,
    B_w_r: jax.Array,
    B_w_gate: jax.Array,
    B_w_up: jax.Array,
    B_w_down: jax.Array,
    c: jax.Array,
    w_mod: jax.Array,
):
    del B_x
    hbm = pl.BlockSpec(memory_space=pl.ANY)
    out = pl.pallas_call(
        _kernel,
        in_specs=[hbm] * 11,
        out_specs=hbm,
        out_shape=jax.ShapeDtypeStruct((S, D), BF16),
        scratch_shapes=[
            pltpu.VMEM((S, D), BF16),
            pltpu.VMEM((H, S, DH), BF16),
            pltpu.VMEM((H, S, DH), BF16),
            pltpu.VMEM((H, D, DH), BF16),
            pltpu.VMEM((H, DH, D), BF16),
            pltpu.VMEM((D, F + PAD), BF16),
            pltpu.VMEM((D, F + PAD), BF16),
            pltpu.VMEM((F, D + PAD), BF16),
            pltpu.VMEM((S + PR, D), BF16),
            pltpu.VMEM((S, D), F32),
            pltpu.VMEM((2 * SUB, D), F32),
            pltpu.VMEM((PR, 128), F32),
            pltpu.VMEM((2, 5, 8, D), F32),
            pltpu.VMEM((8, 128), BF16),
            pltpu.VMEM((8, D), F32),
            pltpu.VMEM((1, D), BF16),
            pltpu.VMEM((8, 128), I32),
            pltpu.VMEM((FILL, DH), F32),
            pltpu.VMEM((2, SUB, DH), F32),
            pltpu.VMEM((2, SUB, DH), F32),
            pltpu.SemaphoreType.DMA((NSEM,)),
        ],
        compiler_params=pltpu.CompilerParams(
            vmem_limit_bytes=120 * 1024 * 1024,
        ),
        name="adaln_mha_mod",
    )(
        A_x.reshape(S, D),
        A_k_cache.reshape(H, S, DH),
        A_v_cache.reshape(H, S, DH),
        A_wq,
        A_wo.reshape(H, DH, D),
        B_w_r.reshape(8, 128),
        B_w_gate,
        B_w_up,
        B_w_down,
        c,
        w_mod,
    )
    return out.reshape(1, S, D)
```

```python
import jax
import jax.numpy as jnp
from jax import lax
import jax.experimental.pallas as pl
import jax.experimental.pallas.tpu as pltpu

S = 2048
D = 1024
H = 32
DH = 128
F = 3584
SUB = 256
NRB = S // SUB
NU = H * NRB
PR = 16
UM = 12
R2 = 8
RAMP = 2 * R2
NM = (NU - RAMP) // UM
HPI = UM // 2
NLOAD = (2 * H - RAMP) // UM
K_MOD = NLOAD
LN_START = 33
FIN_START = 130
FILL = 64
ECH = 128
PAD = 128
MCH = 4
EPS = 1e-5
QSCALE = float(DH ** -0.5) * 1.4426950408889634

F32 = jnp.float32
BF16 = jnp.bfloat16
I32 = jnp.int32
NT = (((1,), (1,)), ((), ()))

C_GA, C_SCALE, C_SHIFT, C_KEEP, C_GB = range(5)


def _r(v):
    return v.astype(BF16).astype(F32)


def _rows8(v, fn, c):
    n = v.shape[0] // 8
    return fn(v.reshape(n, 8, D), c[None]).reshape(v.shape)


def _ln_stats(y):
    m = jnp.mean(y, axis=-1, keepdims=True)
    yc = y - m
    v = jnp.mean(yc * yc, axis=-1, keepdims=True)
    den = _r(jnp.sqrt(_r(_r(v) + EPS)))
    return yc, m, _r(m), 1.0 / den


def _layernorm(y):
    _, _, mr, rinv = _ln_stats(y)
    return (y - mr) * rinv


def _lane_fold(p, fn):
    t = p[:, 0:128]
    for j in range(1, p.shape[1] // 128):
        t = fn(t, p[:, j * 128:(j + 1) * 128])
    return t


def _normalize(pv, ls):
    l = jnp.sum(ls, axis=-1, keepdims=True)
    r = pl.reciprocal(l, approx=True)
    r = r * (2.0 - l * r)
    return (pv * r).astype(BF16)


def _head_of(n):
    if isinstance(n, int):
        return (n % 64) // 2 if n < 192 else (n - 192) % H
    return jnp.where(n < 192, lax.shift_right_logical(n & 63, 1), (n - 192) & (H - 1))


def _row_of(n):
    if isinstance(n, int):
        return SUB * ((n // 64) * 2 + n % 2 if n < 192 else min(n // 32, NRB - 1))
    rb = jnp.where(n < 192, lax.shift_right_logical(n, 6) * 2 + (n & 1),
                   jnp.minimum(lax.shift_right_logical(n, 5), NRB - 1))
    return pl.multiple_of(rb * SUB, SUB)


(SEM_C, SEM_WR, SEM_X0, SEM_XR, SEM_M12, SEM_FFN, SEM_OUT, SEM_FIX,
 SEM_WQ0, SEM_K0, SEM_M0) = range(11)
SEM_RAMP = SEM_M0 + MCH
SEM_MAIN = SEM_RAMP + R2
NSEM = SEM_MAIN + NLOAD


def _kernel(x_hbm, k_hbm, v_hbm, wq_hbm, wo_hbm, wr_hbm, wg_hbm, wu_hbm, wd_hbm,
            c_hbm, wmod_hbm, out_hbm,
            x_buf, k_buf, v_buf, wq_buf, wo_buf, wa_buf, wb_buf, wd_buf,
            act, acc, n_buf, x2_buf, r_buf, coef, wr_buf, sw_buf, rc_buf, c_buf, zero_buf, qa_car, pv_car, ls_car,
            sems):
    def cp(src, dst, slot):
        return pltpu.make_async_copy(src, dst, sems.at[slot])

    def cp_x(b, nb, slot):
        return cp(x_hbm.at[pl.ds(b * SUB, nb * SUB), :],
                  x_buf.at[pl.ds(b * SUB, nb * SUB), :], slot)

    def cp_wq(h, slot):
        col = h * DH if isinstance(h, int) else pl.multiple_of(h * DH, DH)
        return cp(wq_hbm.at[:, pl.ds(col, DH)], wq_buf.at[h], slot)

    def cp_h(src, dst, h0, nh, slot):
        return cp(src.at[pl.ds(h0, nh)], dst.at[pl.ds(h0, nh)], slot)

    def heads(h0, nh, slot, last=False):
        return [cp_h(k_hbm, k_buf, h0, nh, slot), cp_h(v_hbm, v_buf, h0, nh, slot),
                cp_h(wo_hbm, wo_buf, h0 - 1, nh + 1 if last else nh, slot)] + [
            cp_wq(h0 + 1 + j, slot) for j in range(nh - 1 if last else nh)]

    def ramp_heads(j):
        return heads(j, 1, SEM_RAMP + j)

    def main_heads(k, last=False):
        return heads(RAMP // 2 + k * HPI, HPI, SEM_MAIN + k, last)

    cp_k0 = cp_h(k_hbm, k_buf, 0, 1, SEM_K0)
    cp_v0 = [cp_h(v_hbm, v_buf, 0, 1, SEM_RAMP), cp_wq(1, SEM_RAMP)]
    mrows = D // MCH
    cp_m0 = [cp(wmod_hbm.at[pl.ds(j * mrows, mrows), 0:2 * D],
                wa_buf.at[pl.ds(j * mrows, mrows), 0:2 * D], SEM_M0 + j) for j in range(MCH)]
    cp_c = cp(c_hbm, c_buf, SEM_C)
    cp_wr = cp(wr_hbm, wr_buf, SEM_WR)
    cp_m12 = [cp(wmod_hbm.at[:, 2 * D:3 * D], wa_buf.at[:, 2 * D:3 * D], SEM_M12),
              cp(wmod_hbm.at[:, 3 * D:6 * D], wb_buf.at[:, 0:3 * D], SEM_M12)]
    cp_ffn = [cp(wg_hbm, wa_buf.at[:, 0:F], SEM_FFN),
              cp(wu_hbm, wb_buf.at[:, 0:F], SEM_FFN),
              cp(wd_hbm, wd_buf.at[:, 0:D], SEM_FFN)]

    def cp_out(b):
        row = b * SUB if isinstance(b, int) else pl.multiple_of(b * SUB, SUB)
        return cp(act.at[pl.ds(row, SUB), :], out_hbm.at[pl.ds(row, SUB), :], SEM_OUT)

    def silu_c():
        cf = c_buf[...].astype(F32)
        sc = (cf * _r(jax.nn.sigmoid(cf))).astype(BF16)
        return jnp.broadcast_to(sc, (16, D))

    def packed(ref, h):
        return pltpu.bitcast(ref.bitcast(jnp.uint32)[h], BF16)

    def modulate(n, kind):
        n = _rows8(n, jnp.multiply, coef[kind, C_SCALE])
        return _rows8(n, jnp.add, coef[kind, C_SHIFT])

    def ada_ln_router(y, kind):
        yc, m, mr, rinv = _ln_stats(y)
        d = jnp.sum(_rows8(yc, jnp.multiply, sw_buf[...]), axis=-1, keepdims=True)
        r = (d + (m - mr) * rc_buf[0:1, 0:1]) * rinv + rc_buf[1:2, 0:1]
        return modulate((y - mr) * rinv, kind), r

    def resid(a, row, nrows, kind):
        a = _rows8(a, jnp.multiply, coef[kind, C_GA])
        return _r(x_buf[pl.ds(row, nrows), :].astype(F32) + a)

    def piece(src, dst, kind, lane_id):
        y = resid(acc[pl.ds(src, PR), :], src, PR, kind)
        nn = _layernorm(y)
        hh = modulate(nn, kind)
        r = (jnp.sum(_rows8(nn, jnp.multiply, sw_buf[...]), axis=-1, keepdims=True)
             + rc_buf[1:2, 0:1])
        oo = (_rows8(y, jnp.multiply, coef[kind, C_KEEP])
              + _rows8(hh, jnp.multiply, coef[kind, C_GB]))
        act[pl.ds(dst, PR), :] = oo.astype(BF16)
        lane = lax.broadcasted_iota(I32, (PR, 128), 1)
        rn = jnp.where(lane == lane_id, r, r_buf[...])
        r_buf[...] = rn
        return oo, rn

    def unit_piece(n):
        is_ln = jnp.logical_and(n >= LN_START, n < LN_START + (S - 2 * SUB) // PR)
        is_fin = jnp.logical_and(n >= FIN_START, n < FIN_START + (S - SUB) // PR)
        f = n - FIN_START
        src = jnp.where(is_ln, 2 * SUB + (n - LN_START) * PR, jnp.where(is_fin, f * PR, 0))
        dst = jnp.where(jnp.logical_or(is_ln, is_fin), src, S)
        oo, rn = piece(pl.multiple_of(src, PR), pl.multiple_of(dst, PR),
                       is_fin.astype(I32), jnp.where(is_fin, f, -1))
        bits = _lane_fold(pltpu.bitcast(oo, I32), jnp.bitwise_or) | pltpu.bitcast(rn, I32)
        return (bits[0:8] | bits[8:16]) & zero_buf[...]

    def qproj_head(n):
        return jnp.dot(act[pl.ds(_row_of(n), FILL), 0:D // 2],
                       packed(wq_buf, _head_of(n))[0:D // 2], preferred_element_type=F32)

    def qproj_rest(n, qa):
        row = _row_of(n)
        w = packed(wq_buf, _head_of(n))
        row2 = row + FILL if isinstance(row, int) else pl.multiple_of(row + FILL, 16)
        qb = jnp.dot(act[pl.ds(row, SUB), D // 2:D], w[D // 2:D], preferred_element_type=F32)
        qc = jnp.dot(act[pl.ds(row2, SUB - FILL), 0:D // 2], w[0:D // 2],
                     preferred_element_type=F32)
        return ((qb + jnp.concatenate([qa, qc], axis=0)) * QSCALE).astype(BF16)

    def oproj(o, n):
        acc[pl.ds(_row_of(n), SUB), :] += jnp.dot(o, wo_buf[_head_of(n)],
                                                  preferred_element_type=F32)

    def unit_block(n0, nunits, with_piece):
        o = _normalize(pv_car[0], ls_car[0])
        raw = (pv_car[1], ls_car[1])
        qa = qa_car[...]
        for u in range(nunits):
            n = n0 + u
            hd = _head_of(n)
            q = qproj_rest(n, qa)
            z = unit_piece(n) if with_piece else None
            oproj(o, n - 2)
            sc = lax.dot_general(q, packed(k_buf, hd), NT, preferred_element_type=F32)
            qa = qproj_head(n + 1)
            mm = _lane_fold(sc, jnp.maximum)
            if with_piece:
                mb = pltpu.bitcast(mm, I32)
                mm = pltpu.bitcast(jnp.concatenate([mb[0:8] | z, mb[8:]], axis=0), F32)
            m = jnp.max(mm, axis=-1, keepdims=True)
            p = jnp.exp2(sc - m)
            ls = _lane_fold(p, jnp.add)
            pv = jnp.dot(p.astype(BF16), packed(v_buf, hd), preferred_element_type=F32)
            if u + 1 < nunits:
                zb = (pltpu.bitcast(pv, I32).reshape(SUB // 8, 8, 128)
                      & zero_buf[...][None]).reshape(SUB, 128)
                o = _normalize(raw[0], pltpu.bitcast(pltpu.bitcast(raw[1], I32) | zb, F32))
            else:
                pv_car[0] = raw[0]
                ls_car[0] = raw[1]
            raw = (pv, ls)
        pv_car[1] = raw[0]
        ls_car[1] = raw[1]
        qa_car[...] = qa

    def start(cps):
        for c_ in cps:
            c_.start()

    def wait(cps):
        for c_ in cps:
            c_.wait()

    start([cp_c, cp_x(0, 2, SEM_X0)] + cp_m0 + [cp_wq(0, SEM_WQ0), cp_k0] + cp_v0)
    for j in range(1, R2):
        start(ramp_heads(j))
    start([cp_wr])
    n_early = (LN_START - RAMP) // UM
    for k in range(n_early):
        start(main_heads(k))

    def zero_acc(j, carry):
        acc[pl.ds(pl.multiple_of(j * 64, 64), 64), :] = jnp.zeros((64, D), F32)
        return carry

    lax.fori_loop(0, S // 64, zero_acc, 0)
    r_buf[...] = jnp.zeros(r_buf.shape, F32)
    zero_buf[...] = jnp.zeros(zero_buf.shape, I32)
    coef[0, C_GA] = jnp.zeros((8, D), F32)
    coef[0, C_KEEP] = jnp.zeros((8, D), F32)
    coef[0, C_GB] = jnp.ones((8, D), F32)
    coef[1, C_KEEP] = jnp.ones((8, D), F32)
    sw_buf[...] = jnp.zeros(sw_buf.shape, F32)
    rc_buf[...] = jnp.zeros(rc_buf.shape, F32)
    cp_c.wait()
    cp_x(0, 2, SEM_X0).wait()

    def norm_rows(j, carry):
        row = pl.multiple_of(j * 128, 128)
        n_buf[pl.ds(row, 128), :] = _layernorm(x_buf[pl.ds(row, 128), :].astype(F32))
        return carry

    lax.fori_loop(0, 2 * SUB // 128, norm_rows, 0)
    sc16 = silu_c()
    m0 = None
    for j in range(MCH):
        cp_m0[j].wait()
        part = jnp.dot(sc16[:, j * mrows:(j + 1) * mrows],
                       wa_buf[j * mrows:(j + 1) * mrows, 0:2 * D], preferred_element_type=F32)
        m0 = part if m0 is None else m0 + part
    m0 = _r(m0[0:8, :])
    coef[0, C_SHIFT] = m0[:, 0:D]
    coef[0, C_SCALE] = _r(1.0 + m0[:, D:2 * D])

    cp_wq(0, SEM_WQ0).wait()
    h01 = modulate(n_buf[...], 0).astype(BF16)
    act[0:2 * SUB, :] = h01
    q01 = (jnp.dot(h01, packed(wq_buf, 0), preferred_element_type=F32) * QSCALE).astype(BF16)
    cp_k0.wait()
    s01 = lax.dot_general(q01, packed(k_buf, 0), NT, preferred_element_type=F32)
    m01 = jnp.max(_lane_fold(s01, jnp.maximum), axis=-1, keepdims=True)
    wait(cp_v0)
    qa_car[...] = qproj_head(2)
    for u in range(2):
        p = jnp.exp2(s01[u * SUB:(u + 1) * SUB] - m01[u * SUB:(u + 1) * SUB])
        ls_car[u] = _lane_fold(p, jnp.add)
        pv_car[u] = jnp.dot(p.astype(BF16), packed(v_buf, 0), preferred_element_type=F32)

    def ramp2(j, carry):
        wait(ramp_heads(j))
        unit_block(2 * j, 2, False)
        return carry

    lax.fori_loop(1, R2, ramp2, 0)
    start([cp_x(2, NRB - 2, SEM_XR)])
    for k in range(n_early, NLOAD):
        start(main_heads(k, k == NLOAD - 1))
    start(cp_m12)

    def blocks_done(n0):
        return (n0 - FIN_START) // (SUB // PR)

    def main(k, carry):
        n0 = RAMP + k * UM

        @pl.when(k <= K_MOD + 2)
        def _():
            @pl.when(k < NLOAD - 1)
            def _():
                wait(main_heads(k))

            @pl.when(k == NLOAD - 1)
            def _():
                wait(main_heads(NLOAD - 1, True))

            @pl.when(k == n_early)
            def _():
                cp_x(2, NRB - 2, SEM_XR).wait()

            @pl.when(k == K_MOD)
            def _():
                wait(cp_m12 + [cp_wr])
                sc = silu_c()
                m1 = _r(jnp.dot(sc, wa_buf[:, 2 * D:3 * D], preferred_element_type=F32)[0:8, :])
                m2 = _r(jnp.dot(sc, wb_buf[:, 0:3 * D], preferred_element_type=F32)[0:8, :])
                coef[1, C_GA] = m1
                scale = _r(1.0 + m2[:, D:2 * D])
                coef[1, C_SHIFT] = m2[:, 0:D]
                coef[1, C_SCALE] = scale
                coef[1, C_GB] = m2[:, 2 * D:3 * D]
                w8 = wr_buf[...].astype(F32)
                wr = jnp.concatenate([jnp.broadcast_to(w8[j:j + 1, :], (8, 128))
                                      for j in range(D // 128)], axis=1)
                sw_buf[...] = scale * wr
                c1 = jnp.sum(scale * wr, axis=-1, keepdims=True)
                c0 = jnp.sum(m2[:, 0:D] * wr, axis=-1, keepdims=True)
                rid = lax.broadcasted_iota(I32, (8, 128), 0)
                rc_buf[...] = jnp.where(rid == 0, c1, c0)
                start(cp_ffn)

            @pl.when(k == K_MOD + 2)
            def _():
                wait(cp_ffn)

        done = lax.shift_right_arithmetic(n0 - FIN_START, 4)
        done_before = lax.shift_right_arithmetic(n0 - UM - FIN_START, 4)

        @pl.when(jnp.logical_and(done >= 1, done > done_before))
        def _():
            cp_out(jnp.maximum(done - 1, 0)).start()

        unit_block(n0, UM, True)
        return carry

    lax.fori_loop(0, NM, main, 0)

    for b in range(blocks_done(RAMP + (NM - 1) * UM), NRB - 1):
        cp_out(b).start()
    row0 = (NRB - 1) * SUB
    neg = -jnp.inf

    def all_red(v, fn):
        return fn(fn(v, axis=0, keepdims=True), axis=1, keepdims=True)

    lane = lax.broadcasted_iota(I32, (PR, 128), 1)
    ridx = (lane * PR + lax.broadcasted_iota(I32, (PR, 128), 0)).astype(F32)
    rr = jnp.where(lane < row0 // PR, r_buf[...], neg)
    last_old = float(row0 - 1)
    cm1 = all_red(rr, jnp.max)
    ci1 = all_red(jnp.where(rr == cm1, ridx, last_old), jnp.min)
    rr2 = jnp.where(ridx == ci1, neg, rr)
    cm2 = all_red(rr2, jnp.max)
    ci2 = all_red(jnp.where(jnp.logical_and(rr2 == cm2, ridx != ci1), ridx, last_old), jnp.min)
    ci1 = jnp.minimum(ci1, last_old).astype(I32)
    ci2 = jnp.minimum(ci2, last_old).astype(I32)
    for j, ci in enumerate((ci1, ci2)):
        g = pl.multiple_of(lax.shift_right_logical(ci[0, 0], 4) * PR, PR)
        y = resid(acc[pl.ds(g, PR), :], g, PR, 1)
        x2_buf[SUB + j * PR:SUB + (j + 1) * PR, :] = y
        n_buf[SUB + j * PR:SUB + (j + 1) * PR, :] = modulate(_layernorm(y), 1)

    o2 = jnp.concatenate([_normalize(pv_car[0], ls_car[0]),
                          _normalize(pv_car[1], ls_car[1])], axis=1)
    wo2 = jnp.concatenate([wo_buf[H - 2], wo_buf[H - 1]], axis=0)
    r_new = []
    for j in range(SUB // ECH):
        lo, hi = j * ECH, (j + 1) * ECH
        a = acc[row0 + lo:row0 + hi, :] + jnp.dot(o2[lo:hi], wo2, preferred_element_type=F32)
        y = resid(a, row0 + lo, ECH, 1)
        hh, r = ada_ln_router(y, 1)
        x2_buf[lo:hi, :] = y
        n_buf[lo:hi, :] = hh
        act[row0 + lo:row0 + hi, :] = (
            y + _rows8(hh, jnp.multiply, coef[1, C_GB])).astype(BF16)
        r_new.append(r)
    cp_out(NRB - 1).start()

    sub8 = lax.broadcasted_iota(I32, (8, 1), 0)
    big = jnp.int32((S - 1) * 512 + SUB - 1)
    vals = jnp.concatenate(
        r_new + [jnp.where(sub8 == 0, cm1, jnp.where(sub8 == 1, cm2, neg))], axis=0)
    pos = lax.broadcasted_iota(I32, (SUB, 1), 0)
    cc1 = ci1 * 512 + SUB + (ci1 & (PR - 1))
    cc2 = ci2 * 512 + SUB + PR + (ci2 & (PR - 1))
    code = jnp.concatenate(
        [(pos + row0) * 512 + pos,
         jnp.where(sub8 == 0, cc1, jnp.where(sub8 == 1, cc2, big))], axis=0)
    m1 = jnp.max(vals, axis=0, keepdims=True)
    k1 = jnp.min(jnp.where(vals == m1, code, big), axis=0, keepdims=True)
    vals2 = jnp.where(code == k1, neg, vals)
    m2 = jnp.max(vals2, axis=0, keepdims=True)
    k2 = jnp.min(jnp.where(jnp.logical_and(vals2 == m2, code != k1), code, big),
                 axis=0, keepdims=True)
    k1 = k1[0, 0]
    k2 = k2[0, 0]
    i1 = lax.shift_right_logical(k1, 9)
    i2 = lax.shift_right_logical(k2, 9)
    t1 = k1 & 511
    t2 = k2 & 511
    rowid = lax.broadcasted_iota(I32, (PR, D), 0)
    xs = jnp.where(rowid == 0, n_buf[pl.ds(t1, 1), :], n_buf[pl.ds(t2, 1), :]).astype(BF16)

    gt = _r(jnp.dot(xs, wa_buf[:, 0:F], preferred_element_type=F32))
    up = _r(jnp.dot(xs, wb_buf[:, 0:F], preferred_element_type=F32))
    hid = (_r(gt * _r(jax.nn.sigmoid(gt))) * up).astype(BF16)
    y = _r(jnp.dot(hid, wd_buf[:, 0:D], preferred_element_type=F32))
    y1 = _r(y[0:1, :] * _r(jax.nn.sigmoid(_r(m1))))
    y2 = _r(y[1:2, :] * _r(jax.nn.sigmoid(_r(m2))))

    def fix(i, t):
        g = pl.multiple_of(lax.shift_right_logical(i, 4) * PR, PR)
        tg = pl.multiple_of(lax.shift_right_logical(t, 4) * PR, PR)
        rid = rowid + g
        upd = jnp.where(rid == i1, y1, jnp.where(rid == i2, y2, 0.0))
        h2g = n_buf[pl.ds(tg, PR), :] + upd
        return g, (x2_buf[pl.ds(tg, PR), :]
                   + _rows8(h2g, jnp.multiply, coef[1, C_GB])).astype(BF16)

    g1, fix1 = fix(i1, t1)
    g2, fix2 = fix(i2, t2)
    for b in range(NRB):
        cp_out(b).wait()
    act[pl.ds(g1, PR), :] = fix1
    act[pl.ds(g2, PR), :] = fix2
    f1 = cp(act.at[pl.ds(g1, PR), :], out_hbm.at[pl.ds(g1, PR), :], SEM_OUT)
    f2 = cp(act.at[pl.ds(g2, PR), :], out_hbm.at[pl.ds(g2, PR), :], SEM_FIX)
    f1.start()

    @pl.when(g1 != g2)
    def _():
        f2.start()
        f2.wait()

    f1.wait()


@jax.jit
def pallas_adaLN_cond__mha_block_cached__moe_arch_mod__prompt_kernel(
    A_x: jax.Array,
    A_k_cache: jax.Array,
    A_v_cache: jax.Array,
    A_wq: jax.Array,
    A_wo: jax.Array,
    B_x: jax.Array,
    B_w_r: jax.Array,
    B_w_gate: jax.Array,
    B_w_up: jax.Array,
    B_w_down: jax.Array,
    c: jax.Array,
    w_mod: jax.Array,
):
    del B_x
    hbm = pl.BlockSpec(memory_space=pl.ANY)
    out = pl.pallas_call(
        _kernel,
        in_specs=[hbm] * 11,
        out_specs=hbm,
        out_shape=jax.ShapeDtypeStruct((S, D), BF16),
        scratch_shapes=[
            pltpu.VMEM((S, D), BF16),
            pltpu.VMEM((H, S, DH), BF16),
            pltpu.VMEM((H, S, DH), BF16),
            pltpu.VMEM((H, D, DH), BF16),
            pltpu.VMEM((H, DH, D), BF16),
            pltpu.VMEM((D, F + PAD), BF16),
            pltpu.VMEM((D, F + PAD), BF16),
            pltpu.VMEM((F, D + PAD), BF16),
            pltpu.VMEM((S + PR, D), BF16),
            pltpu.VMEM((S, D), F32),
            pltpu.VMEM((2 * SUB, D), F32),
            pltpu.VMEM((SUB + 2 * PR, D), F32),
            pltpu.VMEM((PR, 128), F32),
            pltpu.VMEM((2, 5, 8, D), F32),
            pltpu.VMEM((8, 128), BF16),
            pltpu.VMEM((8, D), F32),
            pltpu.VMEM((8, 128), F32),
            pltpu.VMEM((1, D), BF16),
            pltpu.VMEM((8, 128), I32),
            pltpu.VMEM((FILL, DH), F32),
            pltpu.VMEM((2, SUB, DH), F32),
            pltpu.VMEM((2, SUB, DH), F32),
            pltpu.SemaphoreType.DMA((NSEM,)),
        ],
        compiler_params=pltpu.CompilerParams(
            vmem_limit_bytes=120 * 1024 * 1024,
        ),
        name="adaln_mha_mod",
    )(
        A_x.reshape(S, D),
        A_k_cache.reshape(H, S, DH),
        A_v_cache.reshape(H, S, DH),
        A_wq,
        A_wo.reshape(H, DH, D),
        B_w_r.reshape(8, 128),
        B_w_gate,
        B_w_up,
        B_w_down,
        c,
        w_mod,
    )
    return out.reshape(1, S, D)
```

```python
import jax
import jax.numpy as jnp
from jax import lax
import jax.experimental.pallas as pl
import jax.experimental.pallas.tpu as pltpu

S = 2048
D = 1024
H = 32
DH = 128
F = 3584
SUB = 256
NRB = S // SUB
NU = H * NRB
PR = 16
UM = 12
R2 = 8
RAMP = 2 * R2
NM = (NU - RAMP) // UM
HPI = UM // 2
NLOAD = (2 * H - RAMP) // UM
K_MOD = NLOAD
LN_START = 33
FIN_START = 130
FILL = 64
ECH = 128
PAD = 128
MCH = 4
EPS = 1e-5
QSCALE = float(DH ** -0.5) * 1.4426950408889634

F32 = jnp.float32
BF16 = jnp.bfloat16
I32 = jnp.int32
NT = (((1,), (1,)), ((), ()))

C_GA, C_SCALE, C_SHIFT, C_KEEP, C_GB = range(5)


def _r(v):
    return v.astype(BF16).astype(F32)


def _rows8(v, fn, c):
    n = v.shape[0] // 8
    return fn(v.reshape(n, 8, D), c[None]).reshape(v.shape)


def _ln_stats(y):
    m = jnp.mean(y, axis=-1, keepdims=True)
    yc = y - m
    v = jnp.mean(yc * yc, axis=-1, keepdims=True)
    den = _r(jnp.sqrt(_r(_r(v) + EPS)))
    return yc, m, _r(m), 1.0 / den


def _layernorm(y):
    _, _, mr, rinv = _ln_stats(y)
    return (y - mr) * rinv


def _lane_fold(p, fn):
    t = p[:, 0:128]
    for j in range(1, p.shape[1] // 128):
        t = fn(t, p[:, j * 128:(j + 1) * 128])
    return t


def _normalize(pv, ls):
    l = jnp.sum(ls, axis=-1, keepdims=True)
    r = pl.reciprocal(l, approx=True)
    r = r * (2.0 - l * r)
    return (pv * r).astype(BF16)


def _head_of(n):
    if isinstance(n, int):
        return (n % 64) // 2 if n < 192 else (n - 192) % H
    return jnp.where(n < 192, lax.shift_right_logical(n & 63, 1), (n - 192) & (H - 1))


def _row_of(n):
    if isinstance(n, int):
        return SUB * ((n // 64) * 2 + n % 2 if n < 192 else min(n // 32, NRB - 1))
    rb = jnp.where(n < 192, lax.shift_right_logical(n, 6) * 2 + (n & 1),
                   jnp.minimum(lax.shift_right_logical(n, 5), NRB - 1))
    return pl.multiple_of(rb * SUB, SUB)


(SEM_C, SEM_WR, SEM_X0, SEM_XR, SEM_M12, SEM_FFN, SEM_OUT, SEM_FIX,
 SEM_WQ0, SEM_K0, SEM_M0) = range(11)
SEM_RAMP = SEM_M0 + MCH
SEM_MAIN = SEM_RAMP + R2
NSEM = SEM_MAIN + NLOAD


def _kernel(x_hbm, k_hbm, v_hbm, wq_hbm, wo_hbm, wr_hbm, wg_hbm, wu_hbm, wd_hbm,
            c_hbm, wmod_hbm, out_hbm,
            x_buf, k_buf, v_buf, wq_buf, wo_buf, wa_buf, wb_buf, wd_buf,
            act, acc, n_buf, x2_buf, r_buf, coef, wr_buf, sw_buf, rc_buf, c_buf, zero_buf, qa_car, pv_car, ls_car,
            sems):
    def cp(src, dst, slot):
        return pltpu.make_async_copy(src, dst, sems.at[slot])

    def cp_x(b, nb, slot):
        return cp(x_hbm.at[pl.ds(b * SUB, nb * SUB), :],
                  x_buf.at[pl.ds(b * SUB, nb * SUB), :], slot)

    def cp_wq(h, slot):
        col = h * DH if isinstance(h, int) else pl.multiple_of(h * DH, DH)
        return cp(wq_hbm.at[:, pl.ds(col, DH)], wq_buf.at[h], slot)

    def cp_h(src, dst, h0, nh, slot):
        return cp(src.at[pl.ds(h0, nh)], dst.at[pl.ds(h0, nh)], slot)

    def heads(h0, nh, slot, last=False):
        return [cp_h(k_hbm, k_buf, h0, nh, slot), cp_h(v_hbm, v_buf, h0, nh, slot),
                cp_h(wo_hbm, wo_buf, h0 - 1, nh + 1 if last else nh, slot)] + [
            cp_wq(h0 + 1 + j, slot) for j in range(nh - 1 if last else nh)]

    def ramp_heads(j):
        return heads(j, 1, SEM_RAMP + j)

    def main_heads(k, last=False):
        return heads(RAMP // 2 + k * HPI, HPI, SEM_MAIN + k, last)

    cp_k0 = cp_h(k_hbm, k_buf, 0, 1, SEM_K0)
    cp_v0 = [cp_h(v_hbm, v_buf, 0, 1, SEM_RAMP), cp_wq(1, SEM_RAMP)]
    mrows = D // MCH
    cp_m0 = [cp(wmod_hbm.at[pl.ds(j * mrows, mrows), 0:2 * D],
                wa_buf.at[pl.ds(j * mrows, mrows), 0:2 * D], SEM_M0 + j) for j in range(MCH)]
    cp_c = cp(c_hbm, c_buf, SEM_C)
    cp_wr = cp(wr_hbm, wr_buf, SEM_WR)
    cp_m12 = [cp(wmod_hbm.at[:, 2 * D:3 * D], wa_buf.at[:, 2 * D:3 * D], SEM_M12),
              cp(wmod_hbm.at[:, 3 * D:6 * D], wb_buf.at[:, 0:3 * D], SEM_M12)]
    cp_ffn = [cp(wg_hbm, wa_buf.at[:, 0:F], SEM_FFN),
              cp(wu_hbm, wb_buf.at[:, 0:F], SEM_FFN),
              cp(wd_hbm, wd_buf.at[:, 0:D], SEM_FFN)]

    def cp_out(b):
        row = b * SUB if isinstance(b, int) else pl.multiple_of(b * SUB, SUB)
        return cp(act.at[pl.ds(row, SUB), :], out_hbm.at[pl.ds(row, SUB), :], SEM_OUT)

    def silu_c():
        cf = c_buf[...].astype(F32)
        sc = (cf * _r(jax.nn.sigmoid(cf))).astype(BF16)
        return jnp.broadcast_to(sc, (16, D))

    def packed(ref, h):
        return pltpu.bitcast(ref.bitcast(jnp.uint32)[h], BF16)

    def modulate(n, kind):
        n = _rows8(n, jnp.multiply, coef[kind, C_SCALE])
        return _rows8(n, jnp.add, coef[kind, C_SHIFT])

    def ada_ln_router(y, kind):
        yc, m, mr, rinv = _ln_stats(y)
        d = jnp.sum(_rows8(yc, jnp.multiply, sw_buf[...]), axis=-1, keepdims=True)
        r = (d + (m - mr) * rc_buf[0:1, 0:1]) * rinv
        return modulate((y - mr) * rinv, kind), r

    def resid(a, row, nrows, kind):
        a = _rows8(a, jnp.multiply, coef[kind, C_GA])
        return _r(x_buf[pl.ds(row, nrows), :].astype(F32) + a)

    def piece(src, dst, kind, lane_id):
        y = resid(acc[pl.ds(src, PR), :], src, PR, kind)
        nn = _layernorm(y)
        hh = modulate(nn, kind)
        r = jnp.sum(_rows8(nn, jnp.multiply, sw_buf[...]), axis=-1, keepdims=True)
        oo = (_rows8(y, jnp.multiply, coef[kind, C_KEEP])
              + _rows8(hh, jnp.multiply, coef[kind, C_GB]))
        act[pl.ds(dst, PR), :] = oo.astype(BF16)
        lane = lax.broadcasted_iota(I32, (PR, 128), 1)
        rn = jnp.where(lane == lane_id, r, r_buf[...])
        r_buf[...] = rn
        return oo, rn

    def unit_piece(n):
        is_ln = jnp.logical_and(n >= LN_START, n < LN_START + (S - 2 * SUB) // PR)
        is_fin = jnp.logical_and(n >= FIN_START, n < FIN_START + (S - SUB) // PR)
        f = n - FIN_START
        src = jnp.where(is_ln, 2 * SUB + (n - LN_START) * PR, jnp.where(is_fin, f * PR, 0))
        dst = jnp.where(jnp.logical_or(is_ln, is_fin), src, S)
        oo, rn = piece(pl.multiple_of(src, PR), pl.multiple_of(dst, PR),
                       is_fin.astype(I32), jnp.where(is_fin, f, -1))
        bits = _lane_fold(pltpu.bitcast(oo, I32), jnp.bitwise_or) | pltpu.bitcast(rn, I32)
        return (bits[0:8] | bits[8:16]) & zero_buf[...]

    def qproj_head(n):
        return jnp.dot(act[pl.ds(_row_of(n), FILL), 0:D // 2],
                       packed(wq_buf, _head_of(n))[0:D // 2], preferred_element_type=F32)

    def qproj_rest(n, qa):
        row = _row_of(n)
        w = packed(wq_buf, _head_of(n))
        row2 = row + FILL if isinstance(row, int) else pl.multiple_of(row + FILL, 16)
        qb = jnp.dot(act[pl.ds(row, SUB), D // 2:D], w[D // 2:D], preferred_element_type=F32)
        qc = jnp.dot(act[pl.ds(row2, SUB - FILL), 0:D // 2], w[0:D // 2],
                     preferred_element_type=F32)
        return ((qb + jnp.concatenate([qa, qc], axis=0)) * QSCALE).astype(BF16)

    def oproj(o, n):
        acc[pl.ds(_row_of(n), SUB), :] += jnp.dot(o, wo_buf[_head_of(n)],
                                                  preferred_element_type=F32)

    def unit_block(n0, nunits, with_piece):
        o = _normalize(pv_car[0], ls_car[0])
        raw = (pv_car[1], ls_car[1])
        qa = qa_car[...]
        for u in range(nunits):
            n = n0 + u
            hd = _head_of(n)
            q = qproj_rest(n, qa)
            z = unit_piece(n) if with_piece else None
            oproj(o, n - 2)
            sc = lax.dot_general(q, packed(k_buf, hd), NT, preferred_element_type=F32)
            qa = qproj_head(n + 1)
            mm = _lane_fold(sc, jnp.maximum)
            if with_piece:
                mb = pltpu.bitcast(mm, I32)
                mm = pltpu.bitcast(jnp.concatenate([mb[0:8] | z, mb[8:]], axis=0), F32)
            m = jnp.max(mm, axis=-1, keepdims=True)
            p = jnp.exp2(sc - m)
            ls = _lane_fold(p, jnp.add)
            pv = jnp.dot(p.astype(BF16), packed(v_buf, hd), preferred_element_type=F32)
            if u + 1 < nunits:
                zb = (pltpu.bitcast(pv, I32).reshape(SUB // 8, 8, 128)
                      & zero_buf[...][None]).reshape(SUB, 128)
                o = _normalize(raw[0], pltpu.bitcast(pltpu.bitcast(raw[1], I32) | zb, F32))
            else:
                pv_car[0] = raw[0]
                ls_car[0] = raw[1]
            raw = (pv, ls)
        pv_car[1] = raw[0]
        ls_car[1] = raw[1]
        qa_car[...] = qa

    def start(cps):
        for c_ in cps:
            c_.start()

    def wait(cps):
        for c_ in cps:
            c_.wait()

    start([cp_c, cp_x(0, 2, SEM_X0)] + cp_m0 + [cp_wq(0, SEM_WQ0), cp_k0] + cp_v0)
    for j in range(1, R2):
        start(ramp_heads(j))
    start([cp_wr])
    n_early = (LN_START - RAMP) // UM
    for k in range(n_early):
        start(main_heads(k))

    def zero_acc(j, carry):
        acc[pl.ds(pl.multiple_of(j * 64, 64), 64), :] = jnp.zeros((64, D), F32)
        return carry

    lax.fori_loop(0, S // 64, zero_acc, 0)
    r_buf[...] = jnp.zeros(r_buf.shape, F32)
    zero_buf[...] = jnp.zeros(zero_buf.shape, I32)
    coef[0, C_GA] = jnp.zeros((8, D), F32)
    coef[0, C_KEEP] = jnp.zeros((8, D), F32)
    coef[0, C_GB] = jnp.ones((8, D), F32)
    coef[1, C_KEEP] = jnp.ones((8, D), F32)
    sw_buf[...] = jnp.zeros(sw_buf.shape, F32)
    rc_buf[...] = jnp.zeros(rc_buf.shape, F32)
    cp_c.wait()
    cp_x(0, 2, SEM_X0).wait()

    def norm_rows(j, carry):
        row = pl.multiple_of(j * 128, 128)
        n_buf[pl.ds(row, 128), :] = _layernorm(x_buf[pl.ds(row, 128), :].astype(F32))
        return carry

    lax.fori_loop(0, 2 * SUB // 128, norm_rows, 0)
    sc16 = silu_c()
    m0 = None
    for j in range(MCH):
        cp_m0[j].wait()
        part = jnp.dot(sc16[:, j * mrows:(j + 1) * mrows],
                       wa_buf[j * mrows:(j + 1) * mrows, 0:2 * D], preferred_element_type=F32)
        m0 = part if m0 is None else m0 + part
    m0 = _r(m0[0:8, :])
    coef[0, C_SHIFT] = m0[:, 0:D]
    coef[0, C_SCALE] = _r(1.0 + m0[:, D:2 * D])

    cp_wq(0, SEM_WQ0).wait()
    h01 = modulate(n_buf[...], 0).astype(BF16)
    act[0:2 * SUB, :] = h01
    q01 = (jnp.dot(h01, packed(wq_buf, 0), preferred_element_type=F32) * QSCALE).astype(BF16)
    cp_k0.wait()
    s01 = lax.dot_general(q01, packed(k_buf, 0), NT, preferred_element_type=F32)
    m01 = jnp.max(_lane_fold(s01, jnp.maximum), axis=-1, keepdims=True)
    wait(cp_v0)
    qa_car[...] = qproj_head(2)
    for u in range(2):
        p = jnp.exp2(s01[u * SUB:(u + 1) * SUB] - m01[u * SUB:(u + 1) * SUB])
        ls_car[u] = _lane_fold(p, jnp.add)
        pv_car[u] = jnp.dot(p.astype(BF16), packed(v_buf, 0), preferred_element_type=F32)

    def ramp2(j, carry):
        wait(ramp_heads(j))
        unit_block(2 * j, 2, False)
        return carry

    lax.fori_loop(1, R2, ramp2, 0)
    start([cp_x(2, NRB - 2, SEM_XR)])
    for k in range(n_early, NLOAD):
        start(main_heads(k, k == NLOAD - 1))
    start(cp_m12)

    def blocks_done(n0):
        return (n0 - FIN_START) // (SUB // PR)

    def main(k, carry):
        n0 = RAMP + k * UM

        @pl.when(k <= K_MOD + 2)
        def _():
            @pl.when(k < NLOAD - 1)
            def _():
                wait(main_heads(k))

            @pl.when(k == NLOAD - 1)
            def _():
                wait(main_heads(NLOAD - 1, True))

            @pl.when(k == n_early)
            def _():
                cp_x(2, NRB - 2, SEM_XR).wait()

            @pl.when(k == K_MOD)
            def _():
                wait(cp_m12 + [cp_wr])
                sc = silu_c()
                m1 = _r(jnp.dot(sc, wa_buf[:, 2 * D:3 * D], preferred_element_type=F32)[0:8, :])
                m2 = _r(jnp.dot(sc, wb_buf[:, 0:3 * D], preferred_element_type=F32)[0:8, :])
                coef[1, C_GA] = m1
                scale = _r(1.0 + m2[:, D:2 * D])
                coef[1, C_SHIFT] = m2[:, 0:D]
                coef[1, C_SCALE] = scale
                coef[1, C_GB] = m2[:, 2 * D:3 * D]
                w8 = wr_buf[...].astype(F32)
                wr = jnp.concatenate([jnp.broadcast_to(w8[j:j + 1, :], (8, 128))
                                      for j in range(D // 128)], axis=1)
                sw_buf[...] = scale * wr
                c1 = jnp.sum(scale * wr, axis=-1, keepdims=True)
                c0 = jnp.sum(m2[:, 0:D] * wr, axis=-1, keepdims=True)
                rid = lax.broadcasted_iota(I32, (8, 128), 0)
                rc_buf[...] = jnp.where(rid == 0, c1, c0)
                start(cp_ffn)

            @pl.when(k == K_MOD + 2)
            def _():
                wait(cp_ffn)

        done = lax.shift_right_arithmetic(n0 - FIN_START, 4)
        done_before = lax.shift_right_arithmetic(n0 - UM - FIN_START, 4)

        @pl.when(jnp.logical_and(done >= 1, done > done_before))
        def _():
            cp_out(jnp.maximum(done - 1, 0)).start()

        unit_block(n0, UM, True)
        return carry

    lax.fori_loop(0, NM, main, 0)

    for b in range(blocks_done(RAMP + (NM - 1) * UM), NRB - 1):
        cp_out(b).start()
    row0 = (NRB - 1) * SUB
    neg = -jnp.inf

    def all_red(v, fn):
        return fn(fn(v, axis=0, keepdims=True), axis=1, keepdims=True)

    lane = lax.broadcasted_iota(I32, (PR, 128), 1)
    ridx = (lane * PR + lax.broadcasted_iota(I32, (PR, 128), 0)).astype(F32)
    rr = jnp.where(lane < row0 // PR, r_buf[...], neg)
    last_old = float(row0 - 1)
    cm1 = all_red(rr, jnp.max)
    ci1 = all_red(jnp.where(rr == cm1, ridx, last_old), jnp.min)
    rr2 = jnp.where(ridx == ci1, neg, rr)
    cm2 = all_red(rr2, jnp.max)
    ci2 = all_red(jnp.where(jnp.logical_and(rr2 == cm2, ridx != ci1), ridx, last_old), jnp.min)
    ci1 = jnp.minimum(ci1, last_old).astype(I32)
    ci2 = jnp.minimum(ci2, last_old).astype(I32)
    for j, ci in enumerate((ci1, ci2)):
        g = pl.multiple_of(lax.shift_right_logical(ci[0, 0], 4) * PR, PR)
        y = resid(acc[pl.ds(g, PR), :], g, PR, 1)
        x2_buf[SUB + j * PR:SUB + (j + 1) * PR, :] = y
        n_buf[SUB + j * PR:SUB + (j + 1) * PR, :] = modulate(_layernorm(y), 1)

    o2 = jnp.concatenate([_normalize(pv_car[0], ls_car[0]),
                          _normalize(pv_car[1], ls_car[1])], axis=1)
    wo2 = jnp.concatenate([wo_buf[H - 2], wo_buf[H - 1]], axis=0)
    r_new = []
    for j in range(SUB // ECH):
        lo, hi = j * ECH, (j + 1) * ECH
        a = acc[row0 + lo:row0 + hi, :] + jnp.dot(o2[lo:hi], wo2, preferred_element_type=F32)
        y = resid(a, row0 + lo, ECH, 1)
        hh, r = ada_ln_router(y, 1)
        x2_buf[lo:hi, :] = y
        n_buf[lo:hi, :] = hh
        act[row0 + lo:row0 + hi, :] = (
            y + _rows8(hh, jnp.multiply, coef[1, C_GB])).astype(BF16)
        r_new.append(r)
    cp_out(NRB - 1).start()

    sub8 = lax.broadcasted_iota(I32, (8, 1), 0)
    big = jnp.int32((S - 1) * 512 + SUB - 1)
    vals = jnp.concatenate(
        r_new + [jnp.where(sub8 == 0, cm1, jnp.where(sub8 == 1, cm2, neg))], axis=0)
    pos = lax.broadcasted_iota(I32, (SUB, 1), 0)
    cc1 = ci1 * 512 + SUB + (ci1 & (PR - 1))
    cc2 = ci2 * 512 + SUB + PR + (ci2 & (PR - 1))
    code = jnp.concatenate(
        [(pos + row0) * 512 + pos,
         jnp.where(sub8 == 0, cc1, jnp.where(sub8 == 1, cc2, big))], axis=0)
    m1 = jnp.max(vals, axis=0, keepdims=True)
    k1 = jnp.min(jnp.where(vals == m1, code, big), axis=0, keepdims=True)
    vals2 = jnp.where(code == k1, neg, vals)
    m2 = jnp.max(vals2, axis=0, keepdims=True)
    k2 = jnp.min(jnp.where(jnp.logical_and(vals2 == m2, code != k1), code, big),
                 axis=0, keepdims=True)
    k1 = k1[0, 0]
    k2 = k2[0, 0]
    i1 = lax.shift_right_logical(k1, 9)
    i2 = lax.shift_right_logical(k2, 9)
    t1 = k1 & 511
    t2 = k2 & 511
    rowid = lax.broadcasted_iota(I32, (PR, D), 0)
    xs = jnp.where(rowid == 0, n_buf[pl.ds(t1, 1), :], n_buf[pl.ds(t2, 1), :]).astype(BF16)

    gt = _r(jnp.dot(xs, wa_buf[:, 0:F], preferred_element_type=F32))
    up = _r(jnp.dot(xs, wb_buf[:, 0:F], preferred_element_type=F32))
    hid = (_r(gt * _r(jax.nn.sigmoid(gt))) * up).astype(BF16)
    y = _r(jnp.dot(hid, wd_buf[:, 0:D], preferred_element_type=F32))
    y1 = _r(y[0:1, :] * _r(jax.nn.sigmoid(_r(m1 + rc_buf[1:2, 0:1]))))
    y2 = _r(y[1:2, :] * _r(jax.nn.sigmoid(_r(m2 + rc_buf[1:2, 0:1]))))

    def fix(i, t):
        g = pl.multiple_of(lax.shift_right_logical(i, 4) * PR, PR)
        tg = pl.multiple_of(lax.shift_right_logical(t, 4) * PR, PR)
        rid = rowid + g
        upd = jnp.where(rid == i1, y1, jnp.where(rid == i2, y2, 0.0))
        h2g = n_buf[pl.ds(tg, PR), :] + upd
        return g, (x2_buf[pl.ds(tg, PR), :]
                   + _rows8(h2g, jnp.multiply, coef[1, C_GB])).astype(BF16)

    g1, fix1 = fix(i1, t1)
    g2, fix2 = fix(i2, t2)
    for b in range(NRB):
        cp_out(b).wait()
    act[pl.ds(g1, PR), :] = fix1
    act[pl.ds(g2, PR), :] = fix2
    f1 = cp(act.at[pl.ds(g1, PR), :], out_hbm.at[pl.ds(g1, PR), :], SEM_OUT)
    f2 = cp(act.at[pl.ds(g2, PR), :], out_hbm.at[pl.ds(g2, PR), :], SEM_FIX)
    f1.start()

    @pl.when(g1 != g2)
    def _():
        f2.start()
        f2.wait()

    f1.wait()


@jax.jit
def pallas_adaLN_cond__mha_block_cached__moe_arch_mod__prompt_kernel(
    A_x: jax.Array,
    A_k_cache: jax.Array,
    A_v_cache: jax.Array,
    A_wq: jax.Array,
    A_wo: jax.Array,
    B_x: jax.Array,
    B_w_r: jax.Array,
    B_w_gate: jax.Array,
    B_w_up: jax.Array,
    B_w_down: jax.Array,
    c: jax.Array,
    w_mod: jax.Array,
):
    del B_x
    hbm = pl.BlockSpec(memory_space=pl.ANY)
    out = pl.pallas_call(
        _kernel,
        in_specs=[hbm] * 11,
        out_specs=hbm,
        out_shape=jax.ShapeDtypeStruct((S, D), BF16),
        scratch_shapes=[
            pltpu.VMEM((S, D), BF16),
            pltpu.VMEM((H, S, DH), BF16),
            pltpu.VMEM((H, S, DH), BF16),
            pltpu.VMEM((H, D, DH), BF16),
            pltpu.VMEM((H, DH, D), BF16),
            pltpu.VMEM((D, F + PAD), BF16),
            pltpu.VMEM((D, F + PAD), BF16),
            pltpu.VMEM((F, D + PAD), BF16),
            pltpu.VMEM((S + PR, D), BF16),
            pltpu.VMEM((S, D), F32),
            pltpu.VMEM((2 * SUB, D), F32),
            pltpu.VMEM((SUB + 2 * PR, D), F32),
            pltpu.VMEM((PR, 128), F32),
            pltpu.VMEM((2, 5, 8, D), F32),
            pltpu.VMEM((8, 128), BF16),
            pltpu.VMEM((8, D), F32),
            pltpu.VMEM((8, 128), F32),
            pltpu.VMEM((1, D), BF16),
            pltpu.VMEM((8, 128), I32),
            pltpu.VMEM((FILL, DH), F32),
            pltpu.VMEM((2, SUB, DH), F32),
            pltpu.VMEM((2, SUB, DH), F32),
            pltpu.SemaphoreType.DMA((NSEM,)),
        ],
        compiler_params=pltpu.CompilerParams(
            vmem_limit_bytes=120 * 1024 * 1024,
        ),
        name="adaln_mha_mod",
    )(
        A_x.reshape(S, D),
        A_k_cache.reshape(H, S, DH),
        A_v_cache.reshape(H, S, DH),
        A_wq,
        A_wo.reshape(H, DH, D),
        B_w_r.reshape(8, 128),
        B_w_gate,
        B_w_up,
        B_w_down,
        c,
        w_mod,
    )
    return out.reshape(1, S, D)
```

```python
import jax
import jax.numpy as jnp
from jax import lax
import jax.experimental.pallas as pl
import jax.experimental.pallas.tpu as pltpu

S = 2048
D = 1024
H = 32
DH = 128
F = 3584
SUB = 256
NRB = S // SUB
NU = H * NRB
PR = 16
UM = 12
R2 = 8
RAMP = 2 * R2
NM = (NU - RAMP) // UM
HPI = UM // 2
NLOAD = (2 * H - RAMP) // UM
FIN_START = 130
K_MOD = (FIN_START - RAMP) // UM
LN_START = RAMP + K_MOD * UM - (S - 2 * SUB) // PR
FILL = 64
ECH = 128
PAD = 128
MCH = 4
EPS = 1e-5
QSCALE = float(DH ** -0.5) * 1.4426950408889634

F32 = jnp.float32
BF16 = jnp.bfloat16
I32 = jnp.int32
NT = (((1,), (1,)), ((), ()))

C_GA, C_SCALE, C_SHIFT, C_KEEP, C_GB = range(5)


def _r(v):
    return v.astype(BF16).astype(F32)


def _rows8(v, fn, c):
    n = v.shape[0] // 8
    return fn(v.reshape(n, 8, D), c[None]).reshape(v.shape)


def _ln_stats(y):
    m = jnp.mean(y, axis=-1, keepdims=True)
    yc = y - m
    v = jnp.mean(yc * yc, axis=-1, keepdims=True)
    den = _r(jnp.sqrt(_r(_r(v) + EPS)))
    return yc, m, _r(m), 1.0 / den


def _layernorm(y):
    _, _, mr, rinv = _ln_stats(y)
    return (y - mr) * rinv


def _lane_fold(p, fn):
    t = p[:, 0:128]
    for j in range(1, p.shape[1] // 128):
        t = fn(t, p[:, j * 128:(j + 1) * 128])
    return t


def _normalize(pv, ls):
    l = jnp.sum(ls, axis=-1, keepdims=True)
    r = pl.reciprocal(l, approx=True)
    r = r * (2.0 - l * r)
    return (pv * r).astype(BF16)


def _head_of(n):
    if isinstance(n, int):
        return (n % 64) // 2 if n < 192 else (n - 192) % H
    return jnp.where(n < 192, lax.shift_right_logical(n & 63, 1), (n - 192) & (H - 1))


def _row_of(n):
    if isinstance(n, int):
        return SUB * ((n // 64) * 2 + n % 2 if n < 192 else min(n // 32, NRB - 1))
    rb = jnp.where(n < 192, lax.shift_right_logical(n, 6) * 2 + (n & 1),
                   jnp.minimum(lax.shift_right_logical(n, 5), NRB - 1))
    return pl.multiple_of(rb * SUB, SUB)


(SEM_C, SEM_WR, SEM_X0, SEM_XR, SEM_M12, SEM_FFN, SEM_OUT, SEM_FIX,
 SEM_WQ0, SEM_K0, SEM_M0) = range(11)
SEM_RAMP = SEM_M0 + MCH
SEM_MAIN = SEM_RAMP + R2
NSEM = SEM_MAIN + NLOAD


def _kernel(x_hbm, k_hbm, v_hbm, wq_hbm, wo_hbm, wr_hbm, wg_hbm, wu_hbm, wd_hbm,
            c_hbm, wmod_hbm, out_hbm,
            x_buf, k_buf, v_buf, wq_buf, wo_buf, wa_buf, wb_buf, wd_buf,
            act, acc, n_buf, x2_buf, r_buf, coef, wr_buf, sw_buf, rc_buf, c_buf, zero_buf, qa_car, pv_car, ls_car,
            sems):
    def cp(src, dst, slot):
        return pltpu.make_async_copy(src, dst, sems.at[slot])

    def cp_x(b, nb, slot):
        return cp(x_hbm.at[pl.ds(b * SUB, nb * SUB), :],
                  x_buf.at[pl.ds(b * SUB, nb * SUB), :], slot)

    def cp_wq(h, slot):
        col = h * DH if isinstance(h, int) else pl.multiple_of(h * DH, DH)
        return cp(wq_hbm.at[:, pl.ds(col, DH)], wq_buf.at[h], slot)

    def cp_h(src, dst, h0, nh, slot):
        return cp(src.at[pl.ds(h0, nh)], dst.at[pl.ds(h0, nh)], slot)

    def heads(h0, nh, slot, last=False):
        return [cp_h(k_hbm, k_buf, h0, nh, slot), cp_h(v_hbm, v_buf, h0, nh, slot),
                cp_h(wo_hbm, wo_buf, h0 - 1, nh + 1 if last else nh, slot)] + [
            cp_wq(h0 + 1 + j, slot) for j in range(nh - 1 if last else nh)]

    def ramp_heads(j):
        return heads(j, 1, SEM_RAMP + j)

    def main_heads(k, last=False):
        return heads(RAMP // 2 + k * HPI, HPI, SEM_MAIN + k, last)

    cp_k0 = cp_h(k_hbm, k_buf, 0, 1, SEM_K0)
    cp_v0 = [cp_h(v_hbm, v_buf, 0, 1, SEM_RAMP), cp_wq(1, SEM_RAMP)]
    mrows = D // MCH
    cp_m0 = [cp(wmod_hbm.at[pl.ds(j * mrows, mrows), 0:2 * D],
                wa_buf.at[pl.ds(j * mrows, mrows), 0:2 * D], SEM_M0 + j) for j in range(MCH)]
    cp_c = cp(c_hbm, c_buf, SEM_C)
    cp_wr = cp(wr_hbm, wr_buf, SEM_WR)
    cp_m12 = [cp(wmod_hbm.at[:, 2 * D:3 * D], wa_buf.at[:, 2 * D:3 * D], SEM_M12),
              cp(wmod_hbm.at[:, 3 * D:6 * D], wb_buf.at[:, 0:3 * D], SEM_M12)]
    cp_ffn = [cp(wg_hbm, wa_buf.at[:, 0:F], SEM_FFN),
              cp(wu_hbm, wb_buf.at[:, 0:F], SEM_FFN),
              cp(wd_hbm, wd_buf.at[:, 0:D], SEM_FFN)]

    def cp_out(b):
        row = b * SUB if isinstance(b, int) else pl.multiple_of(b * SUB, SUB)
        return cp(act.at[pl.ds(row, SUB), :], out_hbm.at[pl.ds(row, SUB), :], SEM_OUT)

    def silu_c():
        cf = c_buf[...].astype(F32)
        sc = (cf * _r(jax.nn.sigmoid(cf))).astype(BF16)
        return jnp.broadcast_to(sc, (16, D))

    def packed(ref, h):
        return pltpu.bitcast(ref.bitcast(jnp.uint32)[h], BF16)

    def modulate(n):
        n = _rows8(n, jnp.multiply, coef[C_SCALE])
        return _rows8(n, jnp.add, coef[C_SHIFT])

    def ada_ln_router(y):
        yc, m, mr, rinv = _ln_stats(y)
        d = jnp.sum(_rows8(yc, jnp.multiply, sw_buf[...]), axis=-1, keepdims=True)
        r = (d + (m - mr) * rc_buf[0:1, 0:1]) * rinv
        return modulate((y - mr) * rinv), r

    def resid(a, row, nrows):
        a = _rows8(a, jnp.multiply, coef[C_GA])
        return _r(x_buf[pl.ds(row, nrows), :].astype(F32) + a)

    def piece(src, dst, lane_id):
        y = resid(acc[pl.ds(src, PR), :], src, PR)
        nn = _layernorm(y)
        hh = modulate(nn)
        r = jnp.sum(_rows8(nn, jnp.multiply, sw_buf[...]), axis=-1, keepdims=True)
        oo = (_rows8(y, jnp.multiply, coef[C_KEEP])
              + _rows8(hh, jnp.multiply, coef[C_GB]))
        act[pl.ds(dst, PR), :] = oo.astype(BF16)
        lane = lax.broadcasted_iota(I32, (PR, 128), 1)
        rn = jnp.where(lane == lane_id, r, r_buf[...])
        r_buf[...] = rn
        return oo, rn

    def unit_piece(n):
        is_ln = jnp.logical_and(n >= LN_START, n < LN_START + (S - 2 * SUB) // PR)
        is_fin = jnp.logical_and(n >= FIN_START, n < FIN_START + (S - SUB) // PR)
        f = n - FIN_START
        src = jnp.where(is_ln, 2 * SUB + (n - LN_START) * PR, jnp.where(is_fin, f * PR, 0))
        dst = jnp.where(jnp.logical_or(is_ln, is_fin), src, S)
        oo, rn = piece(pl.multiple_of(src, PR), pl.multiple_of(dst, PR),
                       jnp.where(is_fin, f, -1))
        bits = _lane_fold(pltpu.bitcast(oo, I32), jnp.bitwise_or) | pltpu.bitcast(rn, I32)
        return (bits[0:8] | bits[8:16]) & zero_buf[...]

    def qproj_head(n):
        return jnp.dot(act[pl.ds(_row_of(n), FILL), 0:D // 2],
                       packed(wq_buf, _head_of(n))[0:D // 2], preferred_element_type=F32)

    def qproj_rest(n, qa):
        row = _row_of(n)
        w = packed(wq_buf, _head_of(n))
        row2 = row + FILL if isinstance(row, int) else pl.multiple_of(row + FILL, 16)
        qb = jnp.dot(act[pl.ds(row, SUB), D // 2:D], w[D // 2:D], preferred_element_type=F32)
        qc = jnp.dot(act[pl.ds(row2, SUB - FILL), 0:D // 2], w[0:D // 2],
                     preferred_element_type=F32)
        return ((qb + jnp.concatenate([qa, qc], axis=0)) * QSCALE).astype(BF16)

    def oproj(o, n):
        acc[pl.ds(_row_of(n), SUB), :] += jnp.dot(o, wo_buf[_head_of(n)],
                                                  preferred_element_type=F32)

    def unit_block(n0, nunits, with_piece):
        o = _normalize(pv_car[0], ls_car[0])
        raw = (pv_car[1], ls_car[1])
        qa = qa_car[...]
        for u in range(nunits):
            n = n0 + u
            hd = _head_of(n)
            q = qproj_rest(n, qa)
            z = unit_piece(n) if with_piece else None
            oproj(o, n - 2)
            sc = lax.dot_general(q, packed(k_buf, hd), NT, preferred_element_type=F32)
            qa = qproj_head(n + 1)
            mm = _lane_fold(sc, jnp.maximum)
            if with_piece:
                mb = pltpu.bitcast(mm, I32)
                mm = pltpu.bitcast(jnp.concatenate([mb[0:8] | z, mb[8:]], axis=0), F32)
            m = jnp.max(mm, axis=-1, keepdims=True)
            p = jnp.exp2(sc - m)
            ls = _lane_fold(p, jnp.add)
            pv = jnp.dot(p.astype(BF16), packed(v_buf, hd), preferred_element_type=F32)
            if u + 1 < nunits:
                zb = (pltpu.bitcast(pv, I32).reshape(SUB // 8, 8, 128)
                      & zero_buf[...][None]).reshape(SUB, 128)
                o = _normalize(raw[0], pltpu.bitcast(pltpu.bitcast(raw[1], I32) | zb, F32))
            else:
                pv_car[0] = raw[0]
                ls_car[0] = raw[1]
            raw = (pv, ls)
        pv_car[1] = raw[0]
        ls_car[1] = raw[1]
        qa_car[...] = qa

    def start(cps):
        for c_ in cps:
            c_.start()

    def wait(cps):
        for c_ in cps:
            c_.wait()

    start([cp_c, cp_x(0, 2, SEM_X0)] + cp_m0 + [cp_wq(0, SEM_WQ0), cp_k0] + cp_v0)
    for j in range(1, R2):
        start(ramp_heads(j))
    start([cp_wr])
    n_early = (LN_START - RAMP) // UM
    for k in range(n_early):
        start(main_heads(k))

    def zero_acc(j, carry):
        acc[pl.ds(pl.multiple_of(j * 64, 64), 64), :] = jnp.zeros((64, D), F32)
        return carry

    lax.fori_loop(0, S // 64, zero_acc, 0)
    r_buf[...] = jnp.zeros(r_buf.shape, F32)
    zero_buf[...] = jnp.zeros(zero_buf.shape, I32)
    coef[C_GA] = jnp.zeros((8, D), F32)
    coef[C_KEEP] = jnp.zeros((8, D), F32)
    coef[C_GB] = jnp.ones((8, D), F32)
    sw_buf[...] = jnp.zeros(sw_buf.shape, F32)
    rc_buf[...] = jnp.zeros(rc_buf.shape, F32)
    cp_c.wait()
    cp_x(0, 2, SEM_X0).wait()

    def norm_rows(j, carry):
        row = pl.multiple_of(j * 128, 128)
        n_buf[pl.ds(row, 128), :] = _layernorm(x_buf[pl.ds(row, 128), :].astype(F32))
        return carry

    lax.fori_loop(0, 2 * SUB // 128, norm_rows, 0)
    sc16 = silu_c()
    m0 = None
    for j in range(MCH):
        cp_m0[j].wait()
        part = jnp.dot(sc16[:, j * mrows:(j + 1) * mrows],
                       wa_buf[j * mrows:(j + 1) * mrows, 0:2 * D], preferred_element_type=F32)
        m0 = part if m0 is None else m0 + part
    m0 = _r(m0[0:8, :])
    coef[C_SHIFT] = m0[:, 0:D]
    coef[C_SCALE] = _r(1.0 + m0[:, D:2 * D])

    cp_wq(0, SEM_WQ0).wait()
    h01 = modulate(n_buf[...]).astype(BF16)
    act[0:2 * SUB, :] = h01
    q01 = (jnp.dot(h01, packed(wq_buf, 0), preferred_element_type=F32) * QSCALE).astype(BF16)
    cp_k0.wait()
    s01 = lax.dot_general(q01, packed(k_buf, 0), NT, preferred_element_type=F32)
    m01 = jnp.max(_lane_fold(s01, jnp.maximum), axis=-1, keepdims=True)
    wait(cp_v0)
    qa_car[...] = qproj_head(2)
    for u in range(2):
        p = jnp.exp2(s01[u * SUB:(u + 1) * SUB] - m01[u * SUB:(u + 1) * SUB])
        ls_car[u] = _lane_fold(p, jnp.add)
        pv_car[u] = jnp.dot(p.astype(BF16), packed(v_buf, 0), preferred_element_type=F32)

    def ramp2(j, carry):
        wait(ramp_heads(j))
        unit_block(2 * j, 2, False)
        return carry

    lax.fori_loop(1, R2, ramp2, 0)
    start([cp_x(2, NRB - 2, SEM_XR)])
    for k in range(n_early, NLOAD):
        start(main_heads(k, k == NLOAD - 1))
    start(cp_m12)

    def blocks_done(n0):
        return (n0 - FIN_START) // (SUB // PR)

    def main(k, carry):
        n0 = RAMP + k * UM

        @pl.when(k <= K_MOD + 2)
        def _():
            @pl.when(k < NLOAD - 1)
            def _():
                wait(main_heads(k))

            @pl.when(k == NLOAD - 1)
            def _():
                wait(main_heads(NLOAD - 1, True))

            @pl.when(k == n_early)
            def _():
                cp_x(2, NRB - 2, SEM_XR).wait()

            @pl.when(k == K_MOD)
            def _():
                wait(cp_m12 + [cp_wr])
                sc = silu_c()
                m1 = _r(jnp.dot(sc, wa_buf[:, 2 * D:3 * D], preferred_element_type=F32)[0:8, :])
                m2 = _r(jnp.dot(sc, wb_buf[:, 0:3 * D], preferred_element_type=F32)[0:8, :])
                coef[C_GA] = m1
                coef[C_KEEP] = jnp.ones((8, D), F32)
                scale = _r(1.0 + m2[:, D:2 * D])
                coef[C_SHIFT] = m2[:, 0:D]
                coef[C_SCALE] = scale
                coef[C_GB] = m2[:, 2 * D:3 * D]
                w8 = wr_buf[...].astype(F32)
                wr = jnp.concatenate([jnp.broadcast_to(w8[j:j + 1, :], (8, 128))
                                      for j in range(D // 128)], axis=1)
                sw_buf[...] = scale * wr
                c1 = jnp.sum(scale * wr, axis=-1, keepdims=True)
                c0 = jnp.sum(m2[:, 0:D] * wr, axis=-1, keepdims=True)
                rid = lax.broadcasted_iota(I32, (8, 128), 0)
                rc_buf[...] = jnp.where(rid == 0, c1, c0)
                start(cp_ffn)

            @pl.when(k == K_MOD + 2)
            def _():
                wait(cp_ffn)

        done = lax.shift_right_arithmetic(n0 - FIN_START, 4)
        done_before = lax.shift_right_arithmetic(n0 - UM - FIN_START, 4)

        @pl.when(jnp.logical_and(done >= 1, done > done_before))
        def _():
            cp_out(jnp.maximum(done - 1, 0)).start()

        unit_block(n0, UM, True)
        return carry

    lax.fori_loop(0, NM, main, 0)

    for b in range(blocks_done(RAMP + (NM - 1) * UM), NRB - 1):
        cp_out(b).start()
    row0 = (NRB - 1) * SUB
    neg = -jnp.inf

    def all_red(v, fn):
        return fn(fn(v, axis=0, keepdims=True), axis=1, keepdims=True)

    lane = lax.broadcasted_iota(I32, (PR, 128), 1)
    ridx = (lane * PR + lax.broadcasted_iota(I32, (PR, 128), 0)).astype(F32)
    rr = jnp.where(lane < row0 // PR, r_buf[...], neg)
    last_old = float(row0 - 1)
    cm1 = all_red(rr, jnp.max)
    ci1 = all_red(jnp.where(rr == cm1, ridx, last_old), jnp.min)
    rr2 = jnp.where(ridx == ci1, neg, rr)
    cm2 = all_red(rr2, jnp.max)
    ci2 = all_red(jnp.where(jnp.logical_and(rr2 == cm2, ridx != ci1), ridx, last_old), jnp.min)
    ci1 = jnp.minimum(ci1, last_old).astype(I32)
    ci2 = jnp.minimum(ci2, last_old).astype(I32)
    for j, ci in enumerate((ci1, ci2)):
        g = pl.multiple_of(lax.shift_right_logical(ci[0, 0], 4) * PR, PR)
        y = resid(acc[pl.ds(g, PR), :], g, PR)
        x2_buf[SUB + j * PR:SUB + (j + 1) * PR, :] = y
        n_buf[SUB + j * PR:SUB + (j + 1) * PR, :] = modulate(_layernorm(y))

    o2 = jnp.concatenate([_normalize(pv_car[0], ls_car[0]),
                          _normalize(pv_car[1], ls_car[1])], axis=1)
    wo2 = jnp.concatenate([wo_buf[H - 2], wo_buf[H - 1]], axis=0)
    r_new = []
    for j in range(SUB // ECH):
        lo, hi = j * ECH, (j + 1) * ECH
        a = acc[row0 + lo:row0 + hi, :] + jnp.dot(o2[lo:hi], wo2, preferred_element_type=F32)
        y = resid(a, row0 + lo, ECH)
        hh, r = ada_ln_router(y)
        x2_buf[lo:hi, :] = y
        n_buf[lo:hi, :] = hh
        act[row0 + lo:row0 + hi, :] = (
            y + _rows8(hh, jnp.multiply, coef[C_GB])).astype(BF16)
        r_new.append(r)
    cp_out(NRB - 1).start()

    sub8 = lax.broadcasted_iota(I32, (8, 1), 0)
    big = jnp.int32((S - 1) * 512 + SUB - 1)
    vals = jnp.concatenate(
        r_new + [jnp.where(sub8 == 0, cm1, jnp.where(sub8 == 1, cm2, neg))], axis=0)
    pos = lax.broadcasted_iota(I32, (SUB, 1), 0)
    cc1 = ci1 * 512 + SUB + (ci1 & (PR - 1))
    cc2 = ci2 * 512 + SUB + PR + (ci2 & (PR - 1))
    code = jnp.concatenate(
        [(pos + row0) * 512 + pos,
         jnp.where(sub8 == 0, cc1, jnp.where(sub8 == 1, cc2, big))], axis=0)
    m1 = jnp.max(vals, axis=0, keepdims=True)
    k1 = jnp.min(jnp.where(vals == m1, code, big), axis=0, keepdims=True)
    vals2 = jnp.where(code == k1, neg, vals)
    m2 = jnp.max(vals2, axis=0, keepdims=True)
    k2 = jnp.min(jnp.where(jnp.logical_and(vals2 == m2, code != k1), code, big),
                 axis=0, keepdims=True)
    k1 = k1[0, 0]
    k2 = k2[0, 0]
    i1 = lax.shift_right_logical(k1, 9)
    i2 = lax.shift_right_logical(k2, 9)
    t1 = k1 & 511
    t2 = k2 & 511
    rowid = lax.broadcasted_iota(I32, (PR, D), 0)
    xs = jnp.where(rowid == 0, n_buf[pl.ds(t1, 1), :], n_buf[pl.ds(t2, 1), :]).astype(BF16)

    gt = _r(jnp.dot(xs, wa_buf[:, 0:F], preferred_element_type=F32))
    up = _r(jnp.dot(xs, wb_buf[:, 0:F], preferred_element_type=F32))
    hid = (_r(gt * _r(jax.nn.sigmoid(gt))) * up).astype(BF16)
    y = _r(jnp.dot(hid, wd_buf[:, 0:D], preferred_element_type=F32))
    y1 = _r(y[0:1, :] * _r(jax.nn.sigmoid(_r(m1 + rc_buf[1:2, 0:1]))))
    y2 = _r(y[1:2, :] * _r(jax.nn.sigmoid(_r(m2 + rc_buf[1:2, 0:1]))))

    def fix(i, t):
        g = pl.multiple_of(lax.shift_right_logical(i, 4) * PR, PR)
        tg = pl.multiple_of(lax.shift_right_logical(t, 4) * PR, PR)
        rid = rowid + g
        upd = jnp.where(rid == i1, y1, jnp.where(rid == i2, y2, 0.0))
        h2g = n_buf[pl.ds(tg, PR), :] + upd
        return g, (x2_buf[pl.ds(tg, PR), :]
                   + _rows8(h2g, jnp.multiply, coef[C_GB])).astype(BF16)

    g1, fix1 = fix(i1, t1)
    g2, fix2 = fix(i2, t2)
    for b in range(NRB):
        cp_out(b).wait()
    act[pl.ds(g1, PR), :] = fix1
    act[pl.ds(g2, PR), :] = fix2
    f1 = cp(act.at[pl.ds(g1, PR), :], out_hbm.at[pl.ds(g1, PR), :], SEM_OUT)
    f2 = cp(act.at[pl.ds(g2, PR), :], out_hbm.at[pl.ds(g2, PR), :], SEM_FIX)
    f1.start()

    @pl.when(g1 != g2)
    def _():
        f2.start()
        f2.wait()

    f1.wait()


@jax.jit
def pallas_adaLN_cond__mha_block_cached__moe_arch_mod__prompt_kernel(
    A_x: jax.Array,
    A_k_cache: jax.Array,
    A_v_cache: jax.Array,
    A_wq: jax.Array,
    A_wo: jax.Array,
    B_x: jax.Array,
    B_w_r: jax.Array,
    B_w_gate: jax.Array,
    B_w_up: jax.Array,
    B_w_down: jax.Array,
    c: jax.Array,
    w_mod: jax.Array,
):
    del B_x
    hbm = pl.BlockSpec(memory_space=pl.ANY)
    out = pl.pallas_call(
        _kernel,
        in_specs=[hbm] * 11,
        out_specs=hbm,
        out_shape=jax.ShapeDtypeStruct((S, D), BF16),
        scratch_shapes=[
            pltpu.VMEM((S, D), BF16),
            pltpu.VMEM((H, S, DH), BF16),
            pltpu.VMEM((H, S, DH), BF16),
            pltpu.VMEM((H, D, DH), BF16),
            pltpu.VMEM((H, DH, D), BF16),
            pltpu.VMEM((D, F + PAD), BF16),
            pltpu.VMEM((D, F + PAD), BF16),
            pltpu.VMEM((F, D + PAD), BF16),
            pltpu.VMEM((S + PR, D), BF16),
            pltpu.VMEM((S, D), F32),
            pltpu.VMEM((2 * SUB, D), F32),
            pltpu.VMEM((SUB + 2 * PR, D), F32),
            pltpu.VMEM((PR, 128), F32),
            pltpu.VMEM((5, 8, D), F32),
            pltpu.VMEM((8, 128), BF16),
            pltpu.VMEM((8, D), F32),
            pltpu.VMEM((8, 128), F32),
            pltpu.VMEM((1, D), BF16),
            pltpu.VMEM((8, 128), I32),
            pltpu.VMEM((FILL, DH), F32),
            pltpu.VMEM((2, SUB, DH), F32),
            pltpu.VMEM((2, SUB, DH), F32),
            pltpu.SemaphoreType.DMA((NSEM,)),
        ],
        compiler_params=pltpu.CompilerParams(
            vmem_limit_bytes=120 * 1024 * 1024,
        ),
        name="adaln_mha_mod",
    )(
        A_x.reshape(S, D),
        A_k_cache.reshape(H, S, DH),
        A_v_cache.reshape(H, S, DH),
        A_wq,
        A_wo.reshape(H, DH, D),
        B_w_r.reshape(8, 128),
        B_w_gate,
        B_w_up,
        B_w_down,
        c,
        w_mod,
    )
    return out.reshape(1, S, D)
```

```python
import jax
import jax.numpy as jnp
from jax import lax
import jax.experimental.pallas as pl
import jax.experimental.pallas.tpu as pltpu

S = 2048
D = 1024
H = 32
DH = 128
F = 3584
SUB = 256
NRB = S // SUB
NU = H * NRB
PR = 16
UM = 12
R2 = 8
RAMP = 2 * R2
NM = (NU - RAMP) // UM
HPI = UM // 2
NLOAD = (2 * H - RAMP) // UM
FIN_START = 130
K_MOD = (FIN_START - RAMP) // UM
LN_START = RAMP + K_MOD * UM - (S - 2 * SUB) // PR
FILL = 64
ECH = 64
PAD = 128
MCH = 4
EPS = 1e-5
QSCALE = float(DH ** -0.5) * 1.4426950408889634

F32 = jnp.float32
BF16 = jnp.bfloat16
I32 = jnp.int32
NT = (((1,), (1,)), ((), ()))

C_GA, C_SCALE, C_SHIFT, C_KEEP, C_GB = range(5)


def _r(v):
    return v.astype(BF16).astype(F32)


def _rows8(v, fn, c):
    n = v.shape[0] // 8
    return fn(v.reshape(n, 8, D), c[None]).reshape(v.shape)


def _ln_stats(y):
    m = jnp.mean(y, axis=-1, keepdims=True)
    yc = y - m
    v = jnp.mean(yc * yc, axis=-1, keepdims=True)
    den = _r(jnp.sqrt(_r(_r(v) + EPS)))
    return yc, m, _r(m), 1.0 / den


def _layernorm(y):
    _, _, mr, rinv = _ln_stats(y)
    return (y - mr) * rinv


def _lane_fold(p, fn):
    t = p[:, 0:128]
    for j in range(1, p.shape[1] // 128):
        t = fn(t, p[:, j * 128:(j + 1) * 128])
    return t


def _normalize(pv, ls):
    l = jnp.sum(ls, axis=-1, keepdims=True)
    r = pl.reciprocal(l, approx=True)
    r = r * (2.0 - l * r)
    return (pv * r).astype(BF16)


def _head_of(n):
    if isinstance(n, int):
        return (n % 64) // 2 if n < 192 else (n - 192) % H
    return jnp.where(n < 192, lax.shift_right_logical(n & 63, 1), (n - 192) & (H - 1))


def _row_of(n):
    if isinstance(n, int):
        return SUB * ((n // 64) * 2 + n % 2 if n < 192 else min(n // 32, NRB - 1))
    rb = jnp.where(n < 192, lax.shift_right_logical(n, 6) * 2 + (n & 1),
                   jnp.minimum(lax.shift_right_logical(n, 5), NRB - 1))
    return pl.multiple_of(rb * SUB, SUB)


(SEM_C, SEM_WR, SEM_X0, SEM_XR, SEM_M12, SEM_FFN, SEM_OUT, SEM_FIX,
 SEM_WQ0, SEM_K0, SEM_M0) = range(11)
SEM_RAMP = SEM_M0 + MCH
SEM_MAIN = SEM_RAMP + R2
NSEM = SEM_MAIN + NLOAD


def _kernel(x_hbm, k_hbm, v_hbm, wq_hbm, wo_hbm, wr_hbm, wg_hbm, wu_hbm, wd_hbm,
            c_hbm, wmod_hbm, out_hbm,
            x_buf, k_buf, v_buf, wq_buf, wo_buf, wa_buf, wb_buf, wd_buf,
            act, acc, n_buf, x2_buf, st_buf, r_buf, coef, wr_buf, sw_buf, rc_buf, c_buf, zero_buf, qa_car, pv_car, ls_car,
            sems):
    def cp(src, dst, slot):
        return pltpu.make_async_copy(src, dst, sems.at[slot])

    def cp_x(b, nb, slot):
        return cp(x_hbm.at[pl.ds(b * SUB, nb * SUB), :],
                  x_buf.at[pl.ds(b * SUB, nb * SUB), :], slot)

    def cp_wq(h, slot):
        col = h * DH if isinstance(h, int) else pl.multiple_of(h * DH, DH)
        return cp(wq_hbm.at[:, pl.ds(col, DH)], wq_buf.at[h], slot)

    def cp_h(src, dst, h0, nh, slot):
        return cp(src.at[pl.ds(h0, nh)], dst.at[pl.ds(h0, nh)], slot)

    def heads(h0, nh, slot, last=False):
        return [cp_h(k_hbm, k_buf, h0, nh, slot), cp_h(v_hbm, v_buf, h0, nh, slot),
                cp_h(wo_hbm, wo_buf, h0 - 1, nh + 1 if last else nh, slot)] + [
            cp_wq(h0 + 1 + j, slot) for j in range(nh - 1 if last else nh)]

    def ramp_heads(j):
        return heads(j, 1, SEM_RAMP + j)

    def main_heads(k, last=False):
        return heads(RAMP // 2 + k * HPI, HPI, SEM_MAIN + k, last)

    cp_k0 = cp_h(k_hbm, k_buf, 0, 1, SEM_K0)
    cp_v0 = [cp_h(v_hbm, v_buf, 0, 1, SEM_RAMP), cp_wq(1, SEM_RAMP)]
    mrows = D // MCH
    cp_m0 = [cp(wmod_hbm.at[pl.ds(j * mrows, mrows), 0:2 * D],
                wa_buf.at[pl.ds(j * mrows, mrows), 0:2 * D], SEM_M0 + j) for j in range(MCH)]
    cp_c = cp(c_hbm, c_buf, SEM_C)
    cp_wr = cp(wr_hbm, wr_buf, SEM_WR)
    cp_m12 = [cp(wmod_hbm.at[:, 2 * D:3 * D], wa_buf.at[:, 2 * D:3 * D], SEM_M12),
              cp(wmod_hbm.at[:, 3 * D:6 * D], wb_buf.at[:, 0:3 * D], SEM_M12)]
    cp_ffn = [cp(wg_hbm, wa_buf.at[:, 0:F], SEM_FFN),
              cp(wu_hbm, wb_buf.at[:, 0:F], SEM_FFN),
              cp(wd_hbm, wd_buf.at[:, 0:D], SEM_FFN)]

    def cp_out(b):
        row = b * SUB if isinstance(b, int) else pl.multiple_of(b * SUB, SUB)
        return cp(act.at[pl.ds(row, SUB), :], out_hbm.at[pl.ds(row, SUB), :], SEM_OUT)

    def silu_c():
        cf = c_buf[...].astype(F32)
        sc = (cf * _r(jax.nn.sigmoid(cf))).astype(BF16)
        return jnp.broadcast_to(sc, (16, D))

    def packed(ref, h):
        return pltpu.bitcast(ref.bitcast(jnp.uint32)[h], BF16)

    def modulate(n):
        n = _rows8(n, jnp.multiply, coef[C_SCALE])
        return _rows8(n, jnp.add, coef[C_SHIFT])

    def resid(a, row, nrows):
        a = _rows8(a, jnp.multiply, coef[C_GA])
        return _r(x_buf[pl.ds(row, nrows), :].astype(F32) + a)

    def piece(src, dst, lane_id):
        y = resid(acc[pl.ds(src, PR), :], src, PR)
        nn = _layernorm(y)
        hh = modulate(nn)
        r = jnp.sum(_rows8(nn, jnp.multiply, sw_buf[...]), axis=-1, keepdims=True)
        oo = (_rows8(y, jnp.multiply, coef[C_KEEP])
              + _rows8(hh, jnp.multiply, coef[C_GB]))
        act[pl.ds(dst, PR), :] = oo.astype(BF16)
        lane = lax.broadcasted_iota(I32, (PR, 128), 1)
        rn = jnp.where(lane == lane_id, r, r_buf[...])
        r_buf[...] = rn
        return oo, rn

    def unit_piece(n):
        is_ln = jnp.logical_and(n >= LN_START, n < LN_START + (S - 2 * SUB) // PR)
        is_fin = jnp.logical_and(n >= FIN_START, n < FIN_START + (S - SUB) // PR)
        f = n - FIN_START
        src = jnp.where(is_ln, 2 * SUB + (n - LN_START) * PR, jnp.where(is_fin, f * PR, 0))
        dst = jnp.where(jnp.logical_or(is_ln, is_fin), src, S)
        oo, rn = piece(pl.multiple_of(src, PR), pl.multiple_of(dst, PR),
                       jnp.where(is_fin, f, -1))
        bits = _lane_fold(pltpu.bitcast(oo, I32), jnp.bitwise_or) | pltpu.bitcast(rn, I32)
        return (bits[0:8] | bits[8:16]) & zero_buf[...]

    def qproj_head(n):
        return jnp.dot(act[pl.ds(_row_of(n), FILL), 0:D // 2],
                       packed(wq_buf, _head_of(n))[0:D // 2], preferred_element_type=F32)

    def qproj_rest(n, qa):
        row = _row_of(n)
        w = packed(wq_buf, _head_of(n))
        row2 = row + FILL if isinstance(row, int) else pl.multiple_of(row + FILL, 16)
        qb = jnp.dot(act[pl.ds(row, SUB), D // 2:D], w[D // 2:D], preferred_element_type=F32)
        qc = jnp.dot(act[pl.ds(row2, SUB - FILL), 0:D // 2], w[0:D // 2],
                     preferred_element_type=F32)
        return ((qb + jnp.concatenate([qa, qc], axis=0)) * QSCALE).astype(BF16)

    def oproj(o, n):
        acc[pl.ds(_row_of(n), SUB), :] += jnp.dot(o, wo_buf[_head_of(n)],
                                                  preferred_element_type=F32)

    def unit_block(n0, nunits, with_piece):
        o = _normalize(pv_car[0], ls_car[0])
        raw = (pv_car[1], ls_car[1])
        qa = qa_car[...]
        for u in range(nunits):
            n = n0 + u
            hd = _head_of(n)
            q = qproj_rest(n, qa)
            z = unit_piece(n) if with_piece else None
            oproj(o, n - 2)
            sc = lax.dot_general(q, packed(k_buf, hd), NT, preferred_element_type=F32)
            qa = qproj_head(n + 1)
            mm = _lane_fold(sc, jnp.maximum)
            if with_piece:
                mb = pltpu.bitcast(mm, I32)
                mm = pltpu.bitcast(jnp.concatenate([mb[0:8] | z, mb[8:]], axis=0), F32)
            m = jnp.max(mm, axis=-1, keepdims=True)
            p = jnp.exp2(sc - m)
            ls = _lane_fold(p, jnp.add)
            pv = jnp.dot(p.astype(BF16), packed(v_buf, hd), preferred_element_type=F32)
            if u + 1 < nunits:
                zb = (pltpu.bitcast(pv, I32).reshape(SUB // 8, 8, 128)
                      & zero_buf[...][None]).reshape(SUB, 128)
                o = _normalize(raw[0], pltpu.bitcast(pltpu.bitcast(raw[1], I32) | zb, F32))
            else:
                pv_car[0] = raw[0]
                ls_car[0] = raw[1]
            raw = (pv, ls)
        pv_car[1] = raw[0]
        ls_car[1] = raw[1]
        qa_car[...] = qa

    def start(cps):
        for c_ in cps:
            c_.start()

    def wait(cps):
        for c_ in cps:
            c_.wait()

    start([cp_c, cp_x(0, 2, SEM_X0)] + cp_m0 + [cp_wq(0, SEM_WQ0), cp_k0] + cp_v0)
    for j in range(1, R2):
        start(ramp_heads(j))
    start([cp_wr])
    n_early = (LN_START - RAMP) // UM
    for k in range(n_early):
        start(main_heads(k))

    def zero_acc(j, carry):
        acc[pl.ds(pl.multiple_of(j * 64, 64), 64), :] = jnp.zeros((64, D), F32)
        return carry

    lax.fori_loop(0, S // 64, zero_acc, 0)
    r_buf[...] = jnp.zeros(r_buf.shape, F32)
    zero_buf[...] = jnp.zeros(zero_buf.shape, I32)
    coef[C_GA] = jnp.zeros((8, D), F32)
    coef[C_KEEP] = jnp.zeros((8, D), F32)
    coef[C_GB] = jnp.ones((8, D), F32)
    sw_buf[...] = jnp.zeros(sw_buf.shape, F32)
    rc_buf[...] = jnp.zeros(rc_buf.shape, F32)
    cp_c.wait()
    cp_x(0, 2, SEM_X0).wait()

    def norm_rows(j, carry):
        row = pl.multiple_of(j * 128, 128)
        n_buf[pl.ds(row, 128), :] = _layernorm(x_buf[pl.ds(row, 128), :].astype(F32))
        return carry

    lax.fori_loop(0, 2 * SUB // 128, norm_rows, 0)
    sc16 = silu_c()
    m0 = None
    for j in range(MCH):
        cp_m0[j].wait()
        part = jnp.dot(sc16[:, j * mrows:(j + 1) * mrows],
                       wa_buf[j * mrows:(j + 1) * mrows, 0:2 * D], preferred_element_type=F32)
        m0 = part if m0 is None else m0 + part
    m0 = _r(m0[0:8, :])
    coef[C_SHIFT] = m0[:, 0:D]
    coef[C_SCALE] = _r(1.0 + m0[:, D:2 * D])

    cp_wq(0, SEM_WQ0).wait()
    h01 = modulate(n_buf[...]).astype(BF16)
    act[0:2 * SUB, :] = h01
    q01 = (jnp.dot(h01, packed(wq_buf, 0), preferred_element_type=F32) * QSCALE).astype(BF16)
    cp_k0.wait()
    s01 = lax.dot_general(q01, packed(k_buf, 0), NT, preferred_element_type=F32)
    m01 = jnp.max(_lane_fold(s01, jnp.maximum), axis=-1, keepdims=True)
    wait(cp_v0)
    qa_car[...] = qproj_head(2)
    for u in range(2):
        p = jnp.exp2(s01[u * SUB:(u + 1) * SUB] - m01[u * SUB:(u + 1) * SUB])
        ls_car[u] = _lane_fold(p, jnp.add)
        pv_car[u] = jnp.dot(p.astype(BF16), packed(v_buf, 0), preferred_element_type=F32)

    def ramp2(j, carry):
        wait(ramp_heads(j))
        unit_block(2 * j, 2, False)
        return carry

    lax.fori_loop(1, R2, ramp2, 0)
    start([cp_x(2, NRB - 2, SEM_XR)])
    for k in range(n_early, NLOAD):
        start(main_heads(k, k == NLOAD - 1))
    start(cp_m12)

    def blocks_done(n0):
        return (n0 - FIN_START) // (SUB // PR)

    def main(k, carry):
        n0 = RAMP + k * UM

        @pl.when(k <= K_MOD + 2)
        def _():
            @pl.when(k < NLOAD - 1)
            def _():
                wait(main_heads(k))

            @pl.when(k == NLOAD - 1)
            def _():
                wait(main_heads(NLOAD - 1, True))

            @pl.when(k == n_early)
            def _():
                cp_x(2, NRB - 2, SEM_XR).wait()

            @pl.when(k == K_MOD)
            def _():
                wait(cp_m12 + [cp_wr])
                sc = silu_c()
                m1 = _r(jnp.dot(sc, wa_buf[:, 2 * D:3 * D], preferred_element_type=F32)[0:8, :])
                m2 = _r(jnp.dot(sc, wb_buf[:, 0:3 * D], preferred_element_type=F32)[0:8, :])
                coef[C_GA] = m1
                coef[C_KEEP] = jnp.ones((8, D), F32)
                scale = _r(1.0 + m2[:, D:2 * D])
                coef[C_SHIFT] = m2[:, 0:D]
                coef[C_SCALE] = scale
                coef[C_GB] = m2[:, 2 * D:3 * D]
                w8 = wr_buf[...].astype(F32)
                wr = jnp.concatenate([jnp.broadcast_to(w8[j:j + 1, :], (8, 128))
                                      for j in range(D // 128)], axis=1)
                sw_buf[...] = scale * wr
                c1 = jnp.sum(scale * wr, axis=-1, keepdims=True)
                c0 = jnp.sum(m2[:, 0:D] * wr, axis=-1, keepdims=True)
                rid = lax.broadcasted_iota(I32, (8, 128), 0)
                rc_buf[...] = jnp.where(rid == 0, c1, c0)
                start(cp_ffn)

            @pl.when(k == K_MOD + 2)
            def _():
                wait(cp_ffn)

        done = lax.shift_right_arithmetic(n0 - FIN_START, 4)
        done_before = lax.shift_right_arithmetic(n0 - UM - FIN_START, 4)

        @pl.when(jnp.logical_and(done >= 1, done > done_before))
        def _():
            cp_out(jnp.maximum(done - 1, 0)).start()

        unit_block(n0, UM, True)
        return carry

    lax.fori_loop(0, NM, main, 0)

    for b in range(blocks_done(RAMP + (NM - 1) * UM), NRB - 1):
        cp_out(b).start()
    row0 = (NRB - 1) * SUB
    neg = -jnp.inf

    def keep_rows(y, lo):
        n = y.shape[0]
        yc, m, mr, rinv = _ln_stats(y)
        x2_buf[lo:lo + n, :] = y
        st_buf[0, lo:lo + n, :] = jnp.broadcast_to(mr, (n, 128))
        st_buf[1, lo:lo + n, :] = jnp.broadcast_to(rinv, (n, 128))
        d = jnp.sum(_rows8(yc, jnp.multiply, sw_buf[...]), axis=-1, keepdims=True)
        return (d + (m - mr) * rc_buf[0:1, 0:1]) * rinv

    def parked(lo, n):
        y = x2_buf[pl.ds(lo, n), :]
        mr = st_buf[0, pl.ds(lo, n), :]
        rinv = st_buf[1, pl.ds(lo, n), :]
        return y, jnp.concatenate([(y[:, j * 128:(j + 1) * 128] - mr) * rinv
                                   for j in range(D // 128)], axis=1)

    def all_red(v, fn):
        return fn(fn(v, axis=0, keepdims=True), axis=1, keepdims=True)

    lane = lax.broadcasted_iota(I32, (PR, 128), 1)
    ridx = (lane * PR + lax.broadcasted_iota(I32, (PR, 128), 0)).astype(F32)
    rr = jnp.where(lane < row0 // PR, r_buf[...], neg)
    last_old = float(row0 - 1)
    cm1 = all_red(rr, jnp.max)
    ci1 = all_red(jnp.where(rr == cm1, ridx, last_old), jnp.min)
    rr2 = jnp.where(ridx == ci1, neg, rr)
    cm2 = all_red(rr2, jnp.max)
    ci2 = all_red(jnp.where(jnp.logical_and(rr2 == cm2, ridx != ci1), ridx, last_old), jnp.min)
    ci1 = jnp.minimum(ci1, last_old).astype(I32)
    ci2 = jnp.minimum(ci2, last_old).astype(I32)
    for j, ci in enumerate((ci1, ci2)):
        g = pl.multiple_of(lax.shift_right_logical(ci[0, 0], 4) * PR, PR)
        keep_rows(resid(acc[pl.ds(g, PR), :], g, PR), SUB + j * PR)

    o2 = jnp.concatenate([_normalize(pv_car[0], ls_car[0]),
                          _normalize(pv_car[1], ls_car[1])], axis=1)
    wo2 = jnp.concatenate([wo_buf[H - 2], wo_buf[H - 1]], axis=0)
    r_new = []
    for j in range(SUB // ECH):
        lo, hi = j * ECH, (j + 1) * ECH
        a = acc[row0 + lo:row0 + hi, :] + jnp.dot(o2[lo:hi], wo2, preferred_element_type=F32)
        r_new.append(keep_rows(resid(a, row0 + lo, ECH), lo))

    sub8 = lax.broadcasted_iota(I32, (8, 1), 0)
    big = jnp.int32((S - 1) * 512 + SUB - 1)
    vals = jnp.concatenate(
        r_new + [jnp.where(sub8 == 0, cm1, jnp.where(sub8 == 1, cm2, neg))], axis=0)
    pos = lax.broadcasted_iota(I32, (SUB, 1), 0)
    cc1 = ci1 * 512 + SUB + (ci1 & (PR - 1))
    cc2 = ci2 * 512 + SUB + PR + (ci2 & (PR - 1))
    code = jnp.concatenate(
        [(pos + row0) * 512 + pos,
         jnp.where(sub8 == 0, cc1, jnp.where(sub8 == 1, cc2, big))], axis=0)
    m1 = jnp.max(vals, axis=0, keepdims=True)
    k1 = jnp.min(jnp.where(vals == m1, code, big), axis=0, keepdims=True)
    vals2 = jnp.where(code == k1, neg, vals)
    m2 = jnp.max(vals2, axis=0, keepdims=True)
    k2 = jnp.min(jnp.where(jnp.logical_and(vals2 == m2, code != k1), code, big),
                 axis=0, keepdims=True)
    k1 = k1[0, 0]
    k2 = k2[0, 0]
    i1 = lax.shift_right_logical(k1, 9)
    i2 = lax.shift_right_logical(k2, 9)
    t1 = k1 & 511
    t2 = k2 & 511
    rowid = lax.broadcasted_iota(I32, (PR, D), 0)
    xs = modulate(jnp.where(rowid == 0, parked(t1, 1)[1], parked(t2, 1)[1])).astype(BF16)

    off = pl.multiple_of(jnp.minimum(k2, 0) * 8, 8)
    for j in range(SUB // PR):
        yl, nl = parked(pl.multiple_of(off + j * PR, 8), PR)
        act[row0 + j * PR:row0 + (j + 1) * PR, :] = (
            yl + _rows8(modulate(nl), jnp.multiply, coef[C_GB])).astype(BF16)
    cp_out(NRB - 1).start()

    gt = _r(jnp.dot(xs, wa_buf[:, 0:F], preferred_element_type=F32))
    zt = pltpu.bitcast(act[pl.ds(pl.multiple_of(off * 2, PR), PR), 0:128], I32) & zero_buf[...]
    xb = pltpu.bitcast(xs, I32)
    xs = pltpu.bitcast(jnp.concatenate([xb[:, 0:128] | zt, xb[:, 128:]], axis=1), BF16)
    up = _r(jnp.dot(xs, wb_buf[:, 0:F], preferred_element_type=F32))
    hid = (_r(gt * _r(jax.nn.sigmoid(gt))) * up).astype(BF16)
    y = _r(jnp.dot(hid, wd_buf[:, 0:D], preferred_element_type=F32))
    y1 = _r(y[0:1, :] * _r(jax.nn.sigmoid(_r(m1 + rc_buf[1:2, 0:1]))))
    y2 = _r(y[1:2, :] * _r(jax.nn.sigmoid(_r(m2 + rc_buf[1:2, 0:1]))))

    def fix(i, t):
        g = pl.multiple_of(lax.shift_right_logical(i, 4) * PR, PR)
        tg = pl.multiple_of(lax.shift_right_logical(t, 4) * PR, PR)
        rid = rowid + g
        upd = jnp.where(rid == i1, y1, jnp.where(rid == i2, y2, 0.0))
        yg, ng = parked(tg, PR)
        return g, (yg + _rows8(modulate(ng) + upd, jnp.multiply, coef[C_GB])).astype(BF16)

    g1, fix1 = fix(i1, t1)
    g2, fix2 = fix(i2, t2)
    for b in range(NRB):
        cp_out(b).wait()
    act[pl.ds(g1, PR), :] = fix1
    act[pl.ds(g2, PR), :] = fix2
    f1 = cp(act.at[pl.ds(g1, PR), :], out_hbm.at[pl.ds(g1, PR), :], SEM_OUT)
    f2 = cp(act.at[pl.ds(g2, PR), :], out_hbm.at[pl.ds(g2, PR), :], SEM_FIX)
    f1.start()

    @pl.when(g1 != g2)
    def _():
        f2.start()
        f2.wait()

    f1.wait()


@jax.jit
def pallas_adaLN_cond__mha_block_cached__moe_arch_mod__prompt_kernel(
    A_x: jax.Array,
    A_k_cache: jax.Array,
    A_v_cache: jax.Array,
    A_wq: jax.Array,
    A_wo: jax.Array,
    B_x: jax.Array,
    B_w_r: jax.Array,
    B_w_gate: jax.Array,
    B_w_up: jax.Array,
    B_w_down: jax.Array,
    c: jax.Array,
    w_mod: jax.Array,
):
    del B_x
    hbm = pl.BlockSpec(memory_space=pl.ANY)
    out = pl.pallas_call(
        _kernel,
        in_specs=[hbm] * 11,
        out_specs=hbm,
        out_shape=jax.ShapeDtypeStruct((S, D), BF16),
        scratch_shapes=[
            pltpu.VMEM((S, D), BF16),
            pltpu.VMEM((H, S, DH), BF16),
            pltpu.VMEM((H, S, DH), BF16),
            pltpu.VMEM((H, D, DH), BF16),
            pltpu.VMEM((H, DH, D), BF16),
            pltpu.VMEM((D, F + PAD), BF16),
            pltpu.VMEM((D, F + PAD), BF16),
            pltpu.VMEM((F, D + PAD), BF16),
            pltpu.VMEM((S + PR, D), BF16),
            pltpu.VMEM((S, D), F32),
            pltpu.VMEM((2 * SUB, D), F32),
            pltpu.VMEM((SUB + 2 * PR, D), F32),
            pltpu.VMEM((2, SUB + 2 * PR, 128), F32),
            pltpu.VMEM((PR, 128), F32),
            pltpu.VMEM((5, 8, D), F32),
            pltpu.VMEM((8, 128), BF16),
            pltpu.VMEM((8, D), F32),
            pltpu.VMEM((8, 128), F32),
            pltpu.VMEM((1, D), BF16),
            pltpu.VMEM((8, 128), I32),
            pltpu.VMEM((FILL, DH), F32),
            pltpu.VMEM((2, SUB, DH), F32),
            pltpu.VMEM((2, SUB, DH), F32),
            pltpu.SemaphoreType.DMA((NSEM,)),
        ],
        compiler_params=pltpu.CompilerParams(
            vmem_limit_bytes=120 * 1024 * 1024,
        ),
        name="adaln_mha_mod",
    )(
        A_x.reshape(S, D),
        A_k_cache.reshape(H, S, DH),
        A_v_cache.reshape(H, S, DH),
        A_wq,
        A_wo.reshape(H, DH, D),
        B_w_r.reshape(8, 128),
        B_w_gate,
        B_w_up,
        B_w_down,
        c,
        w_mod,
    )
    return out.reshape(1, S, D)
```

```python
import jax
import jax.numpy as jnp
from jax import lax
import jax.experimental.pallas as pl
import jax.experimental.pallas.tpu as pltpu

S = 2048
D = 1024
H = 32
DH = 128
F = 3584
SUB = 256
NRB = S // SUB
NU = H * NRB
PR = 16
UM = 12
R2 = 8
RAMP = 2 * R2
NM = (NU - RAMP) // UM
HPI = UM // 2
NLOAD = (2 * H - RAMP) // UM
FIN_START = 130
K_MOD = (FIN_START - RAMP) // UM
LN_START = RAMP + K_MOD * UM - (S - 2 * SUB) // PR
FILL = 64
ECH = 64
PAD = 128
MCH = 4
EPS = 1e-5
QSCALE = float(DH ** -0.5) * 1.4426950408889634

F32 = jnp.float32
BF16 = jnp.bfloat16
I32 = jnp.int32
NT = (((1,), (1,)), ((), ()))

C_GA, C_SCALE, C_SHIFT, C_KEEP, C_GB = range(5)


def _r(v):
    return v.astype(BF16).astype(F32)


def _bits(v):
    return lax.bitcast_convert_type(v, I32)


def _float(v):
    return lax.bitcast_convert_type(v, F32)


def _rows8(v, fn, c):
    n = v.shape[0] // 8
    return fn(v.reshape(n, 8, D), c[None]).reshape(v.shape)


def _ln_stats(y):
    m = jnp.mean(y, axis=-1, keepdims=True)
    yc = y - m
    v = jnp.mean(yc * yc, axis=-1, keepdims=True)
    den = _r(jnp.sqrt(_r(_r(v) + EPS)))
    return yc, m, _r(m), 1.0 / den


def _layernorm(y):
    _, _, mr, rinv = _ln_stats(y)
    return (y - mr) * rinv


def _lane_fold(p, fn):
    t = p[:, 0:128]
    for j in range(1, p.shape[1] // 128):
        t = fn(t, p[:, j * 128:(j + 1) * 128])
    return t


def _normalize(pv, ls):
    l = jnp.sum(ls, axis=-1, keepdims=True)
    r = pl.reciprocal(l, approx=True)
    r = r * (2.0 - l * r)
    return (pv * r).astype(BF16)


def _head_of(n):
    if isinstance(n, int):
        return (n % 64) // 2 if n < 192 else (n - 192) % H
    return jnp.where(n < 192, lax.shift_right_logical(n & 63, 1), (n - 192) & (H - 1))


def _row_of(n):
    if isinstance(n, int):
        return SUB * ((n // 64) * 2 + n % 2 if n < 192 else min(n // 32, NRB - 1))
    rb = jnp.where(n < 192, lax.shift_right_logical(n, 6) * 2 + (n & 1),
                   jnp.minimum(lax.shift_right_logical(n, 5), NRB - 1))
    return pl.multiple_of(rb * SUB, SUB)


(SEM_C, SEM_WR, SEM_X0, SEM_XR, SEM_M12, SEM_FFN, SEM_OUT, SEM_FIX,
 SEM_WQ0, SEM_K0, SEM_M0) = range(11)
SEM_RAMP = SEM_M0 + MCH
SEM_MAIN = SEM_RAMP + R2
NSEM = SEM_MAIN + NLOAD


def _kernel(x_hbm, k_hbm, v_hbm, wq_hbm, wo_hbm, wr_hbm, wg_hbm, wu_hbm, wd_hbm,
            c_hbm, wmod_hbm, out_hbm,
            x_buf, k_buf, v_buf, wq_buf, wo_buf, wa_buf, wb_buf, wd_buf,
            act, acc, n_buf, x2_buf, st_buf, r_buf, coef, wr_buf, sw_buf, rc_buf, c_buf, zero_buf, qa_car, pv_car, ls_car,
            sems):
    def cp(src, dst, slot):
        return pltpu.make_async_copy(src, dst, sems.at[slot])

    def cp_x(b, nb, slot):
        return cp(x_hbm.at[pl.ds(b * SUB, nb * SUB), :],
                  x_buf.at[pl.ds(b * SUB, nb * SUB), :], slot)

    def cp_wq(h, slot):
        col = h * DH if isinstance(h, int) else pl.multiple_of(h * DH, DH)
        return cp(wq_hbm.at[:, pl.ds(col, DH)], wq_buf.at[h], slot)

    def cp_h(src, dst, h0, nh, slot):
        return cp(src.at[pl.ds(h0, nh)], dst.at[pl.ds(h0, nh)], slot)

    def heads(h0, nh, slot, last=False):
        return [cp_h(k_hbm, k_buf, h0, nh, slot), cp_h(v_hbm, v_buf, h0, nh, slot),
                cp_h(wo_hbm, wo_buf, h0 - 1, nh + 1 if last else nh, slot)] + [
            cp_wq(h0 + 1 + j, slot) for j in range(nh - 1 if last else nh)]

    def ramp_heads(j):
        return heads(j, 1, SEM_RAMP + j)

    def main_heads(k, last=False):
        return heads(RAMP // 2 + k * HPI, HPI, SEM_MAIN + k, last)

    cp_k0 = cp_h(k_hbm, k_buf, 0, 1, SEM_K0)
    cp_v0 = [cp_h(v_hbm, v_buf, 0, 1, SEM_RAMP), cp_wq(1, SEM_RAMP)]
    mrows = D // MCH
    cp_m0 = [cp(wmod_hbm.at[pl.ds(j * mrows, mrows), 0:2 * D],
                wa_buf.at[pl.ds(j * mrows, mrows), 0:2 * D], SEM_M0 + j) for j in range(MCH)]
    cp_c = cp(c_hbm, c_buf, SEM_C)
    cp_wr = cp(wr_hbm, wr_buf, SEM_WR)
    cp_m12 = [cp(wmod_hbm.at[:, 2 * D:3 * D], wa_buf.at[:, 2 * D:3 * D], SEM_M12),
              cp(wmod_hbm.at[:, 3 * D:6 * D], wb_buf.at[:, 0:3 * D], SEM_M12)]
    cp_ffn = [cp(wg_hbm, wa_buf.at[:, 0:F], SEM_FFN),
              cp(wu_hbm, wb_buf.at[:, 0:F], SEM_FFN),
              cp(wd_hbm, wd_buf.at[:, 0:D], SEM_FFN)]

    row0 = (NRB - 1) * SUB
    cp_out = [cp(act.at[0:row0, :], out_hbm.at[0:row0, :], SEM_OUT),
              cp(act.at[row0:S, :], out_hbm.at[row0:S, :], SEM_OUT)]

    def silu_c():
        cf = c_buf[...].astype(F32)
        sc = (cf * _r(jax.nn.sigmoid(cf))).astype(BF16)
        return jnp.broadcast_to(sc, (16, D))

    def modulate(n):
        n = _rows8(n, jnp.multiply, coef[C_SCALE])
        return _rows8(n, jnp.add, coef[C_SHIFT])

    def resid(a, row, nrows):
        a = _rows8(a, jnp.multiply, coef[C_GA])
        return _r(x_buf[pl.ds(row, nrows), :].astype(F32) + a)

    def piece(src, dst, lane_id):
        y = resid(acc[pl.ds(src, PR), :], src, PR)
        nn = _layernorm(y)
        hh = modulate(nn)
        r = jnp.sum(_rows8(nn, jnp.multiply, sw_buf[...]), axis=-1, keepdims=True)
        oo = (_rows8(y, jnp.multiply, coef[C_KEEP])
              + _rows8(hh, jnp.multiply, coef[C_GB]))
        act[pl.ds(dst, PR), :] = oo.astype(BF16)
        lane = lax.broadcasted_iota(I32, (PR, 128), 1)
        rn = jnp.where(lane == lane_id, r, r_buf[...])
        r_buf[...] = rn
        return oo, rn

    def unit_piece(n):
        is_ln = jnp.logical_and(n >= LN_START, n < LN_START + (S - 2 * SUB) // PR)
        is_fin = jnp.logical_and(n >= FIN_START, n < FIN_START + (S - SUB) // PR)
        f = n - FIN_START
        src = jnp.where(is_ln, 2 * SUB + (n - LN_START) * PR, jnp.where(is_fin, f * PR, 0))
        dst = jnp.where(jnp.logical_or(is_ln, is_fin), src, S)
        oo, rn = piece(pl.multiple_of(src, PR), pl.multiple_of(dst, PR),
                       jnp.where(is_fin, f, -1))
        bits = _lane_fold(_bits(oo), jnp.bitwise_or) | _bits(rn)
        return (bits[0:8] | bits[8:16]) & zero_buf[...]

    def qproj_head(n):
        return jnp.dot(act[pl.ds(_row_of(n), FILL), 0:D // 2],
                       wq_buf[_head_of(n)][0:D // 2], preferred_element_type=F32)

    def qproj_rest(n, qa):
        row = _row_of(n)
        w = wq_buf[_head_of(n)]
        row2 = row + FILL if isinstance(row, int) else pl.multiple_of(row + FILL, 16)
        qb = jnp.dot(act[pl.ds(row, SUB), D // 2:D], w[D // 2:D], preferred_element_type=F32)
        qc = jnp.dot(act[pl.ds(row2, SUB - FILL), 0:D // 2], w[0:D // 2],
                     preferred_element_type=F32)
        return ((qb + jnp.concatenate([qa, qc], axis=0)) * QSCALE).astype(BF16)

    def oproj(o, n):
        acc[pl.ds(_row_of(n), SUB), :] += jnp.dot(o, wo_buf[_head_of(n)],
                                                  preferred_element_type=F32)

    def unit_block(n0, nunits, with_piece):
        o = _normalize(pv_car[0], ls_car[0])
        raw = (pv_car[1], ls_car[1])
        qa = qa_car[...]
        for u in range(nunits):
            n = n0 + u
            hd = _head_of(n)
            q = qproj_rest(n, qa)
            z = unit_piece(n) if with_piece else None
            oproj(o, n - 2)
            sc = lax.dot_general(q, k_buf[hd], NT, preferred_element_type=F32)
            qa = qproj_head(n + 1)
            mm = _lane_fold(sc, jnp.maximum)
            if with_piece:
                mm = jnp.concatenate([_float(_bits(mm[0:8]) | z), mm[8:]], axis=0)
            m = jnp.max(mm, axis=-1, keepdims=True)
            p = jnp.exp2(sc - m)
            ls = _lane_fold(p, jnp.add)
            pv = jnp.dot(p.astype(BF16), v_buf[hd], preferred_element_type=F32)
            if u + 1 < nunits:
                zb = (_bits(pv).reshape(SUB // 8, 8, 128)
                      & zero_buf[...][None]).reshape(SUB, 128)
                o = _normalize(raw[0], _float(_bits(raw[1]) | zb))
            else:
                pv_car[0] = raw[0]
                ls_car[0] = raw[1]
            raw = (pv, ls)
        pv_car[1] = raw[0]
        ls_car[1] = raw[1]
        qa_car[...] = qa

    def start(cps):
        for c_ in cps:
            c_.start()

    def wait(cps):
        for c_ in cps:
            c_.wait()

    start([cp_c, cp_x(0, 2, SEM_X0)] + cp_m0 + [cp_wq(0, SEM_WQ0), cp_k0] + cp_v0)
    for j in range(1, R2):
        start(ramp_heads(j))
    start([cp_wr])
    n_early = (LN_START - RAMP) // UM
    for k in range(n_early):
        start(main_heads(k))

    def zero_acc(j, carry):
        acc[pl.ds(pl.multiple_of(j * 64, 64), 64), :] = jnp.zeros((64, D), F32)
        return carry

    lax.fori_loop(0, S // 64, zero_acc, 0)
    r_buf[...] = jnp.zeros(r_buf.shape, F32)
    zero_buf[...] = jnp.zeros(zero_buf.shape, I32)
    coef[C_GA] = jnp.zeros((8, D), F32)
    coef[C_KEEP] = jnp.zeros((8, D), F32)
    coef[C_GB] = jnp.ones((8, D), F32)
    sw_buf[...] = jnp.zeros(sw_buf.shape, F32)
    rc_buf[...] = jnp.zeros(rc_buf.shape, F32)
    cp_c.wait()
    cp_x(0, 2, SEM_X0).wait()

    def norm_rows(j, carry):
        row = pl.multiple_of(j * 128, 128)
        n_buf[pl.ds(row, 128), :] = _layernorm(x_buf[pl.ds(row, 128), :].astype(F32))
        return carry

    lax.fori_loop(0, 2 * SUB // 128, norm_rows, 0)
    sc16 = silu_c()
    m0 = None
    for j in range(MCH):
        cp_m0[j].wait()
        part = jnp.dot(sc16[:, j * mrows:(j + 1) * mrows],
                       wa_buf[j * mrows:(j + 1) * mrows, 0:2 * D], preferred_element_type=F32)
        m0 = part if m0 is None else m0 + part
    m0 = _r(m0[0:8, :])
    coef[C_SHIFT] = m0[:, 0:D]
    coef[C_SCALE] = _r(1.0 + m0[:, D:2 * D])

    cp_wq(0, SEM_WQ0).wait()
    h01 = modulate(n_buf[...]).astype(BF16)
    act[0:2 * SUB, :] = h01
    q01 = (jnp.dot(h01, wq_buf[0], preferred_element_type=F32) * QSCALE).astype(BF16)
    cp_k0.wait()
    s01 = lax.dot_general(q01, k_buf[0], NT, preferred_element_type=F32)
    m01 = jnp.max(_lane_fold(s01, jnp.maximum), axis=-1, keepdims=True)
    wait(cp_v0)
    qa_car[...] = qproj_head(2)
    for u in range(2):
        p = jnp.exp2(s01[u * SUB:(u + 1) * SUB] - m01[u * SUB:(u + 1) * SUB])
        ls_car[u] = _lane_fold(p, jnp.add)
        pv_car[u] = jnp.dot(p.astype(BF16), v_buf[0], preferred_element_type=F32)

    def ramp2(j, carry):
        wait(ramp_heads(j))
        unit_block(2 * j, 2, False)
        return carry

    lax.fori_loop(1, R2, ramp2, 0)
    start([cp_x(2, NRB - 2, SEM_XR)])
    for k in range(n_early, NLOAD):
        start(main_heads(k, k == NLOAD - 1))
    start(cp_m12)

    assert FIN_START + row0 // PR <= RAMP + (NM - 1) * UM

    def main(k, carry):
        n0 = RAMP + k * UM

        @pl.when(k <= K_MOD + 2)
        def _():
            @pl.when(k < NLOAD - 1)
            def _():
                wait(main_heads(k))

            @pl.when(k == NLOAD - 1)
            def _():
                wait(main_heads(NLOAD - 1, True))

            @pl.when(k == n_early)
            def _():
                cp_x(2, NRB - 2, SEM_XR).wait()

            @pl.when(k == K_MOD)
            def _():
                wait(cp_m12 + [cp_wr])
                sc = silu_c()
                m1 = _r(jnp.dot(sc, wa_buf[:, 2 * D:3 * D], preferred_element_type=F32)[0:8, :])
                m2 = _r(jnp.dot(sc, wb_buf[:, 0:3 * D], preferred_element_type=F32)[0:8, :])
                coef[C_GA] = m1
                coef[C_KEEP] = jnp.ones((8, D), F32)
                scale = _r(1.0 + m2[:, D:2 * D])
                coef[C_SHIFT] = m2[:, 0:D]
                coef[C_SCALE] = scale
                coef[C_GB] = m2[:, 2 * D:3 * D]
                w8 = wr_buf[...].astype(F32)
                wr = jnp.concatenate([jnp.broadcast_to(w8[j:j + 1, :], (8, 128))
                                      for j in range(D // 128)], axis=1)
                sw_buf[...] = scale * wr
                c1 = jnp.sum(scale * wr, axis=-1, keepdims=True)
                c0 = jnp.sum(m2[:, 0:D] * wr, axis=-1, keepdims=True)
                rid = lax.broadcasted_iota(I32, (8, 128), 0)
                rc_buf[...] = jnp.where(rid == 0, c1, c0)
                start(cp_ffn)

            @pl.when(k == K_MOD + 2)
            def _():
                wait(cp_ffn)

        @pl.when(k == NM - 1)
        def _():
            cp_out[0].start()

        unit_block(n0, UM, True)
        return carry

    lax.fori_loop(0, NM, main, 0)

    neg = -jnp.inf

    def keep_rows(y, lo):
        n = y.shape[0]
        yc, m, mr, rinv = _ln_stats(y)
        x2_buf[lo:lo + n, :] = y
        st_buf[0, lo:lo + n, :] = jnp.broadcast_to(mr, (n, 128))
        st_buf[1, lo:lo + n, :] = jnp.broadcast_to(rinv, (n, 128))
        d = jnp.sum(_rows8(yc, jnp.multiply, sw_buf[...]), axis=-1, keepdims=True)
        return (d + (m - mr) * rc_buf[0:1, 0:1]) * rinv

    def parked(lo, n):
        y = x2_buf[pl.ds(lo, n), :]
        mr = st_buf[0, pl.ds(lo, n), :]
        rinv = st_buf[1, pl.ds(lo, n), :]
        return y, jnp.concatenate([(y[:, j * 128:(j + 1) * 128] - mr) * rinv
                                   for j in range(D // 128)], axis=1)

    def all_red(v, fn):
        return fn(fn(v, axis=0, keepdims=True), axis=1, keepdims=True)

    lane = lax.broadcasted_iota(I32, (PR, 128), 1)
    ridx = (lane * PR + lax.broadcasted_iota(I32, (PR, 128), 0)).astype(F32)
    rr = jnp.where(lane < row0 // PR, r_buf[...], neg)
    last_old = float(row0 - 1)
    cm1 = all_red(rr, jnp.max)
    ci1 = all_red(jnp.where(rr == cm1, ridx, last_old), jnp.min)
    rr2 = jnp.where(ridx == ci1, neg, rr)
    cm2 = all_red(rr2, jnp.max)
    ci2 = all_red(jnp.where(jnp.logical_and(rr2 == cm2, ridx != ci1), ridx, last_old), jnp.min)
    ci1 = jnp.minimum(ci1, last_old).astype(I32)
    ci2 = jnp.minimum(ci2, last_old).astype(I32)
    for j, ci in enumerate((ci1, ci2)):
        g = pl.multiple_of(lax.shift_right_logical(ci[0, 0], 4) * PR, PR)
        keep_rows(resid(acc[pl.ds(g, PR), :], g, PR), SUB + j * PR)

    o2 = jnp.concatenate([_normalize(pv_car[0], ls_car[0]),
                          _normalize(pv_car[1], ls_car[1])], axis=1)
    wo2 = jnp.concatenate([wo_buf[H - 2], wo_buf[H - 1]], axis=0)
    r_new = []
    for j in range(SUB // ECH):
        lo, hi = j * ECH, (j + 1) * ECH
        a = acc[row0 + lo:row0 + hi, :] + jnp.dot(o2[lo:hi], wo2, preferred_element_type=F32)
        r_new.append(keep_rows(resid(a, row0 + lo, ECH), lo))

    sub8 = lax.broadcasted_iota(I32, (8, 1), 0)
    big = jnp.int32((S - 1) * 512 + SUB - 1)
    vals = jnp.concatenate(
        r_new + [jnp.where(sub8 == 0, cm1, jnp.where(sub8 == 1, cm2, neg))], axis=0)
    pos = lax.broadcasted_iota(I32, (SUB, 1), 0)
    cc1 = ci1 * 512 + SUB + (ci1 & (PR - 1))
    cc2 = ci2 * 512 + SUB + PR + (ci2 & (PR - 1))
    code = jnp.concatenate(
        [(pos + row0) * 512 + pos,
         jnp.where(sub8 == 0, cc1, jnp.where(sub8 == 1, cc2, big))], axis=0)
    m1 = jnp.max(vals, axis=0, keepdims=True)
    k1 = jnp.min(jnp.where(vals == m1, code, big), axis=0, keepdims=True)
    vals2 = jnp.where(code == k1, neg, vals)
    m2 = jnp.max(vals2, axis=0, keepdims=True)
    k2 = jnp.min(jnp.where(jnp.logical_and(vals2 == m2, code != k1), code, big),
                 axis=0, keepdims=True)
    k1 = k1[0, 0]
    k2 = k2[0, 0]
    i1 = lax.shift_right_logical(k1, 9)
    i2 = lax.shift_right_logical(k2, 9)
    t1 = k1 & 511
    t2 = k2 & 511
    rowid = lax.broadcasted_iota(I32, (PR, D), 0)
    xf = modulate(jnp.where(rowid == 0, parked(t1, 1)[1], parked(t2, 1)[1]))

    off = pl.multiple_of(jnp.minimum(k2, 0) * 8, 8)
    for j in range(SUB // PR):
        yl, nl = parked(pl.multiple_of(off + j * PR, 8), PR)
        act[row0 + j * PR:row0 + (j + 1) * PR, :] = (
            yl + _rows8(modulate(nl), jnp.multiply, coef[C_GB])).astype(BF16)
    cp_out[1].start()

    gt = _r(jnp.dot(xf.astype(BF16), wa_buf[:, 0:F], preferred_element_type=F32))
    zt = _bits(act[pl.ds(pl.multiple_of(off * 2, PR), PR), 0:128].astype(F32))
    zt = jnp.concatenate([zt[0:8] & zero_buf[...], zt[8:16] & zero_buf[...]], axis=0)
    xs = jnp.concatenate([_float(_bits(xf[:, 0:128]) | zt), xf[:, 128:]], axis=1).astype(BF16)
    up = _r(jnp.dot(xs, wb_buf[:, 0:F], preferred_element_type=F32))
    hid = (_r(gt * _r(jax.nn.sigmoid(gt))) * up).astype(BF16)
    y = _r(jnp.dot(hid, wd_buf[:, 0:D], preferred_element_type=F32))
    y1 = _r(y[0:1, :] * _r(jax.nn.sigmoid(_r(m1 + rc_buf[1:2, 0:1]))))
    y2 = _r(y[1:2, :] * _r(jax.nn.sigmoid(_r(m2 + rc_buf[1:2, 0:1]))))

    def fix(i, t):
        g = pl.multiple_of(lax.shift_right_logical(i, 4) * PR, PR)
        tg = pl.multiple_of(lax.shift_right_logical(t, 4) * PR, PR)
        rid = rowid + g
        upd = jnp.where(rid == i1, y1, jnp.where(rid == i2, y2, 0.0))
        yg, ng = parked(tg, PR)
        return g, (yg + _rows8(modulate(ng) + upd, jnp.multiply, coef[C_GB])).astype(BF16)

    g1, fix1 = fix(i1, t1)
    g2, fix2 = fix(i2, t2)
    wait(cp_out)
    act[pl.ds(g1, PR), :] = fix1
    act[pl.ds(g2, PR), :] = fix2
    f1 = cp(act.at[pl.ds(g1, PR), :], out_hbm.at[pl.ds(g1, PR), :], SEM_OUT)
    f2 = cp(act.at[pl.ds(g2, PR), :], out_hbm.at[pl.ds(g2, PR), :], SEM_FIX)
    f1.start()

    @pl.when(g1 != g2)
    def _():
        f2.start()
        f2.wait()

    f1.wait()


@jax.jit
def pallas_adaLN_cond__mha_block_cached__moe_arch_mod__prompt_kernel(
    A_x: jax.Array,
    A_k_cache: jax.Array,
    A_v_cache: jax.Array,
    A_wq: jax.Array,
    A_wo: jax.Array,
    B_x: jax.Array,
    B_w_r: jax.Array,
    B_w_gate: jax.Array,
    B_w_up: jax.Array,
    B_w_down: jax.Array,
    c: jax.Array,
    w_mod: jax.Array,
):
    del B_x
    hbm = pl.BlockSpec(memory_space=pl.ANY)
    out = pl.pallas_call(
        _kernel,
        in_specs=[hbm] * 11,
        out_specs=hbm,
        out_shape=jax.ShapeDtypeStruct((S, D), BF16),
        scratch_shapes=[
            pltpu.VMEM((S, D), BF16),
            pltpu.VMEM((H, S, DH), BF16),
            pltpu.VMEM((H, S, DH), BF16),
            pltpu.VMEM((H, D, DH), BF16),
            pltpu.VMEM((H, DH, D), BF16),
            pltpu.VMEM((D, F + PAD), BF16),
            pltpu.VMEM((D, F + PAD), BF16),
            pltpu.VMEM((F, D + PAD), BF16),
            pltpu.VMEM((S + PR, D), BF16),
            pltpu.VMEM((S, D), F32),
            pltpu.VMEM((2 * SUB, D), F32),
            pltpu.VMEM((SUB + 2 * PR, D), F32),
            pltpu.VMEM((2, SUB + 2 * PR, 128), F32),
            pltpu.VMEM((PR, 128), F32),
            pltpu.VMEM((5, 8, D), F32),
            pltpu.VMEM((8, 128), BF16),
            pltpu.VMEM((8, D), F32),
            pltpu.VMEM((8, 128), F32),
            pltpu.VMEM((1, D), BF16),
            pltpu.VMEM((8, 128), I32),
            pltpu.VMEM((FILL, DH), F32),
            pltpu.VMEM((2, SUB, DH), F32),
            pltpu.VMEM((2, SUB, DH), F32),
            pltpu.SemaphoreType.DMA((NSEM,)),
        ],
        compiler_params=pltpu.CompilerParams(
            vmem_limit_bytes=120 * 1024 * 1024,
            disable_bounds_checks=True,
            disable_semaphore_checks=True,
        ),
        name="adaln_mha_mod",
    )(
        A_x.reshape(S, D),
        A_k_cache.reshape(H, S, DH),
        A_v_cache.reshape(H, S, DH),
        A_wq,
        A_wo.reshape(H, DH, D),
        B_w_r.reshape(8, 128),
        B_w_gate,
        B_w_up,
        B_w_down,
        c,
        w_mod,
    )
    return out.reshape(1, S, D)
```

```python
import jax
import jax.numpy as jnp
from jax import lax
import jax.experimental.pallas as pl
import jax.experimental.pallas.tpu as pltpu

S = 2048
D = 1024
H = 32
DH = 128
F = 3584
SUB = 256
NRB = S // SUB
NU = H * NRB
PR = 16
UM = 12
R2 = 8
RAMP = 2 * R2
NM = (NU - RAMP) // UM
HPI = UM // 2
NLOAD = (2 * H - RAMP) // UM
FIN_START = 130
K_MOD = (FIN_START - RAMP) // UM
LN_START = RAMP + K_MOD * UM - (S - 2 * SUB) // PR
FILL = 64
ECH = 64
PAD = 128
NST = D // 128
MVC = 1280
EPS = 1e-5
QSCALE = float(DH ** -0.5) * 1.4426950408889634

F32 = jnp.float32
BF16 = jnp.bfloat16
I32 = jnp.int32
NT = (((1,), (1,)), ((), ()))

C_GA, C_SCALE, C_SHIFT, C_KEEP, C_GB = range(5)


def _r(v):
    return v.astype(BF16).astype(F32)


def _bits(v):
    return lax.bitcast_convert_type(v, I32)


def _float(v):
    return lax.bitcast_convert_type(v, F32)


def _rows8(v, fn, c):
    n = v.shape[0] // 8
    return fn(v.reshape(n, 8, D), c[None]).reshape(v.shape)


def _ln_stats(y):
    m = jnp.mean(y, axis=-1, keepdims=True)
    yc = y - m
    v = jnp.mean(yc * yc, axis=-1, keepdims=True)
    den = _r(jnp.sqrt(_r(_r(v) + EPS)))
    return yc, m, _r(m), 1.0 / den


def _layernorm(y):
    _, _, mr, rinv = _ln_stats(y)
    return (y - mr) * rinv


def _lane_fold(p, fn):
    t = p[:, 0:128]
    for j in range(1, p.shape[1] // 128):
        t = fn(t, p[:, j * 128:(j + 1) * 128])
    return t


def _normalize(pv, ls):
    l = jnp.sum(ls, axis=-1, keepdims=True)
    r = pl.reciprocal(l, approx=True)
    r = r * (2.0 - l * r)
    return (pv * r).astype(BF16)


def _head_of(n):
    if isinstance(n, int):
        return (n % 64) // 2 if n < 192 else (n - 192) % H
    return jnp.where(n < 192, lax.shift_right_logical(n & 63, 1), (n - 192) & (H - 1))


def _row_of(n):
    if isinstance(n, int):
        return SUB * ((n // 64) * 2 + n % 2 if n < 192 else min(n // 32, NRB - 1))
    rb = jnp.where(n < 192, lax.shift_right_logical(n, 6) * 2 + (n & 1),
                   jnp.minimum(lax.shift_right_logical(n, 5), NRB - 1))
    return pl.multiple_of(rb * SUB, SUB)


(SEM_C, SEM_WR, SEM_X0, SEM_X1, SEM_XR, SEM_M12, SEM_FFN, SEM_OUT, SEM_FIX,
 SEM_K0, SEM_WQE, SEM_H, SEM_M0) = range(13)
SEM_W0 = SEM_M0 + NST
SEM_RAMP = SEM_W0 + NST
SEM_MAIN = SEM_RAMP + R2
NSEM = SEM_MAIN + NLOAD


def _kernel(x_hbm, k_hbm, v_hbm, wq_hbm, wo_hbm, wr_hbm, wg_hbm, wu_hbm, wd_hbm,
            c_hbm, wmod_hbm, out_hbm,
            x_buf, k_buf, v_buf, wq_buf, wo_buf, wa_buf, wb_buf, wd_buf,
            act, acc, n_buf, q_acc, hq_buf, mq_buf, x2_buf, st_buf, r_buf, coef, wr_buf, sw_buf, rc_buf,
            c_buf, sc_buf, scol, zero_buf, qa_car, pv_car, ls_car,
            sems):
    def cp(src, dst, slot):
        return pltpu.make_async_copy(src, dst, sems.at[slot])

    def cp_x(b, nb, slot):
        return cp(x_hbm.at[pl.ds(b * SUB, nb * SUB), :],
                  x_buf.at[pl.ds(b * SUB, nb * SUB), :], slot)

    def cp_wq(h, slot):
        col = h * DH if isinstance(h, int) else pl.multiple_of(h * DH, DH)
        return cp(wq_hbm.at[:, pl.ds(col, DH)], wq_buf.at[h], slot)

    def cp_h(src, dst, h0, nh, slot):
        return cp(src.at[pl.ds(h0, nh)], dst.at[pl.ds(h0, nh)], slot)

    def heads(h0, nh, slot, last=False):
        return [cp_h(k_hbm, k_buf, h0, nh, slot), cp_h(v_hbm, v_buf, h0, nh, slot),
                cp_h(wo_hbm, wo_buf, h0 - 1, nh + 1 if last else nh, slot)] + [
            cp_wq(h0 + 1 + j, slot) for j in range(nh - 1 if last else nh)]

    def ramp_heads(j):
        return [cp_h(k_hbm, k_buf, j, 1, SEM_RAMP + j), cp_h(v_hbm, v_buf, j, 1, SEM_RAMP + j),
                cp_h(wo_hbm, wo_buf, j - 1, 1, SEM_RAMP + j)]

    def main_heads(k, last=False):
        return heads(R2 + k * HPI, HPI, SEM_MAIN + k, last)

    cp_k0 = cp_h(k_hbm, k_buf, 0, 1, SEM_K0)
    cp_v0 = [cp_h(v_hbm, v_buf, 0, 1, SEM_RAMP), cp_wq(R2, SEM_RAMP)]
    cp_wqe = [cp_wq(h, SEM_WQE) for h in range(R2)]

    def lanes(j):
        return pl.ds(j * 128 if isinstance(j, int) else pl.multiple_of(j * 128, 128), 128)

    def cp_m0(j):
        return [cp(wmod_hbm.at[:, lanes(u * NST + j)],
                   v_buf.at[H - NST + j, u * D:(u + 1) * D, :], SEM_M0 + j) for u in range(2)]

    def cp_w0(j):
        return cp(wq_hbm.at[lanes(j), 0:R2 * DH], wb_buf.at[lanes(j), 0:R2 * DH], SEM_W0 + j)

    def cp_hq(j):
        return cp(hq_buf.at[j], act.at[0:2 * SUB, lanes(j)], SEM_H)

    cp_c = cp(c_hbm, c_buf, SEM_C)
    cp_wr = cp(wr_hbm, wr_buf, SEM_WR)
    cp_m12 = [cp(wmod_hbm.at[:, 2 * D:3 * D], wa_buf.at[:, 2 * D:3 * D], SEM_M12),
              cp(wmod_hbm.at[:, 3 * D:6 * D], wb_buf.at[:, 0:3 * D], SEM_M12)]
    cp_ffn = [cp(wg_hbm, wa_buf.at[:, 0:F], SEM_FFN),
              cp(wu_hbm, wb_buf.at[:, 0:F], SEM_FFN),
              cp(wd_hbm, wd_buf.at[:, 0:D], SEM_FFN)]

    row0 = (NRB - 1) * SUB
    cp_out = [cp(act.at[0:row0, :], out_hbm.at[0:row0, :], SEM_OUT),
              cp(act.at[row0:S, :], out_hbm.at[row0:S, :], SEM_OUT)]

    def vpu_matvec(w_ref, ncols):
        parts = []
        zf = None
        for cc in range(0, ncols, 256):
            a = None if zf is None else jnp.concatenate([zf, zf], axis=1)
            for g in range(D // 8):
                wv = w_ref[g * 8:(g + 1) * 8, cc:cc + 256].astype(F32)
                sv = scol[g * 8:(g + 1) * 8, :]
                pr = jnp.concatenate([wv[:, 0:128] * sv, wv[:, 128:256] * sv], axis=1)
                a = pr if a is None else a + pr
            zf = _float(_lane_fold(_bits(a), jnp.bitwise_or) & zero_buf[...])
            parts.append(a)
        return jnp.sum(jnp.concatenate(parts, axis=1), axis=0, keepdims=True)

    def modulate(n):
        n = _rows8(n, jnp.multiply, coef[C_SCALE])
        return _rows8(n, jnp.add, coef[C_SHIFT])

    def resid(a, row, nrows):
        a = _rows8(a, jnp.multiply, coef[C_GA])
        return _r(x_buf[pl.ds(row, nrows), :].astype(F32) + a)

    def piece(src, dst, lane_id):
        y = resid(acc[pl.ds(src, PR), :], src, PR)
        nn = _layernorm(y)
        hh = modulate(nn)
        r = jnp.sum(_rows8(nn, jnp.multiply, sw_buf[...]), axis=-1, keepdims=True)
        oo = (_rows8(y, jnp.multiply, coef[C_KEEP])
              + _rows8(hh, jnp.multiply, coef[C_GB]))
        act[pl.ds(dst, PR), :] = oo.astype(BF16)
        lane = lax.broadcasted_iota(I32, (PR, 128), 1)
        rn = jnp.where(lane == lane_id, r, r_buf[...])
        r_buf[...] = rn
        return oo, rn

    def unit_piece(n):
        is_ln = jnp.logical_and(n >= LN_START, n < LN_START + (S - 2 * SUB) // PR)
        is_fin = jnp.logical_and(n >= FIN_START, n < FIN_START + (S - SUB) // PR)
        f = n - FIN_START
        src = jnp.where(is_ln, 2 * SUB + (n - LN_START) * PR, jnp.where(is_fin, f * PR, 0))
        dst = jnp.where(jnp.logical_or(is_ln, is_fin), src, S)
        oo, rn = piece(pl.multiple_of(src, PR), pl.multiple_of(dst, PR),
                       jnp.where(is_fin, f, -1))
        bits = _lane_fold(_bits(oo), jnp.bitwise_or) | _bits(rn)
        return (bits[0:8] | bits[8:16]) & zero_buf[...]

    def qproj_head(n):
        return jnp.dot(act[pl.ds(_row_of(n), FILL), 0:D // 2],
                       wq_buf[_head_of(n)][0:D // 2], preferred_element_type=F32)

    def qproj_rest(n, qa):
        row = _row_of(n)
        w = wq_buf[_head_of(n)]
        row2 = row + FILL if isinstance(row, int) else pl.multiple_of(row + FILL, 16)
        qb = jnp.dot(act[pl.ds(row, SUB), D // 2:D], w[D // 2:D], preferred_element_type=F32)
        qc = jnp.dot(act[pl.ds(row2, SUB - FILL), 0:D // 2], w[0:D // 2],
                     preferred_element_type=F32)
        return ((qb + jnp.concatenate([qa, qc], axis=0)) * QSCALE).astype(BF16)

    def oproj(o, n):
        acc[pl.ds(_row_of(n), SUB), :] += jnp.dot(o, wo_buf[_head_of(n)],
                                                  preferred_element_type=F32)

    def unit_block(n0, nunits):
        o = _normalize(pv_car[0], ls_car[0])
        raw = (pv_car[1], ls_car[1])
        qa = qa_car[...]
        for u in range(nunits):
            n = n0 + u
            hd = _head_of(n)
            q = qproj_rest(n, qa)
            z = unit_piece(n)
            oproj(o, n - 2)
            sc = lax.dot_general(q, k_buf[hd], NT, preferred_element_type=F32)
            qa = qproj_head(n + 1)
            mm = _lane_fold(sc, jnp.maximum)
            mm = jnp.concatenate([_float(_bits(mm[0:8]) | z), mm[8:]], axis=0)
            m = jnp.max(mm, axis=-1, keepdims=True)
            p = jnp.exp2(sc - m)
            ls = _lane_fold(p, jnp.add)
            pv = jnp.dot(p.astype(BF16), v_buf[hd], preferred_element_type=F32)
            if u + 1 < nunits:
                zb = (_bits(pv).reshape(SUB // 8, 8, 128)
                      & zero_buf[...][None]).reshape(SUB, 128)
                o = _normalize(raw[0], _float(_bits(raw[1]) | zb))
            else:
                pv_car[0] = raw[0]
                ls_car[0] = raw[1]
            raw = (pv, ls)
        pv_car[1] = raw[0]
        ls_car[1] = raw[1]
        qa_car[...] = qa

    def ramp_block(j):
        o = [_normalize(pv_car[u], ls_car[u]) for u in range(2)]
        w = wo_buf[j - 1]

        def op_part(u, r0, r1, c0, c1):
            acc[u * SUB + r0:u * SUB + r1, c0:c1] += jnp.dot(
                o[u][r0:r1], w[:, c0:c1], preferred_element_type=F32)

        for u in range(2):
            q = (q_acc[j, u * SUB:(u + 1) * SUB, :] * QSCALE).astype(BF16)
            sc = lax.dot_general(q, k_buf[j], NT, preferred_element_type=F32)
            op_part(u, 0, FILL, 0, D // 2)
            m = jnp.max(_lane_fold(sc, jnp.maximum), axis=-1, keepdims=True)
            p = jnp.exp2(sc - m)
            ls_car[u] = _lane_fold(p, jnp.add)
            pv_car[u] = jnp.dot(p.astype(BF16), v_buf[j], preferred_element_type=F32)
            if u == 0:
                for v in range(2):
                    op_part(v, FILL, SUB, 0, D // 2)
                    op_part(v, 0, SUB, D // 2, D)

    def start(cps):
        for c_ in cps:
            c_.start()

    def wait(cps):
        for c_ in cps:
            c_.wait()

    start([cp_c, cp_x(0, 1, SEM_X0), cp_x(1, 1, SEM_X1)])
    for j in range(NST):
        start(cp_m0(j) + [cp_w0(j)])
    start([cp_k0] + cp_v0)
    for j in range(1, R2):
        start(ramp_heads(j))
    start([cp_wr])
    n_early = (LN_START - RAMP) // UM
    for k in range(n_early):
        start(main_heads(k))

    r_buf[...] = jnp.zeros(r_buf.shape, F32)
    zero_buf[...] = jnp.zeros(zero_buf.shape, I32)
    coef[C_GA] = jnp.zeros((8, D), F32)
    coef[C_KEEP] = jnp.zeros((8, D), F32)
    coef[C_GB] = jnp.ones((8, D), F32)
    sw_buf[...] = jnp.zeros(sw_buf.shape, F32)
    q_acc[...] = jnp.zeros(q_acc.shape, F32)
    cp_c.wait()
    cf = c_buf[...].astype(F32)
    sf = _r(cf * _r(jax.nn.sigmoid(cf)))
    sc_buf[...] = jnp.broadcast_to(sf, (16, D)).astype(BF16)
    for j in range(D // 128):
        scol[j * 128:(j + 1) * 128, :] = jnp.broadcast_to(
            sf[:, j * 128:(j + 1) * 128], (128, 128)).T

    def norm_rows(b, carry):
        cp_x(b, 1, SEM_X0 + b).wait()
        for j in range(2):
            row = pl.multiple_of(b * SUB + j * 128, 128)
            nn = _layernorm(x_buf[pl.ds(row, 128), :].astype(F32))
            for t in range(NST):
                n_buf[t, pl.ds(row, 128), :] = nn[:, t * 128:(t + 1) * 128]
        return carry

    lax.fori_loop(0, 2, norm_rows, 0)

    def stage(j, carry):
        wait(cp_m0(j))
        wm = jnp.concatenate([v_buf[H - NST + j, 0:D, :], v_buf[H - NST + j, D:2 * D, :]], axis=1)
        mj = _r(jnp.dot(sc_buf[...], wm, preferred_element_type=F32)[0:8, :])
        mq_buf[j, 0] = mj[:, 0:128]
        mq_buf[j, 1] = _r(1.0 + mj[:, 128:256])
        zr = S // NST
        acc[pl.ds(pl.multiple_of(j * zr, zr), zr), :] = jnp.zeros((zr, D), F32)
        cp_w0(j).wait()
        hj = (n_buf[j].reshape(2 * SUB // 8, 8, 128) * mq_buf[j, 1][None]
              + mq_buf[j, 0][None]).reshape(2 * SUB, 128).astype(BF16)
        hq_buf[j] = hj
        cp_hq(j).start()
        part = jnp.dot(hj, wb_buf[lanes(j), 0:R2 * DH], preferred_element_type=F32)
        for h in range(R2):
            q_acc[h] += part[:, h * DH:(h + 1) * DH]
        return carry

    lax.fori_loop(0, NST, stage, 0)

    cp_k0.wait()
    coef[C_SHIFT] = jnp.concatenate([mq_buf[j, 0] for j in range(NST)], axis=1)
    coef[C_SCALE] = jnp.concatenate([mq_buf[j, 1] for j in range(NST)], axis=1)
    s01 = lax.dot_general((q_acc[0] * QSCALE).astype(BF16), k_buf[0], NT,
                          preferred_element_type=F32)
    m01 = jnp.max(_lane_fold(s01, jnp.maximum), axis=-1, keepdims=True)
    wait(cp_v0)
    qa_car[...] = jnp.dot(
        jnp.concatenate([hq_buf[j, 0:FILL, :] for j in range(NST // 2)], axis=1),
        wq_buf[R2][0:D // 2], preferred_element_type=F32)
    for u in range(2):
        p = jnp.exp2(s01[u * SUB:(u + 1) * SUB] - m01[u * SUB:(u + 1) * SUB])
        ls_car[u] = _lane_fold(p, jnp.add)
        pv_car[u] = jnp.dot(p.astype(BF16), v_buf[0], preferred_element_type=F32)

    def ramp2(j, carry):
        wait(ramp_heads(j))
        ramp_block(j)
        return carry

    lax.fori_loop(1, R2, ramp2, 0)
    start([cp_x(2, NRB - 2, SEM_XR)])
    for k in range(n_early, NLOAD):
        start(main_heads(k, k == NLOAD - 1))
    start(cp_wqe + cp_m12)
    wait([cp_hq(j) for j in range(NST)])

    assert FIN_START + row0 // PR <= RAMP + (NM - 1) * UM

    def main(k, carry):
        n0 = RAMP + k * UM

        @pl.when(k <= K_MOD + 2)
        def _():
            @pl.when(k < NLOAD - 1)
            def _():
                wait(main_heads(k))

            @pl.when(k == NLOAD - 1)
            def _():
                wait(main_heads(NLOAD - 1, True) + cp_wqe)

            @pl.when(k == n_early)
            def _():
                cp_x(2, NRB - 2, SEM_XR).wait()

            @pl.when(k == K_MOD)
            def _():
                wait(cp_m12 + [cp_wr])
                sc = sc_buf[...]
                m2a = jnp.dot(sc, wb_buf[:, MVC:3 * D], preferred_element_type=F32)[0:8, :]
                m1 = _r(jnp.dot(sc, wa_buf[:, 2 * D:3 * D], preferred_element_type=F32)[0:8, :])
                m2b = jnp.broadcast_to(vpu_matvec(wb_buf, MVC), (8, MVC))
                m2 = _r(jnp.concatenate([m2b, m2a], axis=1))
                coef[C_GA] = m1
                coef[C_KEEP] = jnp.ones((8, D), F32)
                scale = _r(1.0 + m2[:, D:2 * D])
                coef[C_SHIFT] = m2[:, 0:D]
                coef[C_SCALE] = scale
                coef[C_GB] = m2[:, 2 * D:3 * D]
                w8 = wr_buf[...].astype(F32)
                wr = jnp.concatenate([jnp.broadcast_to(w8[j:j + 1, :], (8, 128))
                                      for j in range(D // 128)], axis=1)
                sw_buf[...] = scale * wr
                c1 = jnp.sum(scale * wr, axis=-1, keepdims=True)
                c0 = jnp.sum(m2[:, 0:D] * wr, axis=-1, keepdims=True)
                rid = lax.broadcasted_iota(I32, (8, 128), 0)
                rc_buf[...] = jnp.where(rid == 0, c1, c0)
                start(cp_ffn)

            @pl.when(k == K_MOD + 2)
            def _():
                wait(cp_ffn)

        @pl.when(k == NM - 1)
        def _():
            cp_out[0].start()

        unit_block(n0, UM)
        return carry

    lax.fori_loop(0, NM, main, 0)

    neg = -jnp.inf

    def keep_rows(y, lo):
        n = y.shape[0]
        yc, m, mr, rinv = _ln_stats(y)
        x2_buf[lo:lo + n, :] = y
        st_buf[0, lo:lo + n, :] = jnp.broadcast_to(mr, (n, 128))
        st_buf[1, lo:lo + n, :] = jnp.broadcast_to(rinv, (n, 128))
        d = jnp.sum(_rows8(yc, jnp.multiply, sw_buf[...]), axis=-1, keepdims=True)
        return (d + (m - mr) * rc_buf[0:1, 0:1]) * rinv

    def parked(lo, n):
        y = x2_buf[pl.ds(lo, n), :]
        mr = st_buf[0, pl.ds(lo, n), :]
        rinv = st_buf[1, pl.ds(lo, n), :]
        return y, jnp.concatenate([(y[:, j * 128:(j + 1) * 128] - mr) * rinv
                                   for j in range(D // 128)], axis=1)

    def all_red(v, fn):
        return fn(fn(v, axis=0, keepdims=True), axis=1, keepdims=True)

    lane = lax.broadcasted_iota(I32, (PR, 128), 1)
    ridx = (lane * PR + lax.broadcasted_iota(I32, (PR, 128), 0)).astype(F32)
    rr = jnp.where(lane < row0 // PR, r_buf[...], neg)
    last_old = float(row0 - 1)
    cm1 = all_red(rr, jnp.max)
    ci1 = all_red(jnp.where(rr == cm1, ridx, last_old), jnp.min)
    rr2 = jnp.where(ridx == ci1, neg, rr)
    cm2 = all_red(rr2, jnp.max)
    ci2 = all_red(jnp.where(jnp.logical_and(rr2 == cm2, ridx != ci1), ridx, last_old), jnp.min)
    ci1 = jnp.minimum(ci1, last_old).astype(I32)
    ci2 = jnp.minimum(ci2, last_old).astype(I32)
    for j, ci in enumerate((ci1, ci2)):
        g = pl.multiple_of(lax.shift_right_logical(ci[0, 0], 4) * PR, PR)
        keep_rows(resid(acc[pl.ds(g, PR), :], g, PR), SUB + j * PR)

    o2 = jnp.concatenate([_normalize(pv_car[0], ls_car[0]),
                          _normalize(pv_car[1], ls_car[1])], axis=1)
    wo2 = jnp.concatenate([wo_buf[H - 2], wo_buf[H - 1]], axis=0)
    r_new = []
    for j in range(SUB // ECH):
        lo, hi = j * ECH, (j + 1) * ECH
        a = acc[row0 + lo:row0 + hi, :] + jnp.dot(o2[lo:hi], wo2, preferred_element_type=F32)
        r_new.append(keep_rows(resid(a, row0 + lo, ECH), lo))

    sub8 = lax.broadcasted_iota(I32, (8, 1), 0)
    big = jnp.int32((S - 1) * 512 + SUB - 1)
    vals = jnp.concatenate(
        r_new + [jnp.where(sub8 == 0, cm1, jnp.where(sub8 == 1, cm2, neg))], axis=0)
    pos = lax.broadcasted_iota(I32, (SUB, 1), 0)
    cc1 = ci1 * 512 + SUB + (ci1 & (PR - 1))
    cc2 = ci2 * 512 + SUB + PR + (ci2 & (PR - 1))
    code = jnp.concatenate(
        [(pos + row0) * 512 + pos,
         jnp.where(sub8 == 0, cc1, jnp.where(sub8 == 1, cc2, big))], axis=0)
    m1 = jnp.max(vals, axis=0, keepdims=True)
    k1 = jnp.min(jnp.where(vals == m1, code, big), axis=0, keepdims=True)
    vals2 = jnp.where(code == k1, neg, vals)
    m2 = jnp.max(vals2, axis=0, keepdims=True)
    k2 = jnp.min(jnp.where(jnp.logical_and(vals2 == m2, code != k1), code, big),
                 axis=0, keepdims=True)
    k1 = k1[0, 0]
    k2 = k2[0, 0]
    i1 = lax.shift_right_logical(k1, 9)
    i2 = lax.shift_right_logical(k2, 9)
    t1 = k1 & 511
    t2 = k2 & 511
    rowid = lax.broadcasted_iota(I32, (PR, D), 0)
    xf = modulate(jnp.where(rowid == 0, parked(t1, 1)[1], parked(t2, 1)[1]))

    off = pl.multiple_of(jnp.minimum(k2, 0) * 8, 8)
    for j in range(SUB // PR):
        yl, nl = parked(pl.multiple_of(off + j * PR, 8), PR)
        act[row0 + j * PR:row0 + (j + 1) * PR, :] = (
            yl + _rows8(modulate(nl), jnp.multiply, coef[C_GB])).astype(BF16)
    cp_out[1].start()

    gt = _r(jnp.dot(xf.astype(BF16), wa_buf[:, 0:F], preferred_element_type=F32))
    zt = _bits(act[pl.ds(pl.multiple_of(off * 2, PR), PR), 0:128].astype(F32))
    zt = jnp.concatenate([zt[0:8] & zero_buf[...], zt[8:16] & zero_buf[...]], axis=0)
    xs = jnp.concatenate([_float(_bits(xf[:, 0:128]) | zt), xf[:, 128:]], axis=1).astype(BF16)
    up = _r(jnp.dot(xs, wb_buf[:, 0:F], preferred_element_type=F32))
    hid = (_r(gt * _r(jax.nn.sigmoid(gt))) * up).astype(BF16)
    y = _r(jnp.dot(hid, wd_buf[:, 0:D], preferred_element_type=F32))
    y1 = _r(y[0:1, :] * _r(jax.nn.sigmoid(_r(m1 + rc_buf[1:2, 0:1]))))
    y2 = _r(y[1:2, :] * _r(jax.nn.sigmoid(_r(m2 + rc_buf[1:2, 0:1]))))

    def fix(i, t):
        g = pl.multiple_of(lax.shift_right_logical(i, 4) * PR, PR)
        tg = pl.multiple_of(lax.shift_right_logical(t, 4) * PR, PR)
        rid = rowid + g
        upd = jnp.where(rid == i1, y1, jnp.where(rid == i2, y2, 0.0))
        yg, ng = parked(tg, PR)
        return g, (yg + _rows8(modulate(ng) + upd, jnp.multiply, coef[C_GB])).astype(BF16)

    g1, fix1 = fix(i1, t1)
    g2, fix2 = fix(i2, t2)
    wait(cp_out)
    act[pl.ds(g1, PR), :] = fix1
    act[pl.ds(g2, PR), :] = fix2
    f1 = cp(act.at[pl.ds(g1, PR), :], out_hbm.at[pl.ds(g1, PR), :], SEM_OUT)
    f2 = cp(act.at[pl.ds(g2, PR), :], out_hbm.at[pl.ds(g2, PR), :], SEM_FIX)
    f1.start()

    @pl.when(g1 != g2)
    def _():
        f2.start()
        f2.wait()

    f1.wait()


@jax.jit
def pallas_adaLN_cond__mha_block_cached__moe_arch_mod__prompt_kernel(
    A_x: jax.Array,
    A_k_cache: jax.Array,
    A_v_cache: jax.Array,
    A_wq: jax.Array,
    A_wo: jax.Array,
    B_x: jax.Array,
    B_w_r: jax.Array,
    B_w_gate: jax.Array,
    B_w_up: jax.Array,
    B_w_down: jax.Array,
    c: jax.Array,
    w_mod: jax.Array,
):
    del B_x
    hbm = pl.BlockSpec(memory_space=pl.ANY)
    out = pl.pallas_call(
        _kernel,
        in_specs=[hbm] * 11,
        out_specs=hbm,
        out_shape=jax.ShapeDtypeStruct((S, D), BF16),
        scratch_shapes=[
            pltpu.VMEM((S, D), BF16),
            pltpu.VMEM((H, S, DH), BF16),
            pltpu.VMEM((H, S, DH), BF16),
            pltpu.VMEM((H, D, DH), BF16),
            pltpu.VMEM((H, DH, D), BF16),
            pltpu.VMEM((D, F + PAD), BF16),
            pltpu.VMEM((D, F + PAD), BF16),
            pltpu.VMEM((F, D + PAD), BF16),
            pltpu.VMEM((S + PR, D), BF16),
            pltpu.VMEM((S, D), F32),
            pltpu.VMEM((NST, 2 * SUB, 128), F32),
            pltpu.VMEM((R2, 2 * SUB, DH), F32),
            pltpu.VMEM((NST, 2 * SUB, 128), BF16),
            pltpu.VMEM((NST, 2, 8, 128), F32),
            pltpu.VMEM((SUB + 2 * PR, D), F32),
            pltpu.VMEM((2, SUB + 2 * PR, 128), F32),
            pltpu.VMEM((PR, 128), F32),
            pltpu.VMEM((5, 8, D), F32),
            pltpu.VMEM((8, 128), BF16),
            pltpu.VMEM((8, D), F32),
            pltpu.VMEM((8, 128), F32),
            pltpu.VMEM((1, D), BF16),
            pltpu.VMEM((16, D), BF16),
            pltpu.VMEM((D, 128), F32),
            pltpu.VMEM((8, 128), I32),
            pltpu.VMEM((FILL, DH), F32),
            pltpu.VMEM((2, SUB, DH), F32),
            pltpu.VMEM((2, SUB, DH), F32),
            pltpu.SemaphoreType.DMA((NSEM,)),
        ],
        compiler_params=pltpu.CompilerParams(
            vmem_limit_bytes=120 * 1024 * 1024,
            disable_bounds_checks=True,
            disable_semaphore_checks=True,
        ),
        name="adaln_mha_mod",
    )(
        A_x.reshape(S, D),
        A_k_cache.reshape(H, S, DH),
        A_v_cache.reshape(H, S, DH),
        A_wq,
        A_wo.reshape(H, DH, D),
        B_w_r.reshape(8, 128),
        B_w_gate,
        B_w_up,
        B_w_down,
        c,
        w_mod,
    )
    return out.reshape(1, S, D)
```

```python
import jax
import jax.numpy as jnp
from jax import lax
import jax.experimental.pallas as pl
import jax.experimental.pallas.tpu as pltpu

S = 2048
D = 1024
H = 32
DH = 128
F = 3584
SUB = 256
NRB = S // SUB
NU = H * NRB
PR = 16
UM = 12
R2 = 8
RAMP = 2 * R2
NM = (NU - RAMP) // UM
HPI = UM // 2
NLOAD = (2 * H - RAMP) // UM
FIN_START = 130
K_MOD = (FIN_START - RAMP) // UM
LN_START = RAMP + K_MOD * UM - (S - 2 * SUB) // PR
FILL = 64
ECH = 64
PAD = 128
NST = D // 128
MVC = 1280
EPS = 1e-5
QSCALE = float(DH ** -0.5) * 1.4426950408889634

F32 = jnp.float32
BF16 = jnp.bfloat16
I32 = jnp.int32
NT = (((1,), (1,)), ((), ()))

C_GA, C_SCALE, C_SHIFT, C_KEEP, C_GB = range(5)


def _r(v):
    return v.astype(BF16).astype(F32)


def _bits(v):
    return lax.bitcast_convert_type(v, I32)


def _float(v):
    return lax.bitcast_convert_type(v, F32)


def _rows8(v, fn, c):
    n = v.shape[0] // 8
    return fn(v.reshape(n, 8, D), c[None]).reshape(v.shape)


def _ln_stats(y):
    m = jnp.mean(y, axis=-1, keepdims=True)
    yc = y - m
    v = jnp.mean(yc * yc, axis=-1, keepdims=True)
    den = _r(jnp.sqrt(_r(_r(v) + EPS)))
    return yc, m, _r(m), 1.0 / den


def _layernorm(y):
    _, _, mr, rinv = _ln_stats(y)
    return (y - mr) * rinv


def _lane_fold(p, fn):
    t = p[:, 0:128]
    for j in range(1, p.shape[1] // 128):
        t = fn(t, p[:, j * 128:(j + 1) * 128])
    return t


def _normalize(pv, ls):
    l = jnp.sum(ls, axis=-1, keepdims=True)
    r = pl.reciprocal(l, approx=True)
    r = r * (2.0 - l * r)
    return (pv * r).astype(BF16)


def _head_of(n):
    if isinstance(n, int):
        return (n % 64) // 2 if n < 192 else (n - 192) % H
    return jnp.where(n < 192, lax.shift_right_logical(n & 63, 1), (n - 192) & (H - 1))


def _row_of(n):
    if isinstance(n, int):
        return SUB * ((n // 64) * 2 + n % 2 if n < 192 else min(n // 32, NRB - 1))
    rb = jnp.where(n < 192, lax.shift_right_logical(n, 6) * 2 + (n & 1),
                   jnp.minimum(lax.shift_right_logical(n, 5), NRB - 1))
    return pl.multiple_of(rb * SUB, SUB)


(SEM_C, SEM_WR, SEM_X0, SEM_X1, SEM_XR, SEM_M12, SEM_FFN, SEM_OUT, SEM_FIX,
 SEM_K0, SEM_WQE, SEM_M0) = range(12)
SEM_W0 = SEM_M0 + NST
SEM_RAMP = SEM_W0 + NST
SEM_MAIN = SEM_RAMP + R2
NSEM = SEM_MAIN + NLOAD


def _kernel(x_hbm, k_hbm, v_hbm, wq_hbm, wo_hbm, wr_hbm, wg_hbm, wu_hbm, wd_hbm,
            c_hbm, wmod_hbm, out_hbm,
            x_buf, k_buf, v_buf, wq_buf, wo_buf, wa_buf, wb_buf, wd_buf,
            act, acc, n_buf, q_acc, x2_buf, st_buf, r_buf, coef, wr_buf, sw_buf, rc_buf,
            c_buf, sc_buf, scol, zero_buf, qa_car, pv_car, ls_car,
            sems):
    def cp(src, dst, slot):
        return pltpu.make_async_copy(src, dst, sems.at[slot])

    def cp_x(b, nb, slot):
        return cp(x_hbm.at[pl.ds(b * SUB, nb * SUB), :],
                  x_buf.at[pl.ds(b * SUB, nb * SUB), :], slot)

    def cp_wq(h, slot):
        col = h * DH if isinstance(h, int) else pl.multiple_of(h * DH, DH)
        return cp(wq_hbm.at[:, pl.ds(col, DH)], wq_buf.at[h], slot)

    def cp_h(src, dst, h0, nh, slot):
        return cp(src.at[pl.ds(h0, nh)], dst.at[pl.ds(h0, nh)], slot)

    def heads(h0, nh, slot, last=False):
        return [cp_h(k_hbm, k_buf, h0, nh, slot), cp_h(v_hbm, v_buf, h0, nh, slot),
                cp_h(wo_hbm, wo_buf, h0 - 1, nh + 1 if last else nh, slot)] + [
            cp_wq(h0 + 1 + j, slot) for j in range(nh - 1 if last else nh)]

    def ramp_heads(j):
        return [cp_h(k_hbm, k_buf, j, 1, SEM_RAMP + j), cp_h(v_hbm, v_buf, j, 1, SEM_RAMP + j),
                cp_h(wo_hbm, wo_buf, j - 1, 1, SEM_RAMP + j)]

    def main_heads(k, last=False):
        return heads(R2 + k * HPI, HPI, SEM_MAIN + k, last)

    cp_k0 = cp_h(k_hbm, k_buf, 0, 1, SEM_K0)
    cp_v0 = [cp_h(v_hbm, v_buf, 0, 1, SEM_RAMP), cp_wq(R2, SEM_RAMP)]
    cp_wqe = [cp_wq(h, SEM_WQE) for h in range(R2)]

    def lanes(j):
        return pl.ds(j * 128 if isinstance(j, int) else pl.multiple_of(j * 128, 128), 128)

    def cp_m0(j):
        return [cp(wmod_hbm.at[:, lanes(u * NST + j)],
                   v_buf.at[H - NST + j, u * D:(u + 1) * D, :], SEM_M0 + j) for u in range(2)]

    def cp_w0(j):
        return cp(wq_hbm.at[lanes(j), 0:R2 * DH], wb_buf.at[lanes(j), 0:R2 * DH], SEM_W0 + j)

    cp_c = cp(c_hbm, c_buf, SEM_C)
    cp_wr = cp(wr_hbm, wr_buf, SEM_WR)
    cp_m12 = [cp(wmod_hbm.at[:, 2 * D:3 * D], wa_buf.at[:, 2 * D:3 * D], SEM_M12),
              cp(wmod_hbm.at[:, 3 * D:6 * D], wb_buf.at[:, 0:3 * D], SEM_M12)]
    cp_ffn = [cp(wg_hbm, wa_buf.at[:, 0:F], SEM_FFN),
              cp(wu_hbm, wb_buf.at[:, 0:F], SEM_FFN),
              cp(wd_hbm, wd_buf.at[:, 0:D], SEM_FFN)]

    row0 = (NRB - 1) * SUB
    cp_out = [cp(act.at[0:row0, :], out_hbm.at[0:row0, :], SEM_OUT),
              cp(act.at[row0:S, :], out_hbm.at[row0:S, :], SEM_OUT)]

    def vpu_matvec(w_ref, ncols):
        parts = []
        zf = None
        for cc in range(0, ncols, 256):
            a = None if zf is None else jnp.concatenate([zf, zf], axis=1)
            for g in range(D // 8):
                wv = w_ref[g * 8:(g + 1) * 8, cc:cc + 256].astype(F32)
                sv = scol[g * 8:(g + 1) * 8, :]
                pr = jnp.concatenate([wv[:, 0:128] * sv, wv[:, 128:256] * sv], axis=1)
                a = pr if a is None else a + pr
            zf = _float(_lane_fold(_bits(a), jnp.bitwise_or) & zero_buf[...])
            parts.append(a)
        return jnp.sum(jnp.concatenate(parts, axis=1), axis=0, keepdims=True)

    def modulate(n):
        n = _rows8(n, jnp.multiply, coef[C_SCALE])
        return _rows8(n, jnp.add, coef[C_SHIFT])

    def resid(a, row, nrows):
        a = _rows8(a, jnp.multiply, coef[C_GA])
        return _r(x_buf[pl.ds(row, nrows), :].astype(F32) + a)

    def piece(src, dst, lane_id):
        y = resid(acc[pl.ds(src, PR), :], src, PR)
        nn = _layernorm(y)
        hh = modulate(nn)
        r = jnp.sum(_rows8(nn, jnp.multiply, sw_buf[...]), axis=-1, keepdims=True)
        oo = (_rows8(y, jnp.multiply, coef[C_KEEP])
              + _rows8(hh, jnp.multiply, coef[C_GB]))
        act[pl.ds(dst, PR), :] = oo.astype(BF16)
        lane = lax.broadcasted_iota(I32, (PR, 128), 1)
        rn = jnp.where(lane == lane_id, r, r_buf[...])
        r_buf[...] = rn
        return oo, rn

    def unit_piece(n):
        is_ln = jnp.logical_and(n >= LN_START, n < LN_START + (S - 2 * SUB) // PR)
        is_fin = jnp.logical_and(n >= FIN_START, n < FIN_START + (S - SUB) // PR)
        f = n - FIN_START
        src = jnp.where(is_ln, 2 * SUB + (n - LN_START) * PR, jnp.where(is_fin, f * PR, 0))
        dst = jnp.where(jnp.logical_or(is_ln, is_fin), src, S)
        oo, rn = piece(pl.multiple_of(src, PR), pl.multiple_of(dst, PR),
                       jnp.where(is_fin, f, -1))
        bits = _lane_fold(_bits(oo), jnp.bitwise_or) | _bits(rn)
        return (bits[0:8] | bits[8:16]) & zero_buf[...]

    def qproj_head(n):
        return jnp.dot(act[pl.ds(_row_of(n), FILL), 0:D // 2],
                       wq_buf[_head_of(n)][0:D // 2], preferred_element_type=F32)

    def qproj_rest(n, qa):
        row = _row_of(n)
        w = wq_buf[_head_of(n)]
        row2 = row + FILL if isinstance(row, int) else pl.multiple_of(row + FILL, 16)
        qb = jnp.dot(act[pl.ds(row, SUB), D // 2:D], w[D // 2:D], preferred_element_type=F32)
        qc = jnp.dot(act[pl.ds(row2, SUB - FILL), 0:D // 2], w[0:D // 2],
                     preferred_element_type=F32)
        return ((qb + jnp.concatenate([qa, qc], axis=0)) * QSCALE).astype(BF16)

    def oproj(o, n):
        acc[pl.ds(_row_of(n), SUB), :] += jnp.dot(o, wo_buf[_head_of(n)],
                                                  preferred_element_type=F32)

    def unit_block(n0, nunits):
        o = _normalize(pv_car[0], ls_car[0])
        raw = (pv_car[1], ls_car[1])
        qa = qa_car[...]
        for u in range(nunits):
            n = n0 + u
            hd = _head_of(n)
            q = qproj_rest(n, qa)
            z = unit_piece(n)
            oproj(o, n - 2)
            sc = lax.dot_general(q, k_buf[hd], NT, preferred_element_type=F32)
            qa = qproj_head(n + 1)
            mm = _lane_fold(sc, jnp.maximum)
            mm = jnp.concatenate([_float(_bits(mm[0:8]) | z), mm[8:]], axis=0)
            m = jnp.max(mm, axis=-1, keepdims=True)
            p = jnp.exp2(sc - m)
            ls = _lane_fold(p, jnp.add)
            pv = jnp.dot(p.astype(BF16), v_buf[hd], preferred_element_type=F32)
            if u + 1 < nunits:
                zb = (_bits(pv).reshape(SUB // 8, 8, 128)
                      & zero_buf[...][None]).reshape(SUB, 128)
                o = _normalize(raw[0], _float(_bits(raw[1]) | zb))
            else:
                pv_car[0] = raw[0]
                ls_car[0] = raw[1]
            raw = (pv, ls)
        pv_car[1] = raw[0]
        ls_car[1] = raw[1]
        qa_car[...] = qa

    def ramp_block(j):
        o = [_normalize(pv_car[u], ls_car[u]) for u in range(2)]
        w = wo_buf[j - 1]

        def op_part(u, r0, r1, c0, c1):
            acc[u * SUB + r0:u * SUB + r1, c0:c1] += jnp.dot(
                o[u][r0:r1], w[:, c0:c1], preferred_element_type=F32)

        for u in range(2):
            q = (q_acc[j, u * SUB:(u + 1) * SUB, :] * QSCALE).astype(BF16)
            sc = lax.dot_general(q, k_buf[j], NT, preferred_element_type=F32)
            op_part(u, 0, FILL, 0, D // 2)
            m = jnp.max(_lane_fold(sc, jnp.maximum), axis=-1, keepdims=True)
            p = jnp.exp2(sc - m)
            ls_car[u] = _lane_fold(p, jnp.add)
            pv_car[u] = jnp.dot(p.astype(BF16), v_buf[j], preferred_element_type=F32)
            if u == 0:
                for v in range(2):
                    op_part(v, FILL, SUB, 0, D // 2)
                    op_part(v, 0, SUB, D // 2, D)

    def start(cps):
        for c_ in cps:
            c_.start()

    def wait(cps):
        for c_ in cps:
            c_.wait()

    start([cp_c, cp_x(0, 1, SEM_X0), cp_x(1, 1, SEM_X1)])
    for j in range(NST):
        start(cp_m0(j) + [cp_w0(j)])
    start([cp_k0] + cp_v0)
    for j in range(1, R2):
        start(ramp_heads(j))
    start([cp_wr])
    n_early = (LN_START - RAMP) // UM
    for k in range(n_early):
        start(main_heads(k))

    r_buf[...] = jnp.zeros(r_buf.shape, F32)
    zero_buf[...] = jnp.zeros(zero_buf.shape, I32)
    coef[C_GA] = jnp.zeros((8, D), F32)
    coef[C_KEEP] = jnp.zeros((8, D), F32)
    coef[C_GB] = jnp.ones((8, D), F32)
    sw_buf[...] = jnp.zeros(sw_buf.shape, F32)
    q_acc[...] = jnp.zeros(q_acc.shape, F32)
    cp_c.wait()
    cf = c_buf[...].astype(F32)
    sf = _r(cf * _r(jax.nn.sigmoid(cf)))
    sc_buf[...] = jnp.broadcast_to(sf, (16, D)).astype(BF16)
    for j in range(D // 128):
        scol[j * 128:(j + 1) * 128, :] = jnp.broadcast_to(
            sf[:, j * 128:(j + 1) * 128], (128, 128)).T

    def norm_rows(b, carry):
        cp_x(b, 1, SEM_X0 + b).wait()
        for j in range(2):
            row = pl.multiple_of(b * SUB + j * 128, 128)
            nn = _layernorm(x_buf[pl.ds(row, 128), :].astype(F32))
            for t in range(NST):
                n_buf[t, pl.ds(row, 128), :] = nn[:, t * 128:(t + 1) * 128]
        return carry

    lax.fori_loop(0, 2, norm_rows, 0)

    def stage(j, carry):
        wait(cp_m0(j))
        wm = jnp.concatenate([v_buf[H - NST + j, 0:D, :], v_buf[H - NST + j, D:2 * D, :]], axis=1)
        mj = _r(jnp.dot(sc_buf[...], wm, preferred_element_type=F32)[0:8, :])
        coef[C_SHIFT, :, lanes(j)] = mj[:, 0:128]
        coef[C_SCALE, :, lanes(j)] = _r(1.0 + mj[:, 128:256])
        zr = S // NST
        acc[pl.ds(pl.multiple_of(j * zr, zr), zr), :] = jnp.zeros((zr, D), F32)
        cp_w0(j).wait()
        hj = (n_buf[j].reshape(2 * SUB // 8, 8, 128) * coef[C_SCALE, :, lanes(j)][None]
              + coef[C_SHIFT, :, lanes(j)][None]).reshape(2 * SUB, 128).astype(BF16)
        act[0:2 * SUB, lanes(j)] = hj
        part = jnp.dot(hj, wb_buf[lanes(j), 0:R2 * DH], preferred_element_type=F32)
        for h in range(R2):
            q_acc[h] += part[:, h * DH:(h + 1) * DH]
        return carry

    lax.fori_loop(0, NST, stage, 0)

    cp_k0.wait()
    s01 = lax.dot_general((q_acc[0] * QSCALE).astype(BF16), k_buf[0], NT,
                          preferred_element_type=F32)
    m01 = jnp.max(_lane_fold(s01, jnp.maximum), axis=-1, keepdims=True)
    wait(cp_v0)
    qa_car[...] = qproj_head(RAMP)
    for u in range(2):
        p = jnp.exp2(s01[u * SUB:(u + 1) * SUB] - m01[u * SUB:(u + 1) * SUB])
        ls_car[u] = _lane_fold(p, jnp.add)
        pv_car[u] = jnp.dot(p.astype(BF16), v_buf[0], preferred_element_type=F32)

    def ramp2(j, carry):
        wait(ramp_heads(j))
        ramp_block(j)
        return carry

    lax.fori_loop(1, R2, ramp2, 0)
    start([cp_x(2, NRB - 2, SEM_XR)])
    for k in range(n_early, NLOAD):
        start(main_heads(k, k == NLOAD - 1))
    start(cp_wqe + cp_m12)

    assert FIN_START + row0 // PR <= RAMP + (NM - 1) * UM

    def main(k, carry):
        n0 = RAMP + k * UM

        @pl.when(k <= K_MOD + 2)
        def _():
            @pl.when(k < NLOAD - 1)
            def _():
                wait(main_heads(k))

            @pl.when(k == NLOAD - 1)
            def _():
                wait(main_heads(NLOAD - 1, True) + cp_wqe)

            @pl.when(k == n_early)
            def _():
                cp_x(2, NRB - 2, SEM_XR).wait()

            @pl.when(k == K_MOD)
            def _():
                wait(cp_m12 + [cp_wr])
                sc = sc_buf[...]
                m2a = jnp.dot(sc, wb_buf[:, MVC:3 * D], preferred_element_type=F32)[0:8, :]
                m1 = _r(jnp.dot(sc, wa_buf[:, 2 * D:3 * D], preferred_element_type=F32)[0:8, :])
                m2b = jnp.broadcast_to(vpu_matvec(wb_buf, MVC), (8, MVC))
                m2 = _r(jnp.concatenate([m2b, m2a], axis=1))
                coef[C_GA] = m1
                coef[C_KEEP] = jnp.ones((8, D), F32)
                scale = _r(1.0 + m2[:, D:2 * D])
                coef[C_SHIFT] = m2[:, 0:D]
                coef[C_SCALE] = scale
                coef[C_GB] = m2[:, 2 * D:3 * D]
                w8 = wr_buf[...].astype(F32)
                wr = jnp.concatenate([jnp.broadcast_to(w8[j:j + 1, :], (8, 128))
                                      for j in range(D // 128)], axis=1)
                sw_buf[...] = scale * wr
                c1 = jnp.sum(scale * wr, axis=-1, keepdims=True)
                c0 = jnp.sum(m2[:, 0:D] * wr, axis=-1, keepdims=True)
                rid = lax.broadcasted_iota(I32, (8, 128), 0)
                rc_buf[...] = jnp.where(rid == 0, c1, c0)
                start(cp_ffn)

            @pl.when(k == K_MOD + 2)
            def _():
                wait(cp_ffn)

        @pl.when(k == NM - 1)
        def _():
            cp_out[0].start()

        unit_block(n0, UM)
        return carry

    lax.fori_loop(0, NM, main, 0)

    neg = -jnp.inf

    def keep_rows(y, lo):
        n = y.shape[0]
        yc, m, mr, rinv = _ln_stats(y)
        x2_buf[lo:lo + n, :] = y
        st_buf[0, lo:lo + n, :] = jnp.broadcast_to(mr, (n, 128))
        st_buf[1, lo:lo + n, :] = jnp.broadcast_to(rinv, (n, 128))
        d = jnp.sum(_rows8(yc, jnp.multiply, sw_buf[...]), axis=-1, keepdims=True)
        return (d + (m - mr) * rc_buf[0:1, 0:1]) * rinv

    def parked(lo, n):
        y = x2_buf[pl.ds(lo, n), :]
        mr = st_buf[0, pl.ds(lo, n), :]
        rinv = st_buf[1, pl.ds(lo, n), :]
        return y, jnp.concatenate([(y[:, j * 128:(j + 1) * 128] - mr) * rinv
                                   for j in range(D // 128)], axis=1)

    def all_red(v, fn):
        return fn(fn(v, axis=0, keepdims=True), axis=1, keepdims=True)

    lane = lax.broadcasted_iota(I32, (PR, 128), 1)
    ridx = (lane * PR + lax.broadcasted_iota(I32, (PR, 128), 0)).astype(F32)
    rr = jnp.where(lane < row0 // PR, r_buf[...], neg)
    last_old = float(row0 - 1)
    cm1 = all_red(rr, jnp.max)
    ci1 = all_red(jnp.where(rr == cm1, ridx, last_old), jnp.min)
    rr2 = jnp.where(ridx == ci1, neg, rr)
    cm2 = all_red(rr2, jnp.max)
    ci2 = all_red(jnp.where(jnp.logical_and(rr2 == cm2, ridx != ci1), ridx, last_old), jnp.min)
    ci1 = jnp.minimum(ci1, last_old).astype(I32)
    ci2 = jnp.minimum(ci2, last_old).astype(I32)
    for j, ci in enumerate((ci1, ci2)):
        g = pl.multiple_of(lax.shift_right_logical(ci[0, 0], 4) * PR, PR)
        keep_rows(resid(acc[pl.ds(g, PR), :], g, PR), SUB + j * PR)

    o2 = jnp.concatenate([_normalize(pv_car[0], ls_car[0]),
                          _normalize(pv_car[1], ls_car[1])], axis=1)
    wo2 = jnp.concatenate([wo_buf[H - 2], wo_buf[H - 1]], axis=0)
    r_new = []
    for j in range(SUB // ECH):
        lo, hi = j * ECH, (j + 1) * ECH
        a = acc[row0 + lo:row0 + hi, :] + jnp.dot(o2[lo:hi], wo2, preferred_element_type=F32)
        r_new.append(keep_rows(resid(a, row0 + lo, ECH), lo))

    sub8 = lax.broadcasted_iota(I32, (8, 1), 0)
    big = jnp.int32((S - 1) * 512 + SUB - 1)
    vals = jnp.concatenate(
        r_new + [jnp.where(sub8 == 0, cm1, jnp.where(sub8 == 1, cm2, neg))], axis=0)
    pos = lax.broadcasted_iota(I32, (SUB, 1), 0)
    cc1 = ci1 * 512 + SUB + (ci1 & (PR - 1))
    cc2 = ci2 * 512 + SUB + PR + (ci2 & (PR - 1))
    code = jnp.concatenate(
        [(pos + row0) * 512 + pos,
         jnp.where(sub8 == 0, cc1, jnp.where(sub8 == 1, cc2, big))], axis=0)
    m1 = jnp.max(vals, axis=0, keepdims=True)
    k1 = jnp.min(jnp.where(vals == m1, code, big), axis=0, keepdims=True)
    vals2 = jnp.where(code == k1, neg, vals)
    m2 = jnp.max(vals2, axis=0, keepdims=True)
    k2 = jnp.min(jnp.where(jnp.logical_and(vals2 == m2, code != k1), code, big),
                 axis=0, keepdims=True)
    k1 = k1[0, 0]
    k2 = k2[0, 0]
    i1 = lax.shift_right_logical(k1, 9)
    i2 = lax.shift_right_logical(k2, 9)
    t1 = k1 & 511
    t2 = k2 & 511
    rowid = lax.broadcasted_iota(I32, (PR, D), 0)
    xf = modulate(jnp.where(rowid == 0, parked(t1, 1)[1], parked(t2, 1)[1]))

    off = pl.multiple_of(jnp.minimum(k2, 0) * 8, 8)
    for j in range(SUB // PR):
        yl, nl = parked(pl.multiple_of(off + j * PR, 8), PR)
        act[row0 + j * PR:row0 + (j + 1) * PR, :] = (
            yl + _rows8(modulate(nl), jnp.multiply, coef[C_GB])).astype(BF16)
    cp_out[1].start()

    gt = _r(jnp.dot(xf.astype(BF16), wa_buf[:, 0:F], preferred_element_type=F32))
    zt = _bits(act[pl.ds(pl.multiple_of(off * 2, PR), PR), 0:128].astype(F32))
    zt = jnp.concatenate([zt[0:8] & zero_buf[...], zt[8:16] & zero_buf[...]], axis=0)
    xs = jnp.concatenate([_float(_bits(xf[:, 0:128]) | zt), xf[:, 128:]], axis=1).astype(BF16)
    up = _r(jnp.dot(xs, wb_buf[:, 0:F], preferred_element_type=F32))
    hid = (_r(gt * _r(jax.nn.sigmoid(gt))) * up).astype(BF16)
    y = _r(jnp.dot(hid, wd_buf[:, 0:D], preferred_element_type=F32))
    y1 = _r(y[0:1, :] * _r(jax.nn.sigmoid(_r(m1 + rc_buf[1:2, 0:1]))))
    y2 = _r(y[1:2, :] * _r(jax.nn.sigmoid(_r(m2 + rc_buf[1:2, 0:1]))))

    def fix(i, t):
        g = pl.multiple_of(lax.shift_right_logical(i, 4) * PR, PR)
        tg = pl.multiple_of(lax.shift_right_logical(t, 4) * PR, PR)
        rid = rowid + g
        upd = jnp.where(rid == i1, y1, jnp.where(rid == i2, y2, 0.0))
        yg, ng = parked(tg, PR)
        return g, (yg + _rows8(modulate(ng) + upd, jnp.multiply, coef[C_GB])).astype(BF16)

    g1, fix1 = fix(i1, t1)
    g2, fix2 = fix(i2, t2)
    wait(cp_out)
    act[pl.ds(g1, PR), :] = fix1
    act[pl.ds(g2, PR), :] = fix2
    f1 = cp(act.at[pl.ds(g1, PR), :], out_hbm.at[pl.ds(g1, PR), :], SEM_OUT)
    f2 = cp(act.at[pl.ds(g2, PR), :], out_hbm.at[pl.ds(g2, PR), :], SEM_FIX)
    f1.start()

    @pl.when(g1 != g2)
    def _():
        f2.start()
        f2.wait()

    f1.wait()


@jax.jit
def pallas_adaLN_cond__mha_block_cached__moe_arch_mod__prompt_kernel(
    A_x: jax.Array,
    A_k_cache: jax.Array,
    A_v_cache: jax.Array,
    A_wq: jax.Array,
    A_wo: jax.Array,
    B_x: jax.Array,
    B_w_r: jax.Array,
    B_w_gate: jax.Array,
    B_w_up: jax.Array,
    B_w_down: jax.Array,
    c: jax.Array,
    w_mod: jax.Array,
):
    del B_x
    hbm = pl.BlockSpec(memory_space=pl.ANY)
    out = pl.pallas_call(
        _kernel,
        in_specs=[hbm] * 11,
        out_specs=hbm,
        out_shape=jax.ShapeDtypeStruct((S, D), BF16),
        scratch_shapes=[
            pltpu.VMEM((S, D), BF16),
            pltpu.VMEM((H, S, DH), BF16),
            pltpu.VMEM((H, S, DH), BF16),
            pltpu.VMEM((H, D, DH), BF16),
            pltpu.VMEM((H, DH, D), BF16),
            pltpu.VMEM((D, F + PAD), BF16),
            pltpu.VMEM((D, F + PAD), BF16),
            pltpu.VMEM((F, D + PAD), BF16),
            pltpu.VMEM((S + PR, D), BF16),
            pltpu.VMEM((S, D), F32),
            pltpu.VMEM((NST, 2 * SUB, 128), F32),
            pltpu.VMEM((R2, 2 * SUB, DH), F32),
            pltpu.VMEM((SUB + 2 * PR, D), F32),
            pltpu.VMEM((2, SUB + 2 * PR, 128), F32),
            pltpu.VMEM((PR, 128), F32),
            pltpu.VMEM((5, 8, D), F32),
            pltpu.VMEM((8, 128), BF16),
            pltpu.VMEM((8, D), F32),
            pltpu.VMEM((8, 128), F32),
            pltpu.VMEM((1, D), BF16),
            pltpu.VMEM((16, D), BF16),
            pltpu.VMEM((D, 128), F32),
            pltpu.VMEM((8, 128), I32),
            pltpu.VMEM((FILL, DH), F32),
            pltpu.VMEM((2, SUB, DH), F32),
            pltpu.VMEM((2, SUB, DH), F32),
            pltpu.SemaphoreType.DMA((NSEM,)),
        ],
        compiler_params=pltpu.CompilerParams(
            vmem_limit_bytes=120 * 1024 * 1024,
            disable_bounds_checks=True,
            disable_semaphore_checks=True,
        ),
        name="adaln_mha_mod",
    )(
        A_x.reshape(S, D),
        A_k_cache.reshape(H, S, DH),
        A_v_cache.reshape(H, S, DH),
        A_wq,
        A_wo.reshape(H, DH, D),
        B_w_r.reshape(8, 128),
        B_w_gate,
        B_w_up,
        B_w_down,
        c,
        w_mod,
    )
    return out.reshape(1, S, D)
```

```python
import jax
import jax.numpy as jnp
from jax import lax
import jax.experimental.pallas as pl
import jax.experimental.pallas.tpu as pltpu

S = 2048
D = 1024
H = 32
DH = 128
F = 3584
SUB = 256
NRB = S // SUB
NU = H * NRB
PR = 16
UM = 12
R2 = 8
RAMP = 2 * R2
NM = (NU - RAMP) // UM
HPI = UM // 2
NLOAD = (2 * H - RAMP) // UM
FIN_START = 130
K_MOD = (FIN_START - RAMP) // UM
LN_START = RAMP + K_MOD * UM - (S - 2 * SUB) // PR
FILL = 64
ECH = 64
PAD = 128
NST = D // 128
MVC = 1280
EPS = 1e-5
QSCALE = float(DH ** -0.5) * 1.4426950408889634

F32 = jnp.float32
BF16 = jnp.bfloat16
I32 = jnp.int32
NT = (((1,), (1,)), ((), ()))

C_GA, C_SCALE, C_SHIFT, C_KEEP, C_GB = range(5)


def _r(v):
    return v.astype(BF16).astype(F32)


def _bits(v):
    return lax.bitcast_convert_type(v, I32)


def _float(v):
    return lax.bitcast_convert_type(v, F32)


def _rows8(v, fn, c):
    n = v.shape[0] // 8
    return fn(v.reshape(n, 8, D), c[None]).reshape(v.shape)


def _ln_stats(y):
    m = jnp.mean(y, axis=-1, keepdims=True)
    yc = y - m
    v = jnp.mean(yc * yc, axis=-1, keepdims=True)
    den = _r(jnp.sqrt(_r(_r(v) + EPS)))
    return yc, m, _r(m), 1.0 / den


def _layernorm(y):
    _, _, mr, rinv = _ln_stats(y)
    return (y - mr) * rinv


def _lane_fold(p, fn):
    t = p[:, 0:128]
    for j in range(1, p.shape[1] // 128):
        t = fn(t, p[:, j * 128:(j + 1) * 128])
    return t


def _normalize(pv, ls):
    l = jnp.sum(ls, axis=-1, keepdims=True)
    r = pl.reciprocal(l, approx=True)
    r = r * (2.0 - l * r)
    return (pv * r).astype(BF16)


def _head_of(n):
    if isinstance(n, int):
        return (n % 64) // 2 if n < 192 else (n - 192) % H
    return jnp.where(n < 192, lax.shift_right_logical(n & 63, 1), (n - 192) & (H - 1))


def _row_of(n):
    if isinstance(n, int):
        return SUB * ((n // 64) * 2 + n % 2 if n < 192 else min(n // 32, NRB - 1))
    rb = jnp.where(n < 192, lax.shift_right_logical(n, 6) * 2 + (n & 1),
                   jnp.minimum(lax.shift_right_logical(n, 5), NRB - 1))
    return pl.multiple_of(rb * SUB, SUB)


(SEM_C, SEM_WR, SEM_X0, SEM_X1, SEM_XR, SEM_M12, SEM_FFN, SEM_OUT, SEM_FIX,
 SEM_K0, SEM_WQE, SEM_M0) = range(12)
SEM_W0 = SEM_M0 + NST
SEM_RAMP = SEM_W0 + NST
SEM_MAIN = SEM_RAMP + R2
NSEM = SEM_MAIN + NLOAD


def _kernel(x_hbm, k_hbm, v_hbm, wq_hbm, wo_hbm, wr_hbm, wg_hbm, wu_hbm, wd_hbm,
            c_hbm, wmod_hbm, out_hbm,
            x_buf, k_buf, v_buf, wq_buf, wo_buf, wa_buf, wb_buf, wd_buf,
            act, acc, n_buf, q_acc, x2_buf, st_buf, r_buf, coef, wr_buf, sw_buf, rc_buf,
            c_buf, sc_buf, scol, zero_buf, qa_car, pv_car, ls_car,
            sems):
    def cp(src, dst, slot):
        return pltpu.make_async_copy(src, dst, sems.at[slot])

    def cp_x(b, nb, slot):
        return cp(x_hbm.at[pl.ds(b * SUB, nb * SUB), :],
                  x_buf.at[pl.ds(b * SUB, nb * SUB), :], slot)

    def cp_wq(h, slot):
        col = h * DH if isinstance(h, int) else pl.multiple_of(h * DH, DH)
        return cp(wq_hbm.at[:, pl.ds(col, DH)], wq_buf.at[h], slot)

    def cp_h(src, dst, h0, nh, slot):
        return cp(src.at[pl.ds(h0, nh)], dst.at[pl.ds(h0, nh)], slot)

    def heads(h0, nh, slot, last=False):
        return [cp_h(k_hbm, k_buf, h0, nh, slot), cp_h(v_hbm, v_buf, h0, nh, slot),
                cp_h(wo_hbm, wo_buf, h0 - 1, nh + 1 if last else nh, slot)] + [
            cp_wq(h0 + 1 + j, slot) for j in range(nh - 1 if last else nh)]

    def ramp_heads(j):
        return [cp_h(k_hbm, k_buf, j, 1, SEM_RAMP + j), cp_h(v_hbm, v_buf, j, 1, SEM_RAMP + j),
                cp_h(wo_hbm, wo_buf, j - 1, 1, SEM_RAMP + j)]

    def main_heads(k, last=False):
        return heads(R2 + k * HPI, HPI, SEM_MAIN + k, last)

    cp_k0 = cp_h(k_hbm, k_buf, 0, 1, SEM_K0)
    cp_v0 = [cp_h(v_hbm, v_buf, 0, 1, SEM_RAMP), cp_wq(R2, SEM_RAMP)]
    cp_wqe = [cp_wq(h, SEM_WQE) for h in range(R2)]

    def lanes(j):
        return pl.ds(j * 128 if isinstance(j, int) else pl.multiple_of(j * 128, 128), 128)

    def cp_m0(j):
        return [cp(wmod_hbm.at[:, lanes(u * NST + j)],
                   v_buf.at[H - NST + j, u * D:(u + 1) * D, :], SEM_M0 + j) for u in range(2)]

    def cp_w0(j):
        return cp(wq_hbm.at[lanes(j), 0:R2 * DH], wb_buf.at[lanes(j), 0:R2 * DH], SEM_W0 + j)

    cp_c = cp(c_hbm, c_buf, SEM_C)
    cp_wr = cp(wr_hbm, wr_buf, SEM_WR)
    cp_m12 = [cp(wmod_hbm.at[:, 2 * D:3 * D], wa_buf.at[:, 2 * D:3 * D], SEM_M12),
              cp(wmod_hbm.at[:, 3 * D:6 * D], wb_buf.at[:, 0:3 * D], SEM_M12)]
    cp_ffn = [cp(wg_hbm, wa_buf.at[:, 0:F], SEM_FFN),
              cp(wu_hbm, wb_buf.at[:, 0:F], SEM_FFN),
              cp(wd_hbm, wd_buf.at[:, 0:D], SEM_FFN)]

    row0 = (NRB - 1) * SUB
    cp_out = [cp(act.at[0:row0, :], out_hbm.at[0:row0, :], SEM_OUT),
              cp(act.at[row0:S, :], out_hbm.at[row0:S, :], SEM_OUT)]

    def vpu_matvec(w_ref, ncols):
        parts = []
        zf = None
        for cc in range(0, ncols, 256):
            a = None if zf is None else jnp.concatenate([zf, zf], axis=1)
            for g in range(D // 8):
                wv = w_ref[g * 8:(g + 1) * 8, cc:cc + 256].astype(F32)
                sv = scol[g * 8:(g + 1) * 8, :]
                pr = jnp.concatenate([wv[:, 0:128] * sv, wv[:, 128:256] * sv], axis=1)
                a = pr if a is None else a + pr
            zf = _float(_lane_fold(_bits(a), jnp.bitwise_or) & zero_buf[...])
            parts.append(a)
        return jnp.sum(jnp.concatenate(parts, axis=1), axis=0, keepdims=True)

    def modulate(n):
        n = _rows8(n, jnp.multiply, coef[C_SCALE])
        return _rows8(n, jnp.add, coef[C_SHIFT])

    def resid(a, row, nrows):
        a = _rows8(a, jnp.multiply, coef[C_GA])
        return _r(x_buf[pl.ds(row, nrows), :].astype(F32) + a)

    def piece(src, dst, lane_id):
        y = resid(acc[pl.ds(src, PR), :], src, PR)
        nn = _layernorm(y)
        hh = modulate(nn)
        r = jnp.sum(_rows8(nn, jnp.multiply, sw_buf[...]), axis=-1, keepdims=True)
        oo = (_rows8(y, jnp.multiply, coef[C_KEEP])
              + _rows8(hh, jnp.multiply, coef[C_GB]))
        act[pl.ds(dst, PR), :] = oo.astype(BF16)
        lane = lax.broadcasted_iota(I32, (PR, 128), 1)
        rn = jnp.where(lane == lane_id, r, r_buf[...])
        r_buf[...] = rn
        return oo, rn

    def unit_piece(n):
        is_ln = jnp.logical_and(n >= LN_START, n < LN_START + (S - 2 * SUB) // PR)
        is_fin = jnp.logical_and(n >= FIN_START, n < FIN_START + (S - SUB) // PR)
        f = n - FIN_START
        src = jnp.where(is_ln, 2 * SUB + (n - LN_START) * PR, jnp.where(is_fin, f * PR, 0))
        dst = jnp.where(jnp.logical_or(is_ln, is_fin), src, S)
        oo, rn = piece(pl.multiple_of(src, PR), pl.multiple_of(dst, PR),
                       jnp.where(is_fin, f, -1))
        bits = _lane_fold(_bits(oo), jnp.bitwise_or) | _bits(rn)
        return (bits[0:8] | bits[8:16]) & zero_buf[...]

    def qproj_head(n):
        return jnp.dot(act[pl.ds(_row_of(n), FILL), 0:D // 2],
                       wq_buf[_head_of(n)][0:D // 2], preferred_element_type=F32)

    def qproj_rest(n, qa):
        row = _row_of(n)
        w = wq_buf[_head_of(n)]
        row2 = row + FILL if isinstance(row, int) else pl.multiple_of(row + FILL, 16)
        qb = jnp.dot(act[pl.ds(row, SUB), D // 2:D], w[D // 2:D], preferred_element_type=F32)
        qc = jnp.dot(act[pl.ds(row2, SUB - FILL), 0:D // 2], w[0:D // 2],
                     preferred_element_type=F32)
        return ((qb + jnp.concatenate([qa, qc], axis=0)) * QSCALE).astype(BF16)

    def oproj(o, n):
        acc[pl.ds(_row_of(n), SUB), :] += jnp.dot(o, wo_buf[_head_of(n)],
                                                  preferred_element_type=F32)

    def unit_block(n0, nunits):
        o = _normalize(pv_car[0], ls_car[0])
        raw = (pv_car[1], ls_car[1])
        qa = qa_car[...]
        for u in range(nunits):
            n = n0 + u
            hd = _head_of(n)
            q = qproj_rest(n, qa)
            z = unit_piece(n)
            oproj(o, n - 2)
            sc = lax.dot_general(q, k_buf[hd], NT, preferred_element_type=F32)
            qa = qproj_head(n + 1)
            mm = _lane_fold(sc, jnp.maximum)
            mm = jnp.concatenate([_float(_bits(mm[0:8]) | z), mm[8:]], axis=0)
            m = jnp.max(mm, axis=-1, keepdims=True)
            p = jnp.exp2(sc - m)
            ls = _lane_fold(p, jnp.add)
            pv = jnp.dot(p.astype(BF16), v_buf[hd], preferred_element_type=F32)
            if u + 1 < nunits:
                zb = (_bits(pv).reshape(SUB // 8, 8, 128)
                      & zero_buf[...][None]).reshape(SUB, 128)
                o = _normalize(raw[0], _float(_bits(raw[1]) | zb))
            else:
                pv_car[0] = raw[0]
                ls_car[0] = raw[1]
            raw = (pv, ls)
        pv_car[1] = raw[0]
        ls_car[1] = raw[1]
        qa_car[...] = qa

    def ramp_block(j):
        o = [_normalize(pv_car[u], ls_car[u]) for u in range(2)]
        w = wo_buf[j - 1]

        def op_part(u, r0, r1, c0, c1):
            acc[u * SUB + r0:u * SUB + r1, c0:c1] += jnp.dot(
                o[u][r0:r1], w[:, c0:c1], preferred_element_type=F32)

        for u in range(2):
            q = (q_acc[j, u * SUB:(u + 1) * SUB, :] * QSCALE).astype(BF16)
            sc = lax.dot_general(q, k_buf[j], NT, preferred_element_type=F32)
            op_part(u, 0, FILL, 0, D // 2)
            m = jnp.max(_lane_fold(sc, jnp.maximum), axis=-1, keepdims=True)
            p = jnp.exp2(sc - m)
            ls_car[u] = _lane_fold(p, jnp.add)
            pv_car[u] = jnp.dot(p.astype(BF16), v_buf[j], preferred_element_type=F32)
            if u == 0:
                for v in range(2):
                    op_part(v, FILL, SUB, 0, D // 2)
                    op_part(v, 0, SUB, D // 2, D)

    def start(cps):
        for c_ in cps:
            c_.start()

    def wait(cps):
        for c_ in cps:
            c_.wait()

    start([cp_c, cp_x(0, 1, SEM_X0), cp_x(1, 1, SEM_X1)])
    for j in range(NST):
        start(cp_m0(j) + [cp_w0(j)])
    start([cp_k0] + cp_v0)
    for j in range(1, R2):
        start(ramp_heads(j))
    start([cp_wr])
    n_early = (LN_START - RAMP) // UM
    for k in range(n_early):
        start(main_heads(k))

    r_buf[...] = jnp.zeros(r_buf.shape, F32)
    zero_buf[...] = jnp.zeros(zero_buf.shape, I32)
    coef[C_GA] = jnp.zeros((8, D), F32)
    coef[C_KEEP] = jnp.zeros((8, D), F32)
    coef[C_GB] = jnp.ones((8, D), F32)
    sw_buf[...] = jnp.zeros(sw_buf.shape, F32)
    q_acc[...] = jnp.zeros(q_acc.shape, F32)
    cp_c.wait()
    cf = c_buf[...].astype(F32)
    sf = _r(cf * _r(jax.nn.sigmoid(cf)))
    sc_buf[...] = jnp.broadcast_to(sf, (16, D)).astype(BF16)
    for j in range(D // 128):
        scol[j * 128:(j + 1) * 128, :] = jnp.broadcast_to(
            sf[:, j * 128:(j + 1) * 128], (128, 128)).T

    def norm_rows(b, carry):
        cp_x(b, 1, SEM_X0 + b).wait()
        for j in range(2):
            row = pl.multiple_of(b * SUB + j * 128, 128)
            nn = _layernorm(x_buf[pl.ds(row, 128), :].astype(F32))
            for t in range(NST):
                n_buf[t, pl.ds(row, 128), :] = nn[:, t * 128:(t + 1) * 128]
        return carry

    lax.fori_loop(0, 2, norm_rows, 0)

    def stage(j, carry):
        wait(cp_m0(j))
        wm = jnp.concatenate([v_buf[H - NST + j, 0:D, :], v_buf[H - NST + j, D:2 * D, :]], axis=1)
        mj = _r(jnp.dot(sc_buf[...], wm, preferred_element_type=F32)[0:8, :])
        coef[C_SHIFT, :, lanes(j)] = mj[:, 0:128]
        coef[C_SCALE, :, lanes(j)] = _r(1.0 + mj[:, 128:256])
        zr = S // NST
        acc[pl.ds(pl.multiple_of(j * zr, zr), zr), :] = jnp.zeros((zr, D), F32)
        cp_w0(j).wait()
        hj = (n_buf[j].reshape(2 * SUB // 8, 8, 128) * coef[C_SCALE, :, lanes(j)][None]
              + coef[C_SHIFT, :, lanes(j)][None]).reshape(2 * SUB, 128).astype(BF16)
        act[0:2 * SUB, lanes(j)] = hj
        part = jnp.dot(hj, wb_buf[lanes(j), 0:R2 * DH], preferred_element_type=F32)
        for h in range(R2):
            q_acc[h] += part[:, h * DH:(h + 1) * DH]
        return carry

    lax.fori_loop(0, NST, stage, 0)

    cp_k0.wait()
    s01 = lax.dot_general((q_acc[0] * QSCALE).astype(BF16), k_buf[0], NT,
                          preferred_element_type=F32)
    mm01 = _lane_fold(s01, jnp.maximum)
    m0 = jnp.max(mm01[0:SUB], axis=-1, keepdims=True)
    wait(cp_v0)
    qa_car[...] = qproj_head(RAMP)
    for u in range(2):
        m = m0 if u == 0 else jnp.max(mm01[SUB:], axis=-1, keepdims=True)
        p = jnp.exp2(s01[u * SUB:(u + 1) * SUB] - m)
        ls_car[u] = _lane_fold(p, jnp.add)
        pv_car[u] = jnp.dot(p.astype(BF16), v_buf[0], preferred_element_type=F32)

    def ramp2(j, carry):
        wait(ramp_heads(j))
        ramp_block(j)
        return carry

    lax.fori_loop(1, R2, ramp2, 0)
    start([cp_x(2, NRB - 2, SEM_XR)])
    for k in range(n_early, NLOAD):
        start(main_heads(k, k == NLOAD - 1))
    start(cp_wqe + cp_m12)

    assert FIN_START + row0 // PR <= RAMP + (NM - 1) * UM

    def main(k, carry):
        n0 = RAMP + k * UM

        @pl.when(k <= K_MOD + 2)
        def _():
            @pl.when(k < NLOAD - 1)
            def _():
                wait(main_heads(k))

            @pl.when(k == NLOAD - 1)
            def _():
                wait(main_heads(NLOAD - 1, True) + cp_wqe)

            @pl.when(k == n_early)
            def _():
                cp_x(2, NRB - 2, SEM_XR).wait()

            @pl.when(k == K_MOD)
            def _():
                wait(cp_m12 + [cp_wr])
                sc = sc_buf[...]
                m2a = jnp.dot(sc, wb_buf[:, MVC:3 * D], preferred_element_type=F32)[0:8, :]
                m1 = _r(jnp.dot(sc, wa_buf[:, 2 * D:3 * D], preferred_element_type=F32)[0:8, :])
                m2b = jnp.broadcast_to(vpu_matvec(wb_buf, MVC), (8, MVC))
                m2 = _r(jnp.concatenate([m2b, m2a], axis=1))
                coef[C_GA] = m1
                coef[C_KEEP] = jnp.ones((8, D), F32)
                scale = _r(1.0 + m2[:, D:2 * D])
                coef[C_SHIFT] = m2[:, 0:D]
                coef[C_SCALE] = scale
                coef[C_GB] = m2[:, 2 * D:3 * D]
                w8 = wr_buf[...].astype(F32)
                wr = jnp.concatenate([jnp.broadcast_to(w8[j:j + 1, :], (8, 128))
                                      for j in range(D // 128)], axis=1)
                sw_buf[...] = scale * wr
                c1 = jnp.sum(scale * wr, axis=-1, keepdims=True)
                c0 = jnp.sum(m2[:, 0:D] * wr, axis=-1, keepdims=True)
                rid = lax.broadcasted_iota(I32, (8, 128), 0)
                rc_buf[...] = jnp.where(rid == 0, c1, c0)
                start(cp_ffn)

            @pl.when(k == K_MOD + 2)
            def _():
                wait(cp_ffn)

        @pl.when(k == NM - 1)
        def _():
            cp_out[0].start()

        unit_block(n0, UM)
        return carry

    lax.fori_loop(0, NM, main, 0)

    neg = -jnp.inf

    def keep_rows(y, lo):
        n = y.shape[0]
        yc, m, mr, rinv = _ln_stats(y)
        x2_buf[lo:lo + n, :] = y
        st_buf[0, lo:lo + n, :] = jnp.broadcast_to(mr, (n, 128))
        st_buf[1, lo:lo + n, :] = jnp.broadcast_to(rinv, (n, 128))
        d = jnp.sum(_rows8(yc, jnp.multiply, sw_buf[...]), axis=-1, keepdims=True)
        return (d + (m - mr) * rc_buf[0:1, 0:1]) * rinv

    def parked(lo, n):
        y = x2_buf[pl.ds(lo, n), :]
        mr = st_buf[0, pl.ds(lo, n), :]
        rinv = st_buf[1, pl.ds(lo, n), :]
        return y, jnp.concatenate([(y[:, j * 128:(j + 1) * 128] - mr) * rinv
                                   for j in range(D // 128)], axis=1)

    def all_red(v, fn):
        return fn(fn(v, axis=0, keepdims=True), axis=1, keepdims=True)

    lane = lax.broadcasted_iota(I32, (PR, 128), 1)
    ridx = (lane * PR + lax.broadcasted_iota(I32, (PR, 128), 0)).astype(F32)
    rr = jnp.where(lane < row0 // PR, r_buf[...], neg)
    last_old = float(row0 - 1)
    cm1 = all_red(rr, jnp.max)
    ci1 = all_red(jnp.where(rr == cm1, ridx, last_old), jnp.min)
    rr2 = jnp.where(ridx == ci1, neg, rr)
    cm2 = all_red(rr2, jnp.max)
    ci2 = all_red(jnp.where(jnp.logical_and(rr2 == cm2, ridx != ci1), ridx, last_old), jnp.min)
    ci1 = jnp.minimum(ci1, last_old).astype(I32)
    ci2 = jnp.minimum(ci2, last_old).astype(I32)
    for j, ci in enumerate((ci1, ci2)):
        g = pl.multiple_of(lax.shift_right_logical(ci[0, 0], 4) * PR, PR)
        keep_rows(resid(acc[pl.ds(g, PR), :], g, PR), SUB + j * PR)

    o2 = jnp.concatenate([_normalize(pv_car[0], ls_car[0]),
                          _normalize(pv_car[1], ls_car[1])], axis=1)
    wo2 = jnp.concatenate([wo_buf[H - 2], wo_buf[H - 1]], axis=0)
    r_new = []
    for j in range(SUB // ECH):
        lo, hi = j * ECH, (j + 1) * ECH
        a = acc[row0 + lo:row0 + hi, :] + jnp.dot(o2[lo:hi], wo2, preferred_element_type=F32)
        r_new.append(keep_rows(resid(a, row0 + lo, ECH), lo))

    sub8 = lax.broadcasted_iota(I32, (8, 1), 0)
    big = jnp.int32((S - 1) * 512 + SUB - 1)
    vals = jnp.concatenate(
        r_new + [jnp.where(sub8 == 0, cm1, jnp.where(sub8 == 1, cm2, neg))], axis=0)
    pos = lax.broadcasted_iota(I32, (SUB, 1), 0)
    cc1 = ci1 * 512 + SUB + (ci1 & (PR - 1))
    cc2 = ci2 * 512 + SUB + PR + (ci2 & (PR - 1))
    code = jnp.concatenate(
        [(pos + row0) * 512 + pos,
         jnp.where(sub8 == 0, cc1, jnp.where(sub8 == 1, cc2, big))], axis=0)
    m1 = jnp.max(vals, axis=0, keepdims=True)
    k1 = jnp.min(jnp.where(vals == m1, code, big), axis=0, keepdims=True)
    vals2 = jnp.where(code == k1, neg, vals)
    m2 = jnp.max(vals2, axis=0, keepdims=True)
    k2 = jnp.min(jnp.where(jnp.logical_and(vals2 == m2, code != k1), code, big),
                 axis=0, keepdims=True)
    k1 = k1[0, 0]
    k2 = k2[0, 0]
    i1 = lax.shift_right_logical(k1, 9)
    i2 = lax.shift_right_logical(k2, 9)
    t1 = k1 & 511
    t2 = k2 & 511
    rowid = lax.broadcasted_iota(I32, (PR, D), 0)
    xf = modulate(jnp.where(rowid == 0, parked(t1, 1)[1], parked(t2, 1)[1]))

    off = pl.multiple_of(jnp.minimum(k2, 0) * 8, 8)
    for j in range(SUB // PR):
        yl, nl = parked(pl.multiple_of(off + j * PR, 8), PR)
        act[row0 + j * PR:row0 + (j + 1) * PR, :] = (
            yl + _rows8(modulate(nl), jnp.multiply, coef[C_GB])).astype(BF16)
    cp_out[1].start()

    gt = _r(jnp.dot(xf.astype(BF16), wa_buf[:, 0:F], preferred_element_type=F32))
    zt = _bits(act[pl.ds(pl.multiple_of(off * 2, PR), PR), 0:128].astype(F32))
    zt = jnp.concatenate([zt[0:8] & zero_buf[...], zt[8:16] & zero_buf[...]], axis=0)
    xs = jnp.concatenate([_float(_bits(xf[:, 0:128]) | zt), xf[:, 128:]], axis=1).astype(BF16)
    up = _r(jnp.dot(xs, wb_buf[:, 0:F], preferred_element_type=F32))
    hid = (_r(gt * _r(jax.nn.sigmoid(gt))) * up).astype(BF16)
    y = _r(jnp.dot(hid, wd_buf[:, 0:D], preferred_element_type=F32))
    y1 = _r(y[0:1, :] * _r(jax.nn.sigmoid(_r(m1 + rc_buf[1:2, 0:1]))))
    y2 = _r(y[1:2, :] * _r(jax.nn.sigmoid(_r(m2 + rc_buf[1:2, 0:1]))))

    def fix(i, t):
        g = pl.multiple_of(lax.shift_right_logical(i, 4) * PR, PR)
        tg = pl.multiple_of(lax.shift_right_logical(t, 4) * PR, PR)
        rid = rowid + g
        upd = jnp.where(rid == i1, y1, jnp.where(rid == i2, y2, 0.0))
        yg, ng = parked(tg, PR)
        return g, (yg + _rows8(modulate(ng) + upd, jnp.multiply, coef[C_GB])).astype(BF16)

    g1, fix1 = fix(i1, t1)
    g2, fix2 = fix(i2, t2)
    wait(cp_out)
    act[pl.ds(g1, PR), :] = fix1
    act[pl.ds(g2, PR), :] = fix2
    f1 = cp(act.at[pl.ds(g1, PR), :], out_hbm.at[pl.ds(g1, PR), :], SEM_OUT)
    f2 = cp(act.at[pl.ds(g2, PR), :], out_hbm.at[pl.ds(g2, PR), :], SEM_FIX)
    f1.start()

    @pl.when(g1 != g2)
    def _():
        f2.start()
        f2.wait()

    f1.wait()


@jax.jit
def pallas_adaLN_cond__mha_block_cached__moe_arch_mod__prompt_kernel(
    A_x: jax.Array,
    A_k_cache: jax.Array,
    A_v_cache: jax.Array,
    A_wq: jax.Array,
    A_wo: jax.Array,
    B_x: jax.Array,
    B_w_r: jax.Array,
    B_w_gate: jax.Array,
    B_w_up: jax.Array,
    B_w_down: jax.Array,
    c: jax.Array,
    w_mod: jax.Array,
):
    del B_x
    hbm = pl.BlockSpec(memory_space=pl.ANY)
    out = pl.pallas_call(
        _kernel,
        in_specs=[hbm] * 11,
        out_specs=hbm,
        out_shape=jax.ShapeDtypeStruct((S, D), BF16),
        scratch_shapes=[
            pltpu.VMEM((S, D), BF16),
            pltpu.VMEM((H, S, DH), BF16),
            pltpu.VMEM((H, S, DH), BF16),
            pltpu.VMEM((H, D, DH), BF16),
            pltpu.VMEM((H, DH, D), BF16),
            pltpu.VMEM((D, F + PAD), BF16),
            pltpu.VMEM((D, F + PAD), BF16),
            pltpu.VMEM((F, D + PAD), BF16),
            pltpu.VMEM((S + PR, D), BF16),
            pltpu.VMEM((S, D), F32),
            pltpu.VMEM((NST, 2 * SUB, 128), F32),
            pltpu.VMEM((R2, 2 * SUB, DH), F32),
            pltpu.VMEM((SUB + 2 * PR, D), F32),
            pltpu.VMEM((2, SUB + 2 * PR, 128), F32),
            pltpu.VMEM((PR, 128), F32),
            pltpu.VMEM((5, 8, D), F32),
            pltpu.VMEM((8, 128), BF16),
            pltpu.VMEM((8, D), F32),
            pltpu.VMEM((8, 128), F32),
            pltpu.VMEM((1, D), BF16),
            pltpu.VMEM((16, D), BF16),
            pltpu.VMEM((D, 128), F32),
            pltpu.VMEM((8, 128), I32),
            pltpu.VMEM((FILL, DH), F32),
            pltpu.VMEM((2, SUB, DH), F32),
            pltpu.VMEM((2, SUB, DH), F32),
            pltpu.SemaphoreType.DMA((NSEM,)),
        ],
        compiler_params=pltpu.CompilerParams(
            vmem_limit_bytes=120 * 1024 * 1024,
            disable_bounds_checks=True,
            disable_semaphore_checks=True,
        ),
        name="adaln_mha_mod",
    )(
        A_x.reshape(S, D),
        A_k_cache.reshape(H, S, DH),
        A_v_cache.reshape(H, S, DH),
        A_wq,
        A_wo.reshape(H, DH, D),
        B_w_r.reshape(8, 128),
        B_w_gate,
        B_w_up,
        B_w_down,
        c,
        w_mod,
    )
    return out.reshape(1, S, D)
```

```python
import jax
import jax.numpy as jnp
from jax import lax
import jax.experimental.pallas as pl
import jax.experimental.pallas.tpu as pltpu

S = 2048
D = 1024
H = 32
DH = 128
F = 3584
SUB = 256
NRB = S // SUB
NU = H * NRB
PR = 16
UM = 14
GE = 8
R2 = 9
RAMP = 2 * R2
NM = (NU - RAMP) // UM
HPI = UM // 2
NLOAD = (2 * H - RAMP) // UM
FIN_START = 130
K_MOD = (FIN_START - RAMP) // UM
LN_START = RAMP + UM
assert LN_START <= 33 and LN_START + (S - 2 * SUB) // PR <= RAMP + K_MOD * UM
FILL = 64
ECH = 64
PAD = 128
NST = D // 128
MVC = 1280
EPS = 1e-5
QSCALE = float(DH ** -0.5) * 1.4426950408889634

F32 = jnp.float32
BF16 = jnp.bfloat16
I32 = jnp.int32
NT = (((1,), (1,)), ((), ()))

C_GA, C_SCALE, C_SHIFT, C_KEEP, C_GB = range(5)


def _r(v):
    return v.astype(BF16).astype(F32)


def _bits(v):
    return lax.bitcast_convert_type(v, I32)


def _float(v):
    return lax.bitcast_convert_type(v, F32)


def _rows8(v, fn, c):
    n = v.shape[0] // 8
    return fn(v.reshape(n, 8, D), c[None]).reshape(v.shape)


def _ln_stats(y):
    m = jnp.mean(y, axis=-1, keepdims=True)
    yc = y - m
    v = jnp.mean(yc * yc, axis=-1, keepdims=True)
    den = _r(jnp.sqrt(_r(_r(v) + EPS)))
    return yc, m, _r(m), 1.0 / den


def _layernorm(y):
    _, _, mr, rinv = _ln_stats(y)
    return (y - mr) * rinv


def _lane_fold(p, fn):
    t = p[:, 0:128]
    for j in range(1, p.shape[1] // 128):
        t = fn(t, p[:, j * 128:(j + 1) * 128])
    return t


def _normalize(pv, ls):
    l = jnp.sum(ls, axis=-1, keepdims=True)
    r = pl.reciprocal(l, approx=True)
    r = r * (2.0 - l * r)
    return (pv * r).astype(BF16)


def _head_of(n):
    if isinstance(n, int):
        return (n % 64) // 2 if n < 192 else (n - 192) % H
    return jnp.where(n < 192, lax.shift_right_logical(n & 63, 1), (n - 192) & (H - 1))


def _row_of(n):
    if isinstance(n, int):
        return SUB * ((n // 64) * 2 + n % 2 if n < 192 else min(n // 32, NRB - 1))
    rb = jnp.where(n < 192, lax.shift_right_logical(n, 6) * 2 + (n & 1),
                   jnp.minimum(lax.shift_right_logical(n, 5), NRB - 1))
    return pl.multiple_of(rb * SUB, SUB)


(SEM_C, SEM_WR, SEM_X0, SEM_X1, SEM_XR, SEM_M12, SEM_FFN, SEM_OUT, SEM_FIX,
 SEM_K0, SEM_WQE, SEM_M0) = range(12)
SEM_W0 = SEM_M0 + NST
SEM_RAMP = SEM_W0 + NST
SEM_MAIN = SEM_RAMP + R2
NSEM = SEM_MAIN + NLOAD


def _kernel(x_hbm, k_hbm, v_hbm, wq_hbm, wo_hbm, wr_hbm, wg_hbm, wu_hbm, wd_hbm,
            c_hbm, wmod_hbm, out_hbm,
            x_buf, k_buf, v_buf, wq_buf, wo_buf, wa_buf, wb_buf, wd_buf,
            act, acc, n_buf, q_acc, x2_buf, st_buf, r_buf, coef, wr_buf, sw_buf, rc_buf,
            c_buf, sc_buf, scol, zero_buf, qa_car, pv_car, ls_car,
            sems):
    def cp(src, dst, slot):
        return pltpu.make_async_copy(src, dst, sems.at[slot])

    def cp_x(b, nb, slot):
        return cp(x_hbm.at[pl.ds(b * SUB, nb * SUB), :],
                  x_buf.at[pl.ds(b * SUB, nb * SUB), :], slot)

    def cp_wq(h, slot):
        col = h * DH if isinstance(h, int) else pl.multiple_of(h * DH, DH)
        return cp(wq_hbm.at[:, pl.ds(col, DH)], wq_buf.at[h], slot)

    def cp_h(src, dst, h0, nh, slot):
        return cp(src.at[pl.ds(h0, nh)], dst.at[pl.ds(h0, nh)], slot)

    def heads(h0, nh, slot, last=False):
        return [cp_h(k_hbm, k_buf, h0, nh, slot), cp_h(v_hbm, v_buf, h0, nh, slot),
                cp_h(wo_hbm, wo_buf, h0 - 1, nh + 1 if last else nh, slot)] + [
            cp_wq(h0 + 1 + j, slot) for j in range(nh - 1 if last else nh)]

    def ramp_heads(j):
        return [cp_h(k_hbm, k_buf, j, 1, SEM_RAMP + j), cp_h(v_hbm, v_buf, j, 1, SEM_RAMP + j),
                cp_h(wo_hbm, wo_buf, j - 1, 1, SEM_RAMP + j)]

    def main_heads(k, last=False):
        h0 = R2 + k * HPI
        return heads(h0, H - h0 if last else HPI, SEM_MAIN + k, last)

    cp_k0 = cp_h(k_hbm, k_buf, 0, 1, SEM_K0)
    cp_v0 = [cp_h(v_hbm, v_buf, 0, 1, SEM_RAMP)] + [cp_wq(h, SEM_RAMP) for h in range(GE, R2 + 1)]
    cp_wqe = [cp_wq(h, SEM_WQE) for h in range(GE)]

    def lanes(j):
        return pl.ds(j * 128 if isinstance(j, int) else pl.multiple_of(j * 128, 128), 128)

    def cp_m0(j):
        return [cp(wmod_hbm.at[:, lanes(u * NST + j)],
                   v_buf.at[H - NST + j, u * D:(u + 1) * D, :], SEM_M0 + j) for u in range(2)]

    def cp_w0(j):
        return cp(wq_hbm.at[lanes(j), 0:GE * DH], wb_buf.at[lanes(j), 0:GE * DH], SEM_W0 + j)

    cp_c = cp(c_hbm, c_buf, SEM_C)
    cp_wr = cp(wr_hbm, wr_buf, SEM_WR)
    cp_m12 = [cp(wmod_hbm.at[:, 2 * D:3 * D], wa_buf.at[:, 2 * D:3 * D], SEM_M12),
              cp(wmod_hbm.at[:, 3 * D:6 * D], wb_buf.at[:, 0:3 * D], SEM_M12)]
    cp_ffn = [cp(wg_hbm, wa_buf.at[:, 0:F], SEM_FFN),
              cp(wu_hbm, wb_buf.at[:, 0:F], SEM_FFN),
              cp(wd_hbm, wd_buf.at[:, 0:D], SEM_FFN)]

    row0 = (NRB - 1) * SUB
    cp_out = [cp(act.at[0:row0, :], out_hbm.at[0:row0, :], SEM_OUT),
              cp(act.at[row0:S, :], out_hbm.at[row0:S, :], SEM_OUT)]

    def vpu_matvec(w_ref, ncols):
        parts = []
        zf = None
        for cc in range(0, ncols, 256):
            a = None if zf is None else jnp.concatenate([zf, zf], axis=1)
            for g in range(D // 8):
                wv = w_ref[g * 8:(g + 1) * 8, cc:cc + 256].astype(F32)
                sv = scol[g * 8:(g + 1) * 8, :]
                pr = jnp.concatenate([wv[:, 0:128] * sv, wv[:, 128:256] * sv], axis=1)
                a = pr if a is None else a + pr
            zf = _float(_lane_fold(_bits(a), jnp.bitwise_or) & zero_buf[...])
            parts.append(a)
        return jnp.sum(jnp.concatenate(parts, axis=1), axis=0, keepdims=True)

    def modulate(n):
        n = _rows8(n, jnp.multiply, coef[C_SCALE])
        return _rows8(n, jnp.add, coef[C_SHIFT])

    def resid(a, row, nrows):
        a = _rows8(a, jnp.multiply, coef[C_GA])
        return _r(x_buf[pl.ds(row, nrows), :].astype(F32) + a)

    def piece(src, dst, lane_id):
        y = resid(acc[pl.ds(src, PR), :], src, PR)
        nn = _layernorm(y)
        hh = modulate(nn)
        r = jnp.sum(_rows8(nn, jnp.multiply, sw_buf[...]), axis=-1, keepdims=True)
        oo = (_rows8(y, jnp.multiply, coef[C_KEEP])
              + _rows8(hh, jnp.multiply, coef[C_GB]))
        act[pl.ds(dst, PR), :] = oo.astype(BF16)
        lane = lax.broadcasted_iota(I32, (PR, 128), 1)
        rn = jnp.where(lane == lane_id, r, r_buf[...])
        r_buf[...] = rn
        return oo, rn

    def unit_piece(n):
        is_ln = jnp.logical_and(n >= LN_START, n < LN_START + (S - 2 * SUB) // PR)
        is_fin = jnp.logical_and(n >= FIN_START, n < FIN_START + (S - SUB) // PR)
        f = n - FIN_START
        src = jnp.where(is_ln, 2 * SUB + (n - LN_START) * PR, jnp.where(is_fin, f * PR, 0))
        dst = jnp.where(jnp.logical_or(is_ln, is_fin), src, S)
        oo, rn = piece(pl.multiple_of(src, PR), pl.multiple_of(dst, PR),
                       jnp.where(is_fin, f, -1))
        bits = _lane_fold(_bits(oo), jnp.bitwise_or) | _bits(rn)
        return (bits[0:8] | bits[8:16]) & zero_buf[...]

    def qproj_head(n):
        return jnp.dot(act[pl.ds(_row_of(n), FILL), 0:D // 2],
                       wq_buf[_head_of(n)][0:D // 2], preferred_element_type=F32)

    def qproj_rest(n, qa):
        row = _row_of(n)
        w = wq_buf[_head_of(n)]
        row2 = row + FILL if isinstance(row, int) else pl.multiple_of(row + FILL, 16)
        qb = jnp.dot(act[pl.ds(row, SUB), D // 2:D], w[D // 2:D], preferred_element_type=F32)
        qc = jnp.dot(act[pl.ds(row2, SUB - FILL), 0:D // 2], w[0:D // 2],
                     preferred_element_type=F32)
        return ((qb + jnp.concatenate([qa, qc], axis=0)) * QSCALE).astype(BF16)

    def oproj(o, n):
        acc[pl.ds(_row_of(n), SUB), :] += jnp.dot(o, wo_buf[_head_of(n)],
                                                  preferred_element_type=F32)

    def unit_block(n0, nunits):
        o = _normalize(pv_car[0], ls_car[0])
        raw = (pv_car[1], ls_car[1])
        qa = qa_car[...]
        for u in range(nunits):
            n = n0 + u
            hd = _head_of(n)
            q = qproj_rest(n, qa)
            z = unit_piece(n)
            oproj(o, n - 2)
            sc = lax.dot_general(q, k_buf[hd], NT, preferred_element_type=F32)
            qa = qproj_head(n + 1)
            mm = _lane_fold(sc, jnp.maximum)
            mm = jnp.concatenate([_float(_bits(mm[0:8]) | z), mm[8:]], axis=0)
            m = jnp.max(mm, axis=-1, keepdims=True)
            p = jnp.exp2(sc - m)
            ls = _lane_fold(p, jnp.add)
            pv = jnp.dot(p.astype(BF16), v_buf[hd], preferred_element_type=F32)
            if u + 1 < nunits:
                zb = (_bits(pv).reshape(SUB // 8, 8, 128)
                      & zero_buf[...][None]).reshape(SUB, 128)
                o = _normalize(raw[0], _float(_bits(raw[1]) | zb))
            else:
                pv_car[0] = raw[0]
                ls_car[0] = raw[1]
            raw = (pv, ls)
        pv_car[1] = raw[0]
        ls_car[1] = raw[1]
        qa_car[...] = qa

    def ramp_block(j):
        o = [_normalize(pv_car[u], ls_car[u]) for u in range(2)]
        w = wo_buf[j - 1]

        def op_part(u, r0, r1, c0, c1):
            acc[u * SUB + r0:u * SUB + r1, c0:c1] += jnp.dot(
                o[u][r0:r1], w[:, c0:c1], preferred_element_type=F32)

        for u in range(2):
            q = (q_acc[j, u * SUB:(u + 1) * SUB, :] * QSCALE).astype(BF16)
            sc = lax.dot_general(q, k_buf[j], NT, preferred_element_type=F32)
            op_part(u, 0, FILL, 0, D // 2)
            m = jnp.max(_lane_fold(sc, jnp.maximum), axis=-1, keepdims=True)
            p = jnp.exp2(sc - m)
            ls_car[u] = _lane_fold(p, jnp.add)
            pv_car[u] = jnp.dot(p.astype(BF16), v_buf[j], preferred_element_type=F32)
            if u == 0:
                for v in range(2):
                    op_part(v, FILL, SUB, 0, D // 2)
                    op_part(v, 0, SUB, D // 2, D)

    def start(cps):
        for c_ in cps:
            c_.start()

    def wait(cps):
        for c_ in cps:
            c_.wait()

    start([cp_c, cp_x(0, 1, SEM_X0), cp_x(1, 1, SEM_X1)])
    for j in range(NST):
        start(cp_m0(j) + [cp_w0(j)])
    start([cp_k0] + cp_v0)
    for j in range(1, R2):
        start(ramp_heads(j))
    start([cp_wr])
    n_early = (LN_START - RAMP) // UM
    for k in range(n_early):
        start(main_heads(k))

    r_buf[...] = jnp.zeros(r_buf.shape, F32)
    zero_buf[...] = jnp.zeros(zero_buf.shape, I32)
    coef[C_GA] = jnp.zeros((8, D), F32)
    coef[C_KEEP] = jnp.zeros((8, D), F32)
    coef[C_GB] = jnp.ones((8, D), F32)
    sw_buf[...] = jnp.zeros(sw_buf.shape, F32)

    def zero_q(h, carry):
        q_acc[h] = jnp.zeros((2 * SUB, DH), F32)
        return carry

    lax.fori_loop(0, GE, zero_q, 0)
    cp_c.wait()
    cf = c_buf[...].astype(F32)
    sf = _r(cf * _r(jax.nn.sigmoid(cf)))
    sc_buf[...] = jnp.broadcast_to(sf, (16, D)).astype(BF16)
    for j in range(D // 128):
        scol[j * 128:(j + 1) * 128, :] = jnp.broadcast_to(
            sf[:, j * 128:(j + 1) * 128], (128, 128)).T

    def norm_rows(j, carry):
        @pl.when((j & 1) == 0)
        def _():
            b = lax.shift_right_logical(j, 1)
            cp_x(b, 1, SEM_X0 + b).wait()

        row = pl.multiple_of(j * 128, 128)
        nn = _layernorm(x_buf[pl.ds(row, 128), :].astype(F32))
        for t in range(NST):
            n_buf[t, pl.ds(row, 128), :] = nn[:, t * 128:(t + 1) * 128]
        return carry

    lax.fori_loop(0, 2 * SUB // 128, norm_rows, 0)

    def stage(j, carry):
        wait(cp_m0(j))
        wm = jnp.concatenate([v_buf[H - NST + j, 0:D, :], v_buf[H - NST + j, D:2 * D, :]], axis=1)
        mj = _r(jnp.dot(sc_buf[...], wm, preferred_element_type=F32)[0:8, :])
        coef[C_SHIFT, :, lanes(j)] = mj[:, 0:128]
        coef[C_SCALE, :, lanes(j)] = _r(1.0 + mj[:, 128:256])
        zr = S // NST
        acc[pl.ds(pl.multiple_of(j * zr, zr), zr), :] = jnp.zeros((zr, D), F32)
        cp_w0(j).wait()
        hj = (n_buf[j].reshape(2 * SUB // 8, 8, 128) * coef[C_SCALE, :, lanes(j)][None]
              + coef[C_SHIFT, :, lanes(j)][None]).reshape(2 * SUB, 128).astype(BF16)
        act[0:2 * SUB, lanes(j)] = hj
        part = jnp.dot(hj, wb_buf[lanes(j), 0:GE * DH], preferred_element_type=F32)
        for h in range(GE):
            q_acc[h] += part[:, h * DH:(h + 1) * DH]
        return carry

    lax.fori_loop(0, NST, stage, 0)

    cp_k0.wait()
    s01 = lax.dot_general((q_acc[0] * QSCALE).astype(BF16), k_buf[0], NT,
                          preferred_element_type=F32)
    mm01 = _lane_fold(s01, jnp.maximum)
    m0 = jnp.max(mm01[0:SUB], axis=-1, keepdims=True)
    wait(cp_v0)
    qa_car[...] = qproj_head(RAMP)
    for u in range(2):
        m = m0 if u == 0 else jnp.max(mm01[SUB:], axis=-1, keepdims=True)
        p = jnp.exp2(s01[u * SUB:(u + 1) * SUB] - m)
        ls_car[u] = _lane_fold(p, jnp.add)
        pv_car[u] = jnp.dot(p.astype(BF16), v_buf[0], preferred_element_type=F32)
    for h in range(GE, R2):
        q_acc[h] = jnp.dot(act[0:2 * SUB, :], wq_buf[h], preferred_element_type=F32)

    def ramp2(j, carry):
        wait(ramp_heads(j))
        ramp_block(j)
        return carry

    lax.fori_loop(1, R2, ramp2, 0)
    start([cp_x(2, NRB - 2, SEM_XR)])
    for k in range(n_early, NLOAD):
        start(main_heads(k, k == NLOAD - 1))
    start(cp_wqe + cp_m12)

    assert FIN_START + row0 // PR <= RAMP + (NM - 1) * UM

    def main(k, carry):
        n0 = RAMP + k * UM

        @pl.when(k <= K_MOD + 2)
        def _():
            @pl.when(k < NLOAD - 1)
            def _():
                wait(main_heads(k))

            @pl.when(k == NLOAD - 1)
            def _():
                wait(main_heads(NLOAD - 1, True) + cp_wqe)

            @pl.when(k == n_early)
            def _():
                cp_x(2, NRB - 2, SEM_XR).wait()

            @pl.when(k == K_MOD)
            def _():
                wait(cp_m12 + [cp_wr])
                sc = sc_buf[...]
                m2a = jnp.dot(sc, wb_buf[:, MVC:3 * D], preferred_element_type=F32)[0:8, :]
                m1 = _r(jnp.dot(sc, wa_buf[:, 2 * D:3 * D], preferred_element_type=F32)[0:8, :])
                m2b = jnp.broadcast_to(vpu_matvec(wb_buf, MVC), (8, MVC))
                m2 = _r(jnp.concatenate([m2b, m2a], axis=1))
                coef[C_GA] = m1
                coef[C_KEEP] = jnp.ones((8, D), F32)
                scale = _r(1.0 + m2[:, D:2 * D])
                coef[C_SHIFT] = m2[:, 0:D]
                coef[C_SCALE] = scale
                coef[C_GB] = m2[:, 2 * D:3 * D]
                w8 = wr_buf[...].astype(F32)
                wr = jnp.concatenate([jnp.broadcast_to(w8[j:j + 1, :], (8, 128))
                                      for j in range(D // 128)], axis=1)
                sw_buf[...] = scale * wr
                c1 = jnp.sum(scale * wr, axis=-1, keepdims=True)
                c0 = jnp.sum(m2[:, 0:D] * wr, axis=-1, keepdims=True)
                rid = lax.broadcasted_iota(I32, (8, 128), 0)
                rc_buf[...] = jnp.where(rid == 0, c1, c0)
                start(cp_ffn)

            @pl.when(k == K_MOD + 2)
            def _():
                wait(cp_ffn)

        @pl.when(k == NM - 1)
        def _():
            cp_out[0].start()

        unit_block(n0, UM)
        return carry

    lax.fori_loop(0, NM, main, 0)

    neg = -jnp.inf

    def keep_rows(y, lo):
        n = y.shape[0]
        yc, m, mr, rinv = _ln_stats(y)
        x2_buf[lo:lo + n, :] = y
        st_buf[0, lo:lo + n, :] = jnp.broadcast_to(mr, (n, 128))
        st_buf[1, lo:lo + n, :] = jnp.broadcast_to(rinv, (n, 128))
        d = jnp.sum(_rows8(yc, jnp.multiply, sw_buf[...]), axis=-1, keepdims=True)
        return (d + (m - mr) * rc_buf[0:1, 0:1]) * rinv

    def parked(lo, n):
        y = x2_buf[pl.ds(lo, n), :]
        mr = st_buf[0, pl.ds(lo, n), :]
        rinv = st_buf[1, pl.ds(lo, n), :]
        return y, jnp.concatenate([(y[:, j * 128:(j + 1) * 128] - mr) * rinv
                                   for j in range(D // 128)], axis=1)

    def all_red(v, fn):
        return fn(fn(v, axis=0, keepdims=True), axis=1, keepdims=True)

    lane = lax.broadcasted_iota(I32, (PR, 128), 1)
    ridx = (lane * PR + lax.broadcasted_iota(I32, (PR, 128), 0)).astype(F32)
    rr = jnp.where(lane < row0 // PR, r_buf[...], neg)
    last_old = float(row0 - 1)
    cm1 = all_red(rr, jnp.max)
    ci1 = all_red(jnp.where(rr == cm1, ridx, last_old), jnp.min)
    rr2 = jnp.where(ridx == ci1, neg, rr)
    cm2 = all_red(rr2, jnp.max)
    ci2 = all_red(jnp.where(jnp.logical_and(rr2 == cm2, ridx != ci1), ridx, last_old), jnp.min)
    ci1 = jnp.minimum(ci1, last_old).astype(I32)
    ci2 = jnp.minimum(ci2, last_old).astype(I32)
    for j, ci in enumerate((ci1, ci2)):
        g = pl.multiple_of(lax.shift_right_logical(ci[0, 0], 4) * PR, PR)
        keep_rows(resid(acc[pl.ds(g, PR), :], g, PR), SUB + j * PR)

    o2 = jnp.concatenate([_normalize(pv_car[0], ls_car[0]),
                          _normalize(pv_car[1], ls_car[1])], axis=1)
    wo2 = jnp.concatenate([wo_buf[H - 2], wo_buf[H - 1]], axis=0)
    r_new = []
    for j in range(SUB // ECH):
        lo, hi = j * ECH, (j + 1) * ECH
        a = acc[row0 + lo:row0 + hi, :] + jnp.dot(o2[lo:hi], wo2, preferred_element_type=F32)
        r_new.append(keep_rows(resid(a, row0 + lo, ECH), lo))

    sub8 = lax.broadcasted_iota(I32, (8, 1), 0)
    big = jnp.int32((S - 1) * 512 + SUB - 1)
    vals = jnp.concatenate(
        r_new + [jnp.where(sub8 == 0, cm1, jnp.where(sub8 == 1, cm2, neg))], axis=0)
    pos = lax.broadcasted_iota(I32, (SUB, 1), 0)
    cc1 = ci1 * 512 + SUB + (ci1 & (PR - 1))
    cc2 = ci2 * 512 + SUB + PR + (ci2 & (PR - 1))
    code = jnp.concatenate(
        [(pos + row0) * 512 + pos,
         jnp.where(sub8 == 0, cc1, jnp.where(sub8 == 1, cc2, big))], axis=0)
    m1 = jnp.max(vals, axis=0, keepdims=True)
    k1 = jnp.min(jnp.where(vals == m1, code, big), axis=0, keepdims=True)
    vals2 = jnp.where(code == k1, neg, vals)
    m2 = jnp.max(vals2, axis=0, keepdims=True)
    k2 = jnp.min(jnp.where(jnp.logical_and(vals2 == m2, code != k1), code, big),
                 axis=0, keepdims=True)
    k1 = k1[0, 0]
    k2 = k2[0, 0]
    i1 = lax.shift_right_logical(k1, 9)
    i2 = lax.shift_right_logical(k2, 9)
    t1 = k1 & 511
    t2 = k2 & 511
    rowid = lax.broadcasted_iota(I32, (PR, D), 0)
    xf = modulate(jnp.where(rowid == 0, parked(t1, 1)[1], parked(t2, 1)[1]))

    off = pl.multiple_of(jnp.minimum(k2, 0) * 8, 8)
    for j in range(SUB // PR):
        yl, nl = parked(pl.multiple_of(off + j * PR, 8), PR)
        act[row0 + j * PR:row0 + (j + 1) * PR, :] = (
            yl + _rows8(modulate(nl), jnp.multiply, coef[C_GB])).astype(BF16)
    cp_out[1].start()

    gt = _r(jnp.dot(xf.astype(BF16), wa_buf[:, 0:F], preferred_element_type=F32))
    zt = _bits(act[pl.ds(pl.multiple_of(off * 2, PR), PR), 0:128].astype(F32))
    zt = jnp.concatenate([zt[0:8] & zero_buf[...], zt[8:16] & zero_buf[...]], axis=0)
    xs = jnp.concatenate([_float(_bits(xf[:, 0:128]) | zt), xf[:, 128:]], axis=1).astype(BF16)
    up = _r(jnp.dot(xs, wb_buf[:, 0:F], preferred_element_type=F32))
    hid = (_r(gt * _r(jax.nn.sigmoid(gt))) * up).astype(BF16)
    y = _r(jnp.dot(hid, wd_buf[:, 0:D], preferred_element_type=F32))
    y1 = _r(y[0:1, :] * _r(jax.nn.sigmoid(_r(m1 + rc_buf[1:2, 0:1]))))
    y2 = _r(y[1:2, :] * _r(jax.nn.sigmoid(_r(m2 + rc_buf[1:2, 0:1]))))

    def fix(i, t):
        g = pl.multiple_of(lax.shift_right_logical(i, 4) * PR, PR)
        tg = pl.multiple_of(lax.shift_right_logical(t, 4) * PR, PR)
        rid = rowid + g
        upd = jnp.where(rid == i1, y1, jnp.where(rid == i2, y2, 0.0))
        yg, ng = parked(tg, PR)
        return g, (yg + _rows8(modulate(ng) + upd, jnp.multiply, coef[C_GB])).astype(BF16)

    g1, fix1 = fix(i1, t1)
    g2, fix2 = fix(i2, t2)
    wait(cp_out)
    act[pl.ds(g1, PR), :] = fix1
    act[pl.ds(g2, PR), :] = fix2
    f1 = cp(act.at[pl.ds(g1, PR), :], out_hbm.at[pl.ds(g1, PR), :], SEM_OUT)
    f2 = cp(act.at[pl.ds(g2, PR), :], out_hbm.at[pl.ds(g2, PR), :], SEM_FIX)
    f1.start()

    @pl.when(g1 != g2)
    def _():
        f2.start()
        f2.wait()

    f1.wait()


@jax.jit
def pallas_adaLN_cond__mha_block_cached__moe_arch_mod__prompt_kernel(
    A_x: jax.Array,
    A_k_cache: jax.Array,
    A_v_cache: jax.Array,
    A_wq: jax.Array,
    A_wo: jax.Array,
    B_x: jax.Array,
    B_w_r: jax.Array,
    B_w_gate: jax.Array,
    B_w_up: jax.Array,
    B_w_down: jax.Array,
    c: jax.Array,
    w_mod: jax.Array,
):
    del B_x
    hbm = pl.BlockSpec(memory_space=pl.ANY)
    out = pl.pallas_call(
        _kernel,
        in_specs=[hbm] * 11,
        out_specs=hbm,
        out_shape=jax.ShapeDtypeStruct((S, D), BF16),
        scratch_shapes=[
            pltpu.VMEM((S, D), BF16),
            pltpu.VMEM((H, S, DH), BF16),
            pltpu.VMEM((H, S, DH), BF16),
            pltpu.VMEM((H, D, DH), BF16),
            pltpu.VMEM((H, DH, D), BF16),
            pltpu.VMEM((D, F + PAD), BF16),
            pltpu.VMEM((D, F + PAD), BF16),
            pltpu.VMEM((F, D + PAD), BF16),
            pltpu.VMEM((S + PR, D), BF16),
            pltpu.VMEM((S, D), F32),
            pltpu.VMEM((NST, 2 * SUB, 128), F32),
            pltpu.VMEM((R2, 2 * SUB, DH), F32),
            pltpu.VMEM((SUB + 2 * PR, D), F32),
            pltpu.VMEM((2, SUB + 2 * PR, 128), F32),
            pltpu.VMEM((PR, 128), F32),
            pltpu.VMEM((5, 8, D), F32),
            pltpu.VMEM((8, 128), BF16),
            pltpu.VMEM((8, D), F32),
            pltpu.VMEM((8, 128), F32),
            pltpu.VMEM((1, D), BF16),
            pltpu.VMEM((16, D), BF16),
            pltpu.VMEM((D, 128), F32),
            pltpu.VMEM((8, 128), I32),
            pltpu.VMEM((FILL, DH), F32),
            pltpu.VMEM((2, SUB, DH), F32),
            pltpu.VMEM((2, SUB, DH), F32),
            pltpu.SemaphoreType.DMA((NSEM,)),
        ],
        compiler_params=pltpu.CompilerParams(
            vmem_limit_bytes=120 * 1024 * 1024,
            disable_bounds_checks=True,
            disable_semaphore_checks=True,
        ),
        name="adaln_mha_mod",
    )(
        A_x.reshape(S, D),
        A_k_cache.reshape(H, S, DH),
        A_v_cache.reshape(H, S, DH),
        A_wq,
        A_wo.reshape(H, DH, D),
        B_w_r.reshape(8, 128),
        B_w_gate,
        B_w_up,
        B_w_down,
        c,
        w_mod,
    )
    return out.reshape(1, S, D)
```

```python
import jax
import jax.numpy as jnp
from jax import lax
import jax.experimental.pallas as pl
import jax.experimental.pallas.tpu as pltpu

S = 2048
D = 1024
H = 32
DH = 128
F = 3584
SUB = 256
NRB = S // SUB
NU = H * NRB
PR = 16
UM = 14
GE = 8
R2 = 9
RAMP = 2 * R2
NM = (NU - RAMP) // UM
HPI = UM // 2
NLOAD = (2 * H - RAMP) // UM
FIN_START = 130
K_MOD = (FIN_START - RAMP) // UM
LN_START = RAMP + UM
assert LN_START <= 33 and LN_START + (S - 2 * SUB) // PR <= RAMP + K_MOD * UM
FILL = 64
ECH = 64
PAD = 128
NST = D // 128
MVC = 1280
EPS = 1e-5
QSCALE = float(DH ** -0.5) * 1.4426950408889634

F32 = jnp.float32
BF16 = jnp.bfloat16
I32 = jnp.int32
NT = (((1,), (1,)), ((), ()))

C_GA, C_SCALE, C_SHIFT, C_KEEP, C_GB = range(5)


def _r(v):
    return v.astype(BF16).astype(F32)


def _bits(v):
    return lax.bitcast_convert_type(v, I32)


def _float(v):
    return lax.bitcast_convert_type(v, F32)


def _rows8(v, fn, c):
    n = v.shape[0] // 8
    return fn(v.reshape(n, 8, D), c[None]).reshape(v.shape)


def _ln_stats(y):
    m = jnp.mean(y, axis=-1, keepdims=True)
    yc = y - m
    v = jnp.mean(yc * yc, axis=-1, keepdims=True)
    den = _r(jnp.sqrt(_r(_r(v) + EPS)))
    return yc, m, _r(m), 1.0 / den


def _layernorm(y):
    _, _, mr, rinv = _ln_stats(y)
    return (y - mr) * rinv


def _lane_fold(p, fn):
    t = p[:, 0:128]
    for j in range(1, p.shape[1] // 128):
        t = fn(t, p[:, j * 128:(j + 1) * 128])
    return t


def _normalize(pv, ls):
    l = jnp.sum(ls, axis=-1, keepdims=True)
    r = pl.reciprocal(l, approx=True)
    r = r * (2.0 - l * r)
    return (pv * r).astype(BF16)


def _head_of(n):
    if isinstance(n, int):
        return (n % 64) // 2 if n < 192 else (n - 192) % H
    return jnp.where(n < 192, lax.shift_right_logical(n & 63, 1), (n - 192) & (H - 1))


def _row_of(n):
    if isinstance(n, int):
        return SUB * ((n // 64) * 2 + n % 2 if n < 192 else min(n // 32, NRB - 1))
    rb = jnp.where(n < 192, lax.shift_right_logical(n, 6) * 2 + (n & 1),
                   jnp.minimum(lax.shift_right_logical(n, 5), NRB - 1))
    return pl.multiple_of(rb * SUB, SUB)


(SEM_C, SEM_WR, SEM_X0, SEM_X1, SEM_XR, SEM_M12, SEM_FFN, SEM_OUT, SEM_FIX,
 SEM_K0, SEM_WQE, SEM_M0) = range(12)
SEM_W0 = SEM_M0 + NST
SEM_RAMP = SEM_W0 + NST
SEM_MAIN = SEM_RAMP + R2
NSEM = SEM_MAIN + NLOAD


def _kernel(x_hbm, k_hbm, v_hbm, wq_hbm, wo_hbm, wr_hbm, wg_hbm, wu_hbm, wd_hbm,
            c_hbm, wmod_hbm, out_hbm,
            x_buf, k_buf, v_buf, wq_buf, wo_buf, wa_buf, wb_buf, wd_buf,
            act, acc, n_buf, q_acc, x2_buf, st_buf, r_buf, coef, wr_buf, sw_buf, rc_buf,
            c_buf, sc_buf, scol, zero_buf, qa_car, pv_car, ls_car,
            sems):
    def cp(src, dst, slot):
        return pltpu.make_async_copy(src, dst, sems.at[slot])

    def cp_x(b, nb, slot):
        return cp(x_hbm.at[pl.ds(b * SUB, nb * SUB), :],
                  x_buf.at[pl.ds(b * SUB, nb * SUB), :], slot)

    def cp_wq(h, slot):
        col = h * DH if isinstance(h, int) else pl.multiple_of(h * DH, DH)
        return cp(wq_hbm.at[:, pl.ds(col, DH)], wq_buf.at[h], slot)

    def cp_h(src, dst, h0, nh, slot):
        return cp(src.at[pl.ds(h0, nh)], dst.at[pl.ds(h0, nh)], slot)

    def heads(h0, nh, slot, last=False):
        return [cp_h(k_hbm, k_buf, h0, nh, slot), cp_h(v_hbm, v_buf, h0, nh, slot),
                cp_h(wo_hbm, wo_buf, h0 - 1, nh + 1 if last else nh, slot)] + [
            cp_wq(h0 + 1 + j, slot) for j in range(nh - 1 if last else nh)]

    def ramp_heads(j):
        return [cp_h(k_hbm, k_buf, j, 1, SEM_RAMP + j), cp_h(v_hbm, v_buf, j, 1, SEM_RAMP + j),
                cp_h(wo_hbm, wo_buf, j - 1, 1, SEM_RAMP + j)]

    def main_heads(k, last=False):
        h0 = R2 + k * HPI
        return heads(h0, H - h0 if last else HPI, SEM_MAIN + k, last)

    cp_k0 = cp_h(k_hbm, k_buf, 0, 1, SEM_K0)
    cp_v0 = [cp_h(v_hbm, v_buf, 0, 1, SEM_RAMP)] + [cp_wq(h, SEM_RAMP) for h in range(GE, R2 + 1)]
    cp_wqe = [cp_wq(h, SEM_WQE) for h in range(GE)]

    def lanes(j):
        return pl.ds(j * 128 if isinstance(j, int) else pl.multiple_of(j * 128, 128), 128)

    def cp_m0(j):
        return [cp(wmod_hbm.at[:, lanes(u * NST + j)],
                   v_buf.at[H - NST + j, u * D:(u + 1) * D, :], SEM_M0 + j) for u in range(2)]

    def cp_w0(j):
        return cp(wq_hbm.at[lanes(j), 0:GE * DH], wb_buf.at[lanes(j), 0:GE * DH], SEM_W0 + j)

    cp_c = cp(c_hbm, c_buf, SEM_C)
    cp_wr = cp(wr_hbm, wr_buf, SEM_WR)
    cp_m12 = [cp(wmod_hbm.at[:, 2 * D:3 * D], wa_buf.at[:, 2 * D:3 * D], SEM_M12),
              cp(wmod_hbm.at[:, 3 * D:6 * D], wb_buf.at[:, 0:3 * D], SEM_M12)]
    cp_ffn = [cp(wg_hbm, wa_buf.at[:, 0:F], SEM_FFN),
              cp(wu_hbm, wb_buf.at[:, 0:F], SEM_FFN),
              cp(wd_hbm, wd_buf.at[:, 0:D], SEM_FFN)]

    row0 = (NRB - 1) * SUB
    cp_out = [cp(act.at[0:row0, :], out_hbm.at[0:row0, :], SEM_OUT),
              cp(act.at[row0:S, :], out_hbm.at[row0:S, :], SEM_OUT)]

    def vpu_matvec(w_ref, ncols):
        parts = []
        zf = None
        for cc in range(0, ncols, 256):
            a = None if zf is None else jnp.concatenate([zf, zf], axis=1)
            for g in range(D // 8):
                wv = w_ref[g * 8:(g + 1) * 8, cc:cc + 256].astype(F32)
                sv = scol[g * 8:(g + 1) * 8, :]
                pr = jnp.concatenate([wv[:, 0:128] * sv, wv[:, 128:256] * sv], axis=1)
                a = pr if a is None else a + pr
            zf = _float(_lane_fold(_bits(a), jnp.bitwise_or) & zero_buf[...])
            parts.append(a)
        return jnp.sum(jnp.concatenate(parts, axis=1), axis=0, keepdims=True)

    def modulate(n):
        n = _rows8(n, jnp.multiply, coef[C_SCALE])
        return _rows8(n, jnp.add, coef[C_SHIFT])

    def resid(a, row, nrows):
        a = _rows8(a, jnp.multiply, coef[C_GA])
        return _r(x_buf[pl.ds(row, nrows), :].astype(F32) + a)

    def piece(src, dst, lane_id):
        y = resid(acc[pl.ds(src, PR), :], src, PR)
        nn = _layernorm(y)
        hh = modulate(nn)
        r = jnp.sum(_rows8(nn, jnp.multiply, sw_buf[...]), axis=-1, keepdims=True)
        oo = (_rows8(y, jnp.multiply, coef[C_KEEP])
              + _rows8(hh, jnp.multiply, coef[C_GB]))
        act[pl.ds(dst, PR), :] = oo.astype(BF16)
        lane = lax.broadcasted_iota(I32, (PR, 128), 1)
        rn = jnp.where(lane == lane_id, r, r_buf[...])
        r_buf[...] = rn
        return oo, rn

    def unit_piece(n):
        is_ln = jnp.logical_and(n >= LN_START, n < LN_START + (S - 2 * SUB) // PR)
        is_fin = jnp.logical_and(n >= FIN_START, n < FIN_START + (S - SUB) // PR)
        f = n - FIN_START
        src = jnp.where(is_ln, 2 * SUB + (n - LN_START) * PR, jnp.where(is_fin, f * PR, 0))
        dst = jnp.where(jnp.logical_or(is_ln, is_fin), src, S)
        oo, rn = piece(pl.multiple_of(src, PR), pl.multiple_of(dst, PR),
                       jnp.where(is_fin, f, -1))
        bits = _lane_fold(_bits(oo), jnp.bitwise_or) | _bits(rn)
        return (bits[0:8] | bits[8:16]) & zero_buf[...]

    def qproj_head(n):
        return jnp.dot(act[pl.ds(_row_of(n), FILL), 0:D // 2],
                       wq_buf[_head_of(n)][0:D // 2], preferred_element_type=F32)

    def qproj_rest(n, qa):
        row = _row_of(n)
        w = wq_buf[_head_of(n)]
        row2 = row + FILL if isinstance(row, int) else pl.multiple_of(row + FILL, 16)
        qb = jnp.dot(act[pl.ds(row, SUB), D // 2:D], w[D // 2:D], preferred_element_type=F32)
        qc = jnp.dot(act[pl.ds(row2, SUB - FILL), 0:D // 2], w[0:D // 2],
                     preferred_element_type=F32)
        return ((qb + jnp.concatenate([qa, qc], axis=0)) * QSCALE).astype(BF16)

    def oproj(o, n):
        acc[pl.ds(_row_of(n), SUB), :] += jnp.dot(o, wo_buf[_head_of(n)],
                                                  preferred_element_type=F32)

    def unit_block(n0, nunits):
        o = _normalize(pv_car[0], ls_car[0])
        raw = (pv_car[1], ls_car[1])
        qa = qa_car[...]
        for u in range(nunits):
            n = n0 + u
            hd = _head_of(n)
            q = qproj_rest(n, qa)
            z = unit_piece(n)
            oproj(o, n - 2)
            sc = lax.dot_general(q, k_buf[hd], NT, preferred_element_type=F32)
            qa = qproj_head(n + 1)
            mm = _lane_fold(sc, jnp.maximum)
            mm = jnp.concatenate([_float(_bits(mm[0:8]) | z), mm[8:]], axis=0)
            m = jnp.max(mm, axis=-1, keepdims=True)
            p = jnp.exp2(sc - m)
            ls = _lane_fold(p, jnp.add)
            pv = jnp.dot(p.astype(BF16), v_buf[hd], preferred_element_type=F32)
            if u + 1 < nunits:
                zb = (_bits(pv).reshape(SUB // 8, 8, 128)
                      & zero_buf[...][None]).reshape(SUB, 128)
                o = _normalize(raw[0], _float(_bits(raw[1]) | zb))
            else:
                pv_car[0] = raw[0]
                ls_car[0] = raw[1]
            raw = (pv, ls)
        pv_car[1] = raw[0]
        ls_car[1] = raw[1]
        qa_car[...] = qa

    def ramp_block(j):
        o = [_normalize(pv_car[u], ls_car[u]) for u in range(2)]
        w = wo_buf[j - 1]

        def op_part(u, r0, r1, c0, c1):
            acc[u * SUB + r0:u * SUB + r1, c0:c1] += jnp.dot(
                o[u][r0:r1], w[:, c0:c1], preferred_element_type=F32)

        for u in range(2):
            q = (q_acc[j, u * SUB:(u + 1) * SUB, :] * QSCALE).astype(BF16)
            sc = lax.dot_general(q, k_buf[j], NT, preferred_element_type=F32)
            op_part(u, 0, FILL, 0, D // 2)
            m = jnp.max(_lane_fold(sc, jnp.maximum), axis=-1, keepdims=True)
            p = jnp.exp2(sc - m)
            ls_car[u] = _lane_fold(p, jnp.add)
            pv_car[u] = jnp.dot(p.astype(BF16), v_buf[j], preferred_element_type=F32)
            if u == 0:
                for v in range(2):
                    op_part(v, FILL, SUB, 0, D // 2)
                    op_part(v, 0, SUB, D // 2, D)

    def start(cps):
        for c_ in cps:
            c_.start()

    def wait(cps):
        for c_ in cps:
            c_.wait()

    start([cp_c, cp_x(0, 1, SEM_X0), cp_x(1, 1, SEM_X1)])
    for j in range(NST):
        start(cp_m0(j) + [cp_w0(j)])
    start([cp_k0] + cp_v0)
    for j in range(1, R2):
        start(ramp_heads(j))
    start([cp_wr])
    n_early = (LN_START - RAMP) // UM
    for k in range(n_early):
        start(main_heads(k))

    r_buf[...] = jnp.zeros(r_buf.shape, F32)
    zero_buf[...] = jnp.zeros(zero_buf.shape, I32)
    coef[C_GA] = jnp.zeros((8, D), F32)
    coef[C_KEEP] = jnp.zeros((8, D), F32)
    coef[C_GB] = jnp.ones((8, D), F32)
    sw_buf[...] = jnp.zeros(sw_buf.shape, F32)

    def zero_q(h, carry):
        q_acc[h] = jnp.zeros((2 * SUB, DH), F32)
        return carry

    lax.fori_loop(0, GE, zero_q, 0)
    cp_c.wait()
    cf = c_buf[...].astype(F32)
    sf = _r(cf * _r(jax.nn.sigmoid(cf)))
    sc_buf[...] = jnp.broadcast_to(sf, (16, D)).astype(BF16)
    for j in range(D // 128):
        scol[j * 128:(j + 1) * 128, :] = jnp.broadcast_to(
            sf[:, j * 128:(j + 1) * 128], (128, 128)).T

    def norm_rows(j, carry):
        @pl.when((j & 1) == 0)
        def _():
            b = lax.shift_right_logical(j, 1)
            cp_x(b, 1, SEM_X0 + b).wait()

        row = pl.multiple_of(j * 128, 128)
        nn = _layernorm(x_buf[pl.ds(row, 128), :].astype(F32))
        for t in range(NST):
            n_buf[t, pl.ds(row, 128), :] = nn[:, t * 128:(t + 1) * 128]
        return carry

    lax.fori_loop(0, 2 * SUB // 128, norm_rows, 0)

    def stage(j, carry):
        wait(cp_m0(j))
        wm = jnp.concatenate([v_buf[H - NST + j, 0:D, :], v_buf[H - NST + j, D:2 * D, :]], axis=1)
        mj = _r(jnp.dot(sc_buf[...], wm, preferred_element_type=F32)[0:8, :])
        coef[C_SHIFT, :, lanes(j)] = mj[:, 0:128]
        coef[C_SCALE, :, lanes(j)] = _r(1.0 + mj[:, 128:256])
        zr = S // NST
        acc[pl.ds(pl.multiple_of(j * zr, zr), zr), :] = jnp.zeros((zr, D), F32)
        cp_w0(j).wait()
        hj = (n_buf[j].reshape(2 * SUB // 8, 8, 128) * coef[C_SCALE, :, lanes(j)][None]
              + coef[C_SHIFT, :, lanes(j)][None]).reshape(2 * SUB, 128).astype(BF16)
        act[0:2 * SUB, lanes(j)] = hj
        part = jnp.dot(hj, wb_buf[lanes(j), 0:GE * DH], preferred_element_type=F32)
        for h in range(GE):
            q_acc[h] += part[:, h * DH:(h + 1) * DH]
        return carry

    lax.fori_loop(0, NST, stage, 0)

    cp_k0.wait()
    s01 = lax.dot_general((q_acc[0] * QSCALE).astype(BF16), k_buf[0], NT,
                          preferred_element_type=F32)
    mm01 = _lane_fold(s01, jnp.maximum)
    m0 = jnp.max(mm01[0:SUB], axis=-1, keepdims=True)
    wait(cp_v0)
    qa_car[...] = qproj_head(RAMP)
    for u in range(2):
        m = m0 if u == 0 else jnp.max(mm01[SUB:], axis=-1, keepdims=True)
        p = jnp.exp2(s01[u * SUB:(u + 1) * SUB] - m)
        ls_car[u] = _lane_fold(p, jnp.add)
        pv_car[u] = jnp.dot(p.astype(BF16), v_buf[0], preferred_element_type=F32)
    for h in range(GE, R2):
        q_acc[h] = jnp.dot(act[0:2 * SUB, :], wq_buf[h], preferred_element_type=F32)

    def ramp2(j, carry):
        wait(ramp_heads(j))
        ramp_block(j)
        return carry

    lax.fori_loop(1, R2, ramp2, 0)
    start([cp_x(2, NRB - 2, SEM_XR)])
    for k in range(n_early, NLOAD):
        start(main_heads(k, k == NLOAD - 1))
    start(cp_wqe + cp_m12)

    assert FIN_START + row0 // PR <= RAMP + (NM - 1) * UM

    def main(k, carry):
        n0 = RAMP + k * UM

        @pl.when(k <= K_MOD + 2)
        def _():
            @pl.when(k < NLOAD - 1)
            def _():
                wait(main_heads(k))

            @pl.when(k == NLOAD - 1)
            def _():
                wait(main_heads(NLOAD - 1, True) + cp_wqe)

            @pl.when(k == n_early)
            def _():
                cp_x(2, NRB - 2, SEM_XR).wait()

            @pl.when(k == K_MOD)
            def _():
                wait(cp_m12 + [cp_wr])
                sc = sc_buf[...]
                m2a = jnp.dot(sc, wb_buf[:, MVC:3 * D], preferred_element_type=F32)[0:8, :]
                m1 = _r(jnp.dot(sc, wa_buf[:, 2 * D:3 * D], preferred_element_type=F32)[0:8, :])
                m2b = jnp.broadcast_to(vpu_matvec(wb_buf, MVC), (8, MVC))
                m2 = _r(jnp.concatenate([m2b, m2a], axis=1))
                coef[C_GA] = m1
                coef[C_KEEP] = jnp.ones((8, D), F32)
                scale = _r(1.0 + m2[:, D:2 * D])
                coef[C_SHIFT] = m2[:, 0:D]
                coef[C_SCALE] = scale
                coef[C_GB] = m2[:, 2 * D:3 * D]
                w8 = wr_buf[...].astype(F32)
                wr = jnp.concatenate([jnp.broadcast_to(w8[j:j + 1, :], (8, 128))
                                      for j in range(D // 128)], axis=1)
                sw_buf[...] = scale * wr
                c1 = jnp.sum(scale * wr, axis=-1, keepdims=True)
                c0 = jnp.sum(m2[:, 0:D] * wr, axis=-1, keepdims=True)
                rid = lax.broadcasted_iota(I32, (8, 128), 0)
                rc_buf[...] = jnp.where(rid == 0, c1, c0)
                start(cp_ffn)

            @pl.when(k == K_MOD + 2)
            def _():
                wait(cp_ffn)

        @pl.when(k == NM - 1)
        def _():
            cp_out[0].start()

        unit_block(n0, UM)
        return carry

    lax.fori_loop(0, NM, main, 0)

    neg = -jnp.inf

    def keep_rows(y, lo):
        n = y.shape[0]
        yc, m, mr, rinv = _ln_stats(y)
        x2_buf[lo:lo + n, :] = y
        st_buf[0, lo:lo + n, :] = jnp.broadcast_to(mr, (n, 128))
        st_buf[1, lo:lo + n, :] = jnp.broadcast_to(rinv, (n, 128))
        d = jnp.sum(_rows8(yc, jnp.multiply, sw_buf[...]), axis=-1, keepdims=True)
        return _r((d + (m - mr) * rc_buf[0:1, 0:1]) * rinv + rc_buf[1:2, 0:1])

    def parked(lo, n):
        y = x2_buf[pl.ds(lo, n), :]
        mr = st_buf[0, pl.ds(lo, n), :]
        rinv = st_buf[1, pl.ds(lo, n), :]
        return y, jnp.concatenate([(y[:, j * 128:(j + 1) * 128] - mr) * rinv
                                   for j in range(D // 128)], axis=1)

    def all_red(v, fn):
        return fn(fn(v, axis=0, keepdims=True), axis=1, keepdims=True)

    lane = lax.broadcasted_iota(I32, (PR, 128), 1)
    ridx = (lane * PR + lax.broadcasted_iota(I32, (PR, 128), 0)).astype(F32)
    rr = jnp.where(lane < row0 // PR, _r(r_buf[...] + rc_buf[1:2, :]), neg)
    last_old = float(row0 - 1)
    cm1 = all_red(rr, jnp.max)
    ci1 = all_red(jnp.where(rr == cm1, ridx, last_old), jnp.min)
    rr2 = jnp.where(ridx == ci1, neg, rr)
    cm2 = all_red(rr2, jnp.max)
    ci2 = all_red(jnp.where(jnp.logical_and(rr2 == cm2, ridx != ci1), ridx, last_old), jnp.min)
    ci1 = jnp.minimum(ci1, last_old).astype(I32)
    ci2 = jnp.minimum(ci2, last_old).astype(I32)
    for j, ci in enumerate((ci1, ci2)):
        g = pl.multiple_of(lax.shift_right_logical(ci[0, 0], 4) * PR, PR)
        keep_rows(resid(acc[pl.ds(g, PR), :], g, PR), SUB + j * PR)

    o2 = jnp.concatenate([_normalize(pv_car[0], ls_car[0]),
                          _normalize(pv_car[1], ls_car[1])], axis=1)
    wo2 = jnp.concatenate([wo_buf[H - 2], wo_buf[H - 1]], axis=0)
    r_new = []
    for j in range(SUB // ECH):
        lo, hi = j * ECH, (j + 1) * ECH
        a = acc[row0 + lo:row0 + hi, :] + jnp.dot(o2[lo:hi], wo2, preferred_element_type=F32)
        r_new.append(keep_rows(resid(a, row0 + lo, ECH), lo))

    sub8 = lax.broadcasted_iota(I32, (8, 1), 0)
    big = jnp.int32((S - 1) * 512 + SUB - 1)
    vals = jnp.concatenate(
        r_new + [jnp.where(sub8 == 0, cm1, jnp.where(sub8 == 1, cm2, neg))], axis=0)
    pos = lax.broadcasted_iota(I32, (SUB, 1), 0)
    cc1 = ci1 * 512 + SUB + (ci1 & (PR - 1))
    cc2 = ci2 * 512 + SUB + PR + (ci2 & (PR - 1))
    code = jnp.concatenate(
        [(pos + row0) * 512 + pos,
         jnp.where(sub8 == 0, cc1, jnp.where(sub8 == 1, cc2, big))], axis=0)
    m1 = jnp.max(vals, axis=0, keepdims=True)
    k1 = jnp.min(jnp.where(vals == m1, code, big), axis=0, keepdims=True)
    vals2 = jnp.where(code == k1, neg, vals)
    m2 = jnp.max(vals2, axis=0, keepdims=True)
    k2 = jnp.min(jnp.where(jnp.logical_and(vals2 == m2, code != k1), code, big),
                 axis=0, keepdims=True)
    k1 = k1[0, 0]
    k2 = k2[0, 0]
    i1 = lax.shift_right_logical(k1, 9)
    i2 = lax.shift_right_logical(k2, 9)
    t1 = k1 & 511
    t2 = k2 & 511
    rowid = lax.broadcasted_iota(I32, (PR, D), 0)
    xf = modulate(jnp.where(rowid == 0, parked(t1, 1)[1], parked(t2, 1)[1]))

    off = pl.multiple_of(jnp.minimum(k2, 0) * 8, 8)
    for j in range(SUB // PR):
        yl, nl = parked(pl.multiple_of(off + j * PR, 8), PR)
        act[row0 + j * PR:row0 + (j + 1) * PR, :] = (
            yl + _rows8(modulate(nl), jnp.multiply, coef[C_GB])).astype(BF16)
    cp_out[1].start()

    gt = _r(jnp.dot(xf.astype(BF16), wa_buf[:, 0:F], preferred_element_type=F32))
    zt = _bits(act[pl.ds(pl.multiple_of(off * 2, PR), PR), 0:128].astype(F32))
    zt = jnp.concatenate([zt[0:8] & zero_buf[...], zt[8:16] & zero_buf[...]], axis=0)
    xs = jnp.concatenate([_float(_bits(xf[:, 0:128]) | zt), xf[:, 128:]], axis=1).astype(BF16)
    up = _r(jnp.dot(xs, wb_buf[:, 0:F], preferred_element_type=F32))
    hid = (_r(gt * _r(jax.nn.sigmoid(gt))) * up).astype(BF16)
    y = _r(jnp.dot(hid, wd_buf[:, 0:D], preferred_element_type=F32))
    y1 = _r(y[0:1, :] * _r(jax.nn.sigmoid(m1)))
    y2 = _r(y[1:2, :] * _r(jax.nn.sigmoid(m2)))

    def fix(i, t):
        g = pl.multiple_of(lax.shift_right_logical(i, 4) * PR, PR)
        tg = pl.multiple_of(lax.shift_right_logical(t, 4) * PR, PR)
        rid = rowid + g
        upd = jnp.where(rid == i1, y1, jnp.where(rid == i2, y2, 0.0))
        yg, ng = parked(tg, PR)
        return g, (yg + _rows8(modulate(ng) + upd, jnp.multiply, coef[C_GB])).astype(BF16)

    g1, fix1 = fix(i1, t1)
    g2, fix2 = fix(i2, t2)
    wait(cp_out)
    act[pl.ds(g1, PR), :] = fix1
    act[pl.ds(g2, PR), :] = fix2
    f1 = cp(act.at[pl.ds(g1, PR), :], out_hbm.at[pl.ds(g1, PR), :], SEM_OUT)
    f2 = cp(act.at[pl.ds(g2, PR), :], out_hbm.at[pl.ds(g2, PR), :], SEM_FIX)
    f1.start()

    @pl.when(g1 != g2)
    def _():
        f2.start()
        f2.wait()

    f1.wait()


@jax.jit
def pallas_adaLN_cond__mha_block_cached__moe_arch_mod__prompt_kernel(
    A_x: jax.Array,
    A_k_cache: jax.Array,
    A_v_cache: jax.Array,
    A_wq: jax.Array,
    A_wo: jax.Array,
    B_x: jax.Array,
    B_w_r: jax.Array,
    B_w_gate: jax.Array,
    B_w_up: jax.Array,
    B_w_down: jax.Array,
    c: jax.Array,
    w_mod: jax.Array,
):
    del B_x
    hbm = pl.BlockSpec(memory_space=pl.ANY)
    out = pl.pallas_call(
        _kernel,
        in_specs=[hbm] * 11,
        out_specs=hbm,
        out_shape=jax.ShapeDtypeStruct((S, D), BF16),
        scratch_shapes=[
            pltpu.VMEM((S, D), BF16),
            pltpu.VMEM((H, S, DH), BF16),
            pltpu.VMEM((H, S, DH), BF16),
            pltpu.VMEM((H, D, DH), BF16),
            pltpu.VMEM((H, DH, D), BF16),
            pltpu.VMEM((D, F + PAD), BF16),
            pltpu.VMEM((D, F + PAD), BF16),
            pltpu.VMEM((F, D + PAD), BF16),
            pltpu.VMEM((S + PR, D), BF16),
            pltpu.VMEM((S, D), F32),
            pltpu.VMEM((NST, 2 * SUB, 128), F32),
            pltpu.VMEM((R2, 2 * SUB, DH), F32),
            pltpu.VMEM((SUB + 2 * PR, D), F32),
            pltpu.VMEM((2, SUB + 2 * PR, 128), F32),
            pltpu.VMEM((PR, 128), F32),
            pltpu.VMEM((5, 8, D), F32),
            pltpu.VMEM((8, 128), BF16),
            pltpu.VMEM((8, D), F32),
            pltpu.VMEM((8, 128), F32),
            pltpu.VMEM((1, D), BF16),
            pltpu.VMEM((16, D), BF16),
            pltpu.VMEM((D, 128), F32),
            pltpu.VMEM((8, 128), I32),
            pltpu.VMEM((FILL, DH), F32),
            pltpu.VMEM((2, SUB, DH), F32),
            pltpu.VMEM((2, SUB, DH), F32),
            pltpu.SemaphoreType.DMA((NSEM,)),
        ],
        compiler_params=pltpu.CompilerParams(
            vmem_limit_bytes=120 * 1024 * 1024,
            disable_bounds_checks=True,
            disable_semaphore_checks=True,
        ),
        name="adaln_mha_mod",
    )(
        A_x.reshape(S, D),
        A_k_cache.reshape(H, S, DH),
        A_v_cache.reshape(H, S, DH),
        A_wq,
        A_wo.reshape(H, DH, D),
        B_w_r.reshape(8, 128),
        B_w_gate,
        B_w_up,
        B_w_down,
        c,
        w_mod,
    )
    return out.reshape(1, S, D)
```

```python
import jax
import jax.numpy as jnp
from jax import lax
import jax.experimental.pallas as pl
import jax.experimental.pallas.tpu as pltpu

S = 2048
D = 1024
H = 32
DH = 128
F = 3584
SUB = 256
NRB = S // SUB
NU = H * NRB
PR = 16
UM = 14
GE = 8
R2 = 9
RAMP = 2 * R2
NM = (NU - RAMP) // UM
HPI = UM // 2
NLOAD = (2 * H - RAMP) // UM
FIN_START = 130
K_MOD = (FIN_START - RAMP) // UM
LN_START = RAMP + UM
assert LN_START <= 33 and LN_START + (S - 2 * SUB) // PR <= RAMP + K_MOD * UM
FILL = 64
ECH = 64
PAD = 128
NST = D // 128
MVC = 1280
EPS = 1e-5
QSCALE = float(DH ** -0.5) * 1.4426950408889634

F32 = jnp.float32
BF16 = jnp.bfloat16
I32 = jnp.int32
NT = (((1,), (1,)), ((), ()))

C_GA, C_SCALE, C_SHIFT, C_KEEP, C_GB = range(5)


def _r(v):
    return v.astype(BF16).astype(F32)


def _bits(v):
    return lax.bitcast_convert_type(v, I32)


def _float(v):
    return lax.bitcast_convert_type(v, F32)


def _rows8(v, fn, c):
    n = v.shape[0] // 8
    return fn(v.reshape(n, 8, D), c[None]).reshape(v.shape)


def _recip(v):
    r = pl.reciprocal(v, approx=True)
    return r * (2.0 - v * r)


def _ln_stats(y):
    m = jnp.mean(y, axis=-1, keepdims=True)
    yc = y - m
    v = jnp.mean(yc * yc, axis=-1, keepdims=True)
    return yc, m, _r(m), _r(jnp.sqrt(_r(_r(v) + EPS)))


def _layernorm(y):
    _, _, mr, den = _ln_stats(y)
    return (y - mr) * (1.0 / den)


def _lane_fold(p, fn):
    t = p[:, 0:128]
    for j in range(1, p.shape[1] // 128):
        t = fn(t, p[:, j * 128:(j + 1) * 128])
    return t


def _normalize(pv, ls):
    return (pv * _recip(jnp.sum(ls, axis=-1, keepdims=True))).astype(BF16)


def _head_of(n):
    if isinstance(n, int):
        return (n % 64) // 2 if n < 192 else (n - 192) % H
    return jnp.where(n < 192, lax.shift_right_logical(n & 63, 1), (n - 192) & (H - 1))


def _row_of(n):
    if isinstance(n, int):
        return SUB * ((n // 64) * 2 + n % 2 if n < 192 else min(n // 32, NRB - 1))
    rb = jnp.where(n < 192, lax.shift_right_logical(n, 6) * 2 + (n & 1),
                   jnp.minimum(lax.shift_right_logical(n, 5), NRB - 1))
    return pl.multiple_of(rb * SUB, SUB)


(SEM_C, SEM_WR, SEM_X0, SEM_X1, SEM_XR, SEM_M12, SEM_FFN, SEM_OUT, SEM_FIX,
 SEM_K0, SEM_WQE, SEM_M0) = range(12)
SEM_W0 = SEM_M0 + NST
SEM_RAMP = SEM_W0 + NST
SEM_MAIN = SEM_RAMP + R2
NSEM = SEM_MAIN + NLOAD


def _kernel(x_hbm, k_hbm, v_hbm, wq_hbm, wo_hbm, wr_hbm, wg_hbm, wu_hbm, wd_hbm,
            c_hbm, wmod_hbm, out_hbm,
            x_buf, k_buf, v_buf, wq_buf, wo_buf, wa_buf, wb_buf, wd_buf,
            act, acc, n_buf, q_acc, x2_buf, st_buf, r_buf, coef, wr_buf, sw_buf, rc_buf,
            c_buf, sc_buf, scol, zero_buf, qa_car, pv_car, ls_car,
            sems):
    def cp(src, dst, slot):
        return pltpu.make_async_copy(src, dst, sems.at[slot])

    def cp_x(b, nb, slot):
        return cp(x_hbm.at[pl.ds(b * SUB, nb * SUB), :],
                  x_buf.at[pl.ds(b * SUB, nb * SUB), :], slot)

    def cp_wq(h, slot):
        col = h * DH if isinstance(h, int) else pl.multiple_of(h * DH, DH)
        return cp(wq_hbm.at[:, pl.ds(col, DH)], wq_buf.at[h], slot)

    def cp_h(src, dst, h0, nh, slot):
        return cp(src.at[pl.ds(h0, nh)], dst.at[pl.ds(h0, nh)], slot)

    def heads(h0, nh, slot, last=False):
        return [cp_h(k_hbm, k_buf, h0, nh, slot), cp_h(v_hbm, v_buf, h0, nh, slot),
                cp_h(wo_hbm, wo_buf, h0 - 1, nh + 1 if last else nh, slot)] + [
            cp_wq(h0 + 1 + j, slot) for j in range(nh - 1 if last else nh)]

    def ramp_heads(j):
        return [cp_h(k_hbm, k_buf, j, 1, SEM_RAMP + j), cp_h(v_hbm, v_buf, j, 1, SEM_RAMP + j),
                cp_h(wo_hbm, wo_buf, j - 1, 1, SEM_RAMP + j)]

    def main_heads(k, last=False):
        h0 = R2 + k * HPI
        return heads(h0, H - h0 if last else HPI, SEM_MAIN + k, last)

    cp_k0 = cp_h(k_hbm, k_buf, 0, 1, SEM_K0)
    cp_v0 = [cp_h(v_hbm, v_buf, 0, 1, SEM_RAMP)] + [cp_wq(h, SEM_RAMP) for h in range(GE, R2 + 1)]
    cp_wqe = [cp_wq(h, SEM_WQE) for h in range(GE)]

    def lanes(j):
        return pl.ds(j * 128 if isinstance(j, int) else pl.multiple_of(j * 128, 128), 128)

    def cp_m0(j):
        return [cp(wmod_hbm.at[:, lanes(u * NST + j)],
                   v_buf.at[H - NST + j, u * D:(u + 1) * D, :], SEM_M0 + j) for u in range(2)]

    def cp_w0(j):
        return cp(wq_hbm.at[lanes(j), 0:GE * DH], wb_buf.at[lanes(j), 0:GE * DH], SEM_W0 + j)

    cp_c = cp(c_hbm, c_buf, SEM_C)
    cp_wr = cp(wr_hbm, wr_buf, SEM_WR)
    cp_m12 = [cp(wmod_hbm.at[:, 2 * D:3 * D], wa_buf.at[:, 2 * D:3 * D], SEM_M12),
              cp(wmod_hbm.at[:, 3 * D:6 * D], wb_buf.at[:, 0:3 * D], SEM_M12)]
    cp_ffn = [cp(wg_hbm, wa_buf.at[:, 0:F], SEM_FFN),
              cp(wu_hbm, wb_buf.at[:, 0:F], SEM_FFN),
              cp(wd_hbm, wd_buf.at[:, 0:D], SEM_FFN)]

    row0 = (NRB - 1) * SUB
    cp_out = [cp(act.at[0:row0, :], out_hbm.at[0:row0, :], SEM_OUT),
              cp(act.at[row0:S, :], out_hbm.at[row0:S, :], SEM_OUT)]

    def vpu_matvec(w_ref, ncols):
        parts = []
        zf = None
        for cc in range(0, ncols, 256):
            a = None if zf is None else jnp.concatenate([zf, zf], axis=1)
            for g in range(D // 8):
                wv = w_ref[g * 8:(g + 1) * 8, cc:cc + 256].astype(F32)
                sv = scol[g * 8:(g + 1) * 8, :]
                pr = jnp.concatenate([wv[:, 0:128] * sv, wv[:, 128:256] * sv], axis=1)
                a = pr if a is None else a + pr
            zf = _float(_lane_fold(_bits(a), jnp.bitwise_or) & zero_buf[...])
            parts.append(a)
        return jnp.sum(jnp.concatenate(parts, axis=1), axis=0, keepdims=True)

    def modulate(n):
        n = _rows8(n, jnp.multiply, coef[C_SCALE])
        return _rows8(n, jnp.add, coef[C_SHIFT])

    def resid(a, row, nrows):
        a = _rows8(a, jnp.multiply, coef[C_GA])
        return _r(x_buf[pl.ds(row, nrows), :].astype(F32) + a)

    def piece(src, dst, lane_id):
        y = resid(acc[pl.ds(src, PR), :], src, PR)
        nn = _layernorm(y)
        hh = modulate(nn)
        r = jnp.sum(_rows8(nn, jnp.multiply, sw_buf[...]), axis=-1, keepdims=True)
        oo = (_rows8(y, jnp.multiply, coef[C_KEEP])
              + _rows8(hh, jnp.multiply, coef[C_GB]))
        act[pl.ds(dst, PR), :] = oo.astype(BF16)
        lane = lax.broadcasted_iota(I32, (PR, 128), 1)
        rn = jnp.where(lane == lane_id, r, r_buf[...])
        r_buf[...] = rn
        return oo, rn

    def unit_piece(n):
        is_ln = jnp.logical_and(n >= LN_START, n < LN_START + (S - 2 * SUB) // PR)
        is_fin = jnp.logical_and(n >= FIN_START, n < FIN_START + (S - SUB) // PR)
        f = n - FIN_START
        src = jnp.where(is_ln, 2 * SUB + (n - LN_START) * PR, jnp.where(is_fin, f * PR, 0))
        dst = jnp.where(jnp.logical_or(is_ln, is_fin), src, S)
        oo, rn = piece(pl.multiple_of(src, PR), pl.multiple_of(dst, PR),
                       jnp.where(is_fin, f, -1))
        bits = _lane_fold(_bits(oo), jnp.bitwise_or) | _bits(rn)
        return (bits[0:8] | bits[8:16]) & zero_buf[...]

    def qproj_head(n):
        return jnp.dot(act[pl.ds(_row_of(n), FILL), 0:D // 2],
                       wq_buf[_head_of(n)][0:D // 2], preferred_element_type=F32)

    def qproj_rest(n, qa):
        row = _row_of(n)
        w = wq_buf[_head_of(n)]
        row2 = row + FILL if isinstance(row, int) else pl.multiple_of(row + FILL, 16)
        qb = jnp.dot(act[pl.ds(row, SUB), D // 2:D], w[D // 2:D], preferred_element_type=F32)
        qc = jnp.dot(act[pl.ds(row2, SUB - FILL), 0:D // 2], w[0:D // 2],
                     preferred_element_type=F32)
        return ((qb + jnp.concatenate([qa, qc], axis=0)) * QSCALE).astype(BF16)

    def oproj(o, n):
        acc[pl.ds(_row_of(n), SUB), :] += jnp.dot(o, wo_buf[_head_of(n)],
                                                  preferred_element_type=F32)

    def unit_block(n0, nunits):
        o = _normalize(pv_car[0], ls_car[0])
        raw = (pv_car[1], ls_car[1])
        qa = qa_car[...]
        for u in range(nunits):
            n = n0 + u
            hd = _head_of(n)
            q = qproj_rest(n, qa)
            z = unit_piece(n)
            oproj(o, n - 2)
            sc = lax.dot_general(q, k_buf[hd], NT, preferred_element_type=F32)
            qa = qproj_head(n + 1)
            mm = _lane_fold(sc, jnp.maximum)
            mm = jnp.concatenate([_float(_bits(mm[0:8]) | z), mm[8:]], axis=0)
            m = jnp.max(mm, axis=-1, keepdims=True)
            p = jnp.exp2(sc - m)
            ls = _lane_fold(p, jnp.add)
            pv = jnp.dot(p.astype(BF16), v_buf[hd], preferred_element_type=F32)
            if u + 1 < nunits:
                zb = (_bits(pv).reshape(SUB // 8, 8, 128)
                      & zero_buf[...][None]).reshape(SUB, 128)
                o = _normalize(raw[0], _float(_bits(raw[1]) | zb))
            else:
                pv_car[0] = raw[0]
                ls_car[0] = raw[1]
            raw = (pv, ls)
        pv_car[1] = raw[0]
        ls_car[1] = raw[1]
        qa_car[...] = qa

    def ramp_block(j):
        o = [_normalize(pv_car[u], ls_car[u]) for u in range(2)]
        w = wo_buf[j - 1]

        def op_part(u, r0, r1, c0, c1):
            acc[u * SUB + r0:u * SUB + r1, c0:c1] += jnp.dot(
                o[u][r0:r1], w[:, c0:c1], preferred_element_type=F32)

        for u in range(2):
            q = (q_acc[j, u * SUB:(u + 1) * SUB, :] * QSCALE).astype(BF16)
            sc = lax.dot_general(q, k_buf[j], NT, preferred_element_type=F32)
            op_part(u, 0, FILL, 0, D // 2)
            m = jnp.max(_lane_fold(sc, jnp.maximum), axis=-1, keepdims=True)
            p = jnp.exp2(sc - m)
            ls_car[u] = _lane_fold(p, jnp.add)
            pv_car[u] = jnp.dot(p.astype(BF16), v_buf[j], preferred_element_type=F32)
            if u == 0:
                for v in range(2):
                    op_part(v, FILL, SUB, 0, D // 2)
                    op_part(v, 0, SUB, D // 2, D)

    def start(cps):
        for c_ in cps:
            c_.start()

    def wait(cps):
        for c_ in cps:
            c_.wait()

    start([cp_c, cp_x(0, 1, SEM_X0), cp_x(1, 1, SEM_X1)])
    for j in range(NST):
        start(cp_m0(j) + [cp_w0(j)])
    start([cp_k0] + cp_v0)
    for j in range(1, R2):
        start(ramp_heads(j))
    start([cp_wr])
    n_early = (LN_START - RAMP) // UM
    for k in range(n_early):
        start(main_heads(k))

    r_buf[...] = jnp.zeros(r_buf.shape, F32)
    zero_buf[...] = jnp.zeros(zero_buf.shape, I32)
    coef[C_GA] = jnp.zeros((8, D), F32)
    coef[C_KEEP] = jnp.zeros((8, D), F32)
    coef[C_GB] = jnp.ones((8, D), F32)
    sw_buf[...] = jnp.zeros(sw_buf.shape, F32)

    def zero_q(h, carry):
        q_acc[h] = jnp.zeros((2 * SUB, DH), F32)
        return carry

    lax.fori_loop(0, GE, zero_q, 0)
    cp_c.wait()
    cf = c_buf[...].astype(F32)
    sf = _r(cf * _r(jax.nn.sigmoid(cf)))
    sc_buf[...] = jnp.broadcast_to(sf, (16, D)).astype(BF16)
    for j in range(D // 128):
        scol[j * 128:(j + 1) * 128, :] = jnp.broadcast_to(
            sf[:, j * 128:(j + 1) * 128], (128, 128)).T

    def norm_rows(j, carry):
        @pl.when((j & 1) == 0)
        def _():
            b = lax.shift_right_logical(j, 1)
            cp_x(b, 1, SEM_X0 + b).wait()

        row = pl.multiple_of(j * 128, 128)
        nn = _layernorm(x_buf[pl.ds(row, 128), :].astype(F32))
        for t in range(NST):
            n_buf[t, pl.ds(row, 128), :] = nn[:, t * 128:(t + 1) * 128]
        return carry

    lax.fori_loop(0, 2 * SUB // 128, norm_rows, 0)

    def stage(j, carry):
        wait(cp_m0(j))
        wm = jnp.concatenate([v_buf[H - NST + j, 0:D, :], v_buf[H - NST + j, D:2 * D, :]], axis=1)
        mj = _r(jnp.dot(sc_buf[...], wm, preferred_element_type=F32)[0:8, :])
        coef[C_SHIFT, :, lanes(j)] = mj[:, 0:128]
        coef[C_SCALE, :, lanes(j)] = _r(1.0 + mj[:, 128:256])
        zr = S // NST
        acc[pl.ds(pl.multiple_of(j * zr, zr), zr), :] = jnp.zeros((zr, D), F32)
        cp_w0(j).wait()
        hj = (n_buf[j].reshape(2 * SUB // 8, 8, 128) * coef[C_SCALE, :, lanes(j)][None]
              + coef[C_SHIFT, :, lanes(j)][None]).reshape(2 * SUB, 128).astype(BF16)
        act[0:2 * SUB, lanes(j)] = hj
        part = jnp.dot(hj, wb_buf[lanes(j), 0:GE * DH], preferred_element_type=F32)
        for h in range(GE):
            q_acc[h] += part[:, h * DH:(h + 1) * DH]
        return carry

    lax.fori_loop(0, NST, stage, 0)

    cp_k0.wait()
    s01 = lax.dot_general((q_acc[0] * QSCALE).astype(BF16), k_buf[0], NT,
                          preferred_element_type=F32)
    mm01 = _lane_fold(s01, jnp.maximum)
    m0 = jnp.max(mm01[0:SUB], axis=-1, keepdims=True)
    wait(cp_v0)
    qa_car[...] = qproj_head(RAMP)
    for u in range(2):
        m = m0 if u == 0 else jnp.max(mm01[SUB:], axis=-1, keepdims=True)
        p = jnp.exp2(s01[u * SUB:(u + 1) * SUB] - m)
        ls_car[u] = _lane_fold(p, jnp.add)
        pv_car[u] = jnp.dot(p.astype(BF16), v_buf[0], preferred_element_type=F32)
    for h in range(GE, R2):
        q_acc[h] = jnp.dot(act[0:2 * SUB, :], wq_buf[h], preferred_element_type=F32)

    def ramp2(j, carry):
        wait(ramp_heads(j))
        ramp_block(j)
        return carry

    lax.fori_loop(1, R2, ramp2, 0)
    start([cp_x(2, NRB - 2, SEM_XR)])
    for k in range(n_early, NLOAD):
        start(main_heads(k, k == NLOAD - 1))
    start(cp_wqe + cp_m12)

    assert FIN_START + row0 // PR <= RAMP + (NM - 1) * UM

    def main(k, carry):
        n0 = RAMP + k * UM

        @pl.when(k <= K_MOD + 2)
        def _():
            @pl.when(k < NLOAD - 1)
            def _():
                wait(main_heads(k))

            @pl.when(k == NLOAD - 1)
            def _():
                wait(main_heads(NLOAD - 1, True) + cp_wqe)

            @pl.when(k == n_early)
            def _():
                cp_x(2, NRB - 2, SEM_XR).wait()

            @pl.when(k == K_MOD)
            def _():
                wait(cp_m12 + [cp_wr])
                sc = sc_buf[...]
                m2a = jnp.dot(sc, wb_buf[:, MVC:3 * D], preferred_element_type=F32)[0:8, :]
                m1 = _r(jnp.dot(sc, wa_buf[:, 2 * D:3 * D], preferred_element_type=F32)[0:8, :])
                m2b = jnp.broadcast_to(vpu_matvec(wb_buf, MVC), (8, MVC))
                m2 = _r(jnp.concatenate([m2b, m2a], axis=1))
                coef[C_GA] = m1
                coef[C_KEEP] = jnp.ones((8, D), F32)
                scale = _r(1.0 + m2[:, D:2 * D])
                coef[C_SHIFT] = m2[:, 0:D]
                coef[C_SCALE] = scale
                coef[C_GB] = m2[:, 2 * D:3 * D]
                w8 = wr_buf[...].astype(F32)
                wr = jnp.concatenate([jnp.broadcast_to(w8[j:j + 1, :], (8, 128))
                                      for j in range(D // 128)], axis=1)
                sw_buf[...] = scale * wr
                c1 = jnp.sum(scale * wr, axis=-1, keepdims=True)
                c0 = jnp.sum(m2[:, 0:D] * wr, axis=-1, keepdims=True)
                rid = lax.broadcasted_iota(I32, (8, 128), 0)
                rc_buf[...] = jnp.where(rid == 0, c1, c0)
                start(cp_ffn)

            @pl.when(k == K_MOD + 2)
            def _():
                wait(cp_ffn)

        @pl.when(k == NM - 1)
        def _():
            cp_out[0].start()

        unit_block(n0, UM)
        return carry

    lax.fori_loop(0, NM, main, 0)

    neg = -jnp.inf

    def keep_rows(y, lo):
        n = y.shape[0]
        yc, m, mr, den = _ln_stats(y)
        rinv = _recip(den)
        x2_buf[lo:lo + n, :] = y
        st_buf[0, lo:lo + n, :] = jnp.broadcast_to(mr, (n, 128))
        st_buf[1, lo:lo + n, :] = jnp.broadcast_to(rinv, (n, 128))
        d = jnp.sum(_rows8(yc, jnp.multiply, sw_buf[...]), axis=-1, keepdims=True)
        return _r((d + (m - mr) * rc_buf[0:1, 0:1]) * rinv + rc_buf[1:2, 0:1])

    def parked(lo, n):
        y = x2_buf[pl.ds(lo, n), :]
        mr = st_buf[0, pl.ds(lo, n), :]
        rinv = st_buf[1, pl.ds(lo, n), :]
        return y, jnp.concatenate([(y[:, j * 128:(j + 1) * 128] - mr) * rinv
                                   for j in range(D // 128)], axis=1)

    def all_red(v, fn):
        return fn(fn(v, axis=0, keepdims=True), axis=1, keepdims=True)

    lane = lax.broadcasted_iota(I32, (PR, 128), 1)
    ridx = (lane * PR + lax.broadcasted_iota(I32, (PR, 128), 0)).astype(F32)
    rr = jnp.where(lane < row0 // PR, _r(r_buf[...] + rc_buf[1:2, :]), neg)
    last_old = float(row0 - 1)
    cm1 = all_red(rr, jnp.max)
    ci1 = all_red(jnp.where(rr == cm1, ridx, last_old), jnp.min)
    rr2 = jnp.where(ridx == ci1, neg, rr)
    cm2 = all_red(rr2, jnp.max)
    ci2 = all_red(jnp.where(jnp.logical_and(rr2 == cm2, ridx != ci1), ridx, last_old), jnp.min)
    ci1 = jnp.minimum(ci1, last_old).astype(I32)
    ci2 = jnp.minimum(ci2, last_old).astype(I32)
    for j, ci in enumerate((ci1, ci2)):
        g = pl.multiple_of(lax.shift_right_logical(ci[0, 0], 4) * PR, PR)
        keep_rows(resid(acc[pl.ds(g, PR), :], g, PR), SUB + j * PR)

    o2 = jnp.concatenate([_normalize(pv_car[0], ls_car[0]),
                          _normalize(pv_car[1], ls_car[1])], axis=1)
    wo2 = jnp.concatenate([wo_buf[H - 2], wo_buf[H - 1]], axis=0)
    r_new = []
    for j in range(SUB // ECH):
        lo, hi = j * ECH, (j + 1) * ECH
        a = acc[row0 + lo:row0 + hi, :] + jnp.dot(o2[lo:hi], wo2, preferred_element_type=F32)
        r_new.append(keep_rows(resid(a, row0 + lo, ECH), lo))

    sub8 = lax.broadcasted_iota(I32, (8, 1), 0)
    big = jnp.int32((S - 1) * 512 + SUB - 1)
    vals = jnp.concatenate(
        r_new + [jnp.where(sub8 == 0, cm1, jnp.where(sub8 == 1, cm2, neg))], axis=0)
    pos = lax.broadcasted_iota(I32, (SUB, 1), 0)
    cc1 = ci1 * 512 + SUB + (ci1 & (PR - 1))
    cc2 = ci2 * 512 + SUB + PR + (ci2 & (PR - 1))
    code = jnp.concatenate(
        [(pos + row0) * 512 + pos,
         jnp.where(sub8 == 0, cc1, jnp.where(sub8 == 1, cc2, big))], axis=0)
    m1 = jnp.max(vals, axis=0, keepdims=True)
    k1 = jnp.min(jnp.where(vals == m1, code, big), axis=0, keepdims=True)
    vals2 = jnp.where(code == k1, neg, vals)
    m2 = jnp.max(vals2, axis=0, keepdims=True)
    k2 = jnp.min(jnp.where(jnp.logical_and(vals2 == m2, code != k1), code, big),
                 axis=0, keepdims=True)
    k1 = k1[0, 0]
    k2 = k2[0, 0]
    i1 = lax.shift_right_logical(k1, 9)
    i2 = lax.shift_right_logical(k2, 9)
    t1 = k1 & 511
    t2 = k2 & 511
    rowid = lax.broadcasted_iota(I32, (PR, D), 0)
    xf = modulate(jnp.where(rowid == 0, parked(t1, 1)[1], parked(t2, 1)[1]))

    off = pl.multiple_of(jnp.minimum(k2, 0) * 8, 8)
    for j in range(SUB // PR):
        yl, nl = parked(pl.multiple_of(off + j * PR, 8), PR)
        act[row0 + j * PR:row0 + (j + 1) * PR, :] = (
            yl + _rows8(modulate(nl), jnp.multiply, coef[C_GB])).astype(BF16)
    cp_out[1].start()

    gt = _r(jnp.dot(xf.astype(BF16), wa_buf[:, 0:F], preferred_element_type=F32)[0:8])
    zt = _bits(act[pl.ds(pl.multiple_of(off * 2, PR), PR), 0:128].astype(F32))
    zt = jnp.concatenate([zt[0:8] & zero_buf[...], zt[8:16] & zero_buf[...]], axis=0)
    xs = jnp.concatenate([_float(_bits(xf[:, 0:128]) | zt), xf[:, 128:]], axis=1).astype(BF16)
    up = _r(jnp.dot(xs, wb_buf[:, 0:F], preferred_element_type=F32)[0:8])
    hid = _r(gt * _r(jax.nn.sigmoid(gt))) * up
    hid = jnp.concatenate([hid, hid], axis=0).astype(BF16)
    y = _r(jnp.dot(hid, wd_buf[:, 0:D], preferred_element_type=F32)[0:8])
    y1 = _r(y[0:1, :] * _r(jax.nn.sigmoid(m1)))
    y2 = _r(y[1:2, :] * _r(jax.nn.sigmoid(m2)))

    def fix(i, t):
        g = pl.multiple_of(lax.shift_right_logical(i, 4) * PR, PR)
        tg = pl.multiple_of(lax.shift_right_logical(t, 4) * PR, PR)
        rid = rowid + g
        upd = jnp.where(rid == i1, y1, jnp.where(rid == i2, y2, 0.0))
        yg, ng = parked(tg, PR)
        return g, (yg + _rows8(modulate(ng) + upd, jnp.multiply, coef[C_GB])).astype(BF16)

    g1, fix1 = fix(i1, t1)
    g2, fix2 = fix(i2, t2)
    wait(cp_out)
    act[pl.ds(g1, PR), :] = fix1
    act[pl.ds(g2, PR), :] = fix2
    f1 = cp(act.at[pl.ds(g1, PR), :], out_hbm.at[pl.ds(g1, PR), :], SEM_OUT)
    f2 = cp(act.at[pl.ds(g2, PR), :], out_hbm.at[pl.ds(g2, PR), :], SEM_FIX)
    f1.start()

    @pl.when(g1 != g2)
    def _():
        f2.start()
        f2.wait()

    f1.wait()


@jax.jit
def pallas_adaLN_cond__mha_block_cached__moe_arch_mod__prompt_kernel(
    A_x: jax.Array,
    A_k_cache: jax.Array,
    A_v_cache: jax.Array,
    A_wq: jax.Array,
    A_wo: jax.Array,
    B_x: jax.Array,
    B_w_r: jax.Array,
    B_w_gate: jax.Array,
    B_w_up: jax.Array,
    B_w_down: jax.Array,
    c: jax.Array,
    w_mod: jax.Array,
):
    del B_x
    hbm = pl.BlockSpec(memory_space=pl.ANY)
    out = pl.pallas_call(
        _kernel,
        in_specs=[hbm] * 11,
        out_specs=hbm,
        out_shape=jax.ShapeDtypeStruct((S, D), BF16),
        scratch_shapes=[
            pltpu.VMEM((S, D), BF16),
            pltpu.VMEM((H, S, DH), BF16),
            pltpu.VMEM((H, S, DH), BF16),
            pltpu.VMEM((H, D, DH), BF16),
            pltpu.VMEM((H, DH, D), BF16),
            pltpu.VMEM((D, F + PAD), BF16),
            pltpu.VMEM((D, F + PAD), BF16),
            pltpu.VMEM((F, D + PAD), BF16),
            pltpu.VMEM((S + PR, D), BF16),
            pltpu.VMEM((S, D), F32),
            pltpu.VMEM((NST, 2 * SUB, 128), F32),
            pltpu.VMEM((R2, 2 * SUB, DH), F32),
            pltpu.VMEM((SUB + 2 * PR, D), F32),
            pltpu.VMEM((2, SUB + 2 * PR, 128), F32),
            pltpu.VMEM((PR, 128), F32),
            pltpu.VMEM((5, 8, D), F32),
            pltpu.VMEM((8, 128), BF16),
            pltpu.VMEM((8, D), F32),
            pltpu.VMEM((8, 128), F32),
            pltpu.VMEM((1, D), BF16),
            pltpu.VMEM((16, D), BF16),
            pltpu.VMEM((D, 128), F32),
            pltpu.VMEM((8, 128), I32),
            pltpu.VMEM((FILL, DH), F32),
            pltpu.VMEM((2, SUB, DH), F32),
            pltpu.VMEM((2, SUB, DH), F32),
            pltpu.SemaphoreType.DMA((NSEM,)),
        ],
        compiler_params=pltpu.CompilerParams(
            vmem_limit_bytes=120 * 1024 * 1024,
            disable_bounds_checks=True,
            disable_semaphore_checks=True,
        ),
        name="adaln_mha_mod",
    )(
        A_x.reshape(S, D),
        A_k_cache.reshape(H, S, DH),
        A_v_cache.reshape(H, S, DH),
        A_wq,
        A_wo.reshape(H, DH, D),
        B_w_r.reshape(8, 128),
        B_w_gate,
        B_w_up,
        B_w_down,
        c,
        w_mod,
    )
    return out.reshape(1, S, D)
```

```python
import jax
import jax.numpy as jnp
from jax import lax
import jax.experimental.pallas as pl
import jax.experimental.pallas.tpu as pltpu

S = 2048
D = 1024
H = 32
DH = 128
F = 3584
SUB = 256
NRB = S // SUB
NU = H * NRB
PR = 16
UM = 14
GE = 8
R2 = 9
RAMP = 2 * R2
NM = (NU - RAMP) // UM
HPI = UM // 2
NLOAD = (2 * H - RAMP) // UM
FIN_START = 130
K_MOD = (FIN_START - RAMP) // UM
LN_START = RAMP + UM
assert LN_START <= 33 and LN_START + (S - 2 * SUB) // PR <= RAMP + K_MOD * UM
FILL = 64
ECH = 64
PAD = 128
NST = D // 128
MVN = 3
MV_K0 = 2
assert (K_MOD - MV_K0) * MVN >= 4 * D // 256
WW = 2 * F + 256 + PAD
EPS = 1e-5
QSCALE = float(DH ** -0.5) * 1.4426950408889634

F32 = jnp.float32
BF16 = jnp.bfloat16
I32 = jnp.int32
NT = (((1,), (1,)), ((), ()))

C_GA, C_SCALE, C_SHIFT, C_KEEP, C_GB = range(5)


def _r(v):
    return v.astype(BF16).astype(F32)


def _bits(v):
    return lax.bitcast_convert_type(v, I32)


def _float(v):
    return lax.bitcast_convert_type(v, F32)


def _rows8(v, fn, c):
    n = v.shape[0] // 8
    return fn(v.reshape(n, 8, D), c[None]).reshape(v.shape)


def _recip(v):
    r = pl.reciprocal(v, approx=True)
    return r * (2.0 - v * r)


def _ln_stats(y):
    m = jnp.mean(y, axis=-1, keepdims=True)
    yc = y - m
    v = jnp.mean(yc * yc, axis=-1, keepdims=True)
    return yc, m, _r(m), _r(jnp.sqrt(_r(_r(v) + EPS)))


def _layernorm(y):
    _, _, mr, den = _ln_stats(y)
    return (y - mr) * (1.0 / den)


def _lane_fold(p, fn):
    t = p[:, 0:128]
    for j in range(1, p.shape[1] // 128):
        t = fn(t, p[:, j * 128:(j + 1) * 128])
    return t


def _normalize(pv, ls):
    return (pv * _recip(jnp.sum(ls, axis=-1, keepdims=True))).astype(BF16)


def _head_of(n):
    if isinstance(n, int):
        return (n % 64) // 2 if n < 192 else (n - 192) % H
    return jnp.where(n < 192, lax.shift_right_logical(n & 63, 1), (n - 192) & (H - 1))


def _row_of(n):
    if isinstance(n, int):
        return SUB * ((n // 64) * 2 + n % 2 if n < 192 else min(n // 32, NRB - 1))
    rb = jnp.where(n < 192, lax.shift_right_logical(n, 6) * 2 + (n & 1),
                   jnp.minimum(lax.shift_right_logical(n, 5), NRB - 1))
    return pl.multiple_of(rb * SUB, SUB)


(SEM_C, SEM_WR, SEM_X0, SEM_X1, SEM_XR, SEM_M12, SEM_FFN, SEM_OUT, SEM_FIX,
 SEM_K0, SEM_WQE, SEM_M0) = range(12)
SEM_W0 = SEM_M0 + NST
SEM_RAMP = SEM_W0 + NST
SEM_MAIN = SEM_RAMP + R2
NSEM = SEM_MAIN + NLOAD


def _kernel(x_hbm, k_hbm, v_hbm, wq_hbm, wo_hbm, wr_hbm, wg_hbm, wu_hbm, wd_hbm,
            c_hbm, wmod_hbm, out_hbm,
            x_buf, k_buf, v_buf, wq_buf, wo_buf, w_buf, wd_buf,
            act, acc, n_buf, q_acc, x2_buf, st_buf, r_buf, coef, wr_buf, sw_buf, rc_buf,
            c_buf, sc_buf, scol, m_raw, zero_buf, qa_car, pv_car, ls_car,
            sems):
    def cp(src, dst, slot):
        return pltpu.make_async_copy(src, dst, sems.at[slot])

    def cp_x(b, nb, slot):
        return cp(x_hbm.at[pl.ds(b * SUB, nb * SUB), :],
                  x_buf.at[pl.ds(b * SUB, nb * SUB), :], slot)

    def cp_wq(h, slot):
        col = h * DH if isinstance(h, int) else pl.multiple_of(h * DH, DH)
        return cp(wq_hbm.at[:, pl.ds(col, DH)], wq_buf.at[h], slot)

    def cp_h(src, dst, h0, nh, slot):
        return cp(src.at[pl.ds(h0, nh)], dst.at[pl.ds(h0, nh)], slot)

    def heads(h0, nh, slot, last=False):
        return [cp_h(k_hbm, k_buf, h0, nh, slot), cp_h(v_hbm, v_buf, h0, nh, slot),
                cp_h(wo_hbm, wo_buf, h0 - 1, nh + 1 if last else nh, slot)] + [
            cp_wq(h0 + 1 + j, slot) for j in range(nh - 1 if last else nh)]

    def ramp_heads(j):
        return [cp_h(k_hbm, k_buf, j, 1, SEM_RAMP + j), cp_h(v_hbm, v_buf, j, 1, SEM_RAMP + j),
                cp_h(wo_hbm, wo_buf, j - 1, 1, SEM_RAMP + j)]

    def main_heads(k, last=False):
        h0 = R2 + k * HPI
        return heads(h0, H - h0 if last else HPI, SEM_MAIN + k, last)

    cp_k0 = cp_h(k_hbm, k_buf, 0, 1, SEM_K0)
    cp_v0 = [cp_h(v_hbm, v_buf, 0, 1, SEM_RAMP)] + [cp_wq(h, SEM_RAMP) for h in range(GE, R2 + 1)]
    cp_wqe = [cp_wq(h, SEM_WQE) for h in range(GE)]

    def lanes(j):
        return pl.ds(j * 128 if isinstance(j, int) else pl.multiple_of(j * 128, 128), 128)

    def cp_m0(j):
        return [cp(wmod_hbm.at[:, lanes(u * NST + j)],
                   v_buf.at[H - NST + j, u * D:(u + 1) * D, :], SEM_M0 + j) for u in range(2)]

    def cp_w0(j):
        return cp(wq_hbm.at[lanes(j), 0:GE * DH], w_buf.at[lanes(j), 4 * D:4 * D + GE * DH], SEM_W0 + j)

    cp_c = cp(c_hbm, c_buf, SEM_C)
    cp_wr = cp(wr_hbm, wr_buf, SEM_WR)
    cp_m12 = [cp(wmod_hbm.at[:, 2 * D:6 * D], w_buf.at[:, 0:4 * D], SEM_M12)]
    cp_ffn = [cp(wg_hbm, w_buf.at[:, 0:F], SEM_FFN),
              cp(wu_hbm, w_buf.at[:, F:2 * F], SEM_FFN),
              cp(wd_hbm, wd_buf.at[:, 0:D], SEM_FFN)]

    row0 = (NRB - 1) * SUB
    cp_out = [cp(act.at[0:row0, :], out_hbm.at[0:row0, :], SEM_OUT),
              cp(act.at[row0:S, :], out_hbm.at[row0:S, :], SEM_OUT)]

    def mod_slice(idx):
        live = jnp.logical_and(idx >= 0, idx < 4 * D // 256)
        src = pl.multiple_of(jnp.where(live, idx * 256, 2 * F), 128)
        dst = pl.multiple_of(jnp.where(live, idx * 256, 4 * D), 128)
        a = None
        for g in range(D // 8):
            wv = w_buf[g * 8:(g + 1) * 8, pl.ds(src, 256)].astype(F32)
            sv = scol[g * 8:(g + 1) * 8, :]
            pr = jnp.concatenate([wv[:, 0:128] * sv, wv[:, 128:256] * sv], axis=1)
            a = pr if a is None else a + pr
        m_raw[:, pl.ds(dst, 256)] = a
        return _lane_fold(_bits(a), jnp.bitwise_or) & zero_buf[...]

    def modulate(n):
        n = _rows8(n, jnp.multiply, coef[C_SCALE])
        return _rows8(n, jnp.add, coef[C_SHIFT])

    def resid(a, row, nrows):
        a = _rows8(a, jnp.multiply, coef[C_GA])
        return _r(x_buf[pl.ds(row, nrows), :].astype(F32) + a)

    def piece(src, dst, lane_id):
        y = resid(acc[pl.ds(src, PR), :], src, PR)
        nn = _layernorm(y)
        hh = modulate(nn)
        r = jnp.sum(_rows8(nn, jnp.multiply, sw_buf[...]), axis=-1, keepdims=True)
        oo = (_rows8(y, jnp.multiply, coef[C_KEEP])
              + _rows8(hh, jnp.multiply, coef[C_GB]))
        act[pl.ds(dst, PR), :] = oo.astype(BF16)
        lane = lax.broadcasted_iota(I32, (PR, 128), 1)
        rn = jnp.where(lane == lane_id, r, r_buf[...])
        r_buf[...] = rn
        return oo, rn

    def unit_piece(n):
        is_ln = jnp.logical_and(n >= LN_START, n < LN_START + (S - 2 * SUB) // PR)
        is_fin = jnp.logical_and(n >= FIN_START, n < FIN_START + (S - SUB) // PR)
        f = n - FIN_START
        src = jnp.where(is_ln, 2 * SUB + (n - LN_START) * PR, jnp.where(is_fin, f * PR, 0))
        dst = jnp.where(jnp.logical_or(is_ln, is_fin), src, S)
        oo, rn = piece(pl.multiple_of(src, PR), pl.multiple_of(dst, PR),
                       jnp.where(is_fin, f, -1))
        bits = _lane_fold(_bits(oo), jnp.bitwise_or) | _bits(rn)
        return (bits[0:8] | bits[8:16]) & zero_buf[...]

    def qproj_head(n):
        return jnp.dot(act[pl.ds(_row_of(n), FILL), 0:D // 2],
                       wq_buf[_head_of(n)][0:D // 2], preferred_element_type=F32)

    def qproj_rest(n, qa):
        row = _row_of(n)
        w = wq_buf[_head_of(n)]
        row2 = row + FILL if isinstance(row, int) else pl.multiple_of(row + FILL, 16)
        qb = jnp.dot(act[pl.ds(row, SUB), D // 2:D], w[D // 2:D], preferred_element_type=F32)
        qc = jnp.dot(act[pl.ds(row2, SUB - FILL), 0:D // 2], w[0:D // 2],
                     preferred_element_type=F32)
        return ((qb + jnp.concatenate([qa, qc], axis=0)) * QSCALE).astype(BF16)

    def oproj(o, n):
        acc[pl.ds(_row_of(n), SUB), :] += jnp.dot(o, wo_buf[_head_of(n)],
                                                  preferred_element_type=F32)

    def unit_block(k, n0, nunits):
        o = _normalize(pv_car[0], ls_car[0])
        raw = (pv_car[1], ls_car[1])
        qa = qa_car[...]
        for u in range(nunits):
            n = n0 + u
            hd = _head_of(n)
            q = qproj_rest(n, qa)
            z = unit_piece(n)
            if u < MVN:
                z = z | mod_slice((k - MV_K0) * MVN + u)
            oproj(o, n - 2)
            sc = lax.dot_general(q, k_buf[hd], NT, preferred_element_type=F32)
            qa = qproj_head(n + 1)
            mm = _lane_fold(sc, jnp.maximum)
            mm = jnp.concatenate([_float(_bits(mm[0:8]) | z), mm[8:]], axis=0)
            m = jnp.max(mm, axis=-1, keepdims=True)
            p = jnp.exp2(sc - m)
            ls = _lane_fold(p, jnp.add)
            pv = jnp.dot(p.astype(BF16), v_buf[hd], preferred_element_type=F32)
            if u + 1 < nunits:
                zb = (_bits(pv).reshape(SUB // 8, 8, 128)
                      & zero_buf[...][None]).reshape(SUB, 128)
                o = _normalize(raw[0], _float(_bits(raw[1]) | zb))
            else:
                pv_car[0] = raw[0]
                ls_car[0] = raw[1]
            raw = (pv, ls)
        pv_car[1] = raw[0]
        ls_car[1] = raw[1]
        qa_car[...] = qa

    def ramp_block(j):
        o = [_normalize(pv_car[u], ls_car[u]) for u in range(2)]
        w = wo_buf[j - 1]

        def op_part(u, r0, r1, c0, c1):
            acc[u * SUB + r0:u * SUB + r1, c0:c1] += jnp.dot(
                o[u][r0:r1], w[:, c0:c1], preferred_element_type=F32)

        for u in range(2):
            q = (q_acc[j, u * SUB:(u + 1) * SUB, :] * QSCALE).astype(BF16)
            sc = lax.dot_general(q, k_buf[j], NT, preferred_element_type=F32)
            op_part(u, 0, FILL, 0, D // 2)
            m = jnp.max(_lane_fold(sc, jnp.maximum), axis=-1, keepdims=True)
            p = jnp.exp2(sc - m)
            ls_car[u] = _lane_fold(p, jnp.add)
            pv_car[u] = jnp.dot(p.astype(BF16), v_buf[j], preferred_element_type=F32)
            if u == 0:
                for v in range(2):
                    op_part(v, FILL, SUB, 0, D // 2)
                    op_part(v, 0, SUB, D // 2, D)

    def start(cps):
        for c_ in cps:
            c_.start()

    def wait(cps):
        for c_ in cps:
            c_.wait()

    start([cp_c, cp_x(0, 1, SEM_X0), cp_x(1, 1, SEM_X1)])
    for j in range(NST):
        start(cp_m0(j) + [cp_w0(j)])
    start([cp_k0] + cp_v0)
    for j in range(1, R2):
        start(ramp_heads(j))
    start([cp_wr])
    n_early = (LN_START - RAMP) // UM
    for k in range(n_early):
        start(main_heads(k))

    r_buf[...] = jnp.zeros(r_buf.shape, F32)
    zero_buf[...] = jnp.zeros(zero_buf.shape, I32)
    coef[C_GA] = jnp.zeros((8, D), F32)
    coef[C_KEEP] = jnp.zeros((8, D), F32)
    coef[C_GB] = jnp.ones((8, D), F32)
    sw_buf[...] = jnp.zeros(sw_buf.shape, F32)
    w_buf[:, 2 * F:2 * F + 256] = jnp.zeros((D, 256), BF16)

    def zero_q(h, carry):
        q_acc[h] = jnp.zeros((2 * SUB, DH), F32)
        return carry

    lax.fori_loop(0, GE, zero_q, 0)
    cp_c.wait()
    cf = c_buf[...].astype(F32)
    sf = _r(cf * _r(jax.nn.sigmoid(cf)))
    sc_buf[...] = jnp.broadcast_to(sf, (16, D)).astype(BF16)
    for j in range(D // 128):
        scol[j * 128:(j + 1) * 128, :] = jnp.broadcast_to(
            sf[:, j * 128:(j + 1) * 128], (128, 128)).T

    def norm_rows(j, carry):
        @pl.when((j & 1) == 0)
        def _():
            b = lax.shift_right_logical(j, 1)
            cp_x(b, 1, SEM_X0 + b).wait()

        row = pl.multiple_of(j * 128, 128)
        nn = _layernorm(x_buf[pl.ds(row, 128), :].astype(F32))
        for t in range(NST):
            n_buf[t, pl.ds(row, 128), :] = nn[:, t * 128:(t + 1) * 128]
        return carry

    lax.fori_loop(0, 2 * SUB // 128, norm_rows, 0)

    def stage(j, carry):
        wait(cp_m0(j))
        wm = jnp.concatenate([v_buf[H - NST + j, 0:D, :], v_buf[H - NST + j, D:2 * D, :]], axis=1)
        mj = _r(jnp.dot(sc_buf[...], wm, preferred_element_type=F32)[0:8, :])
        coef[C_SHIFT, :, lanes(j)] = mj[:, 0:128]
        coef[C_SCALE, :, lanes(j)] = _r(1.0 + mj[:, 128:256])
        zr = S // NST
        acc[pl.ds(pl.multiple_of(j * zr, zr), zr), :] = jnp.zeros((zr, D), F32)
        cp_w0(j).wait()
        hj = (n_buf[j].reshape(2 * SUB // 8, 8, 128) * coef[C_SCALE, :, lanes(j)][None]
              + coef[C_SHIFT, :, lanes(j)][None]).reshape(2 * SUB, 128).astype(BF16)
        act[0:2 * SUB, lanes(j)] = hj
        part = jnp.dot(hj, w_buf[lanes(j), 4 * D:4 * D + GE * DH], preferred_element_type=F32)
        for h in range(GE):
            q_acc[h] += part[:, h * DH:(h + 1) * DH]
        return carry

    lax.fori_loop(0, NST, stage, 0)

    cp_k0.wait()
    s01 = lax.dot_general((q_acc[0] * QSCALE).astype(BF16), k_buf[0], NT,
                          preferred_element_type=F32)
    mm01 = _lane_fold(s01, jnp.maximum)
    m0 = jnp.max(mm01[0:SUB], axis=-1, keepdims=True)
    wait(cp_v0)
    qa_car[...] = qproj_head(RAMP)
    for u in range(2):
        m = m0 if u == 0 else jnp.max(mm01[SUB:], axis=-1, keepdims=True)
        p = jnp.exp2(s01[u * SUB:(u + 1) * SUB] - m)
        ls_car[u] = _lane_fold(p, jnp.add)
        pv_car[u] = jnp.dot(p.astype(BF16), v_buf[0], preferred_element_type=F32)
    for h in range(GE, R2):
        q_acc[h] = jnp.dot(act[0:2 * SUB, :], wq_buf[h], preferred_element_type=F32)

    def ramp2(j, carry):
        wait(ramp_heads(j))
        ramp_block(j)
        return carry

    lax.fori_loop(1, R2, ramp2, 0)
    start([cp_x(2, NRB - 2, SEM_XR)])
    for k in range(n_early, NLOAD):
        start(main_heads(k, k == NLOAD - 1))
    start(cp_wqe + cp_m12)

    assert FIN_START + row0 // PR <= RAMP + (NM - 1) * UM

    def main(k, carry):
        n0 = RAMP + k * UM

        @pl.when(k <= K_MOD + 2)
        def _():
            @pl.when(k < NLOAD - 1)
            def _():
                wait(main_heads(k))

            @pl.when(k == NLOAD - 1)
            def _():
                wait(main_heads(NLOAD - 1, True) + cp_wqe)

            @pl.when(k == n_early)
            def _():
                cp_x(2, NRB - 2, SEM_XR).wait()

            @pl.when(k == MV_K0)
            def _():
                wait(cp_m12)

            @pl.when(k == K_MOD)
            def _():
                cp_wr.wait()
                mm = _r(jnp.broadcast_to(jnp.sum(m_raw[:, 0:4 * D], axis=0, keepdims=True),
                                         (8, 4 * D)))
                m1 = mm[:, 0:D]
                m2 = mm[:, D:4 * D]
                coef[C_GA] = m1
                coef[C_KEEP] = jnp.ones((8, D), F32)
                scale = _r(1.0 + m2[:, D:2 * D])
                coef[C_SHIFT] = m2[:, 0:D]
                coef[C_SCALE] = scale
                coef[C_GB] = m2[:, 2 * D:3 * D]
                w8 = wr_buf[...].astype(F32)
                wr = jnp.concatenate([jnp.broadcast_to(w8[j:j + 1, :], (8, 128))
                                      for j in range(D // 128)], axis=1)
                sw_buf[...] = scale * wr
                c1 = jnp.sum(scale * wr, axis=-1, keepdims=True)
                c0 = jnp.sum(m2[:, 0:D] * wr, axis=-1, keepdims=True)
                rid = lax.broadcasted_iota(I32, (8, 128), 0)
                rc_buf[...] = jnp.where(rid == 0, c1, c0)
                start(cp_ffn)

            @pl.when(k == K_MOD + 2)
            def _():
                wait(cp_ffn)

        @pl.when(k == NM - 1)
        def _():
            cp_out[0].start()

        unit_block(k, n0, UM)
        return carry

    lax.fori_loop(0, NM, main, 0)

    neg = -jnp.inf

    def keep_rows(y, lo):
        n = y.shape[0]
        yc, m, mr, den = _ln_stats(y)
        rinv = _recip(den)
        x2_buf[lo:lo + n, :] = y
        st_buf[0, lo:lo + n, :] = jnp.broadcast_to(mr, (n, 128))
        st_buf[1, lo:lo + n, :] = jnp.broadcast_to(rinv, (n, 128))
        d = jnp.sum(_rows8(yc, jnp.multiply, sw_buf[...]), axis=-1, keepdims=True)
        return _r((d + (m - mr) * rc_buf[0:1, 0:1]) * rinv + rc_buf[1:2, 0:1])

    def parked(lo, n):
        y = x2_buf[pl.ds(lo, n), :]
        mr = st_buf[0, pl.ds(lo, n), :]
        rinv = st_buf[1, pl.ds(lo, n), :]
        return y, jnp.concatenate([(y[:, j * 128:(j + 1) * 128] - mr) * rinv
                                   for j in range(D // 128)], axis=1)

    def all_red(v, fn):
        return fn(fn(v, axis=0, keepdims=True), axis=1, keepdims=True)

    lane = lax.broadcasted_iota(I32, (PR, 128), 1)
    ridx = (lane * PR + lax.broadcasted_iota(I32, (PR, 128), 0)).astype(F32)
    rr = jnp.where(lane < row0 // PR, _r(r_buf[...] + rc_buf[1:2, :]), neg)
    last_old = float(row0 - 1)
    cm1 = all_red(rr, jnp.max)
    ci1 = all_red(jnp.where(rr == cm1, ridx, last_old), jnp.min)
    rr2 = jnp.where(ridx == ci1, neg, rr)
    cm2 = all_red(rr2, jnp.max)
    ci2 = all_red(jnp.where(jnp.logical_and(rr2 == cm2, ridx != ci1), ridx, last_old), jnp.min)
    ci1 = jnp.minimum(ci1, last_old).astype(I32)
    ci2 = jnp.minimum(ci2, last_old).astype(I32)
    for j, ci in enumerate((ci1, ci2)):
        g = pl.multiple_of(lax.shift_right_logical(ci[0, 0], 4) * PR, PR)
        keep_rows(resid(acc[pl.ds(g, PR), :], g, PR), SUB + j * PR)

    o2 = jnp.concatenate([_normalize(pv_car[0], ls_car[0]),
                          _normalize(pv_car[1], ls_car[1])], axis=1)
    wo2 = jnp.concatenate([wo_buf[H - 2], wo_buf[H - 1]], axis=0)
    r_new = []
    for j in range(SUB // ECH):
        lo, hi = j * ECH, (j + 1) * ECH
        a = acc[row0 + lo:row0 + hi, :] + jnp.dot(o2[lo:hi], wo2, preferred_element_type=F32)
        r_new.append(keep_rows(resid(a, row0 + lo, ECH), lo))

    sub8 = lax.broadcasted_iota(I32, (8, 1), 0)
    big = jnp.int32((S - 1) * 512 + SUB - 1)
    vals = jnp.concatenate(
        r_new + [jnp.where(sub8 == 0, cm1, jnp.where(sub8 == 1, cm2, neg))], axis=0)
    pos = lax.broadcasted_iota(I32, (SUB, 1), 0)
    cc1 = ci1 * 512 + SUB + (ci1 & (PR - 1))
    cc2 = ci2 * 512 + SUB + PR + (ci2 & (PR - 1))
    code = jnp.concatenate(
        [(pos + row0) * 512 + pos,
         jnp.where(sub8 == 0, cc1, jnp.where(sub8 == 1, cc2, big))], axis=0)
    m1 = jnp.max(vals, axis=0, keepdims=True)
    k1 = jnp.min(jnp.where(vals == m1, code, big), axis=0, keepdims=True)
    vals2 = jnp.where(code == k1, neg, vals)
    m2 = jnp.max(vals2, axis=0, keepdims=True)
    k2 = jnp.min(jnp.where(jnp.logical_and(vals2 == m2, code != k1), code, big),
                 axis=0, keepdims=True)
    k1 = k1[0, 0]
    k2 = k2[0, 0]
    i1 = lax.shift_right_logical(k1, 9)
    i2 = lax.shift_right_logical(k2, 9)
    t1 = k1 & 511
    t2 = k2 & 511
    rowid = lax.broadcasted_iota(I32, (PR, D), 0)
    xf = modulate(jnp.where(rowid == 0, parked(t1, 1)[1], parked(t2, 1)[1]))

    off = pl.multiple_of(jnp.minimum(k2, 0) * 8, 8)
    for j in range(SUB // PR):
        yl, nl = parked(pl.multiple_of(off + j * PR, 8), PR)
        act[row0 + j * PR:row0 + (j + 1) * PR, :] = (
            yl + _rows8(modulate(nl), jnp.multiply, coef[C_GB])).astype(BF16)
    cp_out[1].start()

    gt = _r(jnp.dot(xf.astype(BF16), w_buf[:, 0:F], preferred_element_type=F32)[0:8])
    zt = _bits(act[pl.ds(pl.multiple_of(off * 2, PR), PR), 0:128].astype(F32))
    zt = jnp.concatenate([zt[0:8] & zero_buf[...], zt[8:16] & zero_buf[...]], axis=0)
    xs = jnp.concatenate([_float(_bits(xf[:, 0:128]) | zt), xf[:, 128:]], axis=1).astype(BF16)
    up = _r(jnp.dot(xs, w_buf[:, F:2 * F], preferred_element_type=F32)[0:8])
    hid = _r(gt * _r(jax.nn.sigmoid(gt))) * up
    hid = jnp.concatenate([hid, hid], axis=0).astype(BF16)
    y = _r(jnp.dot(hid, wd_buf[:, 0:D], preferred_element_type=F32)[0:8])
    y1 = _r(y[0:1, :] * _r(jax.nn.sigmoid(m1)))
    y2 = _r(y[1:2, :] * _r(jax.nn.sigmoid(m2)))

    def fix(i, t):
        g = pl.multiple_of(lax.shift_right_logical(i, 4) * PR, PR)
        tg = pl.multiple_of(lax.shift_right_logical(t, 4) * PR, PR)
        rid = rowid + g
        upd = jnp.where(rid == i1, y1, jnp.where(rid == i2, y2, 0.0))
        yg, ng = parked(tg, PR)
        return g, (yg + _rows8(modulate(ng) + upd, jnp.multiply, coef[C_GB])).astype(BF16)

    g1, fix1 = fix(i1, t1)
    g2, fix2 = fix(i2, t2)
    wait(cp_out)
    act[pl.ds(g1, PR), :] = fix1
    act[pl.ds(g2, PR), :] = fix2
    f1 = cp(act.at[pl.ds(g1, PR), :], out_hbm.at[pl.ds(g1, PR), :], SEM_OUT)
    f2 = cp(act.at[pl.ds(g2, PR), :], out_hbm.at[pl.ds(g2, PR), :], SEM_FIX)
    f1.start()

    @pl.when(g1 != g2)
    def _():
        f2.start()
        f2.wait()

    f1.wait()


@jax.jit
def pallas_adaLN_cond__mha_block_cached__moe_arch_mod__prompt_kernel(
    A_x: jax.Array,
    A_k_cache: jax.Array,
    A_v_cache: jax.Array,
    A_wq: jax.Array,
    A_wo: jax.Array,
    B_x: jax.Array,
    B_w_r: jax.Array,
    B_w_gate: jax.Array,
    B_w_up: jax.Array,
    B_w_down: jax.Array,
    c: jax.Array,
    w_mod: jax.Array,
):
    del B_x
    hbm = pl.BlockSpec(memory_space=pl.ANY)
    out = pl.pallas_call(
        _kernel,
        in_specs=[hbm] * 11,
        out_specs=hbm,
        out_shape=jax.ShapeDtypeStruct((S, D), BF16),
        scratch_shapes=[
            pltpu.VMEM((S, D), BF16),
            pltpu.VMEM((H, S, DH), BF16),
            pltpu.VMEM((H, S, DH), BF16),
            pltpu.VMEM((H, D, DH), BF16),
            pltpu.VMEM((H, DH, D), BF16),
            pltpu.VMEM((D, WW), BF16),
            pltpu.VMEM((F, D + PAD), BF16),
            pltpu.VMEM((S + PR, D), BF16),
            pltpu.VMEM((S, D), F32),
            pltpu.VMEM((NST, 2 * SUB, 128), F32),
            pltpu.VMEM((R2, 2 * SUB, DH), F32),
            pltpu.VMEM((SUB + 2 * PR, D), F32),
            pltpu.VMEM((2, SUB + 2 * PR, 128), F32),
            pltpu.VMEM((PR, 128), F32),
            pltpu.VMEM((5, 8, D), F32),
            pltpu.VMEM((8, 128), BF16),
            pltpu.VMEM((8, D), F32),
            pltpu.VMEM((8, 128), F32),
            pltpu.VMEM((1, D), BF16),
            pltpu.VMEM((16, D), BF16),
            pltpu.VMEM((D, 128), F32),
            pltpu.VMEM((8, 4 * D + 256), F32),
            pltpu.VMEM((8, 128), I32),
            pltpu.VMEM((FILL, DH), F32),
            pltpu.VMEM((2, SUB, DH), F32),
            pltpu.VMEM((2, SUB, DH), F32),
            pltpu.SemaphoreType.DMA((NSEM,)),
        ],
        compiler_params=pltpu.CompilerParams(
            vmem_limit_bytes=120 * 1024 * 1024,
            disable_bounds_checks=True,
            disable_semaphore_checks=True,
        ),
        name="adaln_mha_mod",
    )(
        A_x.reshape(S, D),
        A_k_cache.reshape(H, S, DH),
        A_v_cache.reshape(H, S, DH),
        A_wq,
        A_wo.reshape(H, DH, D),
        B_w_r.reshape(8, 128),
        B_w_gate,
        B_w_up,
        B_w_down,
        c,
        w_mod,
    )
    return out.reshape(1, S, D)
```

```python
import jax
import jax.numpy as jnp
from jax import lax
import jax.experimental.pallas as pl
import jax.experimental.pallas.tpu as pltpu

S = 2048
D = 1024
H = 32
DH = 128
F = 3584
SUB = 256
NRB = S // SUB
NU = H * NRB
PR = 16
UM = 14
GE = 8
R2 = 9
RAMP = 2 * R2
NM = (NU - RAMP) // UM
HPI = UM // 2
NLOAD = (2 * H - RAMP) // UM
FIN_START = 130
K_MOD = (FIN_START - RAMP) // UM
LN_START = RAMP + UM
assert LN_START <= 33 and LN_START + (S - 2 * SUB) // PR <= RAMP + K_MOD * UM
FILL = 64
ECH = 64
PAD = 128
NST = D // 128
MVN = 3
MV_K0 = 2
assert (K_MOD - MV_K0) * MVN >= 4 * D // 256
WW = 2 * F + 256 + PAD
EPS = 1e-5
QSCALE = float(DH ** -0.5) * 1.4426950408889634

F32 = jnp.float32
BF16 = jnp.bfloat16
I32 = jnp.int32
NT = (((1,), (1,)), ((), ()))

C_GA, C_SCALE, C_SHIFT, C_KEEP, C_GB = range(5)


def _r(v):
    return v.astype(BF16).astype(F32)


def _bits(v):
    return lax.bitcast_convert_type(v, I32)


def _float(v):
    return lax.bitcast_convert_type(v, F32)


def _rows8(v, fn, c):
    n = v.shape[0] // 8
    return fn(v.reshape(n, 8, D), c[None]).reshape(v.shape)


def _recip(v):
    r = pl.reciprocal(v, approx=True)
    return r * (2.0 - v * r)


def _ln_stats(y):
    m = jnp.mean(y, axis=-1, keepdims=True)
    yc = y - m
    v = jnp.mean(yc * yc, axis=-1, keepdims=True)
    return yc, m, _r(m), _r(jnp.sqrt(_r(_r(v) + EPS)))


def _layernorm(y):
    _, _, mr, den = _ln_stats(y)
    return (y - mr) * (1.0 / den)


def _lane_fold(p, fn):
    t = p[:, 0:128]
    for j in range(1, p.shape[1] // 128):
        t = fn(t, p[:, j * 128:(j + 1) * 128])
    return t


def _normalize(pv, ls):
    return (pv * _recip(jnp.sum(ls, axis=-1, keepdims=True))).astype(BF16)


def _head_of(n):
    if isinstance(n, int):
        return (n % 64) // 2 if n < 192 else (n - 192) % H
    return jnp.where(n < 192, lax.shift_right_logical(n & 63, 1), (n - 192) & (H - 1))


def _row_of(n):
    if isinstance(n, int):
        return SUB * ((n // 64) * 2 + n % 2 if n < 192 else min(n // 32, NRB - 1))
    rb = jnp.where(n < 192, lax.shift_right_logical(n, 6) * 2 + (n & 1),
                   jnp.minimum(lax.shift_right_logical(n, 5), NRB - 1))
    return pl.multiple_of(rb * SUB, SUB)


(SEM_C, SEM_WR, SEM_X0, SEM_X1, SEM_XR, SEM_M12, SEM_FFN, SEM_OUT, SEM_FIX,
 SEM_K0, SEM_WQE, SEM_M0) = range(12)
SEM_W0 = SEM_M0 + NST
SEM_RAMP = SEM_W0 + NST
SEM_MAIN = SEM_RAMP + R2
NSEM = SEM_MAIN + NLOAD


def _kernel(x_hbm, k_hbm, v_hbm, wq_hbm, wo_hbm, wr_hbm, wg_hbm, wu_hbm, wd_hbm,
            c_hbm, wmod_hbm, out_hbm,
            x_buf, k_buf, v_buf, wq_buf, wo_buf, w_buf, wd_buf,
            act, acc, n_buf, q_acc, x2_buf, st_buf, r_buf, coef, wr_buf, sw_buf, rc_buf,
            c_buf, sc_buf, scol, m_raw, zero_buf, qa_car, pv_car, ls_car,
            sems):
    def cp(src, dst, slot):
        return pltpu.make_async_copy(src, dst, sems.at[slot])

    def cp_x(b, nb, slot):
        return cp(x_hbm.at[pl.ds(b * SUB, nb * SUB), :],
                  x_buf.at[pl.ds(b * SUB, nb * SUB), :], slot)

    def cp_wq(h, slot):
        col = h * DH if isinstance(h, int) else pl.multiple_of(h * DH, DH)
        return cp(wq_hbm.at[:, pl.ds(col, DH)], wq_buf.at[h], slot)

    def cp_h(src, dst, h0, nh, slot):
        return cp(src.at[pl.ds(h0, nh)], dst.at[pl.ds(h0, nh)], slot)

    def heads(h0, nh, slot, last=False):
        return [cp_h(k_hbm, k_buf, h0, nh, slot), cp_h(v_hbm, v_buf, h0, nh, slot),
                cp_h(wo_hbm, wo_buf, h0 - 1, nh + 1 if last else nh, slot)] + [
            cp_wq(h0 + 1 + j, slot) for j in range(nh - 1 if last else nh)]

    def ramp_heads(j):
        return [cp_h(k_hbm, k_buf, j, 1, SEM_RAMP + j), cp_h(v_hbm, v_buf, j, 1, SEM_RAMP + j),
                cp_h(wo_hbm, wo_buf, j - 1, 1, SEM_RAMP + j)]

    def main_heads(k, last=False):
        h0 = R2 + k * HPI
        return heads(h0, H - h0 if last else HPI, SEM_MAIN + k, last)

    cp_k0 = cp_h(k_hbm, k_buf, 0, 1, SEM_K0)
    cp_v0 = [cp_h(v_hbm, v_buf, 0, 1, SEM_RAMP)] + [cp_wq(h, SEM_RAMP) for h in range(GE, R2 + 1)]
    cp_wqe = [cp_wq(h, SEM_WQE) for h in range(GE)]

    def lanes(j):
        return pl.ds(j * 128 if isinstance(j, int) else pl.multiple_of(j * 128, 128), 128)

    def cp_m0(j):
        return [cp(wmod_hbm.at[:, lanes(u * NST + j)],
                   v_buf.at[H - NST + j, u * D:(u + 1) * D, :], SEM_M0 + j) for u in range(2)]

    def cp_w0(j):
        return cp(wq_hbm.at[lanes(j), 0:GE * DH], w_buf.at[lanes(j), 4 * D:4 * D + GE * DH], SEM_W0 + j)

    cp_c = cp(c_hbm, c_buf, SEM_C)
    cp_wr = cp(wr_hbm, wr_buf, SEM_WR)
    cp_m12 = [cp(wmod_hbm.at[:, 2 * D:6 * D], w_buf.at[:, 0:4 * D], SEM_M12)]
    cp_ffn = [cp(wg_hbm, w_buf.at[:, 0:F], SEM_FFN),
              cp(wu_hbm, w_buf.at[:, F:2 * F], SEM_FFN),
              cp(wd_hbm, wd_buf.at[:, 0:D], SEM_FFN)]

    row0 = (NRB - 1) * SUB
    cp_out = [cp(act.at[0:row0, :], out_hbm.at[0:row0, :], SEM_OUT),
              cp(act.at[row0:S, :], out_hbm.at[row0:S, :], SEM_OUT)]

    def mod_slice(idx):
        live = jnp.logical_and(idx >= 0, idx < 4 * D // 256)
        src = pl.multiple_of(jnp.where(live, idx * 256, 2 * F), 128)
        dst = pl.multiple_of(jnp.where(live, idx * 256, 4 * D), 128)
        a = None
        for g in range(D // 8):
            wv = w_buf[g * 8:(g + 1) * 8, pl.ds(src, 256)].astype(F32)
            sv = scol[g * 8:(g + 1) * 8, :]
            pr = jnp.concatenate([wv[:, 0:128] * sv, wv[:, 128:256] * sv], axis=1)
            a = pr if a is None else a + pr
        m_raw[:, pl.ds(dst, 256)] = a
        return _lane_fold(_bits(a), jnp.bitwise_or) & zero_buf[...]

    def modulate(n):
        n = _rows8(n, jnp.multiply, coef[C_SCALE])
        return _rows8(n, jnp.add, coef[C_SHIFT])

    def resid(a, row, nrows):
        a = _rows8(a, jnp.multiply, coef[C_GA])
        return _r(x_buf[pl.ds(row, nrows), :].astype(F32) + a)

    def piece(src, dst, lane_id):
        y = resid(acc[pl.ds(src, PR), :], src, PR)
        nn = _layernorm(y)
        hh = modulate(nn)
        r = jnp.sum(_rows8(nn, jnp.multiply, sw_buf[...]), axis=-1, keepdims=True)
        oo = (_rows8(y, jnp.multiply, coef[C_KEEP])
              + _rows8(hh, jnp.multiply, coef[C_GB]))
        act[pl.ds(dst, PR), :] = oo.astype(BF16)
        lane = lax.broadcasted_iota(I32, (PR, 128), 1)
        rn = jnp.where(lane == lane_id, r, r_buf[...])
        r_buf[...] = rn
        return oo, rn

    def unit_piece(n):
        is_ln = jnp.logical_and(n >= LN_START, n < LN_START + (S - 2 * SUB) // PR)
        is_fin = jnp.logical_and(n >= FIN_START, n < FIN_START + (S - SUB) // PR)
        f = n - FIN_START
        src = jnp.where(is_ln, 2 * SUB + (n - LN_START) * PR, jnp.where(is_fin, f * PR, 0))
        dst = jnp.where(jnp.logical_or(is_ln, is_fin), src, S)
        oo, rn = piece(pl.multiple_of(src, PR), pl.multiple_of(dst, PR),
                       jnp.where(is_fin, f, -1))
        bits = _lane_fold(_bits(oo), jnp.bitwise_or) | _bits(rn)
        return (bits[0:8] | bits[8:16]) & zero_buf[...]

    def qproj_head(n):
        return jnp.dot(act[pl.ds(_row_of(n), FILL), 0:D // 2],
                       wq_buf[_head_of(n)][0:D // 2], preferred_element_type=F32)

    def qproj_rest(n, qa):
        row = _row_of(n)
        w = wq_buf[_head_of(n)]
        row2 = row + FILL if isinstance(row, int) else pl.multiple_of(row + FILL, 16)
        qb = jnp.dot(act[pl.ds(row, SUB), D // 2:D], w[D // 2:D], preferred_element_type=F32)
        qc = jnp.dot(act[pl.ds(row2, SUB - FILL), 0:D // 2], w[0:D // 2],
                     preferred_element_type=F32)
        return ((qb + jnp.concatenate([qa, qc], axis=0)) * QSCALE).astype(BF16)

    def oproj(o, n):
        acc[pl.ds(_row_of(n), SUB), :] += jnp.dot(o, wo_buf[_head_of(n)],
                                                  preferred_element_type=F32)

    def unit_block(k, n0, nunits):
        o = _normalize(pv_car[0], ls_car[0])
        raw = (pv_car[1], ls_car[1])
        qa = qa_car[...]
        for u in range(nunits):
            n = n0 + u
            hd = _head_of(n)
            q = qproj_rest(n, qa)
            z = unit_piece(n)
            if u < MVN:
                z = z | mod_slice((k - MV_K0) * MVN + u)
            oproj(o, n - 2)
            sc = lax.dot_general(q, k_buf[hd], NT, preferred_element_type=F32)
            qa = qproj_head(n + 1)
            mm = _lane_fold(sc, jnp.maximum)
            mm = jnp.concatenate([_float(_bits(mm[0:8]) | z), mm[8:]], axis=0)
            m = jnp.max(mm, axis=-1, keepdims=True)
            p = jnp.exp2(sc - m)
            ls = _lane_fold(p, jnp.add)
            pv = jnp.dot(p.astype(BF16), v_buf[hd], preferred_element_type=F32)
            if u + 1 < nunits:
                zb = (_bits(pv).reshape(SUB // 8, 8, 128)
                      & zero_buf[...][None]).reshape(SUB, 128)
                o = _normalize(raw[0], _float(_bits(raw[1]) | zb))
            else:
                pv_car[0] = raw[0]
                ls_car[0] = raw[1]
            raw = (pv, ls)
        pv_car[1] = raw[0]
        ls_car[1] = raw[1]
        qa_car[...] = qa

    def early_oproj(u, nrows, w):
        ri = _recip(jnp.sum(ls_car[u, 0:nrows, :], axis=-1, keepdims=True))
        return jnp.dot(pv_car[u, 0:nrows, :].astype(BF16), w, preferred_element_type=F32) * ri

    def ramp_block(j):
        o = [_normalize(pv_car[u], ls_car[u]) for u in range(2)]
        w = wo_buf[j - 1]

        def op_part(u, r0, r1, c0, c1):
            acc[u * SUB + r0:u * SUB + r1, c0:c1] += jnp.dot(
                o[u][r0:r1], w[:, c0:c1], preferred_element_type=F32)

        acc[0:FILL, D // 2:D] += early_oproj(0, FILL, w[:, D // 2:D])
        for u in range(2):
            q = (q_acc[j, u * SUB:(u + 1) * SUB, :] * QSCALE).astype(BF16)
            sc = lax.dot_general(q, k_buf[j], NT, preferred_element_type=F32)
            op_part(u, 0, FILL, 0, D // 2)
            m = jnp.max(_lane_fold(sc, jnp.maximum), axis=-1, keepdims=True)
            p = jnp.exp2(sc - m)
            ls_car[u] = _lane_fold(p, jnp.add)
            pv_car[u] = jnp.dot(p.astype(BF16), v_buf[j], preferred_element_type=F32)
            if u == 0:
                for v in range(2):
                    op_part(v, FILL, SUB, 0, D // 2)
                    op_part(v, FILL if v == 0 else 0, SUB, D // 2, D)

    def start(cps):
        for c_ in cps:
            c_.start()

    def wait(cps):
        for c_ in cps:
            c_.wait()

    start([cp_c, cp_x(0, 1, SEM_X0), cp_x(1, 1, SEM_X1)])
    for j in range(NST):
        start(cp_m0(j) + [cp_w0(j)])
    start([cp_k0] + cp_v0)
    for j in range(1, R2):
        start(ramp_heads(j))
    start([cp_wr])
    n_early = (LN_START - RAMP) // UM
    for k in range(n_early):
        start(main_heads(k))

    r_buf[...] = jnp.zeros(r_buf.shape, F32)
    zero_buf[...] = jnp.zeros(zero_buf.shape, I32)
    coef[C_GA] = jnp.zeros((8, D), F32)
    coef[C_KEEP] = jnp.zeros((8, D), F32)
    coef[C_GB] = jnp.ones((8, D), F32)
    sw_buf[...] = jnp.zeros(sw_buf.shape, F32)
    w_buf[:, 2 * F:2 * F + 256] = jnp.zeros((D, 256), BF16)

    def zero_q(h, carry):
        q_acc[h] = jnp.zeros((2 * SUB, DH), F32)
        return carry

    lax.fori_loop(0, GE, zero_q, 0)
    cp_c.wait()
    cf = c_buf[...].astype(F32)
    sf = _r(cf * _r(jax.nn.sigmoid(cf)))
    sc_buf[...] = jnp.broadcast_to(sf, (16, D)).astype(BF16)
    for j in range(D // 128):
        scol[j * 128:(j + 1) * 128, :] = jnp.broadcast_to(
            sf[:, j * 128:(j + 1) * 128], (128, 128)).T

    def norm_rows(j, carry):
        @pl.when((j & 1) == 0)
        def _():
            b = lax.shift_right_logical(j, 1)
            cp_x(b, 1, SEM_X0 + b).wait()

        row = pl.multiple_of(j * 128, 128)
        nn = _layernorm(x_buf[pl.ds(row, 128), :].astype(F32))
        for t in range(NST):
            n_buf[t, pl.ds(row, 128), :] = nn[:, t * 128:(t + 1) * 128]
        return carry

    lax.fori_loop(0, 2 * SUB // 128, norm_rows, 0)

    def stage(j, carry):
        wait(cp_m0(j))
        wm = jnp.concatenate([v_buf[H - NST + j, 0:D, :], v_buf[H - NST + j, D:2 * D, :]], axis=1)
        mj = _r(jnp.dot(sc_buf[...], wm, preferred_element_type=F32)[0:8, :])
        coef[C_SHIFT, :, lanes(j)] = mj[:, 0:128]
        coef[C_SCALE, :, lanes(j)] = _r(1.0 + mj[:, 128:256])
        zr = S // NST
        acc[pl.ds(pl.multiple_of(j * zr, zr), zr), :] = jnp.zeros((zr, D), F32)
        cp_w0(j).wait()
        hj = (n_buf[j].reshape(2 * SUB // 8, 8, 128) * coef[C_SCALE, :, lanes(j)][None]
              + coef[C_SHIFT, :, lanes(j)][None]).reshape(2 * SUB, 128).astype(BF16)
        act[0:2 * SUB, lanes(j)] = hj
        part = jnp.dot(hj, w_buf[lanes(j), 4 * D:4 * D + GE * DH], preferred_element_type=F32)
        for h in range(GE):
            q_acc[h] += part[:, h * DH:(h + 1) * DH]
        return carry

    lax.fori_loop(0, NST, stage, 0)

    cp_k0.wait()
    s01 = lax.dot_general((q_acc[0] * QSCALE).astype(BF16), k_buf[0], NT,
                          preferred_element_type=F32)
    mm01 = _lane_fold(s01, jnp.maximum)
    m0 = jnp.max(mm01[0:SUB], axis=-1, keepdims=True)
    wait(cp_v0)
    qa_car[...] = qproj_head(RAMP)
    for u in range(2):
        m = m0 if u == 0 else jnp.max(mm01[SUB:], axis=-1, keepdims=True)
        p = jnp.exp2(s01[u * SUB:(u + 1) * SUB] - m)
        ls_car[u] = _lane_fold(p, jnp.add)
        pv_car[u] = jnp.dot(p.astype(BF16), v_buf[0], preferred_element_type=F32)
    for h in range(GE, R2):
        q_acc[h] = jnp.dot(act[0:2 * SUB, :], wq_buf[h], preferred_element_type=F32)

    def ramp2(j, carry):
        wait(ramp_heads(j))
        ramp_block(j)
        return carry

    lax.fori_loop(1, R2, ramp2, 0)
    start([cp_x(2, NRB - 2, SEM_XR)])
    for k in range(n_early, NLOAD):
        start(main_heads(k, k == NLOAD - 1))
    start(cp_wqe + cp_m12)

    assert FIN_START + row0 // PR <= RAMP + (NM - 1) * UM

    def main(k, carry):
        n0 = RAMP + k * UM

        @pl.when(k <= K_MOD + 2)
        def _():
            @pl.when(k < NLOAD - 1)
            def _():
                wait(main_heads(k))

            @pl.when(k == NLOAD - 1)
            def _():
                wait(main_heads(NLOAD - 1, True) + cp_wqe)

            @pl.when(k == n_early)
            def _():
                cp_x(2, NRB - 2, SEM_XR).wait()

            @pl.when(k == MV_K0)
            def _():
                wait(cp_m12)

            @pl.when(k == K_MOD)
            def _():
                cp_wr.wait()
                mm = _r(jnp.broadcast_to(jnp.sum(m_raw[:, 0:4 * D], axis=0, keepdims=True),
                                         (8, 4 * D)))
                m1 = mm[:, 0:D]
                m2 = mm[:, D:4 * D]
                coef[C_GA] = m1
                coef[C_KEEP] = jnp.ones((8, D), F32)
                scale = _r(1.0 + m2[:, D:2 * D])
                coef[C_SHIFT] = m2[:, 0:D]
                coef[C_SCALE] = scale
                coef[C_GB] = m2[:, 2 * D:3 * D]
                w8 = wr_buf[...].astype(F32)
                wr = jnp.concatenate([jnp.broadcast_to(w8[j:j + 1, :], (8, 128))
                                      for j in range(D // 128)], axis=1)
                sw_buf[...] = scale * wr
                c1 = jnp.sum(scale * wr, axis=-1, keepdims=True)
                c0 = jnp.sum(m2[:, 0:D] * wr, axis=-1, keepdims=True)
                rid = lax.broadcasted_iota(I32, (8, 128), 0)
                rc_buf[...] = jnp.where(rid == 0, c1, c0)
                start(cp_ffn)

            @pl.when(k == K_MOD + 2)
            def _():
                wait(cp_ffn)

        @pl.when(k == NM - 1)
        def _():
            cp_out[0].start()

        unit_block(k, n0, UM)
        return carry

    lax.fori_loop(0, NM, main, 0)

    neg = -jnp.inf

    def keep_rows(y, lo):
        n = y.shape[0]
        yc, m, mr, den = _ln_stats(y)
        rinv = _recip(den)
        x2_buf[lo:lo + n, :] = y
        st_buf[0, lo:lo + n, :] = jnp.broadcast_to(mr, (n, 128))
        st_buf[1, lo:lo + n, :] = jnp.broadcast_to(rinv, (n, 128))
        d = jnp.sum(_rows8(yc, jnp.multiply, sw_buf[...]), axis=-1, keepdims=True)
        return _r((d + (m - mr) * rc_buf[0:1, 0:1]) * rinv + rc_buf[1:2, 0:1])

    def parked(lo, n):
        y = x2_buf[pl.ds(lo, n), :]
        mr = st_buf[0, pl.ds(lo, n), :]
        rinv = st_buf[1, pl.ds(lo, n), :]
        return y, jnp.concatenate([(y[:, j * 128:(j + 1) * 128] - mr) * rinv
                                   for j in range(D // 128)], axis=1)

    def all_red(v, fn):
        return fn(fn(v, axis=0, keepdims=True), axis=1, keepdims=True)

    lane = lax.broadcasted_iota(I32, (PR, 128), 1)
    ridx = (lane * PR + lax.broadcasted_iota(I32, (PR, 128), 0)).astype(F32)
    rr = jnp.where(lane < row0 // PR, _r(r_buf[...] + rc_buf[1:2, :]), neg)
    last_old = float(row0 - 1)
    cm1 = all_red(rr, jnp.max)
    ci1 = all_red(jnp.where(rr == cm1, ridx, last_old), jnp.min)
    rr2 = jnp.where(ridx == ci1, neg, rr)
    cm2 = all_red(rr2, jnp.max)
    ci2 = all_red(jnp.where(jnp.logical_and(rr2 == cm2, ridx != ci1), ridx, last_old), jnp.min)
    ci1 = jnp.minimum(ci1, last_old).astype(I32)
    ci2 = jnp.minimum(ci2, last_old).astype(I32)
    for j, ci in enumerate((ci1, ci2)):
        g = pl.multiple_of(lax.shift_right_logical(ci[0, 0], 4) * PR, PR)
        keep_rows(resid(acc[pl.ds(g, PR), :], g, PR), SUB + j * PR)

    o2 = jnp.concatenate([_normalize(pv_car[0], ls_car[0]),
                          _normalize(pv_car[1], ls_car[1])], axis=1)
    wo2 = jnp.concatenate([wo_buf[H - 2], wo_buf[H - 1]], axis=0)
    r_new = []
    for j in range(SUB // ECH):
        lo, hi = j * ECH, (j + 1) * ECH
        a = acc[row0 + lo:row0 + hi, :]
        if j == 0:
            a = a + early_oproj(0, ECH, wo_buf[H - 2]) + early_oproj(1, ECH, wo_buf[H - 1])
        else:
            a = a + jnp.dot(o2[lo:hi], wo2, preferred_element_type=F32)
        r_new.append(keep_rows(resid(a, row0 + lo, ECH), lo))

    sub8 = lax.broadcasted_iota(I32, (8, 1), 0)
    big = jnp.int32((S - 1) * 512 + SUB - 1)
    vals = jnp.concatenate(
        r_new + [jnp.where(sub8 == 0, cm1, jnp.where(sub8 == 1, cm2, neg))], axis=0)
    pos = lax.broadcasted_iota(I32, (SUB, 1), 0)
    cc1 = ci1 * 512 + SUB + (ci1 & (PR - 1))
    cc2 = ci2 * 512 + SUB + PR + (ci2 & (PR - 1))
    code = jnp.concatenate(
        [(pos + row0) * 512 + pos,
         jnp.where(sub8 == 0, cc1, jnp.where(sub8 == 1, cc2, big))], axis=0)
    m1 = jnp.max(vals, axis=0, keepdims=True)
    k1 = jnp.min(jnp.where(vals == m1, code, big), axis=0, keepdims=True)
    vals2 = jnp.where(code == k1, neg, vals)
    m2 = jnp.max(vals2, axis=0, keepdims=True)
    k2 = jnp.min(jnp.where(jnp.logical_and(vals2 == m2, code != k1), code, big),
                 axis=0, keepdims=True)
    k1 = k1[0, 0]
    k2 = k2[0, 0]
    i1 = lax.shift_right_logical(k1, 9)
    i2 = lax.shift_right_logical(k2, 9)
    t1 = k1 & 511
    t2 = k2 & 511
    rowid = lax.broadcasted_iota(I32, (PR, D), 0)
    xf = modulate(jnp.where(rowid == 0, parked(t1, 1)[1], parked(t2, 1)[1]))

    off = pl.multiple_of(jnp.minimum(k2, 0) * 8, 8)
    for j in range(SUB // PR):
        yl, nl = parked(pl.multiple_of(off + j * PR, 8), PR)
        act[row0 + j * PR:row0 + (j + 1) * PR, :] = (
            yl + _rows8(modulate(nl), jnp.multiply, coef[C_GB])).astype(BF16)
    cp_out[1].start()

    gt = _r(jnp.dot(xf.astype(BF16), w_buf[:, 0:F], preferred_element_type=F32)[0:8])
    zt = _bits(act[pl.ds(pl.multiple_of(off * 2, PR), PR), 0:128].astype(F32))
    zt = jnp.concatenate([zt[0:8] & zero_buf[...], zt[8:16] & zero_buf[...]], axis=0)
    xs = jnp.concatenate([_float(_bits(xf[:, 0:128]) | zt), xf[:, 128:]], axis=1).astype(BF16)
    up = _r(jnp.dot(xs, w_buf[:, F:2 * F], preferred_element_type=F32)[0:8])
    hid = _r(gt * _r(jax.nn.sigmoid(gt))) * up
    hid = jnp.concatenate([hid, hid], axis=0).astype(BF16)
    y = _r(jnp.dot(hid, wd_buf[:, 0:D], preferred_element_type=F32)[0:8])
    y1 = _r(y[0:1, :] * _r(jax.nn.sigmoid(m1)))
    y2 = _r(y[1:2, :] * _r(jax.nn.sigmoid(m2)))

    def fix(i, t):
        g = pl.multiple_of(lax.shift_right_logical(i, 4) * PR, PR)
        tg = pl.multiple_of(lax.shift_right_logical(t, 4) * PR, PR)
        rid = rowid + g
        upd = jnp.where(rid == i1, y1, jnp.where(rid == i2, y2, 0.0))
        yg, ng = parked(tg, PR)
        return g, (yg + _rows8(modulate(ng) + upd, jnp.multiply, coef[C_GB])).astype(BF16)

    g1, fix1 = fix(i1, t1)
    g2, fix2 = fix(i2, t2)
    wait(cp_out)
    act[pl.ds(g1, PR), :] = fix1
    act[pl.ds(g2, PR), :] = fix2
    f1 = cp(act.at[pl.ds(g1, PR), :], out_hbm.at[pl.ds(g1, PR), :], SEM_OUT)
    f2 = cp(act.at[pl.ds(g2, PR), :], out_hbm.at[pl.ds(g2, PR), :], SEM_FIX)
    f1.start()

    @pl.when(g1 != g2)
    def _():
        f2.start()
        f2.wait()

    f1.wait()


@jax.jit
def pallas_adaLN_cond__mha_block_cached__moe_arch_mod__prompt_kernel(
    A_x: jax.Array,
    A_k_cache: jax.Array,
    A_v_cache: jax.Array,
    A_wq: jax.Array,
    A_wo: jax.Array,
    B_x: jax.Array,
    B_w_r: jax.Array,
    B_w_gate: jax.Array,
    B_w_up: jax.Array,
    B_w_down: jax.Array,
    c: jax.Array,
    w_mod: jax.Array,
):
    del B_x
    hbm = pl.BlockSpec(memory_space=pl.ANY)
    out = pl.pallas_call(
        _kernel,
        in_specs=[hbm] * 11,
        out_specs=hbm,
        out_shape=jax.ShapeDtypeStruct((S, D), BF16),
        scratch_shapes=[
            pltpu.VMEM((S, D), BF16),
            pltpu.VMEM((H, S, DH), BF16),
            pltpu.VMEM((H, S, DH), BF16),
            pltpu.VMEM((H, D, DH), BF16),
            pltpu.VMEM((H, DH, D), BF16),
            pltpu.VMEM((D, WW), BF16),
            pltpu.VMEM((F, D + PAD), BF16),
            pltpu.VMEM((S + PR, D), BF16),
            pltpu.VMEM((S, D), F32),
            pltpu.VMEM((NST, 2 * SUB, 128), F32),
            pltpu.VMEM((R2, 2 * SUB, DH), F32),
            pltpu.VMEM((SUB + 2 * PR, D), F32),
            pltpu.VMEM((2, SUB + 2 * PR, 128), F32),
            pltpu.VMEM((PR, 128), F32),
            pltpu.VMEM((5, 8, D), F32),
            pltpu.VMEM((8, 128), BF16),
            pltpu.VMEM((8, D), F32),
            pltpu.VMEM((8, 128), F32),
            pltpu.VMEM((1, D), BF16),
            pltpu.VMEM((16, D), BF16),
            pltpu.VMEM((D, 128), F32),
            pltpu.VMEM((8, 4 * D + 256), F32),
            pltpu.VMEM((8, 128), I32),
            pltpu.VMEM((FILL, DH), F32),
            pltpu.VMEM((2, SUB, DH), F32),
            pltpu.VMEM((2, SUB, DH), F32),
            pltpu.SemaphoreType.DMA((NSEM,)),
        ],
        compiler_params=pltpu.CompilerParams(
            vmem_limit_bytes=120 * 1024 * 1024,
            disable_bounds_checks=True,
            disable_semaphore_checks=True,
        ),
        name="adaln_mha_mod",
    )(
        A_x.reshape(S, D),
        A_k_cache.reshape(H, S, DH),
        A_v_cache.reshape(H, S, DH),
        A_wq,
        A_wo.reshape(H, DH, D),
        B_w_r.reshape(8, 128),
        B_w_gate,
        B_w_up,
        B_w_down,
        c,
        w_mod,
    )
    return out.reshape(1, S, D)
```
